```python
import jax
import jax.numpy as jnp

def _softmax(x, axis=-1):
    return jax.nn.softmax(x, axis=axis)
def _gelu(x):
    return jax.nn.gelu(x, approximate=True)
def _silu(x):
    return jax.nn.silu(x)
def _sigmoid(x):
    return jax.nn.sigmoid(x)
def _layernorm(x, axis=-1, eps=1e-5):
    m = jnp.mean(x, axis=axis, keepdims=True)
    v = jnp.var(x, axis=axis, keepdims=True)
    return (x - m) / jnp.sqrt(v + eps)
def _scatter_add(tgt, idx, src, axis=0):
    return tgt.at[idx].add(src)
def _segment_sum(src, seg, n):
    return jax.ops.segment_sum(src, seg, n)
class _Rng:
    def __init__(self, key):
        self._k = key
    def _next(self):
        self._k, sub = jax.random.split(self._k)
        return sub
    def normal(self, shape):
        return jax.random.normal(self._next(), shape, dtype=jnp.bfloat16)
    def randint(self, lo, hi, shape):
        return jax.random.randint(self._next(), shape, lo, hi, dtype=jnp.int32)
    def uniform(self, shape, lo=0.0, hi=1.0):
        return jax.random.uniform(self._next(), shape, jnp.bfloat16, lo, hi)
    def permutation(self, n):
        return jax.random.permutation(self._next(), n)


kernel_name = 'interleave_layers__softmax_full_mha__ssm_conv_h3__prompt'

def setup_inputs():
    _rng = _Rng(jax.random.key(int.from_bytes(__import__("os").urandom(4), "little")))
    _w = (lambda a: (lambda t: t.astype(jnp.bfloat16) if jnp.issubdtype(t.dtype, jnp.floating) else t)(jnp.asarray(a)))
    def _A_setup():
        B, S, D = 1, 2048, 1024
        return {
            "x": _w((lambda *s: _rng.normal(s) * 0.05)(B, S, D)),
            "wqkv": _w((lambda *s: _rng.normal(s) * 0.05)(D, 3 * D)),
            "wo": _w((lambda *s: _rng.normal(s) * 0.05)(D, D)),
        }
    _A_in = _A_setup()

    def _B_setup():
        B, S, D = 1, 2048, 1024
        ks = 4
        return {
            "q": _w((lambda *s: _rng.normal(s) * 0.05)(B, S, D)),
            "k": _w((lambda *s: _rng.normal(s) * 0.05)(B, S, D)),
            "v": _w((lambda *s: _rng.normal(s) * 0.05)(B, S, D)),
            "shift_k": _w((lambda *s: _rng.normal(s) * 0.05)(D, ks) * 0.5),
            "ssm_k": _w((lambda *s: _rng.normal(s) * 0.05)(D, S) * (1.0 / S ** 0.5)),
            "ssm_D": _w((lambda *s: _rng.normal(s) * 0.05)(D)),
        }
    _B_in = _B_setup()

    return {
        "A_x": _A_in["x"],
        "A_wqkv": _A_in["wqkv"],
        "A_wo": _A_in["wo"],
        "B_q": _B_in["q"],
        "B_k": _B_in["k"],
        "B_v": _B_in["v"],
        "B_shift_k": _B_in["shift_k"],
        "B_ssm_k": _B_in["ssm_k"],
        "B_ssm_D": _B_in["ssm_D"],
    }

def reference(A_x, A_wqkv, A_wo, B_q, B_k, B_v, B_shift_k, B_ssm_k, B_ssm_D):
    def _A_ref(x, wqkv, wo):
        B, S, D = x.shape
        H = 32; Dh = D // H
        qkv = (lambda x, *d: x.transpose(*d))((x @ wqkv).reshape(B, S, 3, H, Dh), 2, 0, 3, 1, 4)
        q, k, v = qkv[0], qkv[1], qkv[2]
        scale = Dh ** -0.5
        scores = jnp.einsum("bhqd,bhkd->bhqk", q, k) * scale
        p = _softmax(scores, axis=-1)
        o = jnp.einsum("bhqk,bhkd->bhqd", p, v)
        return (lambda x, *d: x.transpose(*d))(o, 0, 2, 1, 3).reshape(B, S, D) @ wo

    def _B_ref(q, k, v, shift_k, ssm_k, ssm_D):
        B, S, D = q.shape
        ks = shift_k.shape[-1]
        k_pad = jnp.pad(k, ((0, 0), (ks - 1, 0), (0, 0)))
        k_shift = jnp.zeros_like(k)
        for t in range(ks):
            k_shift = k_shift + k_pad[:, t:t + S, :] * shift_k[:, ks - 1 - t][None, None, :]
        kv = k_shift * v
        L = 2 * S
        kv_pad = jnp.pad(kv, ((0, 0), (0, S), (0, 0)))
        kf_pad = jnp.pad(ssm_k, ((0, 0), (0, S)))
        kv_f = (lambda x, axes=(-2,-1): jnp.fft.rfft2(x.astype(jnp.float32), axes=axes))(kv_pad[:, None, :, :], axes=(1, 2))
        kf_f = (lambda x, axes=(-2,-1): jnp.fft.rfft2(x.astype(jnp.float32), axes=axes))(kf_pad[:, None, :], axes=(1, 2))
        kf_f = (lambda x, *d: x.transpose(*d))(kf_f, 1, 2, 0)
        y_f = kv_f * kf_f[None, :, :, :]
        y = (lambda x, s, axes=(-2,-1): jnp.fft.irfft2(x, s=s, axes=axes).astype(jnp.bfloat16))(y_f, (1, L), axes=(1, 2))[:, 0, :S, :]
        y = y + kv * ssm_D[None, None, :]
        return q * y

    x = A_x
    x = x + _A_ref(_layernorm(x, axis=-1), A_wqkv, A_wo)
    x = x + _B_ref(_layernorm(x, axis=-1), B_k, B_v, B_shift_k, B_ssm_k, B_ssm_D)
    x = x + _A_ref(_layernorm(x, axis=-1), A_wqkv, A_wo)
    x = x + _B_ref(_layernorm(x, axis=-1), B_k, B_v, B_shift_k, B_ssm_k, B_ssm_D)
    return x
```

```python
import functools
import numpy as np
import jax
import jax.numpy as jnp
from jax import lax
import jax.experimental.pallas as pl
import jax.experimental.pallas.tpu as pltpu

S = 2048
D = 1024
H = 32
DH = 32
G = 8
NQ = 16
HS = S // 2
CH = HS // 4
UNR = 2
TRIG = 20
RC = 256
NRC = S // RC
NC = 16
EPS = 1e-5
NZ = 2 + 8 * UNR
QSCALE = float(DH ** -0.5 * np.log2(np.e))

bf = jnp.bfloat16
f32 = jnp.float32
u32 = jnp.uint32
NT = (((1,), (1,)), ((), ()))


def _dft_mats():
    n = np.arange(128)
    f = np.concatenate([np.arange(0, 128, 2), np.arange(1, 128, 2)])
    ang = 2.0 * np.pi * np.outer(f + 0.5, n) / 256.0
    fwd = np.concatenate([np.cos(ang), -np.sin(ang)], axis=0)
    inv = fwd.T / 128.0
    return fwd.astype(np.float32), inv.astype(np.float32)


def _tree_sum(p):
    n = p.shape[0] // 8
    x = p.reshape(n, 8, 128)
    while n > 1:
        x = x.reshape(n // 2, 2, 8, 128)
        x = x[:, 0] + x[:, 1]
        n //= 2
    return x[0]


def _ln(x):
    m = jnp.mean(x, axis=-1, keepdims=True)
    xc = x - m
    v = jnp.mean(xc * xc, axis=-1, keepdims=True)
    return xc * lax.rsqrt(v + EPS)


def _pack(x):
    return pltpu.bitcast(x.astype(bf), u32)


def _unpack(x):
    return pltpu.bitcast(x, bf)


def _kernel(x_in, wqkv, wo, bk, bv, shk, ssmk, ssmd, fwd_ref, inv_ref, out_ref,
            x_s, y_s, qt_s, k_s, vt_s, o_s, a1, a2, b1, b2, fin, kf_s, u_s, g_s, z_ref):
    for i in range(NZ):
        z_ref[i] = 0
    fin[...] = jnp.ones(fin.shape, f32)

    kf_s[0:8, :] = jnp.zeros((8, 128), f32)
    eye8 = (lax.broadcasted_iota(jnp.int32, (8, 4), 0) == lax.broadcasted_iota(jnp.int32, (8, 4), 1)).astype(bf)

    def conv_block(cb, carry):
        c0 = pl.multiple_of(cb * 128, 128)
        cs = pl.ds(c0, 128)
        taps = lax.dot_general(eye8, shk[cs, :], NT, preferred_element_type=f32)
        dvec = ssmd[:, cs].astype(f32)
        kf_s[8:8 + S, :] = bk[0, :, cs].astype(f32)
        fwd = fwd_ref[...]
        inv = inv_ref[...]
        for j in range(NC):
            r0 = j * 128
            ks = kf_s[8 + r0:8 + r0 + 128, :] * taps[0:1]
            for t in range(1, 4):
                ks = ks + kf_s[8 + r0 - t:8 + r0 - t + 128, :] * taps[t:t + 1]
            kv = (ks * bv[0, r0:r0 + 128, cs].astype(f32)).astype(bf)
            y_s[cb, r0:r0 + 128, :] = kv.astype(f32) * dvec
            u_s[j] = jnp.dot(fwd, kv, preferred_element_type=f32)
        hprev = None
        for m in range(NC):
            hm = lax.dot_general(fwd, ssmk[cs, m * 128:(m + 1) * 128], NT, preferred_element_type=f32)
            if hprev is None:
                g_s[m] = hm
            else:
                gr = jnp.concatenate([hm[0:64] - hprev[128:192], hm[64:128] + hprev[192:256]], axis=0)
                gi = jnp.concatenate([hm[128:192] + hprev[0:64], hm[192:256] - hprev[64:128]], axis=0)
                g_s[m] = jnp.concatenate([gr, gi], axis=0)
            hprev = hm
        for i in range(NC):
            zr = None
            zi = None
            for j in range(i + 1):
                ur = u_s[j, 0:128, :]
                ui = u_s[j, 128:256, :]
                gr = g_s[i - j, 0:128, :]
                gi = g_s[i - j, 128:256, :]
                tr = ur * gr - ui * gi
                ti = ur * gi + ui * gr
                zr = tr if zr is None else zr + tr
                zi = ti if zi is None else zi + ti
            zz = jnp.concatenate([zr, zi], axis=0).astype(bf)
            y_s[cb, i * 128:(i + 1) * 128, :] += jnp.dot(inv, zz, preferred_element_type=f32)
        return carry

    lax.fori_loop(0, G, conv_block, 0)

    def qkv_proj(h, c):
        r2 = pl.multiple_of(c * (RC // 2), RC // 2)
        q = jnp.dot(h, wqkv[:, 0:D], preferred_element_type=f32) * QSCALE
        for t in range(RC // 128):
            qt_s[c * (RC // 128) + t] = _pack(q[t * 128:(t + 1) * 128, :].T)
        k = jnp.dot(h, wqkv[:, D:2 * D], preferred_element_type=f32)
        for g in range(G):
            k_s[g, pl.ds(r2, RC // 2), :] = _pack(k[:, g * 128:(g + 1) * 128])
        v = jnp.dot(h, wqkv[:, 2 * D:3 * D], preferred_element_type=f32)
        for t in range(RC // 128):
            vt_s[c * (RC // 128) + t] = _pack(v[t * 128:(t + 1) * 128, :].T)

    def out_proj_gate(c):
        r0 = pl.multiple_of(c * RC, RC)
        r2 = pl.multiple_of(c * (RC // 2), RC // 2)
        o = jnp.concatenate([_unpack(o_s[g, pl.ds(r2, RC // 2), :]) for g in range(G)], axis=1)
        x1 = x_s[pl.ds(r0, RC), :] + jnp.dot(o, wo[...], preferred_element_type=f32)
        y = jnp.concatenate([y_s[g, pl.ds(r0, RC), :] for g in range(G)], axis=1)
        return x1 + _ln(x1) * y

    def phase1(c, carry):
        r0 = pl.multiple_of(c * RC, RC)
        x = x_in[0, pl.ds(r0, RC), :].astype(f32)
        x_s[pl.ds(r0, RC), :] = x
        qkv_proj(_ln(x).astype(bf), c)
        return carry

    def phase2(c, carry):
        r0 = pl.multiple_of(c * RC, RC)
        x2 = out_proj_gate(c)
        x_s[pl.ds(r0, RC), :] = x2
        qkv_proj(_ln(x2).astype(bf), c)
        return carry

    def phase3(c, carry):
        r0 = pl.multiple_of(c * RC, RC)
        out_ref[0, pl.ds(r0, RC), :] = out_proj_gate(c).astype(bf)
        return carry

    zero16 = jnp.zeros((16, 128), u32)

    def qk(g, j, hh, half, dst, z, zk=0, dep=None):
        qt = qt_s[j, pl.ds(pl.multiple_of(g * 64 + hh * 16, 16), 16), :]
        w = _unpack(jnp.concatenate([qt if i == hh else zero16 for i in range(4)], axis=0))
        m = None
        first = None
        trig = None
        for c in range(4):
            r0 = half * HS + c * CH
            ku = k_s[g + zk, r0 // 2:(r0 + CH) // 2, :]
            if dep is not None:
                ku = jnp.concatenate([ku[:CH // 2 - 8], ku[CH // 2 - 8:] | dep], axis=0)
            s = jnp.dot(_unpack(ku), w, preferred_element_type=f32)
            dst[z, c * CH:(c + 1) * CH, :] = s
            mc = jnp.max(s.reshape(CH // 8, 8, 128), axis=0)
            m = mc if m is None else jnp.maximum(m, mc)
            f = pltpu.bitcast(s[0:8], u32)
            first = f if first is None else first | f
            if c == 3:
                trig = pltpu.bitcast(s[TRIG * 8:TRIG * 8 + 8], u32)
        return m, first, trig

    def fullmax(m1, m2):
        return jnp.max(jnp.maximum(m1, m2), axis=0, keepdims=True)

    def sm_pv(g, hh, half, src, m, z2, dep, trig, trig2):
        mb = jnp.broadcast_to(m, (8, 128))
        ps = []
        for i, tr in enumerate((trig, trig2)):
            mi = mb
            if tr is not None:
                mi = pltpu.bitcast(pltpu.bitcast(mb, u32) | tr, f32)
            x = src[z2, i * HS // 2:(i + 1) * HS // 2, :]
            ps.append(jnp.exp2(x.reshape(HS // 16, 8, 128) - mi[None]).reshape(HS // 2, 128))
        p = jnp.concatenate(ps, axis=0)
        l = _tree_sum(p)
        rs = pl.ds(pl.multiple_of(g * 64 + hh * 16, 16), 16)
        dep2 = jnp.concatenate([dep, dep], axis=0)
        vu = jnp.concatenate([vt_s[half * 8 + t, rs, :] | dep2 for t in range(8)], axis=1)
        o = jnp.dot(_unpack(vu), p.astype(bf), preferred_element_type=f32)
        return o, l

    def store_o(g, j, parts):
        outs = [parts[2 * h] * (1.0 / jnp.sum(parts[2 * h + 1], axis=0, keepdims=True)) for h in range(4)]
        ot = jnp.concatenate(outs, axis=0)
        o_s[g, pl.ds(pl.multiple_of(j * 64, 64), 64), :] = _pack(ot.T)

    def finalize(g, j, slot):
        x = fin[slot]
        parts = []
        for hh in range(4):
            parts += [x[hh * 40: hh * 40 + 32], x[hh * 40 + 32: hh * 40 + 40]]
        store_o(g, j, parts)

    def attention():
        ma = fullmax(qk(0, 0, 0, 0, a1, 0)[0], qk(0, 0, 0, 1, a2, 0)[0])
        mb1 = qk(0, 0, 1, 0, b1, 0)[0]
        bufs = {(0, 0): a1, (0, 1): a2, (1, 0): b1, (1, 1): b2}

        def body(it, carry):
            ma, mb1 = carry
            z1 = z_ref[0]
            z2 = z_ref[1]
            zv = jnp.full((8, 128), z1, jnp.int32).astype(u32)
            tp = jnp.maximum(it * UNR - 1, 0)
            finalize(tp // NQ, tp % NQ, z2)
            do = None
            ptrig = None
            for u in range(UNR):
                zk = [z_ref[2 + 8 * u + i] for i in range(8)]
                t = it * UNR + u
                g = t // NQ
                j = t % NQ
                tn = jnp.minimum(t + 1, G * NQ - 1)
                gn = tn // NQ
                jn = tn % NQ
                qks = [(g, j, 1, 1), (g, j, 2, 0), (g, j, 2, 1), (g, j, 3, 0), (g, j, 3, 1),
                       (gn, jn, 0, 0), (gn, jn, 0, 1), (gn, jn, 1, 0)]
                mfull = {0: ma}
                mpart = {1: mb1}
                os_, ls_ = {}, {}
                for n in range(8):
                    qg, qj, qh, qhalf = qks[n]
                    key = qh if n < 5 else qh + 4
                    mp, first, trig = qk(qg, qj, qh, qhalf, bufs[(qh % 2, qhalf)], z1, zk[n], do)
                    if qhalf == 0:
                        mpart[key] = mp
                    else:
                        mfull[key] = fullmax(mpart[key], mp)
                    ph, phalf = n // 2, n % 2
                    o, l = sm_pv(g, ph, phalf, bufs[(ph % 2, phalf)], mfull[ph], z2, first & zv, ptrig, do)
                    ptrig = trig & zv
                    do = pltpu.bitcast(o[24:32], u32) & zv
                    os_[(ph, phalf)] = o
                    ls_[(ph, phalf)] = l
                ma = mfull[4]
                mb1 = mpart[5]
                parts = []
                for h in range(4):
                    parts += [os_[(h, 0)] + os_[(h, 1)], ls_[(h, 0)] + ls_[(h, 1)]]
                if u == UNR - 1:
                    fin[z1] = jnp.concatenate(parts, axis=0)
                else:
                    store_o(g, j, parts)
            return ma, mb1

        lax.fori_loop(0, G * NQ // UNR, body, (ma, mb1))
        finalize(G - 1, NQ - 1, 0)

    lax.fori_loop(0, NRC, phase1, 0)
    attention()
    lax.fori_loop(0, NRC, phase2, 0)
    attention()
    lax.fori_loop(0, NRC, phase3, 0)


@jax.jit
def pallas_interleave_layers__softmax_full_mha__ssm_conv_h3__prompt_kernel(A_x, A_wqkv, A_wo, B_q, B_k, B_v, B_shift_k, B_ssm_k, B_ssm_D):
    fwd, inv = _dft_mats()
    fwd = jnp.asarray(fwd, dtype=bf)
    inv = jnp.asarray(inv, dtype=bf)
    scratch = [
        pltpu.VMEM((S, D), f32),
        pltpu.VMEM((G, S, 128), f32),
        pltpu.VMEM((NQ, D // 2, 128), u32),
        pltpu.VMEM((G, S // 2, 128), u32),
        pltpu.VMEM((NQ, D // 2, 128), u32),
        pltpu.VMEM((G, S // 2, 128), u32),
        pltpu.VMEM((1, HS, 128), f32), pltpu.VMEM((1, HS, 128), f32),
        pltpu.VMEM((1, HS, 128), f32), pltpu.VMEM((1, HS, 128), f32),
        pltpu.VMEM((1, 160, 128), f32),
        pltpu.VMEM((S + 8, 128), f32),
        pltpu.VMEM((NC, 256, 128), f32),
        pltpu.VMEM((NC, 256, 128), f32),
        pltpu.SMEM((NZ,), jnp.int32),
    ]
    return pl.pallas_call(
        _kernel,
        out_shape=jax.ShapeDtypeStruct((1, S, D), bf),
        scratch_shapes=scratch,
        compiler_params=pltpu.CompilerParams(vmem_limit_bytes=120 * 2**20),
    )(A_x, A_wqkv, A_wo, B_k, B_v, B_shift_k, B_ssm_k, B_ssm_D.reshape(1, D), fwd, inv)
```

```python
import functools
import numpy as np
import jax
import jax.numpy as jnp
from jax import lax
import jax.experimental.pallas as pl
import jax.experimental.pallas.tpu as pltpu

S = 2048
D = 1024
H = 32
DH = 32
G = 8
NQ = 16
HS = S // 2
CH = HS // 4
UNR = 4
TA = (17, 21, 25, 29)
TB = (0, 0, 4, 8)
RC = 256
NRC = S // RC
NC = 16
EPS = 1e-5
NZ = 2 + 8 * UNR
QSCALE = float(DH ** -0.5 * np.log2(np.e))

bf = jnp.bfloat16
f32 = jnp.float32
u32 = jnp.uint32
NT = (((1,), (1,)), ((), ()))


def _dft_mats():
    n = np.arange(128)
    f = np.concatenate([np.arange(0, 128, 2), np.arange(1, 128, 2)])
    ang = 2.0 * np.pi * np.outer(f + 0.5, n) / 256.0
    fwd = np.concatenate([np.cos(ang), -np.sin(ang)], axis=0)
    inv = fwd.T / 128.0
    return fwd.astype(np.float32), inv.astype(np.float32)


def _tree_sum(p):
    n = p.shape[0] // 8
    x = p.reshape(n, 8, 128)
    while n > 1:
        x = x.reshape(n // 2, 2, 8, 128)
        x = x[:, 0] + x[:, 1]
        n //= 2
    return x[0]


def _ln(x):
    m = jnp.mean(x, axis=-1, keepdims=True)
    xc = x - m
    v = jnp.mean(xc * xc, axis=-1, keepdims=True)
    return xc * lax.rsqrt(v + EPS)


def _pack(x):
    return pltpu.bitcast(x.astype(bf), u32)


def _unpack(x):
    return pltpu.bitcast(x, bf)


def _kernel(x_hbm, wqkv_hbm, wo_hbm, bk_hbm, bv_hbm, shk, ssmk_hbm, ssmd, fwd_ref, inv_ref, out_hbm,
            x_s, y_s, qt_s, k_s, vt_s, o_s, a1, a2, b1, b2, fin, kf_s, u_s, g_s, z_ref,
            x_in, wqkv, wo, bk, bv, ssmk, out_s, sem_c, sem_x, sem_w, sem_o):
    def conv_copies(cb):
        cs = pl.ds(pl.multiple_of(cb * 128, 128), 128)
        return [pltpu.make_async_copy(bk_hbm.at[0, :, cs], bk.at[cb], sem_c.at[0, cb]),
                pltpu.make_async_copy(bv_hbm.at[0, :, cs], bv.at[cb], sem_c.at[1, cb]),
                pltpu.make_async_copy(ssmk_hbm.at[cs, :], ssmk.at[cs, :], sem_c.at[2, cb])]

    def x_copy(c):
        rs = pl.ds(pl.multiple_of(c * RC, RC), RC)
        return pltpu.make_async_copy(x_hbm.at[0, rs, :], x_in.at[rs, :], sem_x.at[c])

    def w_copy(c):
        rs = pl.ds(pl.multiple_of(c * 128, 128), 128)
        return pltpu.make_async_copy(wqkv_hbm.at[rs, :], wqkv.at[rs, :], sem_w.at[c])

    def wo_copy():
        return pltpu.make_async_copy(wo_hbm, wo, sem_w.at[G])

    def out_copy(c):
        rs = pl.ds(pl.multiple_of(c * RC, RC), RC)
        return pltpu.make_async_copy(out_s.at[rs, :], out_hbm.at[0, rs, :], sem_o.at[c])

    for cb in range(2):
        for cp in conv_copies(cb):
            cp.start()
    for i in range(NZ):
        z_ref[i] = 0
    fin[...] = jnp.ones(fin.shape, f32)

    kf_s[0:8, :] = jnp.zeros((8, 128), f32)
    eye8 = (lax.broadcasted_iota(jnp.int32, (8, 4), 0) == lax.broadcasted_iota(jnp.int32, (8, 4), 1)).astype(bf)

    def conv_block(cb, carry):
        c0 = pl.multiple_of(cb * 128, 128)
        cs = pl.ds(c0, 128)

        @pl.when(cb + 2 < G)
        def _():
            for cp in conv_copies(cb + 2):
                cp.start()
        w_copy(cb).start()
        x_copy(cb).start()
        for cp in conv_copies(cb):
            cp.wait()
        taps = lax.dot_general(eye8, shk[cs, :], NT, preferred_element_type=f32)
        dvec = ssmd[:, cs].astype(f32)
        kf_s[8:8 + S, :] = bk[cb].astype(f32)
        fwd = fwd_ref[...]
        inv = inv_ref[...]
        for j in range(NC):
            r0 = j * 128
            ks = kf_s[8 + r0:8 + r0 + 128, :] * taps[0:1]
            for t in range(1, 4):
                ks = ks + kf_s[8 + r0 - t:8 + r0 - t + 128, :] * taps[t:t + 1]
            kv = (ks * bv[cb, r0:r0 + 128, :].astype(f32)).astype(bf)
            y_s[cb, r0:r0 + 128, :] = kv.astype(f32) * dvec
            u_s[j] = jnp.dot(fwd, kv, preferred_element_type=f32)
        hprev = None
        for m in range(NC):
            hm = lax.dot_general(fwd, ssmk[cs, m * 128:(m + 1) * 128], NT, preferred_element_type=f32)
            if hprev is None:
                g_s[m] = hm
            else:
                gr = jnp.concatenate([hm[0:64] - hprev[128:192], hm[64:128] + hprev[192:256]], axis=0)
                gi = jnp.concatenate([hm[128:192] + hprev[0:64], hm[192:256] - hprev[64:128]], axis=0)
                g_s[m] = jnp.concatenate([gr, gi], axis=0)
            hprev = hm
        for i in range(NC):
            zr = None
            zi = None
            for j in range(i + 1):
                ur = u_s[j, 0:128, :]
                ui = u_s[j, 128:256, :]
                gr = g_s[i - j, 0:128, :]
                gi = g_s[i - j, 128:256, :]
                tr = ur * gr - ui * gi
                ti = ur * gi + ui * gr
                zr = tr if zr is None else zr + tr
                zi = ti if zi is None else zi + ti
            zz = jnp.concatenate([zr, zi], axis=0).astype(bf)
            y_s[cb, i * 128:(i + 1) * 128, :] += jnp.dot(inv, zz, preferred_element_type=f32)
        return carry

    lax.fori_loop(0, G, conv_block, 0)
    wo_copy().start()
    for c in range(G):
        w_copy(c).wait()

    def qkv_proj(h, c):
        r2 = pl.multiple_of(c * (RC // 2), RC // 2)
        q = jnp.dot(h, wqkv[:, 0:D], preferred_element_type=f32) * QSCALE
        for t in range(RC // 128):
            qt_s[c * (RC // 128) + t] = _pack(q[t * 128:(t + 1) * 128, :].T)
        k = jnp.dot(h, wqkv[:, D:2 * D], preferred_element_type=f32)
        for g in range(G):
            k_s[g, pl.ds(r2, RC // 2), :] = _pack(k[:, g * 128:(g + 1) * 128])
        v = jnp.dot(h, wqkv[:, 2 * D:3 * D], preferred_element_type=f32)
        for t in range(RC // 128):
            vt_s[c * (RC // 128) + t] = _pack(v[t * 128:(t + 1) * 128, :].T)

    def out_proj_gate(c):
        r0 = pl.multiple_of(c * RC, RC)
        r2 = pl.multiple_of(c * (RC // 2), RC // 2)
        o = jnp.concatenate([_unpack(o_s[g, pl.ds(r2, RC // 2), :]) for g in range(G)], axis=1)
        x1 = x_s[pl.ds(r0, RC), :] + jnp.dot(o, wo[...], preferred_element_type=f32)
        y = jnp.concatenate([y_s[g, pl.ds(r0, RC), :] for g in range(G)], axis=1)
        return x1 + _ln(x1) * y

    def phase1(c, carry):
        r0 = pl.multiple_of(c * RC, RC)
        x_copy(c).wait()
        x = x_in[pl.ds(r0, RC), :].astype(f32)
        x_s[pl.ds(r0, RC), :] = x
        qkv_proj(_ln(x).astype(bf), c)
        return carry

    def phase2(c, carry):
        r0 = pl.multiple_of(c * RC, RC)
        x2 = out_proj_gate(c)
        x_s[pl.ds(r0, RC), :] = x2
        qkv_proj(_ln(x2).astype(bf), c)
        return carry

    def phase3(c, carry):
        r0 = pl.multiple_of(c * RC, RC)
        out_s[pl.ds(r0, RC), :] = out_proj_gate(c).astype(bf)
        out_copy(c).start()
        return carry

    zero16 = jnp.zeros((16, 128), u32)

    def qk(g, j, hh, half, dst, z, zk=0, dep=None):
        qt = qt_s[j, pl.ds(pl.multiple_of(g * 64 + hh * 16, 16), 16), :]
        w = _unpack(jnp.concatenate([qt if i == hh else zero16 for i in range(4)], axis=0))
        m = None
        first = None
        trig = None
        for c in range(4):
            r0 = half * HS + c * CH
            ku = k_s[g + zk, r0 // 2:(r0 + CH) // 2, :]
            if dep is not None:
                ku = jnp.concatenate([ku[:CH // 2 - 8], ku[CH // 2 - 8:] | dep], axis=0)
            s = jnp.dot(_unpack(ku), w, preferred_element_type=f32)
            dst[z, c * CH:(c + 1) * CH, :] = s
            mc = jnp.max(s.reshape(CH // 8, 8, 128), axis=0)
            m = mc if m is None else jnp.maximum(m, mc)
            f = pltpu.bitcast(s[0:8], u32)
            first = f if first is None else first | f
            if c == 3:
                trig = s
        return m, first, trig

    def fullmax(m1, m2):
        return jnp.max(jnp.maximum(m1, m2), axis=0, keepdims=True)

    def sm_pv(g, hh, half, src, m, z2, dep, trigs):
        mb = jnp.broadcast_to(m, (8, 128))
        mbu = pltpu.bitcast(mb, u32)
        ms = [mb if tr is None else pltpu.bitcast(mbu | tr, f32) for tr in trigs]
        ng = len(trigs) // 2
        gr = 128 // ng
        ps = []
        for t in range(8):
            for kk in range(ng):
                mi = ms[(t // 4) * ng + (ng - 1 - kk)]
                x = src[z2, t * 128 + kk * gr:t * 128 + (kk + 1) * gr, :]
                ps.append(jnp.exp2(x.reshape(gr // 8, 8, 128) - mi[None]).reshape(gr, 128))
        p = jnp.concatenate(ps, axis=0)
        l = _tree_sum(p)
        rs = pl.ds(pl.multiple_of(g * 64 + hh * 16, 16), 16)
        dep2 = jnp.concatenate([dep, dep], axis=0)
        vu = jnp.concatenate([vt_s[half * 8 + t, rs, :] | dep2 for t in range(8)], axis=1)
        o = jnp.dot(_unpack(vu), p.astype(bf), preferred_element_type=f32)
        return o, l

    def store_o(g, j, parts):
        outs = [parts[2 * h] * (1.0 / jnp.sum(parts[2 * h + 1], axis=0, keepdims=True)) for h in range(4)]
        ot = jnp.concatenate(outs, axis=0)
        o_s[g, pl.ds(pl.multiple_of(j * 64, 64), 64), :] = _pack(ot.T)

    def finalize(g, j, slot):
        x = fin[slot]
        parts = []
        for hh in range(4):
            parts += [x[hh * 40: hh * 40 + 32], x[hh * 40 + 32: hh * 40 + 40]]
        store_o(g, j, parts)

    def attention():
        ma = fullmax(qk(0, 0, 0, 0, a1, 0)[0], qk(0, 0, 0, 1, a2, 0)[0])
        mb1 = qk(0, 0, 1, 0, b1, 0)[0]
        bufs = {(0, 0): a1, (0, 1): a2, (1, 0): b1, (1, 1): b2}

        def body(it, carry):
            ma, mb1 = carry
            z1 = z_ref[0]
            z2 = z_ref[1]
            zv = jnp.full((8, 128), z1, jnp.int32).astype(u32)
            tp = jnp.maximum(it * UNR - 1, 0)
            finalize(tp // NQ, tp % NQ, z2)
            do = None
            ptrig = None
            po = None
            for u in range(UNR):
                zk = [z_ref[2 + 8 * u + i] for i in range(8)]
                t = it * UNR + u
                g = t // NQ
                j = t % NQ
                tn = jnp.minimum(t + 1, G * NQ - 1)
                gn = tn // NQ
                jn = tn % NQ
                qks = [(g, j, 1, 1), (g, j, 2, 0), (g, j, 2, 1), (g, j, 3, 0), (g, j, 3, 1),
                       (gn, jn, 0, 0), (gn, jn, 0, 1), (gn, jn, 1, 0)]
                mfull = {0: ma}
                mpart = {1: mb1}
                os_, ls_ = {}, {}
                for n in range(8):
                    qg, qj, qh, qhalf = qks[n]
                    key = qh if n < 5 else qh + 4
                    mp, first, trig = qk(qg, qj, qh, qhalf, bufs[(qh % 2, qhalf)], z1, zk[n], do)
                    if qhalf == 0:
                        mpart[key] = mp
                    else:
                        mfull[key] = fullmax(mpart[key], mp)
                    ph, phalf = n // 2, n % 2
                    def tg(sv, i):
                        return None if sv is None else pltpu.bitcast(sv[i * 8:i * 8 + 8], u32) & zv
                    trigs = [tg(ptrig, i) for i in TA] + [tg(po, TB[0])] + [tg(trig, i) for i in TB[1:]]
                    o, l = sm_pv(g, ph, phalf, bufs[(ph % 2, phalf)], mfull[ph], z2, first & zv, trigs)
                    ptrig = trig
                    po = o
                    do = pltpu.bitcast(o[24:32], u32) & zv
                    os_[(ph, phalf)] = o
                    ls_[(ph, phalf)] = l
                ma = mfull[4]
                mb1 = mpart[5]
                parts = []
                for h in range(4):
                    parts += [os_[(h, 0)] + os_[(h, 1)], ls_[(h, 0)] + ls_[(h, 1)]]
                if u == UNR - 1:
                    fin[z1] = jnp.concatenate(parts, axis=0)
                else:
                    store_o(g, j, parts)
            return ma, mb1

        lax.fori_loop(0, G * NQ // UNR, body, (ma, mb1))
        finalize(G - 1, NQ - 1, 0)

    lax.fori_loop(0, NRC, phase1, 0)
    attention()
    wo_copy().wait()
    lax.fori_loop(0, NRC, phase2, 0)
    attention()
    lax.fori_loop(0, NRC, phase3, 0)
    for c in range(NRC):
        out_copy(c).wait()


@jax.jit
def pallas_interleave_layers__softmax_full_mha__ssm_conv_h3__prompt_kernel(A_x, A_wqkv, A_wo, B_q, B_k, B_v, B_shift_k, B_ssm_k, B_ssm_D):
    fwd, inv = _dft_mats()
    fwd = jnp.asarray(fwd, dtype=bf)
    inv = jnp.asarray(inv, dtype=bf)
    scratch = [
        pltpu.VMEM((S, D), f32),
        pltpu.VMEM((G, S, 128), f32),
        pltpu.VMEM((NQ, D // 2, 128), u32),
        pltpu.VMEM((G, S // 2, 128), u32),
        pltpu.VMEM((NQ, D // 2, 128), u32),
        pltpu.VMEM((G, S // 2, 128), u32),
        pltpu.VMEM((1, HS, 128), f32), pltpu.VMEM((1, HS, 128), f32),
        pltpu.VMEM((1, HS, 128), f32), pltpu.VMEM((1, HS, 128), f32),
        pltpu.VMEM((1, 160, 128), f32),
        pltpu.VMEM((S + 8, 128), f32),
        pltpu.VMEM((NC, 256, 128), f32),
        pltpu.VMEM((NC, 256, 128), f32),
        pltpu.SMEM((NZ,), jnp.int32),
        pltpu.VMEM((S, D), bf),
        pltpu.VMEM((D, 3 * D), bf),
        pltpu.VMEM((D, D), bf),
        pltpu.VMEM((G, S, 128), bf),
        pltpu.VMEM((G, S, 128), bf),
        pltpu.VMEM((D, S), bf),
        pltpu.VMEM((S, D), bf),
        pltpu.SemaphoreType.DMA((3, G)),
        pltpu.SemaphoreType.DMA((NRC,)),
        pltpu.SemaphoreType.DMA((G + 1,)),
        pltpu.SemaphoreType.DMA((NRC,)),
    ]
    hbm = pl.BlockSpec(memory_space=pl.ANY)
    vm = pl.BlockSpec(memory_space=pltpu.VMEM)
    return pl.pallas_call(
        _kernel,
        out_shape=jax.ShapeDtypeStruct((1, S, D), bf),
        in_specs=[hbm, hbm, hbm, hbm, hbm, vm, hbm, vm, vm, vm],
        out_specs=hbm,
        scratch_shapes=scratch,
        compiler_params=pltpu.CompilerParams(vmem_limit_bytes=120 * 2**20),
    )(A_x, A_wqkv, A_wo, B_k, B_v, B_shift_k, B_ssm_k, B_ssm_D.reshape(1, D), fwd, inv)
```

```python
import numpy as np
import jax
import jax.numpy as jnp
from jax import lax
import jax.experimental.pallas as pl
import jax.experimental.pallas.tpu as pltpu

S = 2048
D = 1024
DH = 32
G = 8
NQ = 16
HS = S // 2
CH = HS // 4
UNR = 4
TA = (17, 21, 25, 29)
TB = (0, 0, 4, 8)
RC = 256
NRC = S // RC
NP = RC // 16
NC = 16
EPS = 1e-5
MIDW = 0
SKIP = ''
IM = 136
CS = 288
GO = 16 * 288 + 16
LAZY = 1
ONLY = '1a23'
RG = 2
SPAN0 = 8
SPAN_TILES = 16
INV0 = 14
KV0 = 15
NZ = 2 + 8 * UNR
QSCALE = float(DH ** -0.5 * np.log2(np.e))

bf = jnp.bfloat16
f32 = jnp.float32
u32 = jnp.uint32
i32 = jnp.int32
NT = (((1,), (1,)), ((), ()))


def _dft_mats():
    n = np.arange(128)
    f = np.concatenate([np.arange(0, 128, 2), np.arange(1, 128, 2)])
    ang = 2.0 * np.pi * np.outer(f + 0.5, n) / 256.0
    fwd = np.concatenate([np.cos(ang), -np.sin(ang)], axis=0)
    inv = fwd.T / 128.0
    return fwd.astype(np.float32), inv.astype(np.float32)


def _tree_sum(p):
    n = p.shape[0] // 8
    x = p.reshape(n, 8, 128)
    while n > 1:
        x = x.reshape(n // 2, 2, 8, 128)
        x = x[:, 0] + x[:, 1]
        n //= 2
    return x[0]


def _ln(x):
    m = jnp.mean(x, axis=-1, keepdims=True)
    xc = x - m
    v = jnp.mean(xc * xc, axis=-1, keepdims=True)
    return xc * lax.rsqrt(v + EPS)


def _pack(x):
    return pltpu.bitcast(x.astype(bf), u32)


def _unpack(x):
    return pltpu.bitcast(x, bf)


def _tok(v, zv):
    v = v if v.dtype == u32 else pltpu.bitcast(v, u32)
    acc = None
    for r in range(v.shape[0] // 8):
        for c in range(v.shape[1] // 128):
            p = v[r * 8:(r + 1) * 8, c * 128:(c + 1) * 128]
            acc = p if acc is None else acc | p
    return acc & zv


def _gate(w, toks):
    if not toks:
        return w
    wu = pltpu.bitcast(w, u32)
    h0 = wu[0:8]
    for t in toks:
        h0 = h0 | jnp.tile(t, (1, wu.shape[1] // 128))
    return _unpack(jnp.concatenate([h0, wu[8:]], axis=0))


def _tick(v, k, z0):
    return pltpu.bitcast(v[8 * k:8 * k + 8, 0:128], i32)[0, 0] & z0


def _kernel(x_hbm, wqkv_hbm, wo_hbm, bk_hbm, bv_hbm, shk, ssmk_hbm, ssmd, fwd_ref, inv_ref, out_hbm,
            x_s, y_s, qt_s, k_s, vt_s, o_s, a1, a2, b1, b2, fin, kf_s, kv_s, taps_s, ug_s, hr_s, zb_s,
            h_s, z_ref, x_in, wqkv, wo, bk, bv, ssmk, out_s, sem_c, sem_x, sem_w, sem_o):
    def kv_copies(cb):
        cs = pl.ds(pl.multiple_of(cb * 128, 128), 128)
        return [pltpu.make_async_copy(bk_hbm.at[0, :, cs], bk.at[cb], sem_c.at[0, cb]),
                pltpu.make_async_copy(bv_hbm.at[0, :, cs], bv.at[cb], sem_c.at[1, cb])]

    def h_copy(cb):
        cs = pl.ds(pl.multiple_of(cb * 128, 128), 128)
        return pltpu.make_async_copy(ssmk_hbm.at[cs, :], ssmk.at[cs, :], sem_c.at[2, cb])

    def x_copy(c):
        rs = pl.ds(pl.multiple_of(c * RC, RC), RC)
        return pltpu.make_async_copy(x_hbm.at[0, rs, :], x_in.at[0, rs, :], sem_x.at[c])

    def w_copy(c):
        cs = pl.ds(c * D, D)
        return pltpu.make_async_copy(wqkv_hbm.at[:, cs], wqkv.at[:, cs], sem_w.at[c])

    def wo_copy():
        return pltpu.make_async_copy(wo_hbm, wo, sem_w.at[3])

    def out_copy(c):
        rs = pl.ds(pl.multiple_of(c * RC, RC), RC)
        return pltpu.make_async_copy(out_s.at[rs, :], out_hbm.at[0, rs, :], sem_o.at[c])

    x_copy(0).start()
    for cp in kv_copies(0):
        cp.start()
    h_copy(0).start()
    for c in (0, 2, 1):
        w_copy(c).start()
    def blk_start(c):
        x_copy(c).start()
        for cp in kv_copies(c):
            cp.start()
        h_copy(c).start()

    blk_start(1)
    if LAZY == 0:
        for c in range(2, G):
            blk_start(c)
        wo_copy().start()

    for i in range(NZ):
        z_ref[i] = 0
    fin[...] = jnp.ones(fin.shape, f32)
    kf_s[0, 0:8, :] = jnp.zeros((8, 128), f32)
    eye8 = (lax.broadcasted_iota(i32, (8, 4), 0) == lax.broadcasted_iota(i32, (8, 4), 1)).astype(bf)
    for cb in range(G):
        taps = lax.dot_general(eye8, shk[cb * 128:(cb + 1) * 128, :], NT, preferred_element_type=f32)
        dv = ssmd[:, cb * 128:(cb + 1) * 128].astype(f32)
        row = lax.broadcasted_iota(i32, (8, 128), 0)
        taps_s[cb] = jnp.where(row == 4, jnp.broadcast_to(dv, (8, 128)), taps)

    TILES = [(0, n) for n in range(8)] + [(2, n) for n in range(8)] + [(1, n) for n in range(8)]

    def qkv_tile(h, c, idx, toks, zv):
        kind, n = TILES[idx]
        col = kind * D + n * 128
        wa = _gate(wqkv[0:D // 2, col:col + 128], toks)
        ra = jnp.dot(h[:, 0:D // 2], wa, preferred_element_type=f32)
        rb = jnp.dot(h[:, D // 2:D], wqkv[D // 2:D, col:col + 128], preferred_element_type=f32)
        r = ra + rb
        if kind == 1:
            r2 = pl.multiple_of(c * (RC // 2), RC // 2)
            k_s[n, pl.ds(r2, RC // 2), :] = _pack(r)
            return ra, None
        dst = qt_s if kind == 0 else vt_s
        if kind == 0:
            r = r * QSCALE
        pks = []
        for t in range(RC // 128):
            pk = _pack(r[t * 128:(t + 1) * 128, :].T)
            dst[c * (RC // 128) + t, n * 64:(n + 1) * 64, :] = pk
            pks.append(pk)
        return ra, _tok(jnp.concatenate(pks, axis=0), zv)

    def piece_rows(c, p):
        return pl.ds(pl.multiple_of(c * RC + p * 16, 16), 16)

    def ln1_piece(cn, p, zt):
        rows = piece_rows(cn, p)
        x = x_in[zt, rows, :].astype(f32)
        x_s[0, rows, :] = x
        hp = _pack(_ln(x))
        h_s[p * 8:(p + 1) * 8, :] = hp
        return hp

    def gated_x(cn, p, zt):
        rows = piece_rows(cn, p)
        x1 = x_s[zt, rows, :]
        y = jnp.concatenate([y_s[g, rows, :] for g in range(G)], axis=1)
        return x1 + _ln(x1) * y

    def ln2_piece(cn, p, zt):
        x2 = gated_x(cn, p, zt)
        x_s[zt, piece_rows(cn, p), :] = x2
        hp = _pack(_ln(x2))
        h_s[p * 8:(p + 1) * 8, :] = hp
        return hp

    def out_piece(c, p, zt):
        out_s[piece_rows(c, p), :] = gated_x(c, p, zt).astype(bf)

    def kv_item(src, dst, j, zt):
        r0 = j * 128
        tp = taps_s[src]
        kf_s[zt, 8 + r0:8 + r0 + 128, :] = bk[src + zt, r0:r0 + 128, :].astype(f32)
        ks = kf_s[zt, 8 + r0:8 + r0 + 128, :] * tp[0:1]
        for t in range(1, 4):
            ks = ks + kf_s[zt, 8 + r0 - t:8 + r0 - t + 128, :] * tp[t:t + 1]
        kv = ks * bv[src + zt, r0:r0 + 128, :].astype(f32)
        y_s[dst, r0:r0 + 128, :] = kv * tp[4:5]
        kv_s[j * 64:(j + 1) * 64, :] = _pack(kv)

    def oproj_tile(o, cn, n, z1):
        rows = pl.ds(pl.multiple_of(cn * RC, RC), RC)
        cols = slice(n * 128, (n + 1) * 128)
        r = jnp.dot(o, wo[:, cols], preferred_element_type=f32)
        x_s[z1, rows, cols] = x_s[z1, rows, cols] + r
        return r

    def load_o(cn):
        r2 = pl.multiple_of(cn * (RC // 2), RC // 2)
        return jnp.concatenate([_unpack(o_s[g, pl.ds(r2, RC // 2), :]) for g in range(G)], axis=1)

    def phase1(c, carry):
        cn = jnp.minimum(c + 1, NRC - 1)

        if 'w' not in ONLY:
            if not MIDW:
                @pl.when(c + 1 < NRC)
                def _():
                    x_copy(c + 1).wait()
                    for cp in kv_copies(c + 1):
                        cp.wait()
            h_copy(c).wait()
        if LAZY:
            @pl.when(c + 2 < NRC)
            def _():
                blk_start(c + 2)

            @pl.when(c + 2 == NRC)
            def _():
                wo_copy().start()
        z0 = z_ref[0]
        z1 = z_ref[1]
        zv = jnp.full((8, 128), z0, i32).astype(u32)
        h = _unpack(h_s[...])
        cs = pl.ds(pl.multiple_of(c * 128, 128), 128)
        fwd = fwd_ref[...]
        def put(ref, off, v):
            ref[z1, off:off + 128, :] = v[0:128]
            ref[z1, off + IM:off + IM + 128, :] = v[128:256]

        for j in range(NC):
            put(ug_s, j * CS, jnp.dot(fwd, _unpack(kv_s[j * 64:(j + 1) * 64, :]), preferred_element_type=f32))
        for m in range(NC):
            put(hr_s, m * CS, lax.dot_general(fwd, ssmk[cs, m * 128:(m + 1) * 128], NT, preferred_element_type=f32))
        for r in range(0, 128, 8):
            for m in range(NC):
                o0 = m * CS + r
                hre = hr_s[z0, o0:o0 + 8, :]
                him = hr_s[z0, o0 + IM:o0 + IM + 8, :]
                if m > 0 and r < 64:
                    gre, gim = hre - pim, him + pre
                elif m > 0:
                    gre, gim = hre + pim, him - pre
                else:
                    gre, gim = hre, him
                ug_s[z1, GO + o0:GO + o0 + 8, :] = gre
                ug_s[z1, GO + o0 + IM:GO + o0 + IM + 8, :] = gim
                pre, pim = hre, him

        def spec_item(ib, r):
            zt = z_ref[2 + ib]
            gc = {}
            zr = [None] * 4
            zi = [None] * 4
            for j in range(4 * ib + 4):
                ou = j * CS + r
                ur = ug_s[zt, ou:ou + 8, :]
                ui = ug_s[zt, ou + IM:ou + IM + 8, :]
                for q in range(4):
                    m = 4 * ib + q - j
                    if m < 0:
                        continue
                    if m not in gc:
                        og = GO + m * CS + r
                        gc[m] = (ug_s[zt, og:og + 8, :], ug_s[zt, og + IM:og + IM + 8, :])
                    gr, gi = gc[m]
                    tr = ur * gr - ui * gi
                    ti = ur * gi + ui * gr
                    zr[q] = tr if zr[q] is None else zr[q] + tr
                    zi[q] = ti if zi[q] is None else zi[q] + ti
            return zr, zi

        items = [(ib, rp) for ib in range(4) for rp in range(8)]
        tot = sum(10 + 16 * ib for ib, _ in items)
        at = {}
        acc_w = 0
        for it in items:
            at.setdefault(acc_w * SPAN_TILES // tot, []).append(it)
            acc_w += 10 + 16 * it[0]
        inv_at = {}
        deps = {}
        for n in range(24):
            if MIDW and n % 8 == 0:
                @pl.when(c == 0)
                def _():
                    w_copy(TILES[n][0]).wait()
            if MIDW and n == KV0:
                @pl.when(c + 1 < NRC)
                def _():
                    x_copy(c + 1).wait()
                    for cp in kv_copies(c + 1):
                        cp.wait()
            ra, done = qkv_tile(h, c, n, deps.get(n), zv)
            if done is not None and n + 3 < 24:
                deps.setdefault(n + 3, []).append(done)
            if KV0 <= n < KV0 + 8:
                for e in range(2):
                    p = 2 * (n - KV0) + e
                    hp = ln1_piece(cn, p, _tick(ra, 16 * e, z0))
                    if n + 2 < 24:
                        deps.setdefault(n + 2, []).append(_tok(hp, zv))
                    kv_item(cn, c + 1, p, _tick(ra, 16 * e + 8, z0))
            for (ib, rp) in (at.get(n, []) if 's' not in SKIP else []):
                zr0, zi0 = spec_item(ib, 16 * rp)
                zr1, zi1 = spec_item(ib, 16 * rp + 8)
                for q in range(4):
                    i = 4 * ib + q
                    zb_s[i][z1, rp * 8:rp * 8 + 8, :] = _pack(jnp.concatenate([zr0[q], zr1[q]], axis=0))
                    zb_s[i][z1, 64 + rp * 8:64 + rp * 8 + 8, :] = _pack(jnp.concatenate([zi0[q], zi1[q]], axis=0))
                    if rp == 7:
                        inv_at.setdefault(min(max(n + 2, INV0 + i // 2), 23), []).append(i)
            for i in inv_at.get(n, []):
                rel = pltpu.bitcast(ra[0:8], u32) & zv
                zz = _unpack(zb_s[i][z0])
                ys = []
                for hh in range(2):
                    lhs = _gate(inv_ref[hh * 64:(hh + 1) * 64, :], [rel])
                    yy = jnp.dot(lhs, zz, preferred_element_type=f32)
                    rows = pl.ds(i * 128 + hh * 64, 64)
                    yy = yy + y_s[c, rows, :]
                    y_s[c, rows, :] = yy
                    ys.append(yy)
                if n + 2 < 24:
                    deps.setdefault(n + 2, []).append(_tok(jnp.concatenate(ys, axis=0), zv))
        return carry

    def phase2_body(c, nxt):
        z0 = z_ref[0]
        z1 = z_ref[1]
        zv = jnp.full((8, 128), z0, i32).astype(u32)
        h = _unpack(h_s[...])
        if nxt:
            o = load_o(c + 1)
            for n in range(8):
                oproj_tile(o, c + 1, n, z1)
        deps = {}
        for n in range(24):
            ra, done = qkv_tile(h, c, n, deps.get(n), zv)
            if done is not None and n + 3 < 24:
                deps.setdefault(n + 3, []).append(done)
            if nxt and 1 <= n < 1 + NP:
                hp = ln2_piece(c + 1, n - 1, _tick(ra, 0, z0))
                deps.setdefault(n + 3, []).append(_tok(hp, zv))

    def phase2():
        o = load_o(0)
        for n in range(8):
            oproj_tile(o, 0, n, z_ref[1])
        z0 = z_ref[0]
        for p in range(NP):
            ln2_piece(0, p, z0)

        def body(c, carry):
            phase2_body(c, True)
            return carry
        lax.fori_loop(0, (NRC - 1) * 1, lambda c, x: body(c % (NRC - 1), x), 0)
        phase2_body(NRC - 1, False)

    def phase3():
        o = load_o(0)
        for n in range(8):
            oproj_tile(o, 0, n, z_ref[1])

        def body(c, carry):
            z0 = z_ref[0]
            z1 = z_ref[1]
            o = load_o(c + 1)
            for n in range(8):
                out_piece(c, 2 * n, z0)
                out_piece(c, 2 * n + 1, z0)
                oproj_tile(o, c + 1, n, z1)
            out_copy(c).start()
            return carry
        lax.fori_loop(0, NRC - 1, body, 0)
        z0 = z_ref[0]
        for p in range(NP):
            out_piece(NRC - 1, p, z0)
        out_copy(NRC - 1).start()

    zero16 = jnp.zeros((16, 128), u32)

    def qk(g, j, hh, half, dst, z, zk=0, dep=None):
        qt = qt_s[j, pl.ds(pl.multiple_of(g * 64 + hh * 16, 16), 16), :]
        w = _unpack(jnp.concatenate([qt if i == hh else zero16 for i in range(4)], axis=0))
        m = None
        first = None
        last = None
        for c in range(4):
            r0 = half * HS + c * CH
            ku = k_s[g + zk, r0 // 2:(r0 + CH) // 2, :]
            if dep is not None:
                ku = jnp.concatenate([ku[:CH // 2 - 8], ku[CH // 2 - 8:] | dep], axis=0)
            s = jnp.dot(_unpack(ku), w, preferred_element_type=f32)
            dst[z, c * CH:(c + 1) * CH, :] = s
            mc = jnp.max(s.reshape(CH // 8, 8, 128), axis=0)
            m = mc if m is None else jnp.maximum(m, mc)
            f = pltpu.bitcast(s[0:8], u32)
            first = f if first is None else first | f
            last = s
        return m, first, last

    def fullmax(m1, m2):
        return jnp.max(jnp.maximum(m1, m2), axis=0, keepdims=True)

    def sm_pv(g, hh, half, src, m, z2, dep, trigs):
        mb = jnp.broadcast_to(m, (8, 128))
        mbu = pltpu.bitcast(mb, u32)
        ms = [mb if tr is None else pltpu.bitcast(mbu | tr, f32) for tr in trigs]
        ng = len(trigs) // 2
        gr = 128 // ng
        ps = []
        for t in range(8):
            for kk in range(ng):
                mi = ms[(t // 4) * ng + (ng - 1 - kk)]
                x = src[z2, t * 128 + kk * gr:t * 128 + (kk + 1) * gr, :]
                ps.append(jnp.exp2(x.reshape(gr // 8, 8, 128) - mi[None]).reshape(gr, 128))
        p = jnp.concatenate(ps, axis=0)
        l = _tree_sum(p)
        rs = pl.ds(pl.multiple_of(g * 64 + hh * 16, 16), 16)
        dep2 = jnp.concatenate([dep, dep], axis=0)
        vu = jnp.concatenate([vt_s[half * 8 + t, rs, :] | dep2 for t in range(8)], axis=1)
        o = jnp.dot(_unpack(vu), p.astype(bf), preferred_element_type=f32)
        return o, l

    def store_o(g, j, parts):
        outs = [parts[2 * h] * (1.0 / jnp.sum(parts[2 * h + 1], axis=0, keepdims=True)) for h in range(4)]
        ot = jnp.concatenate(outs, axis=0)
        o_s[g, pl.ds(pl.multiple_of(j * 64, 64), 64), :] = _pack(ot.T)

    def finalize(g, j, slot):
        x = fin[slot]
        parts = []
        for hh in range(4):
            parts += [x[hh * 40: hh * 40 + 32], x[hh * 40 + 32: hh * 40 + 40]]
        store_o(g, j, parts)

    def attention():
        ma = fullmax(qk(0, 0, 0, 0, a1, 0)[0], qk(0, 0, 0, 1, a2, 0)[0])
        mb1 = qk(0, 0, 1, 0, b1, 0)[0]
        bufs = {(0, 0): a1, (0, 1): a2, (1, 0): b1, (1, 1): b2}

        def body(it, carry):
            ma, mb1 = carry
            z1 = z_ref[0]
            z2 = z_ref[1]
            zv = jnp.full((8, 128), z1, i32).astype(u32)
            tp = jnp.maximum(it * UNR - 1, 0)
            finalize(tp // NQ, tp % NQ, z2)
            do = None
            ps = None
            po = None

            def tg(sv, i):
                return None if sv is None else pltpu.bitcast(sv[i * 8:i * 8 + 8], u32) & zv

            for u in range(UNR):
                zk = [z_ref[2 + 8 * u + i] for i in range(8)]
                t = it * UNR + u
                g = t // NQ
                j = t % NQ
                tn = jnp.minimum(t + 1, G * NQ - 1)
                gn = tn // NQ
                jn = tn % NQ
                qks = [(g, j, 1, 1), (g, j, 2, 0), (g, j, 2, 1), (g, j, 3, 0), (g, j, 3, 1),
                       (gn, jn, 0, 0), (gn, jn, 0, 1), (gn, jn, 1, 0)]
                mfull = {0: ma}
                mpart = {1: mb1}
                os_, ls_ = {}, {}
                for n in range(8):
                    qg, qj, qh, qhalf = qks[n]
                    key = qh if n < 5 else qh + 4
                    mp, first, cs_ = qk(qg, qj, qh, qhalf, bufs[(qh % 2, qhalf)], z1, zk[n], do)
                    if qhalf == 0:
                        mpart[key] = mp
                    else:
                        mfull[key] = fullmax(mpart[key], mp)
                    ph, phalf = n // 2, n % 2
                    trigs = [tg(ps, i) for i in TA] + [tg(po, TB[0])] + [tg(cs_, i) for i in TB[1:]]
                    o, l = sm_pv(g, ph, phalf, bufs[(ph % 2, phalf)], mfull[ph], z2, first & zv, trigs)
                    ps = cs_
                    po = o
                    do = tg(o, 3)
                    os_[(ph, phalf)] = o
                    ls_[(ph, phalf)] = l
                ma = mfull[4]
                mb1 = mpart[5]
                parts = []
                for h in range(4):
                    parts += [os_[(h, 0)] + os_[(h, 1)], ls_[(h, 0)] + ls_[(h, 1)]]
                if u == UNR - 1:
                    fin[z1] = jnp.concatenate(parts, axis=0)
                else:
                    store_o(g, j, parts)
            return ma, mb1

        lax.fori_loop(0, G * NQ // UNR, body, (ma, mb1))
        finalize(G - 1, NQ - 1, 0)

    x_copy(0).wait()
    for p in range(NP):
        ln1_piece(0, p, 0)
    for cp in kv_copies(0):
        cp.wait()
    for j in range(NC):
        kv_item(0, 0, j, z_ref[0])
    if not MIDW:
        for c in range(3):
            w_copy(c).wait()
    if '1' not in ONLY or 'w' in ONLY:
        h_copy(0).wait()
        for c in range(1, G):
            x_copy(c).wait()
            for cp in kv_copies(c):
                cp.wait()
            h_copy(c).wait()
    if '1' in ONLY:
        lax.fori_loop(0, NRC * 1, lambda c, x: phase1(c % NRC, x), 0)
    if 'a' in ONLY:
        attention()
    wo_copy().wait()
    if '2' in ONLY:
        phase2()
    if 'a' in ONLY:
        attention()
    if '3' in ONLY:
        phase3()
    else:
        for c in range(NRC):
            out_copy(c).start()
    for c in range(NRC):
        out_copy(c).wait()


@jax.jit
def pallas_interleave_layers__softmax_full_mha__ssm_conv_h3__prompt_kernel(A_x, A_wqkv, A_wo, B_q, B_k, B_v, B_shift_k, B_ssm_k, B_ssm_D):
    fwd, inv = _dft_mats()
    fwd = jnp.asarray(fwd, dtype=bf)
    inv = jnp.asarray(inv, dtype=bf)
    scratch = [
        pltpu.VMEM((1, S, D), f32),
        pltpu.VMEM((G + 1, S, 128), f32),
        pltpu.VMEM((NQ, D // 2, 128), u32),
        pltpu.VMEM((G, S // 2, 128), u32),
        pltpu.VMEM((NQ, D // 2, 128), u32),
        pltpu.VMEM((G, S // 2, 128), u32),
        pltpu.VMEM((1, HS, 128), f32), pltpu.VMEM((1, HS, 128), f32),
        pltpu.VMEM((1, HS, 128), f32), pltpu.VMEM((1, HS, 128), f32),
        pltpu.VMEM((1, 160, 128), f32),
        pltpu.VMEM((1, S + 8, 128), f32),
        pltpu.VMEM((S // 2, 128), u32),
        pltpu.VMEM((G, 8, 128), f32),
        pltpu.VMEM((1, 2 * NC * CS + 32, 128), f32),
        pltpu.VMEM((1, NC * CS, 128), f32),
        [pltpu.VMEM((1, 128, 128), u32) for _ in range(NC)],
        pltpu.VMEM((RC // 2, D), u32),
        pltpu.SMEM((NZ,), i32),
        pltpu.VMEM((1, S, D), bf),
        pltpu.VMEM((D, 3 * D), bf),
        pltpu.VMEM((D, D), bf),
        pltpu.VMEM((G, S, 128), bf),
        pltpu.VMEM((G, S, 128), bf),
        pltpu.VMEM((D, S), bf),
        pltpu.VMEM((S, D), bf),
        pltpu.SemaphoreType.DMA((3, G)),
        pltpu.SemaphoreType.DMA((NRC,)),
        pltpu.SemaphoreType.DMA((4,)),
        pltpu.SemaphoreType.DMA((NRC,)),
    ]
    hbm = pl.BlockSpec(memory_space=pl.ANY)
    vm = pl.BlockSpec(memory_space=pltpu.VMEM)
    return pl.pallas_call(
        _kernel,
        out_shape=jax.ShapeDtypeStruct((1, S, D), bf),
        in_specs=[hbm, hbm, hbm, hbm, hbm, vm, hbm, vm, vm, vm],
        out_specs=hbm,
        scratch_shapes=scratch,
        compiler_params=pltpu.CompilerParams(vmem_limit_bytes=120 * 2**20),
    )(A_x, A_wqkv, A_wo, B_k, B_v, B_shift_k, B_ssm_k, B_ssm_D.reshape(1, D), fwd, inv)
```

```python
import numpy as np
import jax
import jax.numpy as jnp
from jax import lax
import jax.experimental.pallas as pl
import jax.experimental.pallas.tpu as pltpu

S = 2048
D = 1024
DH = 32
G = 8
NQ = 16
HS = S // 2
CH = HS // 4
UNR = 4
TA = (17, 21, 25, 29)
TB = (0, 0, 4, 8)
RC = 256
NRC = S // RC
NP = RC // 16
NC = 16
EPS = 1e-5
ORD = 1
NOBC = 1
TAILG = 1
CHAIN = 1
CTICK = 0
SKIP = ''
IM = 136
CS = 416
GO = 16 * 416 + 24
LAZY = 1
ONLY = '1a23'
RG = 2
SPAN0 = 8
SPAN_TILES = 16
INV0 = 14
KV0 = 6
NZ = 2 + 8 * UNR
QSCALE = float(DH ** -0.5 * np.log2(np.e))

bf = jnp.bfloat16
f32 = jnp.float32
u32 = jnp.uint32
i32 = jnp.int32
NT = (((1,), (1,)), ((), ()))


def _dft_mats():
    n = np.arange(128)
    f = np.concatenate([np.arange(0, 128, 2), np.arange(1, 128, 2)])
    ang = 2.0 * np.pi * np.outer(f + 0.5, n) / 256.0
    fwd = np.concatenate([np.cos(ang), -np.sin(ang)], axis=0)
    inv = fwd.T / 128.0
    re, im = fwd[0:128], fwd[128:256]
    fwd = np.concatenate([im, re, im - re, im + re], axis=0)

    def pack_rows(a):
        u = np.ascontiguousarray(a, dtype=np.float32).view(np.uint32)
        u = (u + 0x7FFF + ((u >> 16) & 1)) >> 16
        return (u[0::2] | (u[1::2] << 16)).astype(np.uint32)
    return pack_rows(fwd), pack_rows(inv)


def _tree_sum(p):
    n = p.shape[0] // 8
    x = p.reshape(n, 8, 128)
    while n > 1:
        x = x.reshape(n // 2, 2, 8, 128)
        x = x[:, 0] + x[:, 1]
        n //= 2
    return x[0]


def _ln(x):
    m = jnp.mean(x, axis=-1, keepdims=True)
    xc = x - m
    v = jnp.mean(xc * xc, axis=-1, keepdims=True)
    return xc * lax.rsqrt(v + EPS)


def _pack(x):
    return pltpu.bitcast(x.astype(bf), u32)


def _unpack(x):
    return pltpu.bitcast(x, bf)


def _tok(v, zv):
    v = v if v.dtype == u32 else pltpu.bitcast(v, u32)
    acc = None
    for r in range(v.shape[0] // 8):
        for c in range(v.shape[1] // 128):
            p = v[r * 8:(r + 1) * 8, c * 128:(c + 1) * 128]
            acc = p if acc is None else acc | p
    return acc & zv


def _gate(w, toks):
    if not toks:
        return w
    wu = pltpu.bitcast(w, u32)
    h0 = wu[0:8]
    for t in toks:
        h0 = h0 | jnp.tile(t, (1, wu.shape[1] // 128))
    return _unpack(jnp.concatenate([h0, wu[8:]], axis=0))


def _tick(v, k, z0):
    return pltpu.bitcast(v[8 * k:8 * k + 8, 0:128], i32)[0, 0] & z0


def _kernel(x_hbm, wqkv_hbm, wo_hbm, bk_hbm, bv_hbm, shk_hbm, ssmk_hbm, ssmd_hbm, fwd_hbm, inv_hbm, out_hbm,
            x_s, y_s, qt_s, k_s, vt_s, o_s, a1, a2, b1, b2, fin, kf_s, taps_s, ug_a, ug_b, zb_a, zb_b, pb_a, pb_b,
            h_s, z_ref, x_in, wqkv, wo, bk, bv, ssmk, out_s, shk, ssmd, fwd_ref, inv_ref,
            sem_c, sem_x, sem_w, sem_o, sem_s):
    def kv_copies(cb):
        cs = pl.ds(pl.multiple_of(cb * 128, 128), 128)
        return [pltpu.make_async_copy(bk_hbm.at[0, :, cs], bk.at[cb], sem_c.at[0, cb]),
                pltpu.make_async_copy(bv_hbm.at[0, :, cs], bv.at[cb], sem_c.at[1, cb])]

    def h_copy(cb):
        cs = pl.ds(pl.multiple_of(cb * 128, 128), 128)
        return pltpu.make_async_copy(ssmk_hbm.at[cs, :], ssmk.at[cs, :], sem_c.at[2, cb])

    def x_copy(c):
        rs = pl.ds(pl.multiple_of(c * RC, RC), RC)
        return pltpu.make_async_copy(x_hbm.at[0, rs, :], x_in.at[0, rs, :], sem_x.at[c])

    def w_copy(c):
        rs = pl.ds(pl.multiple_of(c * 128, 128), 128)
        return pltpu.make_async_copy(wqkv_hbm.at[rs, :], wqkv.at[rs, :], sem_w.at[c])

    def wo_copy():
        return pltpu.make_async_copy(wo_hbm, wo, sem_w.at[G])

    def out_copy(c):
        rs = pl.ds(pl.multiple_of(c * RC, RC), RC)
        return pltpu.make_async_copy(out_s.at[rs, :], out_hbm.at[0, rs, :], sem_o.at[c])

    def conv_start(c):
        h_copy(c).start()
        for cp in kv_copies(c):
            cp.start()

    def conv_wait(c):
        h_copy(c).wait()
        for cp in kv_copies(c):
            cp.wait()

    small = [pltpu.make_async_copy(src, dst, sem_s.at[i]) for i, (src, dst) in enumerate(
        ((fwd_hbm, fwd_ref), (shk_hbm, shk), (ssmd_hbm, ssmd), (inv_hbm, inv_ref)))]
    h_copy(0).start()
    for cp in small:
        cp.start()
    for cp in kv_copies(0):
        cp.start()
    conv_start(1)

    for i in range(NZ):
        z_ref[i] = 0
    fin[...] = jnp.ones(fin.shape, f32)
    kf_s[0, 0:8, :] = jnp.zeros((8, 128), f32)
    zb_b[...] = jnp.zeros(zb_b.shape, u32)
    for cp in small:
        cp.wait()
    taps = shk[...].astype(f32)
    dall = ssmd[...].astype(f32)
    for cb in range(G):
        for t in range(4):
            taps_s[cb, 8 * t:8 * t + 8, :] = jnp.broadcast_to(taps[t:t + 1, cb * 128:(cb + 1) * 128], (8, 128))
        taps_s[cb, 32:40, :] = jnp.broadcast_to(dall[cb:cb + 1, :], (8, 128))

    TILES = [(0, n) for n in range(8)] + [(2, n) for n in range(8)] + [(1, n) for n in range(8)]

    def qkv_tile(h, c, idx, toks, zv):
        kind, n = TILES[idx]
        col = kind * D + n * 128
        wa = _gate(wqkv[0:D // 2, col:col + 128], toks)
        ra = jnp.dot(h[:, 0:D // 2], wa, preferred_element_type=f32)
        rb = jnp.dot(h[:, D // 2:D], wqkv[D // 2:D, col:col + 128], preferred_element_type=f32)
        r = ra + rb
        if kind == 1:
            r2 = pl.multiple_of(c * (RC // 2), RC // 2)
            k_s[n, pl.ds(r2, RC // 2), :] = _pack(r)
            return ra, None
        dst = qt_s if kind == 0 else vt_s
        if kind == 0:
            r = r * QSCALE
        pks = []
        for t in range(RC // 128):
            pk = _pack(r[t * 128:(t + 1) * 128, :].T)
            dst[c * (RC // 128) + t, n * 64:(n + 1) * 64, :] = pk
            pks.append(pk)
        return ra, _tok(jnp.concatenate(pks, axis=0), zv)

    def piece_rows(c, p):
        return pl.ds(pl.multiple_of(c * RC + p * 16, 16), 16)

    def ln1_piece(cn, p, zt):
        rows = piece_rows(cn, p)
        x = x_in[zt, rows, :].astype(f32)
        x_s[0, rows, :] = x
        hp = _pack(_ln(x))
        h_s[p * 8:(p + 1) * 8, :] = hp
        return hp

    def gated_x(cn, p, zt):
        rows = piece_rows(cn, p)
        x1 = x_s[zt, rows, :]
        y = jnp.concatenate([y_s[0, g, rows, :] + y_s[1, g, rows, :] for g in range(G)], axis=1)
        return x1 + _ln(x1) * y

    def ln2_piece(cn, p, zt):
        x2 = gated_x(cn, p, zt)
        x_s[zt, piece_rows(cn, p), :] = x2
        hp = _pack(_ln(x2))
        h_s[p * 8:(p + 1) * 8, :] = hp
        return hp

    def out_piece(c, p, zt):
        out_s[piece_rows(c, p), :] = gated_x(c, p, zt).astype(bf)

    zts = [pl.multiple_of((z_ref[2 + ib] & 1) * 32, 32) for ib in range(4)]

    def prep_h(cb, pb):
        cs = pl.ds(pl.multiple_of(cb * 128, 128), 128)
        for j in range(NC):
            pb[HS + j * 64:HS + (j + 1) * 64, :] = pltpu.bitcast(ssmk[cs, j * 128:(j + 1) * 128], u32)

    def prep_kv(cb, pb):
        zs = z_ref[1]
        tp = taps_s[cb]
        for j in range(NC):
            r0 = j * 128
            kf_s[zs, 8 + r0:8 + r0 + 128, :] = bk[cb, r0:r0 + 128, :].astype(f32)
            ks = None
            for t in range(4):
                term = kf_s[zs, 8 + r0 - t:8 + r0 - t + 128, :].reshape(16, 8, 128) * tp[8 * t:8 * t + 8][None]
                ks = term if ks is None else ks + term
            pb[j * 64:(j + 1) * 64, :] = _pack(ks.reshape(128, 128) * bv[cb, r0:r0 + 128, :].astype(f32))

    def fwd_h(pb, ug):
        for m in range(NC):
            hm = lax.dot_general(_unpack(fwd_ref[0, 64:256, :]),
                                 _unpack(pb[HS + m * 64:HS + (m + 1) * 64, :]), NT, preferred_element_type=f32)
            for e in range(3):
                o = GO + m * CS + e * IM
                ug[o:o + 128, :] = hm[e * 128:(e + 1) * 128]

    def fwd_u(pb, ug):
        for j in range(NC):
            u = jnp.dot(_unpack(fwd_ref[0, 0:128, :]), _unpack(pb[j * 64:(j + 1) * 64, :]),
                        preferred_element_type=f32)
            ug[j * CS:j * CS + 128, :] = u[128:256]
            ug[j * CS + IM:j * CS + IM + 128, :] = u[0:128]

    def add_skip(cb, ug):
        dv = taps_s[cb, 32:40, :][None]
        for e, sg in ((0, 1.0), (1, -1.0), (2, 1.0)):
            o = GO + e * IM
            v = ug[o:o + 128, :].reshape(16, 8, 128)
            ug[o:o + 128, :] = (v + dv if sg > 0 else v - dv).reshape(128, 128)

    def spec_item(ug, ib, r, zt):
        gc = {}
        k1 = [None] * 4
        k2 = [None] * 4
        k3 = [None] * 4
        for j in range(4 * ib + 4):
            ou = j * CS + r
            ua = ug[pl.ds(zt + ou, 8), :]
            ub = ug[pl.ds(zt + ou + IM, 8), :]
            us = ua + ub
            for q in range(4):
                m = 4 * ib + q - j
                if m < 0:
                    continue
                if m not in gc:
                    og = GO + m * CS + r
                    gc[m] = tuple(ug[pl.ds(zt + og + e * IM, 8), :] for e in range(3))
                g0, g1, g2 = gc[m]
                t1, t2, t3 = g0 * us, ua * g1, ub * g2
                k1[q] = t1 if k1[q] is None else k1[q] + t1
                k2[q] = t2 if k2[q] is None else k2[q] + t2
                k3[q] = t3 if k3[q] is None else k3[q] + t3
        return [k1[q] - k3[q] for q in range(4)], [k1[q] + k2[q] for q in range(4)]

    def overlap_add(yr, yi, prev, r):
        zr, zi = [], []
        for q in range(4):
            if prev is None:
                zr.append(yr[q])
                zi.append(yi[q])
            elif r < 64:
                zr.append(yr[q] - prev[1])
                zi.append(yi[q] + prev[0])
            else:
                zr.append(yr[q] + prev[1])
                zi.append(yi[q] - prev[0])
            prev = (yr[q], yi[q])
        return zr, zi, prev

    def conv_spec_rows(ug, zb, rp):
        p0 = p1 = None
        for ib in range(4):
            zt = zts[ib]
            zr0, zi0, p0 = overlap_add(*spec_item(ug, ib, 16 * rp, zt), p0, 16 * rp)
            zr1, zi1, p1 = overlap_add(*spec_item(ug, ib, 16 * rp + 8, zt), p1, 16 * rp)
            for q in range(4):
                o = (4 * ib + q) * 128 + rp * 8
                zb[o:o + 8, :] = _pack(jnp.concatenate([zr0[q], zr1[q]], axis=0))
                zb[o + 64:o + 72, :] = _pack(jnp.concatenate([zi0[q], zi1[q]], axis=0))

    def conv_inv(cb, zb):
        for i in range(NC):
            for e in range(2):
                y = jnp.dot(_unpack(inv_ref[0, :, e * 128:(e + 1) * 128]),
                            _unpack(zb[i * 128 + e * 64:i * 128 + (e + 1) * 64, :]), preferred_element_type=f32)
                y_s[e, cb, i * 128:(i + 1) * 128, :] = y
        return y

    def conv_main(c, ug_cur, ug_nxt, zb_cur, zb_prev, pb_nxt):
        if ORD == 1:
            for rp in range(8):
                conv_spec_rows(ug_cur, zb_cur, rp)
        if ORD == 2:
            conv_inv((c + G) % (G + 1), zb_prev)
        if pb_nxt is not None:
            fwd_h(pb_nxt, ug_nxt)
            fwd_u(pb_nxt, ug_nxt)
        if ORD != 2:
            conv_inv((c + G) % (G + 1), zb_prev)
        if ORD != 1:
            for rp in range(8):
                conv_spec_rows(ug_cur, zb_cur, rp)

    def fence(fn):
        @pl.when(z_ref[0] == 0)
        def _():
            fn()

    def conv_half(c, ug_cur, ug_nxt, zb_cur, zb_prev, pb_nxt, pb_new):
        @pl.when(c + 3 < G)
        def _():
            conv_start(c + 3)
        w_copy(c).start()
        conv_main(c, ug_cur, ug_nxt, zb_cur, zb_prev, pb_nxt)
        fence(lambda: h_copy(c + 2).wait())
        add_skip(c + 1, ug_nxt)
        prep_h(c + 2, pb_new)
        for cp in kv_copies(c + 2):
            cp.wait()
        prep_kv(c + 2, pb_new)

        @pl.when(c >= 1)
        def _():
            w_copy(c - 1).wait()

    def conv():
        h_copy(0).wait()
        prep_h(0, pb_a)
        fwd_h(pb_a, ug_a)
        for cp in kv_copies(0):
            cp.wait()
        conv_start(2)
        add_skip(0, ug_a)
        prep_kv(0, pb_a)
        fwd_u(pb_a, ug_a)
        conv_wait(1)
        prep_h(1, pb_b)
        prep_kv(1, pb_b)

        def body(p, carry):
            conv_half(2 * p, ug_a, ug_b, zb_a, zb_b, pb_b, pb_a)
            conv_half(2 * p + 1, ug_b, ug_a, zb_b, zb_a, pb_a, pb_b)
            return carry
        lax.fori_loop(0, G // 2 - 1, body, 0)
        w_copy(G - 2).start()
        w_copy(G - 1).start()
        x_copy(0).start()
        conv_main(G - 2, ug_a, ug_b, zb_a, zb_b, pb_b)
        x_copy(1).start()
        fence(lambda: w_copy(G - 3).wait())
        add_skip(G - 1, ug_b)
        fence(lambda: w_copy(G - 2).wait())
        conv_main(G - 1, ug_b, ug_a, zb_b, zb_a, None)
        fence(lambda: x_copy(0).wait())
        conv_inv(G - 1, zb_b)
        for p in range(NP):
            ln1_piece(0, p, 0)
        w_copy(G - 1).wait()

    def oproj_tile(o, cn, n, z1):
        rows = pl.ds(pl.multiple_of(cn * RC, RC), RC)
        cols = slice(n * 128, (n + 1) * 128)
        r = jnp.dot(o, wo[:, cols], preferred_element_type=f32)
        x_s[z1, rows, cols] = x_s[z1, rows, cols] + r
        return r

    def load_o(cn):
        r2 = pl.multiple_of(cn * (RC // 2), RC // 2)
        return jnp.concatenate([_unpack(o_s[g, pl.ds(r2, RC // 2), :]) for g in range(G)], axis=1)

    def phase1(c, carry):
        cn = jnp.minimum(c + 1, NRC - 1)

        @pl.when(c + 1 < NRC)
        def _():
            x_copy(c + 1).wait()

        @pl.when(c + 2 < NRC)
        def _():
            x_copy(c + 2).start()

        @pl.when(c + 2 == NRC)
        def _():
            wo_copy().start()
        z0 = z_ref[0]
        zv = jnp.full((8, 128), z0, i32).astype(u32)
        h = _unpack(h_s[...])
        deps = {}
        for n in range(24):
            ra, done = qkv_tile(h, c, n, deps.get(n), zv)
            if done is not None and n + 3 < 24:
                deps.setdefault(n + 3, []).append(done)
            if 2 <= n < 2 + NP:
                hp = ln1_piece(cn, n - 2, _tick(ra, 16, z0))
                deps.setdefault(n + 3, []).append(_tok(hp, zv))
        return carry

    def phase2_body(c, nxt):
        z0 = z_ref[0]
        z1 = z_ref[1]
        zv = jnp.full((8, 128), z0, i32).astype(u32)
        h = _unpack(h_s[...])
        if nxt:
            o = load_o(c + 1)
            for n in range(8):
                oproj_tile(o, c + 1, n, z1)
        deps = {}
        for n in range(24):
            ra, done = qkv_tile(h, c, n, deps.get(n), zv)
            if done is not None and n + 3 < 24:
                deps.setdefault(n + 3, []).append(done)
            if nxt and 1 <= n < 1 + NP:
                hp = ln2_piece(c + 1, n - 1, _tick(ra, 0, z0))
                deps.setdefault(n + 3, []).append(_tok(hp, zv))

    def phase2():
        o = load_o(0)
        for n in range(8):
            oproj_tile(o, 0, n, z_ref[1])
        z0 = z_ref[0]
        for p in range(NP):
            ln2_piece(0, p, z0)

        def body(c, carry):
            phase2_body(c, True)
            return carry
        lax.fori_loop(0, (NRC - 1) * 1, lambda c, x: body(c % (NRC - 1), x), 0)
        phase2_body(NRC - 1, False)

    def phase3():
        o = load_o(0)
        for n in range(8):
            oproj_tile(o, 0, n, z_ref[1])

        def body(c, carry):
            z0 = z_ref[0]
            z1 = z_ref[1]
            o = load_o(c + 1)
            for n in range(8):
                out_piece(c, 2 * n, z0)
                out_piece(c, 2 * n + 1, z0)
                oproj_tile(o, c + 1, n, z1)
            out_copy(c).start()
            return carry
        lax.fori_loop(0, NRC - 1, body, 0)
        z0 = z_ref[0]
        for p in range(NP):
            out_piece(NRC - 1, p, z0)
        out_copy(NRC - 1).start()

    zero16 = jnp.zeros((16, 128), u32)

    def qk(g, j, hh, half, dst, z, zk=0, dep=None):
        qt = qt_s[j, pl.ds(pl.multiple_of(g * 64 + hh * 16, 16), 16), :]
        w = _unpack(jnp.concatenate([qt if i == hh else zero16 for i in range(4)], axis=0))
        m = None
        first = None
        last = None
        for c in range(4):
            r0 = half * HS + c * CH
            ku = k_s[g + zk, r0 // 2:(r0 + CH) // 2, :]
            if dep is not None:
                ku = jnp.concatenate([ku[:CH // 2 - 8], ku[CH // 2 - 8:] | dep], axis=0)
            s = jnp.dot(_unpack(ku), w, preferred_element_type=f32)
            dst[z, c * CH:(c + 1) * CH, :] = s
            mc = jnp.max(s.reshape(CH // 8, 8, 128), axis=0)
            m = mc if m is None else jnp.maximum(m, mc)
            f = pltpu.bitcast(s[0:8], u32)
            first = f if first is None else first | f
            last = s
        return m, first, last

    def fullmax(m1, m2):
        return jnp.max(jnp.maximum(m1, m2), axis=0, keepdims=True)

    def sm_pv(g, hh, half, src, m, z2, dep, trigs):
        mb = jnp.broadcast_to(m, (8, 128))
        mbu = pltpu.bitcast(mb, u32)
        ms = [mb if tr is None else pltpu.bitcast(mbu | tr, f32) for tr in trigs]
        ng = len(trigs) // 2
        gr = 128 // ng
        ps = []
        for t in range(8):
            for kk in range(ng):
                mi = ms[(t // 4) * ng + (ng - 1 - kk)]
                x = src[z2, t * 128 + kk * gr:t * 128 + (kk + 1) * gr, :]
                ps.append(jnp.exp2(x.reshape(gr // 8, 8, 128) - mi[None]).reshape(gr, 128))
        p = jnp.concatenate(ps, axis=0)
        l = _tree_sum(p)
        rs = pl.ds(pl.multiple_of(g * 64 + hh * 16, 16), 16)
        dep2 = jnp.concatenate([dep, dep], axis=0)
        vu = jnp.concatenate([vt_s[half * 8 + t, rs, :] | dep2 for t in range(8)], axis=1)
        o = jnp.dot(_unpack(vu), p.astype(bf), preferred_element_type=f32)
        return o, l

    def store_o(g, j, parts):
        outs = [parts[2 * h] * (1.0 / jnp.sum(parts[2 * h + 1], axis=0, keepdims=True)) for h in range(4)]
        ot = jnp.concatenate(outs, axis=0)
        o_s[g, pl.ds(pl.multiple_of(j * 64, 64), 64), :] = _pack(ot.T)

    def finalize(g, j, slot):
        x = fin[slot]
        parts = []
        for hh in range(4):
            parts += [x[hh * 40: hh * 40 + 32], x[hh * 40 + 32: hh * 40 + 40]]
        store_o(g, j, parts)

    def attention():
        ma = fullmax(qk(0, 0, 0, 0, a1, 0)[0], qk(0, 0, 0, 1, a2, 0)[0])
        mb1 = qk(0, 0, 1, 0, b1, 0)[0]
        bufs = {(0, 0): a1, (0, 1): a2, (1, 0): b1, (1, 1): b2}

        def body(it, carry):
            ma, mb1 = carry
            z1 = z_ref[0]
            z2 = z_ref[1]
            zv = jnp.full((8, 128), z1, i32).astype(u32)
            tp = jnp.maximum(it * UNR - 1, 0)
            finalize(tp // NQ, tp % NQ, z2)
            do = None
            ps = None
            po = None

            def tg(sv, i):
                return None if sv is None else pltpu.bitcast(sv[i * 8:i * 8 + 8], u32) & zv

            for u in range(UNR):
                zk = [z_ref[2 + 8 * u + i] for i in range(8)]
                t = it * UNR + u
                g = t // NQ
                j = t % NQ
                tn = jnp.minimum(t + 1, G * NQ - 1)
                gn = tn // NQ
                jn = tn % NQ
                qks = [(g, j, 1, 1), (g, j, 2, 0), (g, j, 2, 1), (g, j, 3, 0), (g, j, 3, 1),
                       (gn, jn, 0, 0), (gn, jn, 0, 1), (gn, jn, 1, 0)]
                mfull = {0: ma}
                mpart = {1: mb1}
                os_, ls_ = {}, {}
                for n in range(8):
                    qg, qj, qh, qhalf = qks[n]
                    key = qh if n < 5 else qh + 4
                    mp, first, cs_ = qk(qg, qj, qh, qhalf, bufs[(qh % 2, qhalf)], z1, zk[n], do)
                    if qhalf == 0:
                        mpart[key] = mp
                    else:
                        mfull[key] = fullmax(mpart[key], mp)
                    ph, phalf = n // 2, n % 2
                    trigs = [tg(ps, i) for i in TA] + [tg(po, TB[0])] + [tg(cs_, i) for i in TB[1:]]
                    o, l = sm_pv(g, ph, phalf, bufs[(ph % 2, phalf)], mfull[ph], z2, first & zv, trigs)
                    ps = cs_
                    po = o
                    do = tg(o, 3)
                    os_[(ph, phalf)] = o
                    ls_[(ph, phalf)] = l
                ma = mfull[4]
                mb1 = mpart[5]
                parts = []
                for h in range(4):
                    parts += [os_[(h, 0)] + os_[(h, 1)], ls_[(h, 0)] + ls_[(h, 1)]]
                if u == UNR - 1:
                    fin[z1] = jnp.concatenate(parts, axis=0)
                else:
                    store_o(g, j, parts)
            return ma, mb1

        lax.fori_loop(0, G * NQ // UNR * 1, lambda i, c: body(i % (G * NQ // UNR), c), (ma, mb1))
        finalize(G - 1, NQ - 1, 0)

    conv()
    if '1' in ONLY:
        lax.fori_loop(0, NRC, phase1, 0)
    else:
        x_copy(1).wait()
        wo_copy().start()
    if 'a' in ONLY:
        attention()
    wo_copy().wait()
    if '2' in ONLY:
        phase2()
    if 'a' in ONLY:
        attention()
    if '3' in ONLY:
        phase3()
    else:
        out_s[0:8, 0:128] = (y_s[0, 7, 0:8, :] + y_s[1, 7, 0:8, :] + pltpu.bitcast(h_s[0:8, 0:128], f32)).astype(bf)
        for c in range(NRC):
            out_copy(c).start()
    for c in range(NRC):
        out_copy(c).wait()


@jax.jit
def pallas_interleave_layers__softmax_full_mha__ssm_conv_h3__prompt_kernel(A_x, A_wqkv, A_wo, B_q, B_k, B_v, B_shift_k, B_ssm_k, B_ssm_D):
    fwd, inv = _dft_mats()
    fwd = jnp.asarray(fwd[None])
    inv = jnp.asarray(inv[None])
    scratch = [
        pltpu.VMEM((1, S, D), f32),
        pltpu.VMEM((2, G + 1, S, 128), f32),
        pltpu.VMEM((NQ, D // 2, 128), u32),
        pltpu.VMEM((G, S // 2, 128), u32),
        pltpu.VMEM((NQ, D // 2, 128), u32),
        pltpu.VMEM((G, S // 2, 128), u32),
        pltpu.VMEM((1, HS, 128), f32), pltpu.VMEM((1, HS, 128), f32),
        pltpu.VMEM((1, HS, 128), f32), pltpu.VMEM((1, HS, 128), f32),
        pltpu.VMEM((1, 160, 128), f32),
        pltpu.VMEM((1, S + 8, 128), f32),
        pltpu.VMEM((G, 40, 128), f32),
        pltpu.VMEM((2 * NC * CS + 64, 128), f32),
        pltpu.VMEM((2 * NC * CS + 64, 128), f32),
        pltpu.VMEM((NC * 128, 128), u32),
        pltpu.VMEM((NC * 128, 128), u32),
        pltpu.VMEM((S, 128), u32),
        pltpu.VMEM((S, 128), u32),
        pltpu.VMEM((RC // 2, D), u32),
        pltpu.SMEM((NZ,), i32),
        pltpu.VMEM((1, S, D), bf),
        pltpu.VMEM((D, 3 * D), bf),
        pltpu.VMEM((D, D), bf),
        pltpu.VMEM((G, S, 128), bf),
        pltpu.VMEM((G, S, 128), bf),
        pltpu.VMEM((D, S), bf),
        pltpu.VMEM((S, D), bf),
        pltpu.VMEM((4, D), bf),
        pltpu.VMEM((G, 128), bf),
        pltpu.VMEM((1, 256, 128), u32),
        pltpu.VMEM((1, 64, 256), u32),
        pltpu.SemaphoreType.DMA((3, G)),
        pltpu.SemaphoreType.DMA((NRC,)),
        pltpu.SemaphoreType.DMA((G + 1,)),
        pltpu.SemaphoreType.DMA((NRC,)),
        pltpu.SemaphoreType.DMA((4,)),
    ]
    hbm = pl.BlockSpec(memory_space=pl.ANY)
    return pl.pallas_call(
        _kernel,
        out_shape=jax.ShapeDtypeStruct((1, S, D), bf),
        in_specs=[hbm] * 10,
        out_specs=hbm,
        scratch_shapes=scratch,
        compiler_params=pltpu.CompilerParams(vmem_limit_bytes=120 * 2**20, disable_bounds_checks=bool(NOBC)),
    )(A_x, A_wqkv, A_wo, B_k, B_v, B_shift_k.T, B_ssm_k, B_ssm_D.reshape(G, 128), fwd, inv)
```

```python
import numpy as np
import jax
import jax.numpy as jnp
from jax import lax
import jax.experimental.pallas as pl
import jax.experimental.pallas.tpu as pltpu

S = 2048
D = 1024
DH = 32
G = 8
NQ = 16
HS = S // 2
CH = HS // 4
UNR = 4
TA = (17, 21, 25, 29)
TB = (0, 0, 4, 8)
RC = 256
NRC = S // RC
NP = RC // 16
NC = 16
EPS = 1e-5
DV = 1
SCOPES = 0
MERGE = 0
GIB = 3
NINV = 16
PQ = 4
P3 = [[0, 1, 2], [3, 4, 5], [6, 7], [8, 9], [10, 11], [12, 13], [14, 15], []]
ORD = 1
NOBC = 1
TAILG = 1
CHAIN = 1
CTICK = 0
SKIP = ''
IM = 136
CS = 416
GO = 16 * 416 + 24
LAZY = 1
ONLY = '1a23'
RG = 2
SPAN0 = 8
SPAN_TILES = 16
INV0 = 14
KV0 = 6
NZ = 2 + 8 * UNR
QSCALE = float(DH ** -0.5 * np.log2(np.e))

bf = jnp.bfloat16
f32 = jnp.float32
u32 = jnp.uint32
i32 = jnp.int32
NT = (((1,), (1,)), ((), ()))


def scope(name):
    import contextlib
    return jax.named_scope(name) if SCOPES else contextlib.nullcontext()


def _dft_mats():
    n = np.arange(128)
    f = np.concatenate([np.arange(0, 128, 2), np.arange(1, 128, 2)])
    ang = 2.0 * np.pi * np.outer(f + 0.5, n) / 256.0
    fwd = np.concatenate([np.cos(ang), -np.sin(ang)], axis=0)
    inv = fwd.T / 128.0
    re, im = fwd[0:128], fwd[128:256]
    fwd = np.concatenate([im, re, im - re, im + re], axis=0)

    def pack_rows(a):
        u = np.ascontiguousarray(a, dtype=np.float32).view(np.uint32)
        u = (u + 0x7FFF + ((u >> 16) & 1)) >> 16
        return (u[0::2] | (u[1::2] << 16)).astype(np.uint32)
    return pack_rows(fwd), pack_rows(inv)


def _tree_sum(p):
    n = p.shape[0] // 8
    x = p.reshape(n, 8, 128)
    while n > 1:
        x = x.reshape(n // 2, 2, 8, 128)
        x = x[:, 0] + x[:, 1]
        n //= 2
    return x[0]


def _ln(x):
    m = jnp.mean(x, axis=-1, keepdims=True)
    xc = x - m
    v = jnp.mean(xc * xc, axis=-1, keepdims=True)
    return xc * lax.rsqrt(v + EPS)


def _pack(x):
    return pltpu.bitcast(x.astype(bf), u32)


def _unpack(x):
    return pltpu.bitcast(x, bf)


def _tok(v, zv):
    v = v if v.dtype == u32 else pltpu.bitcast(v, u32)
    acc = None
    for r in range(v.shape[0] // 8):
        for c in range(v.shape[1] // 128):
            p = v[r * 8:(r + 1) * 8, c * 128:(c + 1) * 128]
            acc = p if acc is None else acc | p
    return acc & zv


def _gate(w, toks):
    if not toks:
        return w
    wu = pltpu.bitcast(w, u32)
    h0 = wu[0:8]
    for t in toks:
        h0 = h0 | jnp.tile(t, (1, wu.shape[1] // 128))
    return _unpack(jnp.concatenate([h0, wu[8:]], axis=0))


def _tick(v, k, z0):
    return pltpu.bitcast(v[8 * k:8 * k + 8, 0:128], i32)[0, 0] & z0


def _kernel(x_hbm, wqkv_hbm, wo_hbm, bk_hbm, bv_hbm, shk_hbm, ssmk_hbm, ssmd_hbm, fwd_hbm, inv_hbm, out_hbm,
            x_s, y_s, qt_s, k_s, vt_s, o_s, a1, a2, b1, b2, fin, kf_s, taps_s, ug_a, ug_b, zb_a, zb_b, pb_a, pb_b,
            h_s, z_ref, x_in, wqkv, wo, bk, bv, ssmk, out_s, shk, ssmd, fwd_ref, inv_ref,
            sem_c, sem_x, sem_w, sem_o, sem_s):
    def kv_copies(cb):
        cs = pl.ds(pl.multiple_of(cb * 128, 128), 128)
        return [pltpu.make_async_copy(bk_hbm.at[0, :, cs], bk.at[cb], sem_c.at[0, cb]),
                pltpu.make_async_copy(bv_hbm.at[0, :, cs], bv.at[cb], sem_c.at[1, cb])]

    def h_copy(cb):
        cs = pl.ds(pl.multiple_of(cb * 128, 128), 128)
        return pltpu.make_async_copy(ssmk_hbm.at[cs, :], ssmk.at[cs, :], sem_c.at[2, cb])

    def x_copy(c):
        rs = pl.ds(pl.multiple_of(c * RC, RC), RC)
        return pltpu.make_async_copy(x_hbm.at[0, rs, :], x_in.at[0, rs, :], sem_x.at[c])

    def w_copy(c):
        rs = pl.ds(pl.multiple_of(c * 128, 128), 128)
        return pltpu.make_async_copy(wqkv_hbm.at[rs, :], wqkv.at[rs, :], sem_w.at[c])

    def wo_copy():
        return pltpu.make_async_copy(wo_hbm, wo, sem_w.at[G])

    def out_copy(c):
        rs = pl.ds(pl.multiple_of(c * RC, RC), RC)
        return pltpu.make_async_copy(out_s.at[rs, :], out_hbm.at[0, rs, :], sem_o.at[c])

    def conv_start(c):
        h_copy(c).start()
        for cp in kv_copies(c):
            cp.start()

    def conv_wait(c):
        h_copy(c).wait()
        for cp in kv_copies(c):
            cp.wait()

    small = [pltpu.make_async_copy(src, dst, sem_s.at[i]) for i, (src, dst) in enumerate(
        ((shk_hbm, shk), (ssmd_hbm, ssmd), (fwd_hbm, fwd_ref), (inv_hbm, inv_ref)))]
    h_copy(0).start()
    small[2].start()
    if DV == 1:
        small[0].start()
        small[1].start()
        for cp in kv_copies(0):
            cp.start()

    for i in range(NZ):
        z_ref[i] = 0
    fin[...] = jnp.ones(fin.shape, f32)
    kf_s[0, 0:8, :] = jnp.zeros((8, 128), f32)
    zb_b[...] = jnp.zeros(zb_b.shape, u32)

    def setup_taps():
        taps = shk[...].astype(f32)
        dall = ssmd[...].astype(f32)
        for cb in range(G):
            for t in range(4):
                taps_s[cb, 8 * t:8 * t + 8, :] = jnp.broadcast_to(taps[t:t + 1, cb * 128:(cb + 1) * 128], (8, 128))
            taps_s[cb, 32:40, :] = jnp.broadcast_to(dall[cb:cb + 1, :], (8, 128))

    TILES = [(0, n) for n in range(8)] + [(2, n) for n in range(8)] + [(1, n) for n in range(8)]

    def qkv_tile(h, c, idx, toks, zv):
        kind, n = TILES[idx]
        col = kind * D + n * 128
        wa = _gate(wqkv[0:D // 2, col:col + 128], toks)
        ra = jnp.dot(h[:, 0:D // 2], wa, preferred_element_type=f32)
        rb = jnp.dot(h[:, D // 2:D], wqkv[D // 2:D, col:col + 128], preferred_element_type=f32)
        r = ra + rb
        if kind == 1:
            r2 = pl.multiple_of(c * (RC // 2), RC // 2)
            k_s[n, pl.ds(r2, RC // 2), :] = _pack(r)
            return ra, None
        dst = qt_s if kind == 0 else vt_s
        if kind == 0:
            r = r * QSCALE
        pks = []
        for t in range(RC // 128):
            pk = _pack(r[t * 128:(t + 1) * 128, :].T)
            dst[c * (RC // 128) + t, n * 64:(n + 1) * 64, :] = pk
            pks.append(pk)
        return ra, _tok(jnp.concatenate(pks, axis=0), zv)

    def piece_rows(c, p):
        return pl.ds(pl.multiple_of(c * RC + p * 16, 16), 16)

    def ln1_piece(cn, p, zt):
        rows = piece_rows(cn, p)
        x = x_in[zt, rows, :].astype(f32)
        x_s[0, rows, :] = x
        hp = _pack(_ln(x))
        h_s[p * 8:(p + 1) * 8, :] = hp
        return hp

    def gated_x(cn, p, zt):
        rows = piece_rows(cn, p)
        x1 = x_s[zt, rows, :]
        y = jnp.concatenate([y_s[0, g, rows, :] + y_s[1, g, rows, :] for g in range(G)], axis=1)
        return x1 + _ln(x1) * y

    def ln2_piece(cn, p, zt):
        x2 = gated_x(cn, p, zt)
        x_s[zt, piece_rows(cn, p), :] = x2
        hp = _pack(_ln(x2))
        h_s[p * 8:(p + 1) * 8, :] = hp
        return hp

    def out_piece(c, p, zt):
        v = gated_x(c, p, zt)
        out_s[piece_rows(c, p), :] = v.astype(bf)
        return v

    zts = [pl.multiple_of((z_ref[2 + ib] & 1) * 32, 32) for ib in range(4)]

    def prep_h(cb, pb):
        cs = pl.ds(pl.multiple_of(cb * 128, 128), 128)
        for j in range(NC):
            pb[HS + j * 64:HS + (j + 1) * 64, :] = pltpu.bitcast(ssmk[cs, j * 128:(j + 1) * 128], u32)

    def prep_kv(cb, pb, with_h=False):
        zs = z_ref[1]
        tp = taps_s[cb]
        cs = pl.ds(pl.multiple_of(cb * 128, 128), 128)
        for j in range(NC):
            r0 = j * 128
            if with_h:
                hu = pltpu.bitcast(ssmk[cs, r0:r0 + 128], u32)
                pb[HS + j * 64:HS + (j + 1) * 64, :] = hu
            kf_s[zs, 8 + r0:8 + r0 + 128, :] = bk[cb, r0:r0 + 128, :].astype(f32)
            ks = None
            for t in range(4):
                term = kf_s[zs, 8 + r0 - t:8 + r0 - t + 128, :].reshape(16, 8, 128) * tp[8 * t:8 * t + 8][None]
                ks = term if ks is None else ks + term
            kv = _pack(ks.reshape(128, 128) * bv[cb, r0:r0 + 128, :].astype(f32))
            pb[j * 64:(j + 1) * 64, :] = kv

    def fwd_h(pb, ug):
        for m in range(NC):
            hm = lax.dot_general(_unpack(fwd_ref[0, 64:256, :]),
                                 _unpack(pb[HS + m * 64:HS + (m + 1) * 64, :]), NT, preferred_element_type=f32)
            for e in range(3):
                o = GO + m * CS + e * IM
                ug[o:o + 128, :] = hm[e * 128:(e + 1) * 128]

    def fwd_u(pb, ug):
        for j in range(NC):
            u = jnp.dot(_unpack(fwd_ref[0, 0:128, :]), _unpack(pb[j * 64:(j + 1) * 64, :]),
                        preferred_element_type=f32)
            ug[j * CS:j * CS + 128, :] = u[128:256]
            ug[j * CS + IM:j * CS + IM + 128, :] = u[0:128]

    def add_skip(cb, ug):
        dv = taps_s[cb, 32:40, :][None]
        for e, sg in ((0, 1.0), (1, -1.0), (2, 1.0)):
            o = GO + e * IM
            v = ug[o:o + 128, :].reshape(16, 8, 128)
            ug[o:o + 128, :] = (v + dv if sg > 0 else v - dv).reshape(128, 128)

    def spec_item(ug, ib, r, zt):
        gc = {}
        k1 = [None] * 4
        k2 = [None] * 4
        k3 = [None] * 4
        for j in range(4 * ib + 4):
            ou = j * CS + r
            ua = ug[pl.ds(zt + ou, 8), :]
            ub = ug[pl.ds(zt + ou + IM, 8), :]
            us = ua + ub
            for q in range(4):
                m = 4 * ib + q - j
                if m < 0:
                    continue
                if m not in gc:
                    og = GO + m * CS + r
                    gc[m] = tuple(ug[pl.ds(zt + og + e * IM, 8), :] for e in range(3))
                g0, g1, g2 = gc[m]
                t1, t2, t3 = g0 * us, ua * g1, ub * g2
                k1[q] = t1 if k1[q] is None else k1[q] + t1
                k2[q] = t2 if k2[q] is None else k2[q] + t2
                k3[q] = t3 if k3[q] is None else k3[q] + t3
        return [k1[q] - k3[q] for q in range(4)], [k1[q] + k2[q] for q in range(4)]

    def overlap_add(yr, yi, prev, r):
        zr, zi = [], []
        for q in range(4):
            if prev is None:
                zr.append(yr[q])
                zi.append(yi[q])
            elif r < 64:
                zr.append(yr[q] - prev[1])
                zi.append(yi[q] + prev[0])
            else:
                zr.append(yr[q] + prev[1])
                zi.append(yi[q] - prev[0])
            prev = (yr[q], yi[q])
        return zr, zi, prev

    def conv_spec_rows(ug, zb, rp, gate=None):
        p0 = p1 = None
        for ib in range(4):
            zt = zts[ib]
            if gate is not None and ib >= GIB:
                zt = pl.multiple_of(zt + gate * 32, 32)
            zr0, zi0, p0 = overlap_add(*spec_item(ug, ib, 16 * rp, zt), p0, 16 * rp)
            zr1, zi1, p1 = overlap_add(*spec_item(ug, ib, 16 * rp + 8, zt), p1, 16 * rp)
            for q in range(4):
                o = (4 * ib + q) * 128 + rp * 8
                zb[o:o + 8, :] = _pack(jnp.concatenate([zr0[q], zr1[q]], axis=0))
                zb[o + 64:o + 72, :] = _pack(jnp.concatenate([zi0[q], zi1[q]], axis=0))

    def conv_inv(cb, zb, lo=0, hi=NC):
        for i in range(lo, hi):
            for e in range(2):
                y = jnp.dot(_unpack(inv_ref[0, :, e * 128:(e + 1) * 128]),
                            _unpack(zb[i * 128 + e * 64:i * 128 + (e + 1) * 64, :]), preferred_element_type=f32)
                y_s[e, cb, i * 128:(i + 1) * 128, :] = y
        return y

    def conv_main(c, ug_cur, ug_nxt, zb_cur, zb_prev, pb_nxt, ninv=NC):
        for rp in range(8):
            conv_spec_rows(ug_cur, zb_cur, rp)
        if pb_nxt is not None:
            fwd_h(pb_nxt, ug_nxt)
            fwd_u(pb_nxt, ug_nxt)
        conv_inv((c + G) % (G + 1), zb_prev, 0, ninv)

    def fence(fn):
        @pl.when(z_ref[0] == 0)
        def _():
            fn()

    def conv_half(c, ug_cur, ug_nxt, zb_cur, zb_prev, pb_nxt, pb_new):
        @pl.when(c + 3 < G)
        def _():
            conv_start(c + 3)
        w_copy(c).start()
        if MERGE == 0:
            conv_main(c, ug_cur, ug_nxt, zb_cur, zb_prev, pb_nxt, NINV)
            fence(lambda: h_copy(c + 2).wait())
            for cp in kv_copies(c + 2):
                cp.wait()
            prep_kv(c + 2, pb_new, True)
            add_skip(c + 1, ug_nxt)
        elif MERGE == 1:
            conv_main(c, ug_cur, ug_nxt, zb_cur, zb_prev, pb_nxt, NINV)
            conv_wait(c + 2)
            prep_kv(c + 2, pb_new, True)
            add_skip(c + 1, ug_nxt)
        else:
            for rp in range(8):
                conv_spec_rows(ug_cur, zb_cur, rp)
            conv_wait(c + 2)
            prep_kv(c + 2, pb_new, True)
            fwd_h(pb_nxt, ug_nxt)
            fwd_u(pb_nxt, ug_nxt)
            conv_inv((c + G) % (G + 1), zb_prev)
            add_skip(c + 1, ug_nxt)

        @pl.when(c >= 1)
        def _():
            w_copy(c - 1).wait()

    def conv():
        with scope("s_w0"):
            small[2].wait()
            h_copy(0).wait()
        if DV == 2:
            for cp in kv_copies(0):
                cp.start()
            small[0].start()
            small[1].start()
        conv_start(1)
        small[3].start()
        with scope("s_h0"):
            prep_h(0, pb_a)
            fwd_h(pb_a, ug_a)
        with scope("s_w1"):
            small[0].wait()
            small[1].wait()
            for cp in kv_copies(0):
                cp.wait()
        conv_start(2)
        setup_taps()
        add_skip(0, ug_a)
        prep_kv(0, pb_a)
        fwd_u(pb_a, ug_a)
        with scope("s_w2"):
            conv_wait(1)
            small[3].wait()
        prep_kv(1, pb_b, True)

        def body(p, carry):
            conv_half(2 * p, ug_a, ug_b, zb_a, zb_b, pb_b, pb_a)
            conv_half(2 * p + 1, ug_b, ug_a, zb_b, zb_a, pb_a, pb_b)
            return carry
        lax.fori_loop(0, G // 2 - 1, body, 0)
        w_copy(G - 2).start()
        w_copy(G - 1).start()
        x_copy(0).start()
        conv_main(G - 2, ug_a, ug_b, zb_a, zb_b, pb_b)
        x_copy(1).start()
        fence(lambda: w_copy(G - 3).wait())
        add_skip(G - 1, ug_b)
        fence(lambda: w_copy(G - 2).wait())
        conv_main(G - 1, ug_b, ug_a, zb_b, zb_a, None)
        fence(lambda: x_copy(0).wait())
        conv_inv(G - 1, zb_b)
        for p in range(NP):
            ln1_piece(0, p, 0)
        w_copy(G - 1).wait()

    def oproj_tile(o, cn, n, z1, toks=None, r0=0, nr=RC):
        rows = pl.ds(pl.multiple_of(cn * RC + r0, nr), nr)
        cols = slice(n * 128, (n + 1) * 128)
        r = jnp.dot(o[r0:r0 + nr], _gate(wo[:, cols], toks), preferred_element_type=f32)
        x_s[z1, rows, cols] = x_s[z1, rows, cols] + r
        return r

    def load_o(cn):
        r2 = pl.multiple_of(cn * (RC // 2), RC // 2)
        return jnp.concatenate([_unpack(o_s[g, pl.ds(r2, RC // 2), :]) for g in range(G)], axis=1)

    def phase1(c, carry):
        cn = jnp.minimum(c + 1, NRC - 1)

        @pl.when(c + 1 < NRC)
        def _():
            x_copy(c + 1).wait()

        @pl.when(c + 2 < NRC)
        def _():
            x_copy(c + 2).start()

        @pl.when(c + 2 == NRC)
        def _():
            wo_copy().start()
        z0 = z_ref[0]
        zv = jnp.full((8, 128), z0, i32).astype(u32)
        h = _unpack(h_s[...])
        deps = {}
        for n in range(24):
            ra, done = qkv_tile(h, c, n, deps.get(n), zv)
            if done is not None and n + 3 < 24:
                deps.setdefault(n + 3, []).append(done)
            if 2 <= n < 2 + NP:
                hp = ln1_piece(cn, n - 2, _tick(ra, 16, z0))
                deps.setdefault(n + 3, []).append(_tok(hp, zv))
        return carry

    def phase2_body(c, nxt):
        z0 = z_ref[0]
        z1 = z_ref[1]
        zv = jnp.full((8, 128), z0, i32).astype(u32)
        h = _unpack(h_s[...])
        if nxt:
            o = load_o(c + 1)
            for n in range(8):
                oproj_tile(o, c + 1, n, z1)
        deps = {}
        for n in range(24):
            ra, done = qkv_tile(h, c, n, deps.get(n), zv)
            if done is not None and n + 3 < 24:
                deps.setdefault(n + 3, []).append(done)
            if nxt and 1 <= n < 1 + NP:
                hp = ln2_piece(c + 1, n - 1, _tick(ra, 0, z0))
                deps.setdefault(n + 3, []).append(_tok(hp, zv))

    def phase2():
        o = load_o(0)
        z0 = z_ref[0]
        nq = RC // PQ
        for q in range(PQ):
            for n in range(8):
                oproj_tile(o, 0, n, z0, None, q * nq, nq)
            for p in range(q * NP // PQ, (q + 1) * NP // PQ):
                ln2_piece(0, p, z0)

        def body(c, carry):
            phase2_body(c, True)
            return carry
        lax.fori_loop(0, (NRC - 1) * 1, lambda c, x: body(c % (NRC - 1), x), 0)
        phase2_body(NRC - 1, False)

    def phase3():
        o = load_o(0)
        for n in range(8):
            oproj_tile(o, 0, n, z_ref[1])

        def body(c, carry):
            z0 = z_ref[0]
            z1 = z_ref[1]
            zv = jnp.full((8, 128), z0, i32).astype(u32)
            o = load_o(c + 1)
            deps = {}
            for n in range(8):
                for p in P3[n]:
                    deps.setdefault(n + 1, []).append(_tok(out_piece(c, p, z0), zv))
                oproj_tile(o, c + 1, n, z1, deps.get(n))
            out_copy(c).start()
            return carry
        lax.fori_loop(0, NRC - 1, body, 0)
        z0 = z_ref[0]
        for p in range(NP):
            out_piece(NRC - 1, p, z0)
        out_copy(NRC - 1).start()

    zero16 = jnp.zeros((16, 128), u32)

    def qk(g, j, hh, half, dst, z, zk=0, dep=None):
        qt = qt_s[j, pl.ds(pl.multiple_of(g * 64 + hh * 16, 16), 16), :]
        w = _unpack(jnp.concatenate([qt if i == hh else zero16 for i in range(4)], axis=0))
        m = None
        first = None
        last = None
        for c in range(4):
            r0 = half * HS + c * CH
            ku = k_s[g + zk, r0 // 2:(r0 + CH) // 2, :]
            if dep is not None:
                ku = jnp.concatenate([ku[:CH // 2 - 8], ku[CH // 2 - 8:] | dep], axis=0)
            s = jnp.dot(_unpack(ku), w, preferred_element_type=f32)
            dst[z, c * CH:(c + 1) * CH, :] = s
            mc = jnp.max(s.reshape(CH // 8, 8, 128), axis=0)
            m = mc if m is None else jnp.maximum(m, mc)
            f = pltpu.bitcast(s[0:8], u32)
            first = f if first is None else first | f
            last = s
        return m, first, last

    def fullmax(m1, m2):
        return jnp.max(jnp.maximum(m1, m2), axis=0, keepdims=True)

    def sm_pv(g, hh, half, src, m, z2, dep, trigs):
        mb = jnp.broadcast_to(m, (8, 128))
        mbu = pltpu.bitcast(mb, u32)
        ms = [mb if tr is None else pltpu.bitcast(mbu | tr, f32) for tr in trigs]
        ng = len(trigs) // 2
        gr = 128 // ng
        ps = []
        for t in range(8):
            for kk in range(ng):
                mi = ms[(t // 4) * ng + (ng - 1 - kk)]
                x = src[z2, t * 128 + kk * gr:t * 128 + (kk + 1) * gr, :]
                ps.append(jnp.exp2(x.reshape(gr // 8, 8, 128) - mi[None]).reshape(gr, 128))
        p = jnp.concatenate(ps, axis=0)
        l = _tree_sum(p)
        rs = pl.ds(pl.multiple_of(g * 64 + hh * 16, 16), 16)
        dep2 = jnp.concatenate([dep, dep], axis=0)
        vu = jnp.concatenate([vt_s[half * 8 + t, rs, :] | dep2 for t in range(8)], axis=1)
        o = jnp.dot(_unpack(vu), p.astype(bf), preferred_element_type=f32)
        return o, l

    def store_o(g, j, parts):
        outs = [parts[2 * h] * (1.0 / jnp.sum(parts[2 * h + 1], axis=0, keepdims=True)) for h in range(4)]
        ot = jnp.concatenate(outs, axis=0)
        o_s[g, pl.ds(pl.multiple_of(j * 64, 64), 64), :] = _pack(ot.T)

    def finalize(g, j, slot):
        x = fin[slot]
        parts = []
        for hh in range(4):
            parts += [x[hh * 40: hh * 40 + 32], x[hh * 40 + 32: hh * 40 + 40]]
        store_o(g, j, parts)

    def attention():
        ma = fullmax(qk(0, 0, 0, 0, a1, 0)[0], qk(0, 0, 0, 1, a2, 0)[0])
        mb1 = qk(0, 0, 1, 0, b1, 0)[0]
        bufs = {(0, 0): a1, (0, 1): a2, (1, 0): b1, (1, 1): b2}

        def body(it, carry):
            ma, mb1 = carry
            z1 = z_ref[0]
            z2 = z_ref[1]
            zv = jnp.full((8, 128), z1, i32).astype(u32)
            tp = jnp.maximum(it * UNR - 1, 0)
            finalize(tp // NQ, tp % NQ, z2)
            do = None
            ps = None
            po = None

            def tg(sv, i):
                return None if sv is None else pltpu.bitcast(sv[i * 8:i * 8 + 8], u32) & zv

            for u in range(UNR):
                zk = [z_ref[2 + 8 * u + i] for i in range(8)]
                t = it * UNR + u
                g = t // NQ
                j = t % NQ
                tn = jnp.minimum(t + 1, G * NQ - 1)
                gn = tn // NQ
                jn = tn % NQ
                qks = [(g, j, 1, 1), (g, j, 2, 0), (g, j, 2, 1), (g, j, 3, 0), (g, j, 3, 1),
                       (gn, jn, 0, 0), (gn, jn, 0, 1), (gn, jn, 1, 0)]
                mfull = {0: ma}
                mpart = {1: mb1}
                os_, ls_ = {}, {}
                for n in range(8):
                    qg, qj, qh, qhalf = qks[n]
                    key = qh if n < 5 else qh + 4
                    mp, first, cs_ = qk(qg, qj, qh, qhalf, bufs[(qh % 2, qhalf)], z1, zk[n], do)
                    if qhalf == 0:
                        mpart[key] = mp
                    else:
                        mfull[key] = fullmax(mpart[key], mp)
                    ph, phalf = n // 2, n % 2
                    trigs = [tg(ps, i) for i in TA] + [tg(po, TB[0])] + [tg(cs_, i) for i in TB[1:]]
                    o, l = sm_pv(g, ph, phalf, bufs[(ph % 2, phalf)], mfull[ph], z2, first & zv, trigs)
                    ps = cs_
                    po = o
                    do = tg(o, 3)
                    os_[(ph, phalf)] = o
                    ls_[(ph, phalf)] = l
                ma = mfull[4]
                mb1 = mpart[5]
                parts = []
                for h in range(4):
                    parts += [os_[(h, 0)] + os_[(h, 1)], ls_[(h, 0)] + ls_[(h, 1)]]
                if u == UNR - 1:
                    fin[z1] = jnp.concatenate(parts, axis=0)
                else:
                    store_o(g, j, parts)
            return ma, mb1

        lax.fori_loop(0, G * NQ // UNR * 1, lambda i, c: body(i % (G * NQ // UNR), c), (ma, mb1))
        finalize(G - 1, NQ - 1, 0)

    with scope('S_conv'):
        conv()
    if '1' in ONLY:
        with scope('S_ph1'):
            lax.fori_loop(0, NRC, phase1, 0)
    else:
        x_copy(1).wait()
        wo_copy().start()
    wo_copy().wait()
    if 'a' in ONLY:
        with scope('S_att1'):
            attention()
    if '2' in ONLY:
        with scope('S_ph2'):
            phase2()
    if 'a' in ONLY:
        with scope('S_att2'):
            attention()
    if '3' in ONLY:
        with scope('S_ph3'):
            phase3()
    else:
        out_s[0:8, 0:128] = (y_s[0, 7, 0:8, :] + y_s[1, 7, 0:8, :] + pltpu.bitcast(h_s[0:8, 0:128], f32)).astype(bf)
        for c in range(NRC):
            out_copy(c).start()
    for c in range(NRC):
        out_copy(c).wait()


@jax.jit
def pallas_interleave_layers__softmax_full_mha__ssm_conv_h3__prompt_kernel(A_x, A_wqkv, A_wo, B_q, B_k, B_v, B_shift_k, B_ssm_k, B_ssm_D):
    fwd, inv = _dft_mats()
    fwd = jnp.asarray(fwd[None])
    inv = jnp.asarray(inv[None])
    scratch = [
        pltpu.VMEM((1, S, D), f32),
        pltpu.VMEM((2, G + 1, S, 128), f32),
        pltpu.VMEM((NQ, D // 2, 128), u32),
        pltpu.VMEM((G, S // 2, 128), u32),
        pltpu.VMEM((NQ, D // 2, 128), u32),
        pltpu.VMEM((G, S // 2, 128), u32),
        pltpu.VMEM((1, HS, 128), f32), pltpu.VMEM((1, HS, 128), f32),
        pltpu.VMEM((1, HS, 128), f32), pltpu.VMEM((1, HS, 128), f32),
        pltpu.VMEM((1, 160, 128), f32),
        pltpu.VMEM((1, S + 8, 128), f32),
        pltpu.VMEM((G, 40, 128), f32),
        pltpu.VMEM((2 * NC * CS + 64, 128), f32),
        pltpu.VMEM((2 * NC * CS + 64, 128), f32),
        pltpu.VMEM((NC * 128, 128), u32),
        pltpu.VMEM((NC * 128, 128), u32),
        pltpu.VMEM((S, 128), u32),
        pltpu.VMEM((S, 128), u32),
        pltpu.VMEM((RC // 2, D), u32),
        pltpu.SMEM((NZ,), i32),
        pltpu.VMEM((1, S, D), bf),
        pltpu.VMEM((D, 3 * D), bf),
        pltpu.VMEM((D, D), bf),
        pltpu.VMEM((G, S, 128), bf),
        pltpu.VMEM((G, S, 128), bf),
        pltpu.VMEM((D, S), bf),
        pltpu.VMEM((S, D), bf),
        pltpu.VMEM((4, D), bf),
        pltpu.VMEM((G, 128), bf),
        pltpu.VMEM((1, 256, 128), u32),
        pltpu.VMEM((1, 64, 256), u32),
        pltpu.SemaphoreType.DMA((3, G)),
        pltpu.SemaphoreType.DMA((NRC,)),
        pltpu.SemaphoreType.DMA((G + 1,)),
        pltpu.SemaphoreType.DMA((NRC,)),
        pltpu.SemaphoreType.DMA((4,)),
    ]
    hbm = pl.BlockSpec(memory_space=pl.ANY)
    return pl.pallas_call(
        _kernel,
        out_shape=jax.ShapeDtypeStruct((1, S, D), bf),
        in_specs=[hbm] * 10,
        out_specs=hbm,
        scratch_shapes=scratch,
        compiler_params=pltpu.CompilerParams(vmem_limit_bytes=120 * 2**20, disable_bounds_checks=bool(NOBC)),
    )(A_x, A_wqkv, A_wo, B_k, B_v, B_shift_k.T, B_ssm_k, B_ssm_D.reshape(G, 128), fwd, inv)
```

```python
import numpy as np
import jax
import jax.numpy as jnp
from jax import lax
import jax.experimental.pallas as pl
import jax.experimental.pallas.tpu as pltpu

S = 2048
D = 1024
DH = 32
G = 8
NQ = 16
HS = S // 2
CH = HS // 4
UNR = 8
TA = (17, 21, 25, 29)
TB = (0, 0, 4, 8)
RC = 256
NRC = S // RC
NP = RC // 16
NC = 16
EPS = 1e-5
PDL = 0
DV = 1
SCOPES = 0
MERGE = 0
GIB = 3
NINV = 16
PQ = 2
P3 = [[0, 1, 2], [3, 4, 5], [6, 7], [8, 9], [10, 11], [12, 13], [14, 15], []]
ORD = 1
NOBC = 1
TAILG = 1
CHAIN = 1
CTICK = 0
SKIP = ''
IM = 136
CS = 416
GO = 16 * 416 + 24
LAZY = 1
ONLY = '1a23'
RG = 2
SPAN0 = 8
SPAN_TILES = 16
INV0 = 14
KV0 = 6
NZ = 2 + 8 * UNR
QSCALE = float(DH ** -0.5 * np.log2(np.e))

bf = jnp.bfloat16
f32 = jnp.float32
u32 = jnp.uint32
i32 = jnp.int32
NT = (((1,), (1,)), ((), ()))


def scope(name):
    import contextlib
    return jax.named_scope(name) if SCOPES else contextlib.nullcontext()


def _dft_mats():
    n = np.arange(128)
    f = np.concatenate([np.arange(0, 128, 2), np.arange(1, 128, 2)])
    ang = 2.0 * np.pi * np.outer(f + 0.5, n) / 256.0
    fwd = np.concatenate([np.cos(ang), -np.sin(ang)], axis=0)
    inv = fwd.T / 128.0
    re, im = fwd[0:128], fwd[128:256]
    fwd = np.concatenate([im, re, im - re, im + re], axis=0)

    def pack_rows(a):
        u = np.ascontiguousarray(a, dtype=np.float32).view(np.uint32)
        u = (u + 0x7FFF + ((u >> 16) & 1)) >> 16
        return (u[0::2] | (u[1::2] << 16)).astype(np.uint32)
    return pack_rows(fwd), pack_rows(inv)


def _tree_sum(p):
    n = p.shape[0] // 8
    x = p.reshape(n, 8, 128)
    while n > 1:
        x = x.reshape(n // 2, 2, 8, 128)
        x = x[:, 0] + x[:, 1]
        n //= 2
    return x[0]


def _ln(x):
    m = jnp.mean(x, axis=-1, keepdims=True)
    xc = x - m
    v = jnp.mean(xc * xc, axis=-1, keepdims=True)
    return xc * lax.rsqrt(v + EPS)


def _pack(x):
    return pltpu.bitcast(x.astype(bf), u32)


def _unpack(x):
    return pltpu.bitcast(x, bf)


def _tok(v, zv):
    v = v if v.dtype == u32 else pltpu.bitcast(v, u32)
    acc = None
    for r in range(v.shape[0] // 8):
        for c in range(v.shape[1] // 128):
            p = v[r * 8:(r + 1) * 8, c * 128:(c + 1) * 128]
            acc = p if acc is None else acc | p
    return acc & zv


def _gate(w, toks):
    if not toks:
        return w
    wu = pltpu.bitcast(w, u32)
    h0 = wu[0:8]
    for t in toks:
        h0 = h0 | jnp.tile(t, (1, wu.shape[1] // 128))
    return _unpack(jnp.concatenate([h0, wu[8:]], axis=0))


def _tick(v, k, z0):
    return pltpu.bitcast(v[8 * k:8 * k + 8, 0:128], i32)[0, 0] & z0


def _kernel(x_hbm, wqkv_hbm, wo_hbm, bk_hbm, bv_hbm, shk_hbm, ssmk_hbm, ssmd_hbm, fwd_hbm, inv_hbm, out_hbm,
            x_s, y_s, qt_s, k_s, vt_s, o_s, a1, a2, b1, b2, fin, kf_s, taps_s, ug_a, ug_b, zb_a, zb_b, pb_a, pb_b,
            h_s, z_ref, x_in, wqkv, wo, bk, bv, ssmk, out_s, shk, ssmd, fwd_ref, inv_ref,
            sem_c, sem_x, sem_w, sem_o, sem_s):
    def kv_copies(cb):
        cs = pl.ds(pl.multiple_of(cb * 128, 128), 128)
        return [pltpu.make_async_copy(bk_hbm.at[0, :, cs], bk.at[cb], sem_c.at[0, cb]),
                pltpu.make_async_copy(bv_hbm.at[0, :, cs], bv.at[cb], sem_c.at[1, cb])]

    def h_copy(cb):
        cs = pl.ds(pl.multiple_of(cb * 128, 128), 128)
        return pltpu.make_async_copy(ssmk_hbm.at[cs, :], ssmk.at[cs, :], sem_c.at[2, cb])

    def x_copy(c):
        rs = pl.ds(pl.multiple_of(c * RC, RC), RC)
        return pltpu.make_async_copy(x_hbm.at[0, rs, :], x_in.at[0, rs, :], sem_x.at[c])

    def w_copy(c):
        rs = pl.ds(pl.multiple_of(c * 128, 128), 128)
        return pltpu.make_async_copy(wqkv_hbm.at[rs, :], wqkv.at[rs, :], sem_w.at[c])

    def wo_copy():
        return pltpu.make_async_copy(wo_hbm, wo, sem_w.at[G])

    def out_copy(c):
        rs = pl.ds(pl.multiple_of(c * RC, RC), RC)
        return pltpu.make_async_copy(out_s.at[rs, :], out_hbm.at[0, rs, :], sem_o.at[c])

    def conv_start(c):
        h_copy(c).start()
        for cp in kv_copies(c):
            cp.start()

    def conv_wait(c):
        h_copy(c).wait()
        for cp in kv_copies(c):
            cp.wait()

    small = [pltpu.make_async_copy(src, dst, sem_s.at[i]) for i, (src, dst) in enumerate(
        ((shk_hbm, shk), (ssmd_hbm, ssmd), (fwd_hbm, fwd_ref), (inv_hbm, inv_ref)))]
    h_copy(0).start()
    small[2].start()
    if DV == 1:
        small[0].start()
        small[1].start()
        for cp in kv_copies(0):
            cp.start()

    for i in range(NZ):
        z_ref[i] = 0
    fin[...] = jnp.ones(fin.shape, f32)
    kf_s[0, 0:8, :] = jnp.zeros((8, 128), f32)
    zb_b[...] = jnp.zeros(zb_b.shape, u32)

    def setup_taps():
        taps = shk[...].astype(f32)
        dall = ssmd[...].astype(f32)
        for cb in range(G):
            for t in range(4):
                taps_s[cb, 8 * t:8 * t + 8, :] = jnp.broadcast_to(taps[t:t + 1, cb * 128:(cb + 1) * 128], (8, 128))
            taps_s[cb, 32:40, :] = jnp.broadcast_to(dall[cb:cb + 1, :], (8, 128))

    TILES = [(0, n) for n in range(8)] + [(2, n) for n in range(8)] + [(1, n) for n in range(8)]

    def qkv_tile(h, c, idx, toks, zv):
        kind, n = TILES[idx]
        col = kind * D + n * 128
        wa = _gate(wqkv[0:D // 2, col:col + 128], toks)
        ra = jnp.dot(h[:, 0:D // 2], wa, preferred_element_type=f32)
        rb = jnp.dot(h[:, D // 2:D], wqkv[D // 2:D, col:col + 128], preferred_element_type=f32)
        r = ra + rb
        if kind == 1:
            r2 = pl.multiple_of(c * (RC // 2), RC // 2)
            k_s[n, pl.ds(r2, RC // 2), :] = _pack(r)
            return ra, None
        dst = qt_s if kind == 0 else vt_s
        if kind == 0:
            r = r * QSCALE
        pks = []
        for t in range(RC // 128):
            pk = _pack(r[t * 128:(t + 1) * 128, :].T)
            dst[c * (RC // 128) + t, n * 64:(n + 1) * 64, :] = pk
            pks.append(pk)
        return ra, _tok(jnp.concatenate(pks, axis=0), zv)

    def piece_rows(c, p):
        return pl.ds(pl.multiple_of(c * RC + p * 16, 16), 16)

    def ln1_piece(cn, p, zt):
        rows = piece_rows(cn, p)
        hp = _pack(_ln(x_in[zt, rows, :].astype(f32)))
        h_s[p * 8:(p + 1) * 8, :] = hp
        return hp

    def gated_x(cn, p, zt):
        rows = piece_rows(cn, p)
        x1 = x_s[zt, rows, :]
        y = jnp.concatenate([y_s[0, g, rows, :] + y_s[1, g, rows, :] for g in range(G)], axis=1)
        return x1 + _ln(x1) * y

    def ln2_piece(cn, p, zt):
        x2 = gated_x(cn, p, zt)
        x_s[zt, piece_rows(cn, p), :] = x2
        hp = _pack(_ln(x2))
        h_s[p * 8:(p + 1) * 8, :] = hp
        return hp

    def out_piece(c, p, zt):
        v = gated_x(c, p, zt)
        out_s[piece_rows(c, p), :] = v.astype(bf)
        return v

    zts = [pl.multiple_of((z_ref[2 + ib] & 1) * 32, 32) for ib in range(4)]

    def prep_h(cb, pb):
        cs = pl.ds(pl.multiple_of(cb * 128, 128), 128)
        for j in range(NC):
            pb[HS + j * 64:HS + (j + 1) * 64, :] = pltpu.bitcast(ssmk[cs, j * 128:(j + 1) * 128], u32)

    def prep_kv(cb, pb, with_h=False):
        zs = z_ref[1]
        tp = taps_s[cb]
        cs = pl.ds(pl.multiple_of(cb * 128, 128), 128)
        for j in range(NC):
            r0 = j * 128
            if with_h:
                hu = pltpu.bitcast(ssmk[cs, r0:r0 + 128], u32)
                pb[HS + j * 64:HS + (j + 1) * 64, :] = hu
            kf_s[zs, 8 + r0:8 + r0 + 128, :] = bk[cb, r0:r0 + 128, :].astype(f32)
            ks = None
            for t in range(4):
                term = kf_s[zs, 8 + r0 - t:8 + r0 - t + 128, :].reshape(16, 8, 128) * tp[8 * t:8 * t + 8][None]
                ks = term if ks is None else ks + term
            kv = _pack(ks.reshape(128, 128) * bv[cb, r0:r0 + 128, :].astype(f32))
            pb[j * 64:(j + 1) * 64, :] = kv

    def fwd_h(pb, ug):
        for m in range(NC):
            hm = lax.dot_general(_unpack(fwd_ref[0, 64:256, :]),
                                 _unpack(pb[HS + m * 64:HS + (m + 1) * 64, :]), NT, preferred_element_type=f32)
            for e in range(3):
                o = GO + m * CS + e * IM
                ug[o:o + 128, :] = hm[e * 128:(e + 1) * 128]

    def fwd_u(pb, ug):
        for j in range(NC):
            u = jnp.dot(_unpack(fwd_ref[0, 0:128, :]), _unpack(pb[j * 64:(j + 1) * 64, :]),
                        preferred_element_type=f32)
            ug[j * CS:j * CS + 128, :] = u[128:256]
            ug[j * CS + IM:j * CS + IM + 128, :] = u[0:128]

    def add_skip(cb, ug):
        dv = taps_s[cb, 32:40, :][None]
        for e, sg in ((0, 1.0), (1, -1.0), (2, 1.0)):
            o = GO + e * IM
            v = ug[o:o + 128, :].reshape(16, 8, 128)
            ug[o:o + 128, :] = (v + dv if sg > 0 else v - dv).reshape(128, 128)

    def spec_item(ug, ib, r, zt):
        gc = {}
        k1 = [None] * 4
        k2 = [None] * 4
        k3 = [None] * 4
        for j in range(4 * ib + 4):
            ou = j * CS + r
            ua = ug[pl.ds(zt + ou, 8), :]
            ub = ug[pl.ds(zt + ou + IM, 8), :]
            us = ua + ub
            for q in range(4):
                m = 4 * ib + q - j
                if m < 0:
                    continue
                if m not in gc:
                    og = GO + m * CS + r
                    gc[m] = tuple(ug[pl.ds(zt + og + e * IM, 8), :] for e in range(3))
                g0, g1, g2 = gc[m]
                t1, t2, t3 = g0 * us, ua * g1, ub * g2
                k1[q] = t1 if k1[q] is None else k1[q] + t1
                k2[q] = t2 if k2[q] is None else k2[q] + t2
                k3[q] = t3 if k3[q] is None else k3[q] + t3
        return [k1[q] - k3[q] for q in range(4)], [k1[q] + k2[q] for q in range(4)]

    def overlap_add(yr, yi, prev, r):
        zr, zi = [], []
        for q in range(4):
            if prev is None:
                zr.append(yr[q])
                zi.append(yi[q])
            elif r < 64:
                zr.append(yr[q] - prev[1])
                zi.append(yi[q] + prev[0])
            else:
                zr.append(yr[q] + prev[1])
                zi.append(yi[q] - prev[0])
            prev = (yr[q], yi[q])
        return zr, zi, prev

    def conv_spec_rows(ug, zb, rp, gate=None):
        p0 = p1 = None
        for ib in range(4):
            zt = zts[ib]
            if gate is not None and ib >= GIB:
                zt = pl.multiple_of(zt + gate * 32, 32)
            zr0, zi0, p0 = overlap_add(*spec_item(ug, ib, 16 * rp, zt), p0, 16 * rp)
            zr1, zi1, p1 = overlap_add(*spec_item(ug, ib, 16 * rp + 8, zt), p1, 16 * rp)
            for q in range(4):
                o = (4 * ib + q) * 128 + rp * 8
                zb[o:o + 8, :] = _pack(jnp.concatenate([zr0[q], zr1[q]], axis=0))
                zb[o + 64:o + 72, :] = _pack(jnp.concatenate([zi0[q], zi1[q]], axis=0))

    def conv_inv(cb, zb, lo=0, hi=NC):
        for i in range(lo, hi):
            for e in range(2):
                y = jnp.dot(_unpack(inv_ref[0, :, e * 128:(e + 1) * 128]),
                            _unpack(zb[i * 128 + e * 64:i * 128 + (e + 1) * 64, :]), preferred_element_type=f32)
                y_s[e, cb, i * 128:(i + 1) * 128, :] = y
        return y

    def conv_main(c, ug_cur, ug_nxt, zb_cur, zb_prev, pb_nxt, ninv=NC):
        for rp in range(8):
            conv_spec_rows(ug_cur, zb_cur, rp)
        if pb_nxt is not None:
            fwd_h(pb_nxt, ug_nxt)
            fwd_u(pb_nxt, ug_nxt)
        conv_inv((c + G) % (G + 1), zb_prev, 0, ninv)

    def fence(fn):
        @pl.when(z_ref[0] == 0)
        def _():
            fn()

    def conv_half(c, ug_cur, ug_nxt, zb_cur, zb_prev, pb_nxt, pb_new):
        @pl.when(c + 3 < G)
        def _():
            conv_start(c + 3)
        w_copy(c).start()
        if MERGE == 0:
            conv_main(c, ug_cur, ug_nxt, zb_cur, zb_prev, pb_nxt, NINV)
            fence(lambda: h_copy(c + 2).wait())
            for cp in kv_copies(c + 2):
                cp.wait()
            prep_kv(c + 2, pb_new, True)
            add_skip(c + 1, ug_nxt)
        elif MERGE == 1:
            conv_main(c, ug_cur, ug_nxt, zb_cur, zb_prev, pb_nxt, NINV)
            conv_wait(c + 2)
            prep_kv(c + 2, pb_new, True)
            add_skip(c + 1, ug_nxt)
        else:
            for rp in range(8):
                conv_spec_rows(ug_cur, zb_cur, rp)
            conv_wait(c + 2)
            prep_kv(c + 2, pb_new, True)
            fwd_h(pb_nxt, ug_nxt)
            fwd_u(pb_nxt, ug_nxt)
            conv_inv((c + G) % (G + 1), zb_prev)
            add_skip(c + 1, ug_nxt)

        @pl.when(c >= 1)
        def _():
            w_copy(c - 1).wait()

    def conv():
        with scope("s_w0"):
            small[2].wait()
            h_copy(0).wait()
        if DV == 2:
            for cp in kv_copies(0):
                cp.start()
            small[0].start()
            small[1].start()
        conv_start(1)
        small[3].start()
        with scope("s_h0"):
            prep_h(0, pb_a)
            fwd_h(pb_a, ug_a)
        with scope("s_w1"):
            small[0].wait()
            small[1].wait()
            for cp in kv_copies(0):
                cp.wait()
        conv_start(2)
        setup_taps()
        add_skip(0, ug_a)
        prep_kv(0, pb_a)
        fwd_u(pb_a, ug_a)
        with scope("s_w2"):
            conv_wait(1)
            small[3].wait()
        prep_kv(1, pb_b, True)

        def body(p, carry):
            conv_half(2 * p, ug_a, ug_b, zb_a, zb_b, pb_b, pb_a)
            conv_half(2 * p + 1, ug_b, ug_a, zb_b, zb_a, pb_a, pb_b)
            return carry
        lax.fori_loop(0, G // 2 - 1, body, 0)
        w_copy(G - 2).start()
        w_copy(G - 1).start()
        x_copy(0).start()
        conv_main(G - 2, ug_a, ug_b, zb_a, zb_b, pb_b)
        x_copy(1).start()
        fence(lambda: w_copy(G - 3).wait())
        add_skip(G - 1, ug_b)
        fence(lambda: w_copy(G - 2).wait())
        conv_main(G - 1, ug_b, ug_a, zb_b, zb_a, None)
        fence(lambda: x_copy(0).wait())
        for p in range(NP):
            ln1_piece(0, p, 0)
        conv_inv(G - 1, zb_b)
        w_copy(G - 1).wait()

    def oproj_tile(o, cn, n, z1, toks=None, r0=0, nr=RC, first=False):
        rows = pl.ds(pl.multiple_of(cn * RC + r0, nr), nr)
        cols = slice(n * 128, (n + 1) * 128)
        r = jnp.dot(o[r0:r0 + nr], _gate(wo[:, cols], toks), preferred_element_type=f32)
        x0 = x_in[0, rows, cols].astype(f32) if first else x_s[z1, rows, cols]
        x_s[z1, rows, cols] = x0 + r
        return r

    def load_o(cn):
        r2 = pl.multiple_of(cn * (RC // 2), RC // 2)
        return jnp.concatenate([_unpack(o_s[g, pl.ds(r2, RC // 2), :]) for g in range(G)], axis=1)

    def phase1(c, carry):
        cn = jnp.minimum(c + 1, NRC - 1)

        @pl.when(c + 1 < NRC)
        def _():
            x_copy(c + 1).wait()

        @pl.when(c + 2 < NRC)
        def _():
            x_copy(c + 2).start()

        @pl.when(c + 2 == NRC)
        def _():
            wo_copy().start()
        z0 = z_ref[0]
        zv = jnp.full((8, 128), z0, i32).astype(u32)
        h = _unpack(h_s[...])
        deps = {}
        for n in range(24):
            ra, done = qkv_tile(h, c, n, deps.get(n), zv)
            if done is not None and n + 3 < 24:
                deps.setdefault(n + 3, []).append(done)
            if 2 <= n < 2 + NP:
                hp = ln1_piece(cn, n - 2, _tick(ra, 16, z0))
                deps.setdefault(n + 3, []).append(_tok(hp, zv))
        return carry

    def phase2_body(c, nxt):
        z0 = z_ref[0]
        z1 = z_ref[1]
        zv = jnp.full((8, 128), z0, i32).astype(u32)
        h = _unpack(h_s[...])
        if nxt:
            o = load_o(c + 1)
            for n in range(8):
                oproj_tile(o, c + 1, n, z1, first=True)
        deps = {}
        for n in range(24):
            ra, done = qkv_tile(h, c, n, deps.get(n), zv)
            if done is not None and n + 3 < 24:
                deps.setdefault(n + 3, []).append(done)
            if nxt and 1 <= n < 1 + NP:
                hp = ln2_piece(c + 1, n - 1, _tick(ra, 0, z0))
                deps.setdefault(n + 3, []).append(_tok(hp, zv))

    def phase2():
        o = load_o(0)
        z0 = z_ref[0]
        nq = RC // PQ
        zv = jnp.full((8, 128), z0, i32).astype(u32)
        pdeps = {}
        for q in range(PQ):
            for n in range(8):
                oproj_tile(o, 0, n, z0, pdeps.get((q, n)), q * nq, nq, True)
            for p in range(q * NP // PQ, (q + 1) * NP // PQ):
                hp = ln2_piece(0, p, z0)
                k = p - q * NP // PQ
                key = (q + 2, 2 * k)
                if PDL and q + 2 < PQ:
                    pdeps.setdefault(key, []).append(_tok(hp, zv))

        def body(c, carry):
            phase2_body(c, True)
            return carry
        lax.fori_loop(0, (NRC - 1) * 1, lambda c, x: body(c % (NRC - 1), x), 0)
        phase2_body(NRC - 1, False)

    def phase3():
        o = load_o(0)
        for n in range(8):
            oproj_tile(o, 0, n, z_ref[1])

        def body(c, carry):
            z0 = z_ref[0]
            z1 = z_ref[1]
            zv = jnp.full((8, 128), z0, i32).astype(u32)
            o = load_o(c + 1)
            deps = {}
            for n in range(8):
                for p in P3[n]:
                    deps.setdefault(n + 1, []).append(_tok(out_piece(c, p, z0), zv))
                oproj_tile(o, c + 1, n, z1, deps.get(n))
            out_copy(c).start()
            return carry
        lax.fori_loop(0, NRC - 1, body, 0)
        z0 = z_ref[0]
        for p in range(NP):
            out_piece(NRC - 1, p, z0)
        out_copy(NRC - 1).start()

    zero16 = jnp.zeros((16, 128), u32)

    def qk(g, j, hh, half, dst, z, zk=0, dep=None):
        qt = qt_s[j, pl.ds(pl.multiple_of(g * 64 + hh * 16, 16), 16), :]
        w = _unpack(jnp.concatenate([qt if i == hh else zero16 for i in range(4)], axis=0))
        m = None
        first = None
        last = None
        for c in range(4):
            r0 = half * HS + c * CH
            ku = k_s[g + zk, r0 // 2:(r0 + CH) // 2, :]
            if dep is not None:
                ku = jnp.concatenate([ku[:CH // 2 - 8], ku[CH // 2 - 8:] | dep], axis=0)
            s = jnp.dot(_unpack(ku), w, preferred_element_type=f32)
            dst[z, c * CH:(c + 1) * CH, :] = s
            mc = jnp.max(s.reshape(CH // 8, 8, 128), axis=0)
            m = mc if m is None else jnp.maximum(m, mc)
            f = pltpu.bitcast(s[0:8], u32)
            first = f if first is None else first | f
            last = s
        return m, first, last

    def fullmax(m1, m2):
        return jnp.max(jnp.maximum(m1, m2), axis=0, keepdims=True)

    def sm_pv(g, hh, half, src, m, z2, dep, trigs):
        mb = jnp.broadcast_to(m, (8, 128))
        mbu = pltpu.bitcast(mb, u32)
        ms = [mb if tr is None else pltpu.bitcast(mbu | tr, f32) for tr in trigs]
        ng = len(trigs) // 2
        gr = 128 // ng
        ps = []
        for t in range(8):
            for kk in range(ng):
                mi = ms[(t // 4) * ng + (ng - 1 - kk)]
                x = src[z2, t * 128 + kk * gr:t * 128 + (kk + 1) * gr, :]
                ps.append(jnp.exp2(x.reshape(gr // 8, 8, 128) - mi[None]).reshape(gr, 128))
        p = jnp.concatenate(ps, axis=0)
        l = _tree_sum(p)
        rs = pl.ds(pl.multiple_of(g * 64 + hh * 16, 16), 16)
        dep2 = jnp.concatenate([dep, dep], axis=0)
        vu = jnp.concatenate([vt_s[half * 8 + t, rs, :] | dep2 for t in range(8)], axis=1)
        o = jnp.dot(_unpack(vu), p.astype(bf), preferred_element_type=f32)
        return o, l

    def store_o(g, j, parts):
        outs = [parts[2 * h] * (1.0 / jnp.sum(parts[2 * h + 1], axis=0, keepdims=True)) for h in range(4)]
        ot = jnp.concatenate(outs, axis=0)
        o_s[g, pl.ds(pl.multiple_of(j * 64, 64), 64), :] = _pack(ot.T)

    def finalize(g, j, slot):
        x = fin[slot]
        parts = []
        for hh in range(4):
            parts += [x[hh * 40: hh * 40 + 32], x[hh * 40 + 32: hh * 40 + 40]]
        store_o(g, j, parts)

    def attention():
        ma = fullmax(qk(0, 0, 0, 0, a1, 0)[0], qk(0, 0, 0, 1, a2, 0)[0])
        mb1 = qk(0, 0, 1, 0, b1, 0)[0]
        bufs = {(0, 0): a1, (0, 1): a2, (1, 0): b1, (1, 1): b2}

        def body(it, carry):
            ma, mb1 = carry
            z1 = z_ref[0]
            z2 = z_ref[1]
            zv = jnp.full((8, 128), z1, i32).astype(u32)
            tp = jnp.maximum(it * UNR - 1, 0)
            finalize(tp // NQ, tp % NQ, z2)
            do = None
            ps = None
            po = None

            def tg(sv, i):
                return None if sv is None else pltpu.bitcast(sv[i * 8:i * 8 + 8], u32) & zv

            for u in range(UNR):
                zk = [z_ref[2 + 8 * u + i] for i in range(8)]
                t = it * UNR + u
                g = t // NQ
                j = t % NQ
                tn = jnp.minimum(t + 1, G * NQ - 1)
                gn = tn // NQ
                jn = tn % NQ
                qks = [(g, j, 1, 1), (g, j, 2, 0), (g, j, 2, 1), (g, j, 3, 0), (g, j, 3, 1),
                       (gn, jn, 0, 0), (gn, jn, 0, 1), (gn, jn, 1, 0)]
                mfull = {0: ma}
                mpart = {1: mb1}
                os_, ls_ = {}, {}
                for n in range(8):
                    qg, qj, qh, qhalf = qks[n]
                    key = qh if n < 5 else qh + 4
                    mp, first, cs_ = qk(qg, qj, qh, qhalf, bufs[(qh % 2, qhalf)], z1, zk[n], do)
                    if qhalf == 0:
                        mpart[key] = mp
                    else:
                        mfull[key] = fullmax(mpart[key], mp)
                    ph, phalf = n // 2, n % 2
                    trigs = [tg(ps, i) for i in TA] + [tg(po, TB[0])] + [tg(cs_, i) for i in TB[1:]]
                    o, l = sm_pv(g, ph, phalf, bufs[(ph % 2, phalf)], mfull[ph], z2, first & zv, trigs)
                    ps = cs_
                    po = o
                    do = tg(o, 3)
                    os_[(ph, phalf)] = o
                    ls_[(ph, phalf)] = l
                ma = mfull[4]
                mb1 = mpart[5]
                parts = []
                for h in range(4):
                    parts += [os_[(h, 0)] + os_[(h, 1)], ls_[(h, 0)] + ls_[(h, 1)]]
                if u == UNR - 1:
                    fin[z1] = jnp.concatenate(parts, axis=0)
                else:
                    store_o(g, j, parts)
            return ma, mb1

        lax.fori_loop(0, G * NQ // UNR * 1, lambda i, c: body(i % (G * NQ // UNR), c), (ma, mb1))
        finalize(G - 1, NQ - 1, 0)

    with scope('S_conv'):
        conv()
    if '1' in ONLY:
        with scope('S_ph1'):
            lax.fori_loop(0, NRC, phase1, 0)
    else:
        x_copy(1).wait()
        wo_copy().start()
    wo_copy().wait()
    if 'a' in ONLY:
        with scope('S_att1'):
            attention()
    if '2' in ONLY:
        with scope('S_ph2'):
            phase2()
    if 'a' in ONLY:
        with scope('S_att2'):
            attention()
    if '3' in ONLY:
        with scope('S_ph3'):
            phase3()
    else:
        out_s[0:8, 0:128] = (y_s[0, 7, 0:8, :] + y_s[1, 7, 0:8, :] + pltpu.bitcast(h_s[0:8, 0:128], f32)).astype(bf)
        for c in range(NRC):
            out_copy(c).start()
    for c in range(NRC):
        out_copy(c).wait()


@jax.jit
def pallas_interleave_layers__softmax_full_mha__ssm_conv_h3__prompt_kernel(A_x, A_wqkv, A_wo, B_q, B_k, B_v, B_shift_k, B_ssm_k, B_ssm_D):
    fwd, inv = _dft_mats()
    fwd = jnp.asarray(fwd[None])
    inv = jnp.asarray(inv[None])
    scratch = [
        pltpu.VMEM((1, S, D), f32),
        pltpu.VMEM((2, G + 1, S, 128), f32),
        pltpu.VMEM((NQ, D // 2, 128), u32),
        pltpu.VMEM((G, S // 2, 128), u32),
        pltpu.VMEM((NQ, D // 2, 128), u32),
        pltpu.VMEM((G, S // 2, 128), u32),
        pltpu.VMEM((1, HS, 128), f32), pltpu.VMEM((1, HS, 128), f32),
        pltpu.VMEM((1, HS, 128), f32), pltpu.VMEM((1, HS, 128), f32),
        pltpu.VMEM((1, 160, 128), f32),
        pltpu.VMEM((1, S + 8, 128), f32),
        pltpu.VMEM((G, 40, 128), f32),
        pltpu.VMEM((2 * NC * CS + 64, 128), f32),
        pltpu.VMEM((2 * NC * CS + 64, 128), f32),
        pltpu.VMEM((NC * 128, 128), u32),
        pltpu.VMEM((NC * 128, 128), u32),
        pltpu.VMEM((S, 128), u32),
        pltpu.VMEM((S, 128), u32),
        pltpu.VMEM((RC // 2, D), u32),
        pltpu.SMEM((NZ,), i32),
        pltpu.VMEM((1, S, D), bf),
        pltpu.VMEM((D, 3 * D), bf),
        pltpu.VMEM((D, D), bf),
        pltpu.VMEM((G, S, 128), bf),
        pltpu.VMEM((G, S, 128), bf),
        pltpu.VMEM((D, S), bf),
        pltpu.VMEM((S, D), bf),
        pltpu.VMEM((4, D), bf),
        pltpu.VMEM((G, 128), bf),
        pltpu.VMEM((1, 256, 128), u32),
        pltpu.VMEM((1, 64, 256), u32),
        pltpu.SemaphoreType.DMA((3, G)),
        pltpu.SemaphoreType.DMA((NRC,)),
        pltpu.SemaphoreType.DMA((G + 1,)),
        pltpu.SemaphoreType.DMA((NRC,)),
        pltpu.SemaphoreType.DMA((4,)),
    ]
    hbm = pl.BlockSpec(memory_space=pl.ANY)
    return pl.pallas_call(
        _kernel,
        out_shape=jax.ShapeDtypeStruct((1, S, D), bf),
        in_specs=[hbm] * 10,
        out_specs=hbm,
        scratch_shapes=scratch,
        compiler_params=pltpu.CompilerParams(vmem_limit_bytes=120 * 2**20, disable_bounds_checks=bool(NOBC)),
    )(A_x, A_wqkv, A_wo, B_k, B_v, B_shift_k.T, B_ssm_k, B_ssm_D.reshape(G, 128), fwd, inv)
```

```python
import numpy as np
import jax
import jax.numpy as jnp
from jax import lax
import jax.experimental.pallas as pl
import jax.experimental.pallas.tpu as pltpu

S = 2048
D = 1024
DH = 32
G = 8
NQ = 16
HS = S // 2
CH = HS // 4
UNR = 8
TA = (17, 21, 25, 29)
TB = (0, 0, 4, 8)
RC = 256
NRC = S // RC
NP = RC // 16
NC = 16
EPS = 1e-5
P3M = 2
R0 = 4
PDL = 0
DV = 1
SCOPES = 0
MERGE = 0
GIB = 3
NINV = 16
PQ = 2
P3 = [[0, 1, 2], [3, 4, 5], [6, 7], [8, 9], [10, 11], [12, 13], [14, 15], []]
ORD = 1
NOBC = 1
TAILG = 1
CHAIN = 1
CTICK = 0
SKIP = ''
IM = 136
CS = 416
GO = 16 * 416 + 24
LAZY = 1
ONLY = '1a23'
RG = 2
SPAN0 = 8
SPAN_TILES = 16
INV0 = 14
KV0 = 6
NZ = 2 + 8 * UNR
QSCALE = float(DH ** -0.5 * np.log2(np.e))

bf = jnp.bfloat16
f32 = jnp.float32
u32 = jnp.uint32
i32 = jnp.int32
NT = (((1,), (1,)), ((), ()))


def scope(name):
    import contextlib
    return jax.named_scope(name) if SCOPES else contextlib.nullcontext()


def _dft_mats():
    n = np.arange(128)
    f = np.concatenate([np.arange(0, 128, 2), np.arange(1, 128, 2)])
    ang = 2.0 * np.pi * np.outer(f + 0.5, n) / 256.0
    fwd = np.concatenate([np.cos(ang), -np.sin(ang)], axis=0)
    inv = fwd.T / 128.0
    re, im = fwd[0:128], fwd[128:256]
    fwd = np.concatenate([im, re, im - re, im + re], axis=0)

    def pack_rows(a):
        u = np.ascontiguousarray(a, dtype=np.float32).view(np.uint32)
        u = (u + 0x7FFF + ((u >> 16) & 1)) >> 16
        return (u[0::2] | (u[1::2] << 16)).astype(np.uint32)
    return pack_rows(fwd), pack_rows(inv)


def _tree_sum(p):
    n = p.shape[0] // 8
    x = p.reshape(n, 8, 128)
    while n > 1:
        x = x.reshape(n // 2, 2, 8, 128)
        x = x[:, 0] + x[:, 1]
        n //= 2
    return x[0]


def _ln(x):
    m = jnp.mean(x, axis=-1, keepdims=True)
    xc = x - m
    v = jnp.mean(xc * xc, axis=-1, keepdims=True)
    return xc * lax.rsqrt(v + EPS)


def _pack(x):
    return pltpu.bitcast(x.astype(bf), u32)


def _unpack(x):
    return pltpu.bitcast(x, bf)


def _tok(v, zv):
    v = v if v.dtype == u32 else pltpu.bitcast(v, u32)
    acc = None
    for r in range(v.shape[0] // 8):
        for c in range(v.shape[1] // 128):
            p = v[r * 8:(r + 1) * 8, c * 128:(c + 1) * 128]
            acc = p if acc is None else acc | p
    return acc & zv


def _gate(w, toks):
    if not toks:
        return w
    wu = pltpu.bitcast(w, u32)
    h0 = wu[0:8]
    for t in toks:
        h0 = h0 | jnp.tile(t, (1, wu.shape[1] // 128))
    return _unpack(jnp.concatenate([h0, wu[8:]], axis=0))


def _tick(v, k, z0):
    return pltpu.bitcast(v[8 * k:8 * k + 8, 0:128], i32)[0, 0] & z0


def _kernel(x_hbm, wqkv_hbm, wo_hbm, bk_hbm, bv_hbm, shk_hbm, ssmk_hbm, ssmd_hbm, fwd_hbm, inv_hbm, out_hbm,
            x_s, y_s, qt_s, k_s, vt_s, o_s, a1, a2, b1, b2, fin, kf_s, taps_s, ug_a, ug_b, zb_a, zb_b, pb_a, pb_b,
            h_s, z_ref, x_in, wqkv, wo, bk, bv, ssmk, out_s, shk, ssmd, fwd_ref, inv_ref,
            sem_c, sem_x, sem_w, sem_o, sem_s):
    def kv_copies(cb):
        cs = pl.ds(pl.multiple_of(cb * 128, 128), 128)
        return [pltpu.make_async_copy(bk_hbm.at[0, :, cs], bk.at[cb], sem_c.at[0, cb]),
                pltpu.make_async_copy(bv_hbm.at[0, :, cs], bv.at[cb], sem_c.at[1, cb])]

    def h_copy(cb):
        cs = pl.ds(pl.multiple_of(cb * 128, 128), 128)
        return pltpu.make_async_copy(ssmk_hbm.at[cs, :], ssmk.at[cs, pl.ds(0, S)], sem_c.at[2, cb])

    def x_copy(c):
        rs = pl.ds(pl.multiple_of(c * RC, RC), RC)
        return pltpu.make_async_copy(x_hbm.at[0, rs, :], x_in.at[0, rs, :], sem_x.at[c])

    def w_copy(c):
        rs = pl.ds(pl.multiple_of(c * 128, 128), 128)
        return pltpu.make_async_copy(wqkv_hbm.at[rs, :], wqkv.at[rs, pl.ds(0, 3 * D)], sem_w.at[c])

    def wo_copy():
        return pltpu.make_async_copy(wo_hbm, wo.at[:, pl.ds(0, D)], sem_w.at[G])

    def out_copy(c):
        rs = pl.ds(pl.multiple_of(c * RC, RC), RC)
        return pltpu.make_async_copy(out_s.at[rs, :], out_hbm.at[0, rs, :], sem_o.at[c])

    def tail_copy(q):
        r0, r1 = ((0, 128), (128, 192), (192, 256))[q]
        rs = pl.ds((NRC - 1) * RC + r0, r1 - r0)
        return pltpu.make_async_copy(out_s.at[rs, :], out_hbm.at[0, rs, :], sem_o.at[NRC - 1 + q])

    def conv_start(c):
        h_copy(c).start()
        for cp in kv_copies(c):
            cp.start()

    def conv_wait(c):
        h_copy(c).wait()
        for cp in kv_copies(c):
            cp.wait()

    small = [pltpu.make_async_copy(src, dst, sem_s.at[i]) for i, (src, dst) in enumerate(
        ((shk_hbm, shk), (ssmd_hbm, ssmd), (fwd_hbm, fwd_ref), (inv_hbm, inv_ref)))]
    h_copy(0).start()
    small[2].start()
    if DV == 1:
        small[0].start()
        small[1].start()
        for cp in kv_copies(0):
            cp.start()

    for i in range(NZ):
        z_ref[i] = 0
    fin[...] = jnp.ones(fin.shape, f32)
    kf_s[0, 0:8, :] = jnp.zeros((8, 128), f32)

    def setup_taps():
        taps = shk[...].astype(f32)
        for cb in range(G):
            for t in range(4):
                taps_s[cb, 8 * t:8 * t + 8, :] = jnp.broadcast_to(taps[t:t + 1, cb * 128:(cb + 1) * 128], (8, 128))

    def setup_skip():
        dall = ssmd[...].astype(f32)
        for cb in range(G):
            taps_s[cb, 32:40, :] = jnp.broadcast_to(dall[cb:cb + 1, :], (8, 128))

    TILES = [(0, n) for n in range(8)] + [(2, n) for n in range(8)] + [(1, n) for n in range(8)]

    def qkv_tile(h, c, idx, toks, zv):
        kind, n = TILES[idx]
        col = kind * D + n * 128
        wa = _gate(wqkv[0:D // 2, col:col + 128], toks)
        ra = jnp.dot(h[:, 0:D // 2], wa, preferred_element_type=f32)
        rb = jnp.dot(h[:, D // 2:D], wqkv[D // 2:D, col:col + 128], preferred_element_type=f32)
        r = ra + rb
        if kind == 1:
            r2 = pl.multiple_of(c * (RC // 2), RC // 2)
            k_s[n, pl.ds(r2, RC // 2), :] = _pack(r)
            return ra, None
        dst = qt_s if kind == 0 else vt_s
        if kind == 0:
            r = r * QSCALE
        pks = []
        for t in range(RC // 128):
            pk = _pack(r[t * 128:(t + 1) * 128, :].T)
            dst[c * (RC // 128) + t, n * 64:(n + 1) * 64, :] = pk
            pks.append(pk)
        return ra, _tok(jnp.concatenate(pks, axis=0), zv)

    def piece_rows(c, p):
        return pl.ds(pl.multiple_of(c * RC + p * 16, 16), 16)

    def ln1_piece(cn, p, zt):
        rows = piece_rows(cn, p)
        hp = _pack(_ln(x_in[zt, rows, :].astype(f32)))
        h_s[p * 8:(p + 1) * 8, :] = hp
        return hp

    def gated_x(cn, p, zt):
        rows = piece_rows(cn, p)
        x1 = x_s[zt, rows, :]
        y = jnp.concatenate([y_s[0, g, rows, :] + y_s[1, g, rows, :] for g in range(G)], axis=1)
        return x1 + _ln(x1) * y

    def ln2_piece(cn, p, zt):
        x2 = gated_x(cn, p, zt)
        x_s[zt, piece_rows(cn, p), :] = x2
        hp = _pack(_ln(x2))
        h_s[p * 8:(p + 1) * 8, :] = hp
        return hp

    def out_piece(c, p, zt):
        v = gated_x(c, p, zt)
        out_s[piece_rows(c, p), :] = v.astype(bf)
        return v

    zts = [pl.multiple_of((z_ref[2 + ib] & 1) * 32, 32) for ib in range(4)]

    def prep_h(cb, pb):
        cs = pl.ds(pl.multiple_of(cb * 128, 128), 128)
        for j in range(NC):
            pb[HS + j * 64:HS + (j + 1) * 64, :] = pltpu.bitcast(ssmk[cs, j * 128:(j + 1) * 128], u32)

    def prep_kv(cb, pb, with_h=False):
        zs = z_ref[1]
        tp = taps_s[cb]
        cs = pl.ds(pl.multiple_of(cb * 128, 128), 128)
        for j in range(NC):
            r0 = j * 128
            if with_h:
                hu = pltpu.bitcast(ssmk[cs, r0:r0 + 128], u32)
                pb[HS + j * 64:HS + (j + 1) * 64, :] = hu
            kf_s[zs, 8 + r0:8 + r0 + 128, :] = bk[cb, r0:r0 + 128, :].astype(f32)
            ks = None
            for t in range(4):
                term = kf_s[zs, 8 + r0 - t:8 + r0 - t + 128, :].reshape(16, 8, 128) * tp[8 * t:8 * t + 8][None]
                ks = term if ks is None else ks + term
            kv = _pack(ks.reshape(128, 128) * bv[cb, r0:r0 + 128, :].astype(f32))
            pb[j * 64:(j + 1) * 64, :] = kv

    def fwd_h(pb, ug):
        for m in range(NC):
            hm = lax.dot_general(_unpack(fwd_ref[0, 64:256, :]),
                                 _unpack(pb[HS + m * 64:HS + (m + 1) * 64, :]), NT, preferred_element_type=f32)
            for e in range(3):
                o = GO + m * CS + e * IM
                ug[o:o + 128, :] = hm[e * 128:(e + 1) * 128]

    def fwd_u(pb, ug):
        for j in range(NC):
            u = jnp.dot(_unpack(fwd_ref[0, 0:128, :]), _unpack(pb[j * 64:(j + 1) * 64, :]),
                        preferred_element_type=f32)
            ug[j * CS:j * CS + 128, :] = u[128:256]
            ug[j * CS + IM:j * CS + IM + 128, :] = u[0:128]

    def add_skip(cb, ug):
        dv = taps_s[cb, 32:40, :][None]
        for e, sg in ((0, 1.0), (1, -1.0), (2, 1.0)):
            o = GO + e * IM
            v = ug[o:o + 128, :].reshape(16, 8, 128)
            ug[o:o + 128, :] = (v + dv if sg > 0 else v - dv).reshape(128, 128)

    def spec_item(ug, ib, r, zt):
        gc = {}
        k1 = [None] * 4
        k2 = [None] * 4
        k3 = [None] * 4
        for j in range(4 * ib + 4):
            ou = j * CS + r
            ua = ug[pl.ds(zt + ou, 8), :]
            ub = ug[pl.ds(zt + ou + IM, 8), :]
            us = ua + ub
            for q in range(4):
                m = 4 * ib + q - j
                if m < 0:
                    continue
                if m not in gc:
                    og = GO + m * CS + r
                    gc[m] = tuple(ug[pl.ds(zt + og + e * IM, 8), :] for e in range(3))
                g0, g1, g2 = gc[m]
                t1, t2, t3 = g0 * us, ua * g1, ub * g2
                k1[q] = t1 if k1[q] is None else k1[q] + t1
                k2[q] = t2 if k2[q] is None else k2[q] + t2
                k3[q] = t3 if k3[q] is None else k3[q] + t3
        return [k1[q] - k3[q] for q in range(4)], [k1[q] + k2[q] for q in range(4)]

    def overlap_add(yr, yi, prev, r):
        zr, zi = [], []
        for q in range(4):
            if prev is None:
                zr.append(yr[q])
                zi.append(yi[q])
            elif r < 64:
                zr.append(yr[q] - prev[1])
                zi.append(yi[q] + prev[0])
            else:
                zr.append(yr[q] + prev[1])
                zi.append(yi[q] - prev[0])
            prev = (yr[q], yi[q])
        return zr, zi, prev

    def conv_spec_rows(ug, zb, rp, gate=None):
        p0 = p1 = None
        for ib in range(4):
            zt = zts[ib]
            if gate is not None and ib >= GIB:
                zt = pl.multiple_of(zt + gate * 32, 32)
            zr0, zi0, p0 = overlap_add(*spec_item(ug, ib, 16 * rp, zt), p0, 16 * rp)
            zr1, zi1, p1 = overlap_add(*spec_item(ug, ib, 16 * rp + 8, zt), p1, 16 * rp)
            for q in range(4):
                o = (4 * ib + q) * 128 + rp * 8
                zb[o:o + 8, :] = _pack(jnp.concatenate([zr0[q], zr1[q]], axis=0))
                zb[o + 64:o + 72, :] = _pack(jnp.concatenate([zi0[q], zi1[q]], axis=0))

    def conv_inv(cb, zb, lo=0, hi=NC):
        for i in range(lo, hi):
            for e in range(2):
                y = jnp.dot(_unpack(inv_ref[0, :, e * 128:(e + 1) * 128]),
                            _unpack(zb[i * 128 + e * 64:i * 128 + (e + 1) * 64, :]), preferred_element_type=f32)
                y_s[e, cb, i * 128:(i + 1) * 128, :] = y
        return y

    def fence(fn):
        @pl.when(z_ref[0] == 0)
        def _():
            fn()

    def conv_half(c, ug_cur, ug_nxt, zb_cur, zb_prev, pb_nxt, pb_new):
        @pl.when(c + 3 < G)
        def _():
            conv_start(c + 3)
        w_copy(c).start()

        @pl.when(c >= G - 3)
        def _():
            x_copy(c - (G - 3)).start()
        for rp in range(8):
            conv_spec_rows(ug_cur, zb_cur, rp)
        fwd_h(pb_nxt, ug_nxt)
        fwd_u(pb_nxt, ug_nxt)
        conv_inv(c - 1, zb_prev)

        @pl.when(c + 2 < G)
        def _():
            w_copy(c - 1).wait()
            conv_wait(c + 2)
            prep_kv(c + 2, pb_new, True)
            add_skip(c + 1, ug_nxt)

        @pl.when(c + 2 >= G)
        def _():
            w_copy(c - 1).wait()
            add_skip(c + 1, ug_nxt)

    def conv():
        with scope("s_w0"):
            small[2].wait()
            h_copy(0).wait()
        conv_start(1)
        small[3].start()
        with scope("s_h0"):
            prep_h(0, pb_a)
            fwd_h(pb_a, ug_a)
        with scope("s_w1"):
            small[0].wait()
            for cp in kv_copies(0):
                cp.wait()
        conv_start(2)
        setup_taps()
        prep_kv(0, pb_a)
        fwd_u(pb_a, ug_a)
        with scope("s_w2"):
            fence(lambda: h_copy(1).wait())
        prep_h(1, pb_b)
        with scope("s_w2b"):
            fence(lambda: small[1].wait())
        setup_skip()
        add_skip(0, ug_a)
        for rp in range(R0):
            conv_spec_rows(ug_a, zb_a, rp)
        fwd_h(pb_b, ug_b)
        with scope("s_w3"):
            fence(lambda: [cp.wait() for cp in kv_copies(1)] and None)
        conv_start(3)
        w_copy(0).start()
        prep_kv(1, pb_b)
        add_skip(1, ug_b)
        fence(lambda: h_copy(2).wait())
        for rp in range(R0, 8):
            conv_spec_rows(ug_a, zb_a, rp)
        fwd_u(pb_b, ug_b)
        fence(lambda: [cp.wait() for cp in kv_copies(2) + [small[3]]] and None)
        prep_kv(2, pb_a, True)

        def body(p, carry):
            conv_half(2 * p + 1, ug_b, ug_a, zb_b, zb_a, pb_a, pb_b)
            conv_half(2 * p + 2, ug_a, ug_b, zb_a, zb_b, pb_b, pb_a)
            return carry
        lax.fori_loop(0, G // 2 - 1, body, 0)
        w_copy(G - 1).start()
        for rp in range(8):
            conv_spec_rows(ug_b, zb_b, rp)
        conv_inv(G - 2, zb_a)
        fence(lambda: x_copy(0).wait())
        for p in range(NP):
            ln1_piece(0, p, 0)
        conv_inv(G - 1, zb_b)
        w_copy(G - 2).wait()
        w_copy(G - 1).wait()

    def oproj_tile(o, cn, n, z1, toks=None, r0=0, nr=RC, first=False):
        rows = pl.ds(pl.multiple_of(cn * RC + r0, nr), nr)
        cols = slice(n * 128, (n + 1) * 128)
        r = jnp.dot(o[r0:r0 + nr], _gate(wo[:, cols], toks), preferred_element_type=f32)
        x0 = x_in[0, rows, cols].astype(f32) if first else x_s[z1, rows, cols]
        x_s[z1, rows, cols] = x0 + r
        return r

    def load_o(cn):
        r2 = pl.multiple_of(cn * (RC // 2), RC // 2)
        return jnp.concatenate([_unpack(o_s[g, pl.ds(r2, RC // 2), :]) for g in range(G)], axis=1)

    def phase1(c, carry):
        cn = jnp.minimum(c + 1, NRC - 1)

        @pl.when(c + 1 < NRC)
        def _():
            x_copy(c + 1).wait()

        @pl.when(c + 2 < NRC)
        def _():
            x_copy(c + 2).start()

        @pl.when(c + 2 == NRC)
        def _():
            wo_copy().start()
        z0 = z_ref[0]
        zv = jnp.full((8, 128), z0, i32).astype(u32)
        h = _unpack(h_s[...])
        deps = {}
        for n in range(24):
            ra, done = qkv_tile(h, c, n, deps.get(n), zv)
            if done is not None and n + 3 < 24:
                deps.setdefault(n + 3, []).append(done)
            if 2 <= n < 2 + NP:
                hp = ln1_piece(cn, n - 2, _tick(ra, 16, z0))
                deps.setdefault(n + 3, []).append(_tok(hp, zv))
        return carry

    def phase2_body(c, nxt):
        z0 = z_ref[0]
        z1 = z_ref[1]
        zv = jnp.full((8, 128), z0, i32).astype(u32)
        h = _unpack(h_s[...])
        if nxt:
            o = load_o(c + 1)
            for n in range(8):
                oproj_tile(o, c + 1, n, z1, first=True)
        deps = {}
        for n in range(24):
            ra, done = qkv_tile(h, c, n, deps.get(n), zv)
            if done is not None and n + 3 < 24:
                deps.setdefault(n + 3, []).append(done)
            if nxt and 1 <= n < 1 + NP:
                hp = ln2_piece(c + 1, n - 1, _tick(ra, 0, z0))
                deps.setdefault(n + 3, []).append(_tok(hp, zv))

    def phase2():
        o = load_o(0)
        z0 = z_ref[0]
        nq = RC // PQ
        zv = jnp.full((8, 128), z0, i32).astype(u32)
        pdeps = {}
        for q in range(PQ):
            for n in range(8):
                oproj_tile(o, 0, n, z0, pdeps.get((q, n)), q * nq, nq, True)
            for p in range(q * NP // PQ, (q + 1) * NP // PQ):
                hp = ln2_piece(0, p, z0)
                k = p - q * NP // PQ
                key = (q + 2, 2 * k)
                if PDL and q + 2 < PQ:
                    pdeps.setdefault(key, []).append(_tok(hp, zv))

        def body(c, carry):
            phase2_body(c, True)
            return carry
        lax.fori_loop(0, (NRC - 1) * 1, lambda c, x: body(c % (NRC - 1), x), 0)
        phase2_body(NRC - 1, False)

    def phase3():
        o = load_o(0)
        for n in range(8):
            oproj_tile(o, 0, n, z_ref[1])

        def body(c, carry):
            z0 = z_ref[0]
            z1 = z_ref[1]
            zv = jnp.full((8, 128), z0, i32).astype(u32)
            o = load_o(c + 1)
            deps = {}
            if P3M == 0:
                for n in range(8):
                    for p in P3[n]:
                        deps.setdefault(n + 1, []).append(_tok(out_piece(c, p, z0), zv))
                    oproj_tile(o, c + 1, n, z1, deps.get(n))
            else:
                p = 0
                for t in range(16):
                    for _ in range(2 if t < P3M else 1):
                        if p < NP:
                            deps.setdefault(t + 2, []).append(_tok(out_piece(c, p, z0), zv))
                            p += 1
                    oproj_tile(o, c + 1, t // 2, z1, deps.get(t), (t % 2) * 128, 128)
            out_copy(c).start()
            return carry
        lax.fori_loop(0, NRC - 2, body, 0)
        c = NRC - 1
        z0 = z_ref[0]
        zv = jnp.full((8, 128), z0, i32).astype(u32)
        o = load_o(c)
        deps = {}
        todo = [(c - 1, p) for p in range(NP)]
        rows = (0, 128, 192, 256)
        t = 0
        for q in range(3):
            for n in range(8):
                for _ in range(2):
                    if todo:
                        cc, p = todo.pop(0)
                        deps.setdefault(t + 2, []).append(_tok(out_piece(cc, p, z0), zv))
                oproj_tile(o, c, n, z0, deps.get(t), rows[q], rows[q + 1] - rows[q])
                t += 1
            if q == 0:
                out_copy(c - 1).start()
            if q == 1:
                tail_copy(0).start()
            for cc, p in todo:
                out_piece(cc, p, z0)
            todo = [(c, p) for p in range(rows[q] // 16, rows[q + 1] // 16)]
        tail_copy(1).start()
        for cc, p in todo:
            out_piece(cc, p, z0)
        tail_copy(2).start()

    zero16 = jnp.zeros((16, 128), u32)

    def qk(g, j, hh, half, dst, z, zk=0, dep=None):
        qt = qt_s[j, pl.ds(pl.multiple_of(g * 64 + hh * 16, 16), 16), :]
        w = _unpack(jnp.concatenate([qt if i == hh else zero16 for i in range(4)], axis=0))
        m = None
        first = None
        last = None
        for c in range(4):
            r0 = half * HS + c * CH
            ku = k_s[g + zk, r0 // 2:(r0 + CH) // 2, :]
            if dep is not None:
                ku = jnp.concatenate([ku[:CH // 2 - 8], ku[CH // 2 - 8:] | dep], axis=0)
            s = jnp.dot(_unpack(ku), w, preferred_element_type=f32)
            dst[z, c * CH:(c + 1) * CH, :] = s
            mc = jnp.max(s.reshape(CH // 8, 8, 128), axis=0)
            m = mc if m is None else jnp.maximum(m, mc)
            f = pltpu.bitcast(s[0:8], u32)
            first = f if first is None else first | f
            last = s
        return m, first, last

    def fullmax(m1, m2):
        return jnp.max(jnp.maximum(m1, m2), axis=0, keepdims=True)

    def sm_pv(g, hh, half, src, m, z2, dep, trigs):
        mb = jnp.broadcast_to(m, (8, 128))
        mbu = pltpu.bitcast(mb, u32)
        ms = [mb if tr is None else pltpu.bitcast(mbu | tr, f32) for tr in trigs]
        ng = len(trigs) // 2
        gr = 128 // ng
        ps = []
        for t in range(8):
            for kk in range(ng):
                mi = ms[(t // 4) * ng + (ng - 1 - kk)]
                x = src[z2, t * 128 + kk * gr:t * 128 + (kk + 1) * gr, :]
                ps.append(jnp.exp2(x.reshape(gr // 8, 8, 128) - mi[None]).reshape(gr, 128))
        p = jnp.concatenate(ps, axis=0)
        l = _tree_sum(p)
        rs = pl.ds(pl.multiple_of(g * 64 + hh * 16, 16), 16)
        dep2 = jnp.concatenate([dep, dep], axis=0)
        vu = jnp.concatenate([vt_s[half * 8 + t, rs, :] | dep2 for t in range(8)], axis=1)
        o = jnp.dot(_unpack(vu), p.astype(bf), preferred_element_type=f32)
        return o, l

    def store_o(g, j, parts):
        outs = [parts[2 * h] * (1.0 / jnp.sum(parts[2 * h + 1], axis=0, keepdims=True)) for h in range(4)]
        ot = jnp.concatenate(outs, axis=0)
        o_s[g, pl.ds(pl.multiple_of(j * 64, 64), 64), :] = _pack(ot.T)

    def finalize(g, j, slot):
        x = fin[slot]
        parts = []
        for hh in range(4):
            parts += [x[hh * 40: hh * 40 + 32], x[hh * 40 + 32: hh * 40 + 40]]
        store_o(g, j, parts)

    def attention():
        ma = fullmax(qk(0, 0, 0, 0, a1, 0)[0], qk(0, 0, 0, 1, a2, 0)[0])
        mb1 = qk(0, 0, 1, 0, b1, 0)[0]
        bufs = {(0, 0): a1, (0, 1): a2, (1, 0): b1, (1, 1): b2}

        def body(it, carry):
            ma, mb1 = carry
            z1 = z_ref[0]
            z2 = z_ref[1]
            zv = jnp.full((8, 128), z1, i32).astype(u32)
            tp = jnp.maximum(it * UNR - 1, 0)
            finalize(tp // NQ, tp % NQ, z2)
            do = None
            ps = None
            po = None

            def tg(sv, i):
                return None if sv is None else pltpu.bitcast(sv[i * 8:i * 8 + 8], u32) & zv

            for u in range(UNR):
                zk = [z_ref[2 + 8 * u + i] for i in range(8)]
                t = it * UNR + u
                g = t // NQ
                j = t % NQ
                tn = jnp.minimum(t + 1, G * NQ - 1)
                gn = tn // NQ
                jn = tn % NQ
                qks = [(g, j, 1, 1), (g, j, 2, 0), (g, j, 2, 1), (g, j, 3, 0), (g, j, 3, 1),
                       (gn, jn, 0, 0), (gn, jn, 0, 1), (gn, jn, 1, 0)]
                mfull = {0: ma}
                mpart = {1: mb1}
                os_, ls_ = {}, {}
                for n in range(8):
                    qg, qj, qh, qhalf = qks[n]
                    key = qh if n < 5 else qh + 4
                    mp, first, cs_ = qk(qg, qj, qh, qhalf, bufs[(qh % 2, qhalf)], z1, zk[n], do)
                    if qhalf == 0:
                        mpart[key] = mp
                    else:
                        mfull[key] = fullmax(mpart[key], mp)
                    ph, phalf = n // 2, n % 2
                    trigs = [tg(ps, i) for i in TA] + [tg(po, TB[0])] + [tg(cs_, i) for i in TB[1:]]
                    o, l = sm_pv(g, ph, phalf, bufs[(ph % 2, phalf)], mfull[ph], z2, first & zv, trigs)
                    ps = cs_
                    po = o
                    do = tg(o, 3)
                    os_[(ph, phalf)] = o
                    ls_[(ph, phalf)] = l
                ma = mfull[4]
                mb1 = mpart[5]
                parts = []
                for h in range(4):
                    parts += [os_[(h, 0)] + os_[(h, 1)], ls_[(h, 0)] + ls_[(h, 1)]]
                if u == UNR - 1:
                    fin[z1] = jnp.concatenate(parts, axis=0)
                else:
                    store_o(g, j, parts)
            return ma, mb1

        lax.fori_loop(0, G * NQ // UNR * 1, lambda i, c: body(i % (G * NQ // UNR), c), (ma, mb1))
        finalize(G - 1, NQ - 1, 0)

    with scope('S_conv'):
        conv()
    if '1' in ONLY:
        with scope('S_ph1'):
            lax.fori_loop(0, NRC, phase1, 0)
    else:
        x_copy(1).wait()
        wo_copy().start()
    wo_copy().wait()
    if 'a' in ONLY:
        with scope('S_att1'):
            attention()
    if '2' in ONLY:
        with scope('S_ph2'):
            phase2()
    if 'a' in ONLY:
        with scope('S_att2'):
            attention()
    if '3' in ONLY:
        with scope('S_ph3'):
            phase3()
    else:
        out_s[0:8, 0:128] = (y_s[0, 7, 0:8, :] + y_s[1, 7, 0:8, :] + pltpu.bitcast(h_s[0:8, 0:128], f32)).astype(bf)
        for c in range(NRC - 1):
            out_copy(c).start()
        for q in range(3):
            tail_copy(q).start()
    for c in range(NRC - 1):
        out_copy(c).wait()
    for q in range(3):
        tail_copy(q).wait()


@jax.jit
def pallas_interleave_layers__softmax_full_mha__ssm_conv_h3__prompt_kernel(A_x, A_wqkv, A_wo, B_q, B_k, B_v, B_shift_k, B_ssm_k, B_ssm_D):
    fwd, inv = _dft_mats()
    fwd = jnp.asarray(fwd[None])
    inv = jnp.asarray(inv[None])
    scratch = [
        pltpu.VMEM((1, S, D), f32),
        pltpu.VMEM((2, G, S, 128), f32),
        pltpu.VMEM((NQ, D // 2, 128), u32),
        pltpu.VMEM((G, S // 2, 128), u32),
        pltpu.VMEM((NQ, D // 2, 128), u32),
        pltpu.VMEM((G, S // 2, 128), u32),
        pltpu.VMEM((1, HS, 128), f32), pltpu.VMEM((1, HS, 128), f32),
        pltpu.VMEM((1, HS, 128), f32), pltpu.VMEM((1, HS, 128), f32),
        pltpu.VMEM((1, 160, 128), f32),
        pltpu.VMEM((1, S + 8, 128), f32),
        pltpu.VMEM((G, 40, 128), f32),
        pltpu.VMEM((2 * NC * CS + 64, 128), f32),
        pltpu.VMEM((2 * NC * CS + 64, 128), f32),
        pltpu.VMEM((NC * 128, 128), u32),
        pltpu.VMEM((NC * 128, 128), u32),
        pltpu.VMEM((S, 128), u32),
        pltpu.VMEM((S, 128), u32),
        pltpu.VMEM((RC // 2, D), u32),
        pltpu.SMEM((NZ,), i32),
        pltpu.VMEM((1, S, D), bf),
        pltpu.VMEM((D, 3 * D + 128), bf),
        pltpu.VMEM((D, D + 128), bf),
        pltpu.VMEM((G, S, 128), bf),
        pltpu.VMEM((G, S, 128), bf),
        pltpu.VMEM((D, S + 128), bf),
        pltpu.VMEM((S, D), bf),
        pltpu.VMEM((4, D), bf),
        pltpu.VMEM((G, 128), bf),
        pltpu.VMEM((1, 256, 128), u32),
        pltpu.VMEM((1, 64, 256), u32),
        pltpu.SemaphoreType.DMA((3, G)),
        pltpu.SemaphoreType.DMA((NRC,)),
        pltpu.SemaphoreType.DMA((G + 1,)),
        pltpu.SemaphoreType.DMA((NRC + 2,)),
        pltpu.SemaphoreType.DMA((4,)),
    ]
    hbm = pl.BlockSpec(memory_space=pl.ANY)
    return pl.pallas_call(
        _kernel,
        out_shape=jax.ShapeDtypeStruct((1, S, D), bf),
        in_specs=[hbm] * 10,
        out_specs=hbm,
        scratch_shapes=scratch,
        compiler_params=pltpu.CompilerParams(vmem_limit_bytes=120 * 2**20, disable_bounds_checks=bool(NOBC)),
    )(A_x, A_wqkv, A_wo, B_k, B_v, B_shift_k.T, B_ssm_k, B_ssm_D.reshape(G, 128), fwd, inv)
```

```python
import numpy as np
import jax
import jax.numpy as jnp
from jax import lax
import jax.experimental.pallas as pl
import jax.experimental.pallas.tpu as pltpu

S = 2048
D = 1024
DH = 32
G = 8
NQ = 16
HS = S // 2
CH = HS // 4
UNR = 8
TA = (17, 21, 25, 29)
TB = (0, 0, 4, 8)
RC = 256
NRC = S // RC
NP = RC // 16
NC = 16
EPS = 1e-5
TICK = 0
P3M = 2
R0 = 4
PDL = 0
DV = 1
SCOPES = 0
MERGE = 0
GIB = 3
NINV = 16
PQ = 2
P3 = [[0, 1, 2], [3, 4, 5], [6, 7], [8, 9], [10, 11], [12, 13], [14, 15], []]
ORD = 1
NOBC = 1
TAILG = 1
CHAIN = 1
CTICK = 0
SKIP = ''
IM = 136
CS = 416
GO = 8
LAZY = 1
ONLY = '1a23'
RG = 2
SPAN0 = 8
SPAN_TILES = 16
INV0 = 14
KV0 = 6
NZ = 2 + 8 * UNR
QSCALE = float(DH ** -0.5 * np.log2(np.e))

bf = jnp.bfloat16
f32 = jnp.float32
u32 = jnp.uint32
i32 = jnp.int32
NT = (((1,), (1,)), ((), ()))


def scope(name):
    import contextlib
    return jax.named_scope(name) if SCOPES else contextlib.nullcontext()


def _dft_mats():
    n = np.arange(128)
    f = np.concatenate([np.arange(0, 128, 2), np.arange(1, 128, 2)])
    ang = 2.0 * np.pi * np.outer(f + 0.5, n) / 256.0
    fwd = np.concatenate([np.cos(ang), -np.sin(ang)], axis=0)
    inv = fwd.T / 128.0
    re, im = fwd[0:128], fwd[128:256]
    fwd = np.concatenate([re, im, re, im - re, im + re], axis=0)

    def pack_rows(a):
        u = np.ascontiguousarray(a, dtype=np.float32).view(np.uint32)
        u = (u + 0x7FFF + ((u >> 16) & 1)) >> 16
        return (u[0::2] | (u[1::2] << 16)).astype(np.uint32)
    return pack_rows(fwd), pack_rows(inv)


def _tree_sum(p):
    n = p.shape[0] // 8
    x = p.reshape(n, 8, 128)
    while n > 1:
        x = x.reshape(n // 2, 2, 8, 128)
        x = x[:, 0] + x[:, 1]
        n //= 2
    return x[0]


def _ln(x):
    m = jnp.mean(x, axis=-1, keepdims=True)
    xc = x - m
    v = jnp.mean(xc * xc, axis=-1, keepdims=True)
    return xc * lax.rsqrt(v + EPS)


def _pack(x):
    return pltpu.bitcast(x.astype(bf), u32)


def _unpack(x):
    return pltpu.bitcast(x, bf)


def _tok(v, zv):
    v = v if v.dtype == u32 else pltpu.bitcast(v, u32)
    while v.shape[1] > 128:
        h = v.shape[1] // 2
        v = v[:, :h] | v[:, h:]
    while v.shape[0] > 8:
        h = v.shape[0] // 2
        v = v[:h] | v[h:]
    return v & zv


def _gate(w, toks):
    if not toks:
        return w
    wu = pltpu.bitcast(w, u32)
    h0 = wu[0:8]
    for t in toks:
        h0 = h0 | jnp.tile(t, (1, wu.shape[1] // 128))
    return _unpack(jnp.concatenate([h0, wu[8:]], axis=0))


def _tick(v, k, z0):
    return pltpu.bitcast(v[8 * k:8 * k + 8, 0:128], i32)[0, 0] & z0


def _kernel(x_hbm, wqkv_hbm, wo_hbm, bk_hbm, bv_hbm, shk_hbm, ssmk_hbm, ssmd_hbm, fwd_hbm, inv_hbm, out_hbm,
            x_s, y_s, qt_s, k_s, vt_s, o_s, a1, a2, b1, b2, fin, kf_s, taps_s, ug_a, ug_b, zb_a, zb_b, pb_a, pb_b,
            h_s, z_ref, x_in, wqkv, wo, bk, bv, ssmk, out_s, shk, ssmd, fwd_ref, inv_ref,
            sem_c, sem_x, sem_w, sem_o, sem_s):
    def kv_copies(cb):
        cs = pl.ds(pl.multiple_of(cb * 128, 128), 128)
        return [pltpu.make_async_copy(bk_hbm.at[0, :, cs], bk.at[cb], sem_c.at[0, cb]),
                pltpu.make_async_copy(bv_hbm.at[0, :, cs], bv.at[cb], sem_c.at[1, cb])]

    def h_copy(cb):
        cs = pl.ds(pl.multiple_of(cb * 128, 128), 128)
        return pltpu.make_async_copy(ssmk_hbm.at[cs, :], ssmk.at[cs, pl.ds(0, S)], sem_c.at[2, cb])

    def x_copy(c):
        rs = pl.ds(pl.multiple_of(c * RC, RC), RC)
        return pltpu.make_async_copy(x_hbm.at[0, rs, :], x_in.at[0, rs, :], sem_x.at[c])

    def w_copy(c):
        rs = pl.ds(pl.multiple_of(c * 128, 128), 128)
        return pltpu.make_async_copy(wqkv_hbm.at[rs, :], wqkv.at[rs, pl.ds(0, 3 * D)], sem_w.at[c])

    def wo_copy():
        return pltpu.make_async_copy(wo_hbm, wo.at[:, pl.ds(0, D)], sem_w.at[G])

    def out_copy(c):
        rs = pl.ds(pl.multiple_of(c * RC, RC), RC)
        return pltpu.make_async_copy(out_s.at[rs, :], out_hbm.at[0, rs, :], sem_o.at[c])

    def tail_copy(q):
        r0, r1 = ((0, 128), (128, 192), (192, 256))[q]
        rs = pl.ds((NRC - 1) * RC + r0, r1 - r0)
        return pltpu.make_async_copy(out_s.at[rs, :], out_hbm.at[0, rs, :], sem_o.at[NRC - 1 + q])

    def conv_start(c):
        h_copy(c).start()
        for cp in kv_copies(c):
            cp.start()

    def conv_wait(c):
        h_copy(c).wait()
        for cp in kv_copies(c):
            cp.wait()

    small = [pltpu.make_async_copy(src, dst, sem_s.at[i]) for i, (src, dst) in enumerate(
        ((shk_hbm, shk), (ssmd_hbm, ssmd), (fwd_hbm, fwd_ref), (inv_hbm, inv_ref)))]
    h_copy(0).start()
    small[2].start()
    if DV == 1:
        small[0].start()
        small[1].start()
        for cp in kv_copies(0):
            cp.start()

    for i in range(NZ):
        z_ref[i] = 0
    fin[...] = jnp.ones(fin.shape, f32)
    kf_s[0, 0:8, :] = jnp.zeros((8, 128), f32)

    def setup_taps():
        taps = shk[...].astype(f32)
        for cb in range(G):
            for t in range(4):
                taps_s[cb, 8 * t:8 * t + 8, :] = jnp.broadcast_to(taps[t:t + 1, cb * 128:(cb + 1) * 128], (8, 128))

    def setup_skip():
        dall = ssmd[...].astype(f32)
        for cb in range(G):
            taps_s[cb, 32:40, :] = jnp.broadcast_to(dall[cb:cb + 1, :], (8, 128))

    TILES = [(0, n) for n in range(8)] + [(2, n) for n in range(8)] + [(1, n) for n in range(8)]

    def qkv_tile(h, c, idx, toks, zv):
        kind, n = TILES[idx]
        col = kind * D + n * 128
        wa = _gate(wqkv[0:D // 2, col:col + 128], toks)
        ra = jnp.dot(h[:, 0:D // 2], wa, preferred_element_type=f32)
        rb = jnp.dot(h[:, D // 2:D], wqkv[D // 2:D, col:col + 128], preferred_element_type=f32)
        r = ra + rb
        if kind == 1:
            r2 = pl.multiple_of(c * (RC // 2), RC // 2)
            k_s[n, pl.ds(r2, RC // 2), :] = _pack(r)
            return ra, None
        dst = qt_s if kind == 0 else vt_s
        if kind == 0:
            r = r * QSCALE
        pks = []
        for t in range(RC // 128):
            pk = _pack(r[t * 128:(t + 1) * 128, :].T)
            dst[c * (RC // 128) + t, n * 64:(n + 1) * 64, :] = pk
            pks.append(pk)
        return ra, _tok(jnp.concatenate(pks, axis=0), zv)

    def piece_rows(c, p):
        return pl.ds(pl.multiple_of(c * RC + p * 16, 16), 16)

    def ln1_piece(cn, p, zt):
        rows = piece_rows(cn, p)
        hp = _pack(_ln(x_in[zt, rows, :].astype(f32)))
        h_s[p * 8:(p + 1) * 8, :] = hp
        return hp

    def gated_x(cn, p, zt):
        rows = piece_rows(cn, p)
        x1 = x_s[zt, rows, :]
        y = jnp.concatenate([y_s[0, g, rows, :] + y_s[1, g, rows, :] for g in range(G)], axis=1)
        return x1 + _ln(x1) * y

    def ln2_piece(cn, p, zt):
        x2 = gated_x(cn, p, zt)
        x_s[zt, piece_rows(cn, p), :] = x2
        hp = _pack(_ln(x2))
        h_s[p * 8:(p + 1) * 8, :] = hp
        return hp

    def out_piece(c, p, zt):
        v = gated_x(c, p, zt)
        out_s[piece_rows(c, p), :] = v.astype(bf)
        return v

    zts = [z_ref[2 + ib] for ib in range(4)]

    def prep_h(cb, pb):
        cs = pl.ds(pl.multiple_of(cb * 128, 128), 128)
        for j in range(NC):
            pb[HS + j * 64:HS + (j + 1) * 64, :] = pltpu.bitcast(ssmk[cs, j * 128:(j + 1) * 128], u32)

    def prep_kv(cb, pb, with_h=False):
        zs = z_ref[1]
        tp = taps_s[cb, 0:32, :]
        cs = pl.ds(pl.multiple_of(cb * 128, 128), 128)
        for j in range(NC):
            r0 = j * 128
            if with_h:
                hu = pltpu.bitcast(ssmk[cs, r0:r0 + 128], u32)
                pb[HS + j * 64:HS + (j + 1) * 64, :] = hu
            kf_s[zs, 8 + r0:8 + r0 + 128, :] = bk[cb, r0:r0 + 128, :].astype(f32)
            ks = None
            for t in range(4):
                term = kf_s[zs, 8 + r0 - t:8 + r0 - t + 128, :].reshape(16, 8, 128) * tp[8 * t:8 * t + 8][None]
                ks = term if ks is None else ks + term
            kv = _pack(ks.reshape(128, 128) * bv[cb, r0:r0 + 128, :].astype(f32))
            pb[j * 64:(j + 1) * 64, :] = kv

    def fwd_h(pb, ug):
        for m in range(NC):
            hm = lax.dot_general(_unpack(fwd_ref[0, 128:320, :]),
                                 _unpack(pb[HS + m * 64:HS + (m + 1) * 64, :]), NT, preferred_element_type=f32)
            ug[0, NC + m, :, GO:GO + 128, :] = hm.reshape(3, 128, 128)

    def fwd_u(pb, ug):
        for j in range(NC):
            u = jnp.dot(_unpack(fwd_ref[0, 0:128, :]), _unpack(pb[j * 64:(j + 1) * 64, :]),
                        preferred_element_type=f32)
            ug[0, j, 0:2, 0:128, :] = u.reshape(2, 128, 128)

    def add_skip(cb, ug):
        dv = taps_s[cb, 32:40, :][None]
        for e, sg in ((0, 1.0), (1, -1.0), (2, 1.0)):
            v = ug[0, NC, e, GO:GO + 128, :].reshape(16, 8, 128)
            ug[0, NC, e, GO:GO + 128, :] = (v + dv if sg > 0 else v - dv).reshape(128, 128)

    def spec_item(ug, ib, r, zt):
        acc = None
        for j in range(4 * ib + 4):
            u = ug[zt, j:j + 1, 0:2, r:r + 8, :]
            u = jnp.concatenate([u[:, 0:1] + u[:, 1:2], u], axis=1)
            q0 = max(0, j - 4 * ib)
            m0 = NC + 4 * ib - j
            t = ug[zt, m0 + q0:m0 + 4, :, GO + r:GO + r + 8, :] * u
            if acc is None:
                acc = t
            elif q0 == 0:
                acc = acc + t
            else:
                acc = jnp.concatenate([acc[:q0], acc[q0:] + t], axis=0)
        return acc[:, 0] - acc[:, 2], acc[:, 0] + acc[:, 1]

    def overlap_add(yr, yi, prev, r):
        n = 1 if prev is None else 0
        pr = yr[:3] if prev is None else jnp.concatenate([prev[0], yr[:3]], axis=0)
        pi = yi[:3] if prev is None else jnp.concatenate([prev[1], yi[:3]], axis=0)
        if r < 64:
            zr, zi = yr[n:] - pi, yi[n:] + pr
        else:
            zr, zi = yr[n:] + pi, yi[n:] - pr
        if prev is None:
            zr = jnp.concatenate([yr[:1], zr], axis=0)
            zi = jnp.concatenate([yi[:1], zi], axis=0)
        return zr, zi, (yr[3:], yi[3:])

    def conv_spec_rows(ug, zb, rp):
        p0 = p1 = None
        for ib in range(4):
            zr0, zi0, p0 = overlap_add(*spec_item(ug, ib, 16 * rp, zts[ib]), p0, 16 * rp)
            zr1, zi1, p1 = overlap_add(*spec_item(ug, ib, 16 * rp + 8, zts[ib]), p1, 16 * rp)
            zb[4 * ib:4 * ib + 4, rp * 8:rp * 8 + 8, :] = _pack(jnp.concatenate([zr0, zr1], axis=1))
            zb[4 * ib:4 * ib + 4, 64 + rp * 8:72 + rp * 8, :] = _pack(jnp.concatenate([zi0, zi1], axis=1))

    def conv_inv(cb, zb, lo=0, hi=NC):
        for i in range(lo, hi):
            for e in range(2):
                y = jnp.dot(_unpack(inv_ref[0, :, e * 128:(e + 1) * 128]),
                            _unpack(zb[i, e * 64:(e + 1) * 64, :]), preferred_element_type=f32)
                y_s[e, cb, i * 128:(i + 1) * 128, :] = y
        return y

    def fence(fn):
        @pl.when(z_ref[0] == 0)
        def _():
            fn()

    def conv_half(c, ug_cur, ug_nxt, zb_cur, zb_prev, pb_nxt, pb_new):
        @pl.when(c + 3 < G)
        def _():
            conv_start(c + 3)
        w_copy(c).start()

        @pl.when(c >= G - 3)
        def _():
            x_copy(c - (G - 3)).start()
        for rp in range(8):
            conv_spec_rows(ug_cur, zb_cur, rp)
        fwd_h(pb_nxt, ug_nxt)
        fwd_u(pb_nxt, ug_nxt)
        conv_inv(c - 1, zb_prev)

        @pl.when(c + 2 < G)
        def _():
            w_copy(c - 1).wait()
            conv_wait(c + 2)
            prep_kv(c + 2, pb_new, True)
            add_skip(c + 1, ug_nxt)

        @pl.when(c + 2 >= G)
        def _():
            w_copy(c - 1).wait()
            add_skip(c + 1, ug_nxt)

    def conv():
        with scope("s_w0"):
            small[2].wait()
            h_copy(0).wait()
        conv_start(1)
        small[3].start()
        with scope("s_h0"):
            prep_h(0, pb_a)
            fwd_h(pb_a, ug_a)
        with scope("s_w1"):
            small[0].wait()
            for cp in kv_copies(0):
                cp.wait()
        conv_start(2)
        setup_taps()
        prep_kv(0, pb_a)
        fwd_u(pb_a, ug_a)
        with scope("s_w2"):
            fence(lambda: h_copy(1).wait())
        prep_h(1, pb_b)
        with scope("s_w2b"):
            fence(lambda: small[1].wait())
        setup_skip()
        add_skip(0, ug_a)
        for rp in range(R0):
            conv_spec_rows(ug_a, zb_a, rp)
        fwd_h(pb_b, ug_b)
        with scope("s_w3"):
            fence(lambda: [cp.wait() for cp in kv_copies(1)] and None)
        conv_start(3)
        w_copy(0).start()
        prep_kv(1, pb_b)
        add_skip(1, ug_b)
        fence(lambda: h_copy(2).wait())
        for rp in range(R0, 8):
            conv_spec_rows(ug_a, zb_a, rp)
        fwd_u(pb_b, ug_b)
        fence(lambda: [cp.wait() for cp in kv_copies(2) + [small[3]]] and None)
        prep_kv(2, pb_a, True)

        def body(p, carry):
            conv_half(2 * p + 1, ug_b, ug_a, zb_b, zb_a, pb_a, pb_b)
            conv_half(2 * p + 2, ug_a, ug_b, zb_a, zb_b, pb_b, pb_a)
            return carry
        lax.fori_loop(0, G // 2 - 1, body, 0)
        w_copy(G - 1).start()
        for rp in range(8):
            conv_spec_rows(ug_b, zb_b, rp)
        conv_inv(G - 2, zb_a)
        fence(lambda: x_copy(0).wait())
        for p in range(NP):
            ln1_piece(0, p, 0)
        conv_inv(G - 1, zb_b)
        w_copy(G - 2).wait()
        w_copy(G - 1).wait()

    def oproj_tile(o, cn, n, z1, toks=None, r0=0, nr=RC, first=False):
        rows = pl.ds(pl.multiple_of(cn * RC + r0, nr), nr)
        cols = slice(n * 128, (n + 1) * 128)
        r = jnp.dot(o[r0:r0 + nr], _gate(wo[:, cols], toks), preferred_element_type=f32)
        x0 = x_in[0, rows, cols].astype(f32) if first else x_s[z1, rows, cols]
        x_s[z1, rows, cols] = x0 + r
        return r

    def load_o(cn):
        r2 = pl.multiple_of(cn * (RC // 2), RC // 2)
        return jnp.concatenate([_unpack(o_s[g, pl.ds(r2, RC // 2), :]) for g in range(G)], axis=1)

    def phase1(c, carry):
        cn = jnp.minimum(c + 1, NRC - 1)

        @pl.when(c + 1 < NRC)
        def _():
            x_copy(c + 1).wait()

        @pl.when(c + 2 < NRC)
        def _():
            x_copy(c + 2).start()

        @pl.when(c + 2 == NRC)
        def _():
            wo_copy().start()
        z0 = z_ref[0]
        zv = jnp.full((8, 128), z0, i32).astype(u32)
        h = _unpack(h_s[...])
        deps = {}
        for n in range(24):
            ra, done = qkv_tile(h, c, n, deps.get(n), zv)
            if done is not None and n + 3 < 24:
                deps.setdefault(n + 3, []).append(done)
            if 2 <= n < 2 + NP:
                hp = ln1_piece(cn, n - 2, _tick(ra, 16, z0) if TICK else 0)
                deps.setdefault(n + 3, []).append(_tok(hp, zv))
        return carry

    def phase2_body(c, nxt):
        z0 = z_ref[0]
        z1 = z_ref[1]
        zv = jnp.full((8, 128), z0, i32).astype(u32)
        h = _unpack(h_s[...])
        if nxt:
            o = load_o(c + 1)
            for n in range(8):
                oproj_tile(o, c + 1, n, z1, first=True)
        deps = {}
        for n in range(24):
            ra, done = qkv_tile(h, c, n, deps.get(n), zv)
            if done is not None and n + 3 < 24:
                deps.setdefault(n + 3, []).append(done)
            if nxt and 1 <= n < 1 + NP:
                hp = ln2_piece(c + 1, n - 1, _tick(ra, 0, z0) if TICK else z0)
                deps.setdefault(n + 3, []).append(_tok(hp, zv))

    def phase2():
        o = load_o(0)
        z0 = z_ref[0]
        nq = RC // PQ
        zv = jnp.full((8, 128), z0, i32).astype(u32)
        pdeps = {}
        for q in range(PQ):
            for n in range(8):
                oproj_tile(o, 0, n, z0, pdeps.get((q, n)), q * nq, nq, True)
            for p in range(q * NP // PQ, (q + 1) * NP // PQ):
                hp = ln2_piece(0, p, z0)
                k = p - q * NP // PQ
                key = (q + 2, 2 * k)
                if PDL and q + 2 < PQ:
                    pdeps.setdefault(key, []).append(_tok(hp, zv))

        def body(c, carry):
            phase2_body(c, True)
            return carry
        lax.fori_loop(0, (NRC - 1) * 1, lambda c, x: body(c % (NRC - 1), x), 0)
        phase2_body(NRC - 1, False)

    def phase3():
        o = load_o(0)
        for n in range(8):
            oproj_tile(o, 0, n, z_ref[1])

        def body(c, carry):
            z0 = z_ref[0]
            z1 = z_ref[1]
            zv = jnp.full((8, 128), z0, i32).astype(u32)
            o = load_o(c + 1)
            deps = {}
            if P3M == 0:
                for n in range(8):
                    for p in P3[n]:
                        deps.setdefault(n + 1, []).append(_tok(out_piece(c, p, z0), zv))
                    oproj_tile(o, c + 1, n, z1, deps.get(n))
            else:
                p = 0
                for t in range(16):
                    for _ in range(2 if t < P3M else 1):
                        if p < NP:
                            deps.setdefault(t + 2, []).append(_tok(out_piece(c, p, z0), zv))
                            p += 1
                    oproj_tile(o, c + 1, t // 2, z1, deps.get(t), (t % 2) * 128, 128)
            out_copy(c).start()
            return carry
        lax.fori_loop(0, NRC - 2, body, 0)
        c = NRC - 1
        z0 = z_ref[0]
        zv = jnp.full((8, 128), z0, i32).astype(u32)
        o = load_o(c)
        deps = {}
        todo = [(c - 1, p) for p in range(NP)]
        rows = (0, 128, 192, 256)
        t = 0
        for q in range(3):
            for n in range(8):
                for _ in range(2):
                    if todo:
                        cc, p = todo.pop(0)
                        deps.setdefault(t + 2, []).append(_tok(out_piece(cc, p, z0), zv))
                oproj_tile(o, c, n, z0, deps.get(t), rows[q], rows[q + 1] - rows[q])
                t += 1
            if q == 0:
                out_copy(c - 1).start()
            if q == 1:
                tail_copy(0).start()
            for cc, p in todo:
                out_piece(cc, p, z0)
            todo = [(c, p) for p in range(rows[q] // 16, rows[q + 1] // 16)]
        tail_copy(1).start()
        for cc, p in todo:
            out_piece(cc, p, z0)
        tail_copy(2).start()

    zero16 = jnp.zeros((16, 128), u32)

    def qk(g, j, hh, half, dst, z, zk=0, dep=None):
        qt = qt_s[j, pl.ds(pl.multiple_of(g * 64 + hh * 16, 16), 16), :]
        w = _unpack(jnp.concatenate([qt if i == hh else zero16 for i in range(4)], axis=0))
        m = None
        first = None
        last = None
        kh = k_s[g + zk, half * HS // 2:(half + 1) * HS // 2, :]
        for c in range(4):
            ku = kh[c * CH // 2:(c + 1) * CH // 2]
            if dep is not None:
                ku = jnp.concatenate([ku[:CH // 2 - 8], ku[CH // 2 - 8:] | dep], axis=0)
            s = jnp.dot(_unpack(ku), w, preferred_element_type=f32)
            dst[z, c * CH:(c + 1) * CH, :] = s
            mc = jnp.max(s.reshape(CH // 8, 8, 128), axis=0)
            m = mc if m is None else jnp.maximum(m, mc)
            f = pltpu.bitcast(s[0:8], u32)
            first = f if first is None else first | f
            last = s
        return m, first, last

    def fullmax(m1, m2):
        return jnp.max(jnp.maximum(m1, m2), axis=0, keepdims=True)

    def sm_pv(g, hh, half, src, m, z2, dep, trigs):
        mb = jnp.broadcast_to(m, (8, 128))
        mbu = pltpu.bitcast(mb, u32)
        ms = [mb if tr is None else pltpu.bitcast(mbu | tr, f32) for tr in trigs]
        mm = jnp.stack([jnp.stack([ms[4 * st + 3 - kk] for kk in range(4)]) for st in range(2)])
        x = src[z2].reshape(2, 4, 4, 4, 8, 128)
        p = jnp.exp2(x - mm[:, None, :, None]).reshape(HS, 128)
        l = _tree_sum(p)
        rs = pl.ds(pl.multiple_of(g * 64 + hh * 16, 16), 16)
        dep2 = jnp.concatenate([dep, dep], axis=0)
        vu = vt_s[half * 8:half * 8 + 8, rs, :] | dep2[None]
        vu = jnp.concatenate([vu[t] for t in range(8)], axis=1)
        o = jnp.dot(_unpack(vu), p.astype(bf), preferred_element_type=f32)
        return o, l

    def store_o(g, j, parts):
        outs = [parts[2 * h] * (1.0 / jnp.sum(parts[2 * h + 1], axis=0, keepdims=True)) for h in range(4)]
        ot = jnp.concatenate(outs, axis=0)
        o_s[g, pl.ds(pl.multiple_of(j * 64, 64), 64), :] = _pack(ot.T)

    def finalize(g, j, slot):
        x = fin[slot]
        parts = []
        for hh in range(4):
            parts += [x[hh * 40: hh * 40 + 32], x[hh * 40 + 32: hh * 40 + 40]]
        store_o(g, j, parts)

    def attention():
        ma = fullmax(qk(0, 0, 0, 0, a1, 0)[0], qk(0, 0, 0, 1, a2, 0)[0])
        mb1 = qk(0, 0, 1, 0, b1, 0)[0]
        bufs = {(0, 0): a1, (0, 1): a2, (1, 0): b1, (1, 1): b2}

        def body(it, carry):
            ma, mb1 = carry
            z1 = z_ref[0]
            z2 = z_ref[1]
            zv = jnp.full((8, 128), z1, i32).astype(u32)
            tp = jnp.maximum(it * UNR - 1, 0)
            finalize(tp // NQ, tp % NQ, z2)
            do = None
            ps = None
            po = None

            def tg(sv, i):
                return None if sv is None else pltpu.bitcast(sv[i * 8:i * 8 + 8], u32) & zv

            for u in range(UNR):
                zk = [z_ref[2 + 8 * u + i] for i in range(8)]
                t = it * UNR + u
                g = t // NQ
                j = t % NQ
                tn = jnp.minimum(t + 1, G * NQ - 1)
                gn = tn // NQ
                jn = tn % NQ
                qks = [(g, j, 1, 1), (g, j, 2, 0), (g, j, 2, 1), (g, j, 3, 0), (g, j, 3, 1),
                       (gn, jn, 0, 0), (gn, jn, 0, 1), (gn, jn, 1, 0)]
                mfull = {0: ma}
                mpart = {1: mb1}
                os_, ls_ = {}, {}
                for n in range(8):
                    qg, qj, qh, qhalf = qks[n]
                    key = qh if n < 5 else qh + 4
                    mp, first, cs_ = qk(qg, qj, qh, qhalf, bufs[(qh % 2, qhalf)], z1, zk[n], do)
                    if qhalf == 0:
                        mpart[key] = mp
                    else:
                        mfull[key] = fullmax(mpart[key], mp)
                    ph, phalf = n // 2, n % 2
                    trigs = [tg(ps, i) for i in TA] + [tg(po, TB[0])] + [tg(cs_, i) for i in TB[1:]]
                    o, l = sm_pv(g, ph, phalf, bufs[(ph % 2, phalf)], mfull[ph], z2, first & zv, trigs)
                    ps = cs_
                    po = o
                    do = tg(o, 3)
                    os_[(ph, phalf)] = o
                    ls_[(ph, phalf)] = l
                ma = mfull[4]
                mb1 = mpart[5]
                parts = []
                for h in range(4):
                    parts += [os_[(h, 0)] + os_[(h, 1)], ls_[(h, 0)] + ls_[(h, 1)]]
                if u == UNR - 1:
                    fin[z1] = jnp.concatenate(parts, axis=0)
                else:
                    store_o(g, j, parts)
            return ma, mb1

        lax.fori_loop(0, G * NQ // UNR * 1, lambda i, c: body(i % (G * NQ // UNR), c), (ma, mb1))
        finalize(G - 1, NQ - 1, 0)

    with scope('S_conv'):
        conv()
    if '1' in ONLY:
        with scope('S_ph1'):
            lax.fori_loop(0, NRC, phase1, 0)
    else:
        x_copy(1).wait()
        wo_copy().start()
    wo_copy().wait()
    if 'a' in ONLY:
        with scope('S_att1'):
            attention()
    if '2' in ONLY:
        with scope('S_ph2'):
            phase2()
    if 'a' in ONLY:
        with scope('S_att2'):
            attention()
    if '3' in ONLY:
        with scope('S_ph3'):
            phase3()
    else:
        out_s[0:8, 0:128] = (y_s[0, 7, 0:8, :] + y_s[1, 7, 0:8, :] + pltpu.bitcast(h_s[0:8, 0:128], f32)).astype(bf)
        for c in range(NRC - 1):
            out_copy(c).start()
        for q in range(3):
            tail_copy(q).start()
    for c in range(NRC - 1):
        out_copy(c).wait()
    for q in range(3):
        tail_copy(q).wait()


@jax.jit
def pallas_interleave_layers__softmax_full_mha__ssm_conv_h3__prompt_kernel(A_x, A_wqkv, A_wo, B_q, B_k, B_v, B_shift_k, B_ssm_k, B_ssm_D):
    fwd, inv = _dft_mats()
    fwd = jnp.asarray(fwd[None])
    inv = jnp.asarray(inv[None])
    scratch = [
        pltpu.VMEM((1, S, D), f32),
        pltpu.VMEM((2, G, S, 128), f32),
        pltpu.VMEM((NQ, D // 2, 128), u32),
        pltpu.VMEM((G, S // 2, 128), u32),
        pltpu.VMEM((NQ, D // 2, 128), u32),
        pltpu.VMEM((G, S // 2, 128), u32),
        pltpu.VMEM((1, HS, 128), f32), pltpu.VMEM((1, HS, 128), f32),
        pltpu.VMEM((1, HS, 128), f32), pltpu.VMEM((1, HS, 128), f32),
        pltpu.VMEM((1, 160, 128), f32),
        pltpu.VMEM((1, S + 8, 128), f32),
        pltpu.VMEM((G, 40, 128), f32),
        pltpu.VMEM((1, 2 * NC, 3, IM, 128), f32),
        pltpu.VMEM((1, 2 * NC, 3, IM, 128), f32),
        pltpu.VMEM((NC, 128, 128), u32),
        pltpu.VMEM((NC, 128, 128), u32),
        pltpu.VMEM((S, 128), u32),
        pltpu.VMEM((S, 128), u32),
        pltpu.VMEM((RC // 2, D), u32),
        pltpu.SMEM((NZ,), i32),
        pltpu.VMEM((1, S, D), bf),
        pltpu.VMEM((D, 3 * D + 128), bf),
        pltpu.VMEM((D, D + 128), bf),
        pltpu.VMEM((G, S, 128), bf),
        pltpu.VMEM((G, S, 128), bf),
        pltpu.VMEM((D, S + 128), bf),
        pltpu.VMEM((S, D), bf),
        pltpu.VMEM((4, D), bf),
        pltpu.VMEM((G, 128), bf),
        pltpu.VMEM((1, 320, 128), u32),
        pltpu.VMEM((1, 64, 256), u32),
        pltpu.SemaphoreType.DMA((3, G)),
        pltpu.SemaphoreType.DMA((NRC,)),
        pltpu.SemaphoreType.DMA((G + 1,)),
        pltpu.SemaphoreType.DMA((NRC + 2,)),
        pltpu.SemaphoreType.DMA((4,)),
    ]
    hbm = pl.BlockSpec(memory_space=pl.ANY)
    return pl.pallas_call(
        _kernel,
        out_shape=jax.ShapeDtypeStruct((1, S, D), bf),
        in_specs=[hbm] * 10,
        out_specs=hbm,
        scratch_shapes=scratch,
        compiler_params=pltpu.CompilerParams(vmem_limit_bytes=120 * 2**20, disable_bounds_checks=bool(NOBC)),
    )(A_x, A_wqkv, A_wo, B_k, B_v, B_shift_k.T, B_ssm_k, B_ssm_D.reshape(G, 128), fwd, inv)
```

```python
import numpy as np
import jax
import jax.numpy as jnp
from jax import lax
import jax.experimental.pallas as pl
import jax.experimental.pallas.tpu as pltpu

S = 2048
D = 1024
DH = 32
G = 8
NQ = 16
HS = S // 2
CH = HS // 4
UNR = 8
TA = (17, 21, 25, 29)
TB = (0, 4, 8)
RC = 256
NRC = S // RC
NP = RC // 16
NC = 16
IM = 136
GO = 8
R0 = 4
EPS = 1e-5
NZ = 2 + 8 * UNR
QSCALE = float(DH ** -0.5 * np.log2(np.e))

bf = jnp.bfloat16
f32 = jnp.float32
u32 = jnp.uint32
i32 = jnp.int32
NT = (((1,), (1,)), ((), ()))


def _dft_mats():
    n = np.arange(128)
    f = np.concatenate([np.arange(0, 128, 2), np.arange(1, 128, 2)])
    ang = 2.0 * np.pi * np.outer(f + 0.5, n) / 256.0
    re, im = np.cos(ang), -np.sin(ang)
    inv = np.concatenate([re, im], axis=0).T / 128.0
    fwd = np.concatenate([re, im, re, im - re, im + re], axis=0)

    def pack_rows(a):
        u = np.ascontiguousarray(a, dtype=np.float32).view(np.uint32)
        u = (u + 0x7FFF + ((u >> 16) & 1)) >> 16
        return (u[0::2] | (u[1::2] << 16)).astype(np.uint32)
    return pack_rows(fwd), pack_rows(inv)


def _tree_sum(p):
    n = p.shape[0] // 8
    x = p.reshape(n, 8, 128)
    while n > 1:
        x = x.reshape(n // 2, 2, 8, 128)
        x = x[:, 0] + x[:, 1]
        n //= 2
    return x[0]


def _ln(x):
    m = jnp.mean(x, axis=-1, keepdims=True)
    xc = x - m
    v = jnp.mean(xc * xc, axis=-1, keepdims=True)
    return xc * lax.rsqrt(v + EPS)


def _pack(x):
    return pltpu.bitcast(x.astype(bf), u32)


def _unpack(x):
    return pltpu.bitcast(x, bf)


def _tok(v, zv):
    v = v if v.dtype == u32 else pltpu.bitcast(v, u32)
    while v.shape[1] > 128:
        h = v.shape[1] // 2
        v = v[:, :h] | v[:, h:]
    while v.shape[0] > 8:
        h = v.shape[0] // 2
        v = v[:h] | v[h:]
    return v & zv


def _gate(w, toks):
    if not toks:
        return w
    wu = pltpu.bitcast(w, u32)
    h0 = wu[0:8]
    for t in toks:
        h0 = h0 | t
    return _unpack(jnp.concatenate([h0, wu[8:]], axis=0))


def _kernel(x_hbm, wqkv_hbm, wo_hbm, bk_hbm, bv_hbm, shk_hbm, ssmk_hbm, ssmd_hbm, fwd_hbm, inv_hbm, out_hbm,
            x_s, y_s, qt_s, k_s, vt_s, o_s, a1, a2, b1, b2, fin, kf_s, taps_s, ug_a, ug_b, zb_a, zb_b,
            pb_a, pb_b, h_s, z_ref, x_in, wqkv, wo, bk, bv, ssmk, out_s, shk, ssmd, fwd_ref, inv_ref,
            sem_c, sem_x, sem_w, sem_o, sem_s):
    def kv_copies(cb):
        cs = pl.ds(pl.multiple_of(cb * 128, 128), 128)
        return [pltpu.make_async_copy(bk_hbm.at[0, :, cs], bk.at[cb], sem_c.at[0, cb]),
                pltpu.make_async_copy(bv_hbm.at[0, :, cs], bv.at[cb], sem_c.at[1, cb])]

    def h_copy(cb):
        cs = pl.ds(pl.multiple_of(cb * 128, 128), 128)
        return pltpu.make_async_copy(ssmk_hbm.at[cs, :], ssmk.at[cs, pl.ds(0, S)], sem_c.at[2, cb])

    def x_copy(c):
        rs = pl.ds(pl.multiple_of(c * RC, RC), RC)
        return pltpu.make_async_copy(x_hbm.at[0, rs, :], x_in.at[rs, :], sem_x.at[c])

    def w_copy(c):
        rs = pl.ds(pl.multiple_of(c * 128, 128), 128)
        return pltpu.make_async_copy(wqkv_hbm.at[rs, :], wqkv.at[rs, pl.ds(0, 3 * D)], sem_w.at[c])

    def wo_copy():
        return pltpu.make_async_copy(wo_hbm, wo.at[:, pl.ds(0, D)], sem_w.at[G])

    def out_copy(c):
        rs = pl.ds(pl.multiple_of(c * RC, RC), RC)
        return pltpu.make_async_copy(out_s.at[rs, :], out_hbm.at[0, rs, :], sem_o.at[c])

    TAIL = (0, 128, 192, 256)

    def tail_copy(q):
        rs = pl.ds((NRC - 1) * RC + TAIL[q], TAIL[q + 1] - TAIL[q])
        return pltpu.make_async_copy(out_s.at[rs, :], out_hbm.at[0, rs, :], sem_o.at[NRC - 1 + q])

    def conv_start(c):
        h_copy(c).start()
        for cp in kv_copies(c):
            cp.start()

    def wait_all(cps):
        for cp in cps:
            cp.wait()

    shk_cp, ssmd_cp, fwd_cp, inv_cp = [
        pltpu.make_async_copy(src, dst, sem_s.at[i]) for i, (src, dst) in enumerate(
            ((shk_hbm, shk), (ssmd_hbm, ssmd), (fwd_hbm, fwd_ref), (inv_hbm, inv_ref)))]
    h_copy(0).start()
    fwd_cp.start()
    shk_cp.start()
    ssmd_cp.start()
    for cp in kv_copies(0):
        cp.start()

    for i in range(NZ):
        z_ref[i] = 0
    fin[...] = jnp.ones(fin.shape, f32)
    kf_s[0, 0:8, :] = jnp.zeros((8, 128), f32)

    def zero_vreg():
        return jnp.full((8, 128), z_ref[0], i32).astype(u32)

    def fence(cps):
        @pl.when(z_ref[0] == 0)
        def _():
            wait_all(cps)

    TILES = [(0, n) for n in range(8)] + [(2, n) for n in range(8)] + [(1, n) for n in range(8)]

    def qkv_tile(h, c, idx, toks, zv):
        kind, n = TILES[idx]
        col = kind * D + n * 128
        r = jnp.dot(h, _gate(wqkv[:, col:col + 128], toks), preferred_element_type=f32)
        if kind == 1:
            k_s[n, pl.ds(pl.multiple_of(c * (RC // 2), RC // 2), RC // 2), :] = _pack(r)
            return None
        dst = qt_s if kind == 0 else vt_s
        if kind == 0:
            r = r * QSCALE
        pks = []
        for t in range(RC // 128):
            pk = _pack(r[t * 128:(t + 1) * 128, :].T)
            dst[c * (RC // 128) + t, n * 64:(n + 1) * 64, :] = pk
            pks.append(pk)
        return _tok(jnp.concatenate(pks, axis=0), zv)

    def qkv_proj(h, c, piece_fn, first_piece):
        zv = zero_vreg()
        deps = {}
        for n in range(24):
            done = qkv_tile(h, c, n, deps.get(n), zv)
            if done is not None:
                deps.setdefault(n + 3, []).append(done)
            if piece_fn is not None and first_piece <= n < first_piece + NP:
                deps.setdefault(n + 3, []).append(_tok(piece_fn(n - first_piece), zv))

    def piece_rows(c, p):
        return pl.ds(pl.multiple_of(c * RC + p * 16, 16), 16)

    def ln1_piece(c, p):
        hp = _pack(_ln(x_in[piece_rows(c, p), :].astype(f32)))
        h_s[p * 8:(p + 1) * 8, :] = hp
        return hp

    def gated_x(c, p, z):
        rows = piece_rows(c, p)
        x1 = x_s[z, rows, :]
        y = jnp.concatenate([y_s[0, g, rows, :] + y_s[1, g, rows, :] for g in range(G)], axis=1)
        return x1 + _ln(x1) * y

    def ln2_piece(c, p, z):
        x2 = gated_x(c, p, z)
        x_s[z, piece_rows(c, p), :] = x2
        hp = _pack(_ln(x2))
        h_s[p * 8:(p + 1) * 8, :] = hp
        return hp

    def out_piece(c, p, z):
        v = gated_x(c, p, z)
        out_s[piece_rows(c, p), :] = v.astype(bf)
        return v

    def load_o(c):
        rs = pl.ds(pl.multiple_of(c * (RC // 2), RC // 2), RC // 2)
        return jnp.concatenate([_unpack(o_s[g, rs, :]) for g in range(G)], axis=1)

    def oproj_tile(o, c, n, z, toks=None, r0=0, nr=RC, first=False):
        rows = pl.ds(pl.multiple_of(c * RC + r0, nr), nr)
        cols = slice(n * 128, (n + 1) * 128)
        r = jnp.dot(o[r0:r0 + nr], _gate(wo[:, cols], toks), preferred_element_type=f32)
        x0 = x_in[rows, cols].astype(f32) if first else x_s[z, rows, cols]
        x_s[z, rows, cols] = x0 + r

    zts = [z_ref[2 + ib] for ib in range(4)]

    def setup_taps():
        taps = shk[...].astype(f32)
        for cb in range(G):
            for t in range(4):
                taps_s[cb, 8 * t:8 * t + 8, :] = jnp.broadcast_to(taps[t:t + 1, cb * 128:(cb + 1) * 128], (8, 128))

    def setup_skip():
        dall = ssmd[...].astype(f32)
        for cb in range(G):
            taps_s[cb, 32:40, :] = jnp.broadcast_to(dall[cb:cb + 1, :], (8, 128))

    def prep_h_chunk(cb, pb, j):
        cs = pl.ds(pl.multiple_of(cb * 128, 128), 128)
        pb[HS + j * 64:HS + (j + 1) * 64, :] = pltpu.bitcast(ssmk[cs, j * 128:(j + 1) * 128], u32)

    def prep_h(cb, pb):
        for j in range(NC):
            prep_h_chunk(cb, pb, j)

    def prep_kv(cb, pb, with_h):
        zs = z_ref[1]
        tp = taps_s[cb, 0:32, :]
        for j in range(NC):
            r0 = j * 128
            if with_h:
                prep_h_chunk(cb, pb, j)
            kf_s[zs, 8 + r0:8 + r0 + 128, :] = bk[cb, r0:r0 + 128, :].astype(f32)
            ks = None
            for t in range(4):
                term = kf_s[zs, 8 + r0 - t:8 + r0 - t + 128, :].reshape(16, 8, 128) * tp[8 * t:8 * t + 8][None]
                ks = term if ks is None else ks + term
            pb[j * 64:(j + 1) * 64, :] = _pack(ks.reshape(128, 128) * bv[cb, r0:r0 + 128, :].astype(f32))

    def fwd_h(pb, ug):
        for m in range(NC):
            hm = lax.dot_general(_unpack(fwd_ref[128:320, :]), _unpack(pb[HS + m * 64:HS + (m + 1) * 64, :]),
                                 NT, preferred_element_type=f32)
            ug[0, NC + m, :, GO:GO + 128, :] = hm.reshape(3, 128, 128)

    def fwd_u(pb, ug):
        for j in range(NC):
            u = jnp.dot(_unpack(fwd_ref[0:128, :]), _unpack(pb[j * 64:(j + 1) * 64, :]),
                        preferred_element_type=f32)
            ug[0, j, 0:2, 0:128, :] = u.reshape(2, 128, 128)

    def add_skip(cb, ug):
        dv = taps_s[cb, 32:40, :][None]
        for e in range(3):
            v = ug[0, NC, e, GO:GO + 128, :].reshape(16, 8, 128)
            ug[0, NC, e, GO:GO + 128, :] = (v - dv if e == 1 else v + dv).reshape(128, 128)

    def spec_item(ug, ib, r):
        zt = zts[ib]
        acc = None
        for j in range(4 * ib + 4):
            u = ug[zt, j:j + 1, 0:2, r:r + 8, :]
            u = jnp.concatenate([u[:, 0:1] + u[:, 1:2], u], axis=1)
            q0 = max(0, j - 4 * ib)
            m0 = NC + 4 * ib - j
            t = ug[zt, m0 + q0:m0 + 4, :, GO + r:GO + r + 8, :] * u
            if acc is None:
                acc = t
            elif q0 == 0:
                acc = acc + t
            else:
                acc = jnp.concatenate([acc[:q0], acc[q0:] + t], axis=0)
        return acc[:, 0] - acc[:, 2], acc[:, 0] + acc[:, 1]

    def overlap_add(yr, yi, prev, r):
        n = 1 if prev is None else 0
        pr = yr[:3] if prev is None else jnp.concatenate([prev[0], yr[:3]], axis=0)
        pi = yi[:3] if prev is None else jnp.concatenate([prev[1], yi[:3]], axis=0)
        if r < 64:
            zr, zi = yr[n:] - pi, yi[n:] + pr
        else:
            zr, zi = yr[n:] + pi, yi[n:] - pr
        if prev is None:
            zr = jnp.concatenate([yr[:1], zr], axis=0)
            zi = jnp.concatenate([yi[:1], zi], axis=0)
        return zr, zi, (yr[3:], yi[3:])

    def conv_spec(ug, zb, lo=0, hi=8):
        for rp in range(lo, hi):
            p0 = p1 = None
            for ib in range(4):
                zr0, zi0, p0 = overlap_add(*spec_item(ug, ib, 16 * rp), p0, 16 * rp)
                zr1, zi1, p1 = overlap_add(*spec_item(ug, ib, 16 * rp + 8), p1, 16 * rp)
                zb[4 * ib:4 * ib + 4, rp * 8:rp * 8 + 8, :] = _pack(jnp.concatenate([zr0, zr1], axis=1))
                zb[4 * ib:4 * ib + 4, 64 + rp * 8:72 + rp * 8, :] = _pack(jnp.concatenate([zi0, zi1], axis=1))

    def conv_inv(cb, zb):
        for i in range(NC):
            for e in range(2):
                y_s[e, cb, i * 128:(i + 1) * 128, :] = jnp.dot(
                    _unpack(inv_ref[:, e * 128:(e + 1) * 128]), _unpack(zb[i, e * 64:(e + 1) * 64, :]),
                    preferred_element_type=f32)

    def conv_step(c, ug_cur, ug_nxt, zb_cur, zb_prev, pb_nxt, pb_new):
        @pl.when(c + 3 < G)
        def _():
            conv_start(c + 3)
        w_copy(c).start()

        @pl.when(c >= G - 3)
        def _():
            x_copy(c - (G - 3)).start()
        conv_spec(ug_cur, zb_cur)
        fwd_h(pb_nxt, ug_nxt)
        fwd_u(pb_nxt, ug_nxt)
        conv_inv(c - 1, zb_prev)

        @pl.when(c + 2 < G)
        def _():
            wait_all([w_copy(c - 1), h_copy(c + 2)] + kv_copies(c + 2))
            prep_kv(c + 2, pb_new, True)
            add_skip(c + 1, ug_nxt)

        @pl.when(c + 2 >= G)
        def _():
            w_copy(c - 1).wait()
            add_skip(c + 1, ug_nxt)

    def conv():
        wait_all([fwd_cp, h_copy(0)])
        conv_start(1)
        inv_cp.start()
        prep_h(0, pb_a)
        fwd_h(pb_a, ug_a)
        wait_all([shk_cp] + kv_copies(0))
        conv_start(2)
        setup_taps()
        prep_kv(0, pb_a, False)
        fwd_u(pb_a, ug_a)
        fence([h_copy(1)])
        prep_h(1, pb_b)
        fence([ssmd_cp])
        setup_skip()
        add_skip(0, ug_a)
        conv_spec(ug_a, zb_a, 0, R0)
        fwd_h(pb_b, ug_b)
        fence(kv_copies(1))
        conv_start(3)
        w_copy(0).start()
        prep_kv(1, pb_b, False)
        add_skip(1, ug_b)
        fence([h_copy(2)])
        conv_spec(ug_a, zb_a, R0, 8)
        fwd_u(pb_b, ug_b)
        fence(kv_copies(2) + [inv_cp])
        prep_kv(2, pb_a, True)

        def body(p, carry):
            conv_step(2 * p + 1, ug_b, ug_a, zb_b, zb_a, pb_a, pb_b)
            conv_step(2 * p + 2, ug_a, ug_b, zb_a, zb_b, pb_b, pb_a)
            return carry
        lax.fori_loop(0, G // 2 - 1, body, 0)
        w_copy(G - 1).start()
        conv_spec(ug_b, zb_b)
        conv_inv(G - 2, zb_a)
        fence([x_copy(0)])
        for p in range(NP):
            ln1_piece(0, p)
        conv_inv(G - 1, zb_b)
        wait_all([w_copy(G - 2), w_copy(G - 1)])

    def phase1():
        def body(c, carry):
            @pl.when(c + 1 < NRC)
            def _():
                x_copy(c + 1).wait()

            @pl.when(c + 2 < NRC)
            def _():
                x_copy(c + 2).start()

            @pl.when(c + 2 == NRC)
            def _():
                wo_copy().start()
            cn = jnp.minimum(c + 1, NRC - 1)
            qkv_proj(_unpack(h_s[...]), c, lambda p: ln1_piece(cn, p), 2)
            return carry
        lax.fori_loop(0, NRC, body, 0)
        wo_copy().wait()

    def phase2():
        o = load_o(0)
        z0 = z_ref[0]
        for q in range(2):
            for n in range(8):
                oproj_tile(o, 0, n, z0, None, q * (RC // 2), RC // 2, True)
            for p in range(q * NP // 2, (q + 1) * NP // 2):
                ln2_piece(0, p, z0)

        def body(c, carry):
            z0 = z_ref[0]
            z1 = z_ref[1]
            h = _unpack(h_s[...])
            o = load_o(c + 1)
            for n in range(8):
                oproj_tile(o, c + 1, n, z1, first=True)
            qkv_proj(h, c, lambda p: ln2_piece(c + 1, p, z0), 1)
            return carry
        lax.fori_loop(0, NRC - 1, body, 0)
        qkv_proj(_unpack(h_s[...]), NRC - 1, None, 0)

    def phase3():
        o = load_o(0)
        for n in range(8):
            oproj_tile(o, 0, n, z_ref[1])

        def body(c, carry):
            z0 = z_ref[0]
            z1 = z_ref[1]
            zv = zero_vreg()
            o = load_o(c + 1)
            deps = {}
            p = 0
            for t in range(16):
                for _ in range(2 if t < 2 else 1):
                    if p < NP:
                        deps.setdefault(t + 2, []).append(_tok(out_piece(c, p, z0), zv))
                        p += 1
                oproj_tile(o, c + 1, t // 2, z1, deps.get(t), (t % 2) * 128, 128)
            out_copy(c).start()
            return carry
        lax.fori_loop(0, NRC - 2, body, 0)

        c = NRC - 1
        z0 = z_ref[0]
        zv = zero_vreg()
        o = load_o(c)
        deps = {}
        todo = [(c - 1, p) for p in range(NP)]
        for q in range(3):
            for n in range(8):
                t = 8 * q + n
                for cc, p in todo[2 * n:2 * n + 2]:
                    deps.setdefault(t + 2, []).append(_tok(out_piece(cc, p, z0), zv))
                oproj_tile(o, c, n, z0, deps.get(t), TAIL[q], TAIL[q + 1] - TAIL[q])
            (out_copy(c - 1) if q == 0 else tail_copy(q - 1)).start()
            todo = [(c, p) for p in range(TAIL[q] // 16, TAIL[q + 1] // 16)]
        for cc, p in todo:
            out_piece(cc, p, z0)
        tail_copy(2).start()
        wait_all([out_copy(i) for i in range(NRC - 1)] + [tail_copy(q) for q in range(3)])

    zero16 = jnp.zeros((16, 128), u32)

    def qk(g, j, hh, half, dst, z, zk=0, dep=None):
        qt = qt_s[j, pl.ds(pl.multiple_of(g * 64 + hh * 16, 16), 16), :]
        w = _unpack(jnp.concatenate([qt if i == hh else zero16 for i in range(4)], axis=0))
        kh = k_s[g + zk, half * HS // 2:(half + 1) * HS // 2, :]
        m = first = s = None
        for c in range(4):
            ku = kh[c * CH // 2:(c + 1) * CH // 2]
            if dep is not None:
                ku = jnp.concatenate([ku[:CH // 2 - 8], ku[CH // 2 - 8:] | dep], axis=0)
            s = jnp.dot(_unpack(ku), w, preferred_element_type=f32)
            dst[z, c * CH:(c + 1) * CH, :] = s
            mc = jnp.max(s.reshape(CH // 8, 8, 128), axis=0)
            m = mc if m is None else jnp.maximum(m, mc)
            f = pltpu.bitcast(s[0:8], u32)
            first = f if first is None else first | f
        return m, first, s

    def fullmax(m1, m2):
        return jnp.max(jnp.maximum(m1, m2), axis=0, keepdims=True)

    def sm_pv(g, hh, half, src, m, z, dep, trigs):
        mb = jnp.broadcast_to(m, (8, 128))
        mbu = pltpu.bitcast(mb, u32)
        ms = [mb if tr is None else pltpu.bitcast(mbu | tr, f32) for tr in trigs]
        mm = jnp.stack([jnp.stack([ms[4 * st + 3 - kk] for kk in range(4)]) for st in range(2)])
        x = src[z].reshape(2, 4, 4, 4, 8, 128)
        p = jnp.exp2(x - mm[:, None, :, None]).reshape(HS, 128)
        rs = pl.ds(pl.multiple_of(g * 64 + hh * 16, 16), 16)
        vu = vt_s[half * 8:half * 8 + 8, rs, :] | jnp.concatenate([dep, dep], axis=0)[None]
        vu = jnp.concatenate([vu[t] for t in range(8)], axis=1)
        l = _tree_sum(p)
        return jnp.dot(_unpack(vu), p.astype(bf), preferred_element_type=f32), l

    def store_o(g, j, parts):
        outs = [parts[2 * h] * (1.0 / jnp.sum(parts[2 * h + 1], axis=0, keepdims=True)) for h in range(4)]
        o_s[g, pl.ds(pl.multiple_of(j * 64, 64), 64), :] = _pack(jnp.concatenate(outs, axis=0).T)

    def finalize(g, j, slot):
        x = fin[slot]
        parts = []
        for hh in range(4):
            parts += [x[hh * 40:hh * 40 + 32], x[hh * 40 + 32:hh * 40 + 40]]
        store_o(g, j, parts)

    def attention():
        ma = fullmax(qk(0, 0, 0, 0, a1, 0)[0], qk(0, 0, 0, 1, a2, 0)[0])
        mb1 = qk(0, 0, 1, 0, b1, 0)[0]
        bufs = {(0, 0): a1, (0, 1): a2, (1, 0): b1, (1, 1): b2}
        nit = G * NQ // UNR

        def tile_of(t):
            return lax.shift_right_logical(t, 4), t & (NQ - 1)

        def body(it, carry):
            ma, mb1 = carry
            z1 = z_ref[0]
            z2 = z_ref[1]
            zv = zero_vreg()
            g, j0 = tile_of(it * UNR)
            finalize(*tile_of(jnp.maximum(it * UNR - 1, 0)), z2)
            do = ps = po = None

            def tg(sv, i):
                return None if sv is None else pltpu.bitcast(sv[i * 8:i * 8 + 8], u32) & zv

            for u in range(UNR):
                j = j0 + u
                gn, jn = (g, j + 1) if u < UNR - 1 else tile_of(jnp.minimum(it + 1, nit - 1) * UNR)
                qks = [(g, j, 1, 1), (g, j, 2, 0), (g, j, 2, 1), (g, j, 3, 0), (g, j, 3, 1),
                       (gn, jn, 0, 0), (gn, jn, 0, 1), (gn, jn, 1, 0)]
                mfull = {0: ma}
                mpart = {1: mb1}
                res = []
                for n in range(8):
                    qg, qj, qh, qhalf = qks[n]
                    key = qh if n < 5 else qh + 4
                    mp, first, cs = qk(qg, qj, qh, qhalf, bufs[(qh % 2, qhalf)], z1, z_ref[2 + 8 * u + n], do)
                    if qhalf == 0:
                        mpart[key] = mp
                    else:
                        mfull[key] = fullmax(mpart[key], mp)
                    ph, phalf = n // 2, n % 2
                    trigs = [tg(ps, i) for i in TA] + [tg(po, 0)] + [tg(cs, i) for i in TB]
                    o, l = sm_pv(g, ph, phalf, bufs[(ph % 2, phalf)], mfull[ph], z2, first & zv, trigs)
                    ps, po, do = cs, o, tg(o, 3)
                    res.append((o, l))
                ma = mfull[4]
                mb1 = mpart[5]
                parts = []
                for h in range(4):
                    parts += [res[2 * h][0] + res[2 * h + 1][0], res[2 * h][1] + res[2 * h + 1][1]]
                if u == UNR - 1:
                    fin[z1] = jnp.concatenate(parts, axis=0)
                else:
                    store_o(g, j, parts)
            return ma, mb1

        lax.fori_loop(0, nit, body, (ma, mb1))
        finalize(G - 1, NQ - 1, 0)

    conv()
    phase1()
    attention()
    phase2()
    attention()
    phase3()


@jax.jit
def pallas_interleave_layers__softmax_full_mha__ssm_conv_h3__prompt_kernel(
        A_x, A_wqkv, A_wo, B_q, B_k, B_v, B_shift_k, B_ssm_k, B_ssm_D):
    del B_q
    fwd, inv = _dft_mats()
    scratch = [
        pltpu.VMEM((1, S, D), f32),
        pltpu.VMEM((2, G, S, 128), f32),
        pltpu.VMEM((NQ, D // 2, 128), u32),
        pltpu.VMEM((G, S // 2, 128), u32),
        pltpu.VMEM((NQ, D // 2, 128), u32),
        pltpu.VMEM((G, S // 2, 128), u32),
        pltpu.VMEM((1, HS, 128), f32), pltpu.VMEM((1, HS, 128), f32),
        pltpu.VMEM((1, HS, 128), f32), pltpu.VMEM((1, HS, 128), f32),
        pltpu.VMEM((1, 160, 128), f32),
        pltpu.VMEM((1, S + 8, 128), f32),
        pltpu.VMEM((G, 40, 128), f32),
        pltpu.VMEM((1, 2 * NC, 3, IM, 128), f32),
        pltpu.VMEM((1, 2 * NC, 3, IM, 128), f32),
        pltpu.VMEM((NC, 128, 128), u32),
        pltpu.VMEM((NC, 128, 128), u32),
        pltpu.VMEM((S, 128), u32),
        pltpu.VMEM((S, 128), u32),
        pltpu.VMEM((RC // 2, D), u32),
        pltpu.SMEM((NZ,), i32),
        pltpu.VMEM((S, D), bf),
        pltpu.VMEM((D, 3 * D + 128), bf),
        pltpu.VMEM((D, D + 128), bf),
        pltpu.VMEM((G, S, 128), bf),
        pltpu.VMEM((G, S, 128), bf),
        pltpu.VMEM((D, S + 128), bf),
        pltpu.VMEM((S, D), bf),
        pltpu.VMEM((4, D), bf),
        pltpu.VMEM((G, 128), bf),
        pltpu.VMEM((320, 128), u32),
        pltpu.VMEM((64, 256), u32),
        pltpu.SemaphoreType.DMA((3, G)),
        pltpu.SemaphoreType.DMA((NRC,)),
        pltpu.SemaphoreType.DMA((G + 1,)),
        pltpu.SemaphoreType.DMA((NRC + 2,)),
        pltpu.SemaphoreType.DMA((4,)),
    ]
    hbm = pl.BlockSpec(memory_space=pl.ANY)
    return pl.pallas_call(
        _kernel,
        out_shape=jax.ShapeDtypeStruct((1, S, D), bf),
        in_specs=[hbm] * 10,
        out_specs=hbm,
        scratch_shapes=scratch,
        compiler_params=pltpu.CompilerParams(vmem_limit_bytes=120 * 2**20, disable_bounds_checks=True),
    )(A_x, A_wqkv, A_wo, B_k, B_v, B_shift_k.T, B_ssm_k, B_ssm_D.reshape(G, 128),
      jnp.asarray(fwd), jnp.asarray(inv))
```

```python
import numpy as np
import jax
import jax.numpy as jnp
from jax import lax
import jax.experimental.pallas as pl
import jax.experimental.pallas.tpu as pltpu

S = 2048
D = 1024
DH = 32
G = 8
NQ = 16
HS = S // 2
CH = HS // 4
UNR = 8
TA = (17, 21, 25, 29)
TB = (0, 4, 8)
RC = 256
NRC = S // RC
NP = RC // 16
NC = 16
IM = 136
GO = 8
R0 = 4
EPS = 1e-5
NZ = 2 + 8 * UNR
QSCALE = float(DH ** -0.5 * np.log2(np.e))

bf = jnp.bfloat16
f32 = jnp.float32
u32 = jnp.uint32
i32 = jnp.int32
NT = (((1,), (1,)), ((), ()))


def _dft_mats():
    n = np.arange(128)
    f = np.concatenate([np.arange(0, 128, 2), np.arange(1, 128, 2)])
    ang = 2.0 * np.pi * np.outer(f + 0.5, n) / 256.0
    re, im = np.cos(ang), -np.sin(ang)
    inv = np.concatenate([re, im], axis=0).T / 128.0
    fwd = np.concatenate([re, im, re, im - re, im + re], axis=0)

    def pack_rows(a):
        u = np.ascontiguousarray(a, dtype=np.float32).view(np.uint32)
        u = (u + 0x7FFF + ((u >> 16) & 1)) >> 16
        return (u[0::2] | (u[1::2] << 16)).astype(np.uint32)
    return pack_rows(fwd), pack_rows(inv)


def _tree_sum(p):
    n = p.shape[0] // 8
    x = p.reshape(n, 8, 128)
    while n > 1:
        x = x.reshape(n // 2, 2, 8, 128)
        x = x[:, 0] + x[:, 1]
        n //= 2
    return x[0]


def _ln(x):
    m = jnp.mean(x, axis=-1, keepdims=True)
    xc = x - m
    v = jnp.mean(xc * xc, axis=-1, keepdims=True)
    return xc * lax.rsqrt(v + EPS)


def _pack(x):
    return pltpu.bitcast(x.astype(bf), u32)


def _unpack(x):
    return pltpu.bitcast(x, bf)


def _tok(v, zv):
    v = v if v.dtype == u32 else pltpu.bitcast(v, u32)
    while v.shape[1] > 128:
        h = v.shape[1] // 2
        v = v[:, :h] | v[:, h:]
    while v.shape[0] > 8:
        h = v.shape[0] // 2
        v = v[:h] | v[h:]
    return v & zv


def _gate(w, toks):
    if not toks:
        return w
    wu = pltpu.bitcast(w, u32)
    h0 = wu[0:8]
    for t in toks:
        h0 = h0 | t
    return _unpack(jnp.concatenate([h0, wu[8:]], axis=0))


def _kernel(x_hbm, wqkv_hbm, wo_hbm, bk_hbm, bv_hbm, shk_hbm, ssmk_hbm, ssmd_hbm, fwd_hbm, inv_hbm, out_hbm,
            x_s, y_s, qt_s, k_s, vt_s, o_s, a1, a2, b1, b2, fin, kf_s, taps_s, ug_a, ug_b, zb_a, zb_b,
            pb_a, pb_b, h_s, z_ref, x_in, wqkv, wo, bk, bv, ssmk, out_s, shk, ssmd, fwd_ref, inv_ref,
            sem_c, sem_x, sem_w, sem_o, sem_s):
    def kv_copies(cb):
        cs = pl.ds(pl.multiple_of(cb * 128, 128), 128)
        return [pltpu.make_async_copy(bk_hbm.at[0, :, cs], bk.at[cb], sem_c.at[0, cb]),
                pltpu.make_async_copy(bv_hbm.at[0, :, cs], bv.at[cb], sem_c.at[1, cb])]

    def h_copy(cb):
        cs = pl.ds(pl.multiple_of(cb * 128, 128), 128)
        return pltpu.make_async_copy(ssmk_hbm.at[cs, :], ssmk.at[cs, pl.ds(0, S)], sem_c.at[2, cb])

    def x_copy(c):
        rs = pl.ds(pl.multiple_of(c * RC, RC), RC)
        return pltpu.make_async_copy(x_hbm.at[0, rs, :], x_in.at[rs, :], sem_x.at[c])

    def w_copy(c):
        rs = pl.ds(pl.multiple_of(c * 128, 128), 128)
        return pltpu.make_async_copy(wqkv_hbm.at[rs, :], wqkv.at[rs, pl.ds(0, 3 * D)], sem_w.at[c])

    def wo_copy():
        return pltpu.make_async_copy(wo_hbm, wo.at[:, pl.ds(0, D)], sem_w.at[G])

    def out_copy(c):
        rs = pl.ds(pl.multiple_of(c * RC, RC), RC)
        return pltpu.make_async_copy(out_s.at[rs, :], out_hbm.at[0, rs, :], sem_o.at[c])

    TAIL = (0, 128, 192, 256)

    def tail_copy(q):
        rs = pl.ds((NRC - 1) * RC + TAIL[q], TAIL[q + 1] - TAIL[q])
        return pltpu.make_async_copy(out_s.at[rs, :], out_hbm.at[0, rs, :], sem_o.at[NRC - 1 + q])

    def conv_start(c):
        h_copy(c).start()
        for cp in kv_copies(c):
            cp.start()

    def wait_all(cps):
        for cp in cps:
            cp.wait()

    shk_cp, ssmd_cp, fwd_cp, inv_cp = [
        pltpu.make_async_copy(src, dst, sem_s.at[i]) for i, (src, dst) in enumerate(
            ((shk_hbm, shk), (ssmd_hbm, ssmd), (fwd_hbm, fwd_ref), (inv_hbm, inv_ref)))]
    h_copy(0).start()
    fwd_cp.start()
    shk_cp.start()
    ssmd_cp.start()
    for cp in kv_copies(0):
        cp.start()

    for i in range(NZ):
        z_ref[i] = 0
    fin[...] = jnp.ones(fin.shape, f32)
    for buf in (a2, b1, b2):
        buf[...] = jnp.zeros(buf.shape, f32)
    kf_s[0, 0:8, :] = jnp.zeros((8, 128), f32)

    def zero_vreg():
        return jnp.full((8, 128), z_ref[0], i32).astype(u32)

    def fence(cps):
        @pl.when(z_ref[0] == 0)
        def _():
            wait_all(cps)

    TILES = [(0, n) for n in range(8)] + [(2, n) for n in range(8)] + [(1, n) for n in range(8)]

    def qkv_tile(h, c, idx, toks, zv):
        kind, n = TILES[idx]
        col = kind * D + n * 128
        r = jnp.dot(h, _gate(wqkv[:, col:col + 128], toks), preferred_element_type=f32)
        if kind == 1:
            k_s[n, pl.ds(pl.multiple_of(c * (RC // 2), RC // 2), RC // 2), :] = _pack(r)
            return None
        dst = qt_s if kind == 0 else vt_s
        if kind == 0:
            r = r * QSCALE
        pks = []
        for t in range(RC // 128):
            pk = _pack(r[t * 128:(t + 1) * 128, :].T)
            dst[c * (RC // 128) + t, n * 64:(n + 1) * 64, :] = pk
            pks.append(pk)
        return _tok(jnp.concatenate(pks, axis=0), zv)

    def qkv_proj(h, c, piece_fn, first_piece):
        zv = zero_vreg()
        deps = {}
        for n in range(24):
            done = qkv_tile(h, c, n, deps.get(n), zv)
            if done is not None:
                deps.setdefault(n + 3, []).append(done)
            if piece_fn is not None and first_piece <= n < first_piece + NP:
                deps.setdefault(n + 3, []).append(_tok(piece_fn(n - first_piece), zv))

    def piece_rows(c, p):
        return pl.ds(pl.multiple_of(c * RC + p * 16, 16), 16)

    def ln1_piece(c, p):
        hp = _pack(_ln(x_in[piece_rows(c, p), :].astype(f32)))
        h_s[p * 8:(p + 1) * 8, :] = hp
        return hp

    def gated_x(c, p, z):
        rows = piece_rows(c, p)
        x1 = x_s[z, rows, :]
        y = jnp.concatenate([y_s[0, g, rows, :] + y_s[1, g, rows, :] for g in range(G)], axis=1)
        return x1 + _ln(x1) * y

    def ln2_piece(c, p, z):
        x2 = gated_x(c, p, z)
        x_s[z, piece_rows(c, p), :] = x2
        hp = _pack(_ln(x2))
        h_s[p * 8:(p + 1) * 8, :] = hp
        return hp

    def out_piece(c, p, z):
        v = gated_x(c, p, z)
        out_s[piece_rows(c, p), :] = v.astype(bf)
        return v

    def load_o(c):
        rs = pl.ds(pl.multiple_of(c * (RC // 2), RC // 2), RC // 2)
        return jnp.concatenate([_unpack(o_s[g, rs, :]) for g in range(G)], axis=1)

    def oproj_tile(o, c, n, z, toks=None, r0=0, nr=RC, first=False):
        rows = pl.ds(pl.multiple_of(c * RC + r0, nr), nr)
        cols = slice(n * 128, (n + 1) * 128)
        r = jnp.dot(o[r0:r0 + nr], _gate(wo[:, cols], toks), preferred_element_type=f32)
        x0 = x_in[rows, cols].astype(f32) if first else x_s[z, rows, cols]
        x_s[z, rows, cols] = x0 + r
        return r

    zts = [z_ref[2 + ib] for ib in range(4)]

    def setup_taps():
        taps = shk[...].astype(f32)
        for cb in range(G):
            for t in range(4):
                taps_s[cb, 8 * t:8 * t + 8, :] = jnp.broadcast_to(taps[t:t + 1, cb * 128:(cb + 1) * 128], (8, 128))

    def setup_skip():
        dall = ssmd[...].astype(f32)
        for cb in range(G):
            taps_s[cb, 32:40, :] = jnp.broadcast_to(dall[cb:cb + 1, :], (8, 128))

    def prep_h_chunk(cb, pb, j):
        cs = pl.ds(pl.multiple_of(cb * 128, 128), 128)
        pb[HS + j * 64:HS + (j + 1) * 64, :] = pltpu.bitcast(ssmk[cs, j * 128:(j + 1) * 128], u32)

    def prep_h(cb, pb):
        for j in range(NC):
            prep_h_chunk(cb, pb, j)

    def prep_kv(cb, pb, with_h):
        zs = z_ref[1]
        tp = taps_s[cb, 0:32, :]
        for j in range(NC):
            r0 = j * 128
            if with_h:
                prep_h_chunk(cb, pb, j)
            kf_s[zs, 8 + r0:8 + r0 + 128, :] = bk[cb, r0:r0 + 128, :].astype(f32)
            ks = None
            for t in range(4):
                term = kf_s[zs, 8 + r0 - t:8 + r0 - t + 128, :].reshape(16, 8, 128) * tp[8 * t:8 * t + 8][None]
                ks = term if ks is None else ks + term
            pb[j * 64:(j + 1) * 64, :] = _pack(ks.reshape(128, 128) * bv[cb, r0:r0 + 128, :].astype(f32))

    def fwd_h(pb, ug):
        for m in range(NC):
            hm = lax.dot_general(_unpack(fwd_ref[128:320, :]), _unpack(pb[HS + m * 64:HS + (m + 1) * 64, :]),
                                 NT, preferred_element_type=f32)
            ug[0, NC + m, :, GO:GO + 128, :] = hm.reshape(3, 128, 128)

    def fwd_u(pb, ug):
        for j in range(NC):
            u = jnp.dot(_unpack(fwd_ref[0:128, :]), _unpack(pb[j * 64:(j + 1) * 64, :]),
                        preferred_element_type=f32)
            ug[0, j, 0:2, 0:128, :] = u.reshape(2, 128, 128)

    def add_skip(cb, ug):
        dv = taps_s[cb, 32:40, :][None]
        for e in range(3):
            v = ug[0, NC, e, GO:GO + 128, :].reshape(16, 8, 128)
            ug[0, NC, e, GO:GO + 128, :] = (v - dv if e == 1 else v + dv).reshape(128, 128)

    def spec_item(ug, ib, r):
        zt = zts[ib]
        acc = None
        for j in range(4 * ib + 4):
            u = ug[zt, j:j + 1, 0:2, r:r + 8, :]
            u = jnp.concatenate([u[:, 0:1] + u[:, 1:2], u], axis=1)
            q0 = max(0, j - 4 * ib)
            m0 = NC + 4 * ib - j
            t = ug[zt, m0 + q0:m0 + 4, :, GO + r:GO + r + 8, :] * u
            if acc is None:
                acc = t
            elif q0 == 0:
                acc = acc + t
            else:
                acc = jnp.concatenate([acc[:q0], acc[q0:] + t], axis=0)
        return acc[:, 0] - acc[:, 2], acc[:, 0] + acc[:, 1]

    def overlap_add(yr, yi, prev, r):
        n = 1 if prev is None else 0
        pr = yr[:3] if prev is None else jnp.concatenate([prev[0], yr[:3]], axis=0)
        pi = yi[:3] if prev is None else jnp.concatenate([prev[1], yi[:3]], axis=0)
        if r < 64:
            zr, zi = yr[n:] - pi, yi[n:] + pr
        else:
            zr, zi = yr[n:] + pi, yi[n:] - pr
        if prev is None:
            zr = jnp.concatenate([yr[:1], zr], axis=0)
            zi = jnp.concatenate([yi[:1], zi], axis=0)
        return zr, zi, (yr[3:], yi[3:])

    def conv_spec(ug, zb, lo=0, hi=8):
        for rp in range(lo, hi):
            p0 = p1 = None
            for ib in range(4):
                zr0, zi0, p0 = overlap_add(*spec_item(ug, ib, 16 * rp), p0, 16 * rp)
                zr1, zi1, p1 = overlap_add(*spec_item(ug, ib, 16 * rp + 8), p1, 16 * rp)
                zb[4 * ib:4 * ib + 4, rp * 8:rp * 8 + 8, :] = _pack(jnp.concatenate([zr0, zr1], axis=1))
                zb[4 * ib:4 * ib + 4, 64 + rp * 8:72 + rp * 8, :] = _pack(jnp.concatenate([zi0, zi1], axis=1))

    def conv_inv(cb, zb):
        for i in range(NC):
            for e in range(2):
                y_s[e, cb, i * 128:(i + 1) * 128, :] = jnp.dot(
                    _unpack(inv_ref[:, e * 128:(e + 1) * 128]), _unpack(zb[i, e * 64:(e + 1) * 64, :]),
                    preferred_element_type=f32)

    def conv_step(c, ug_cur, ug_nxt, zb_cur, zb_prev, pb_nxt, pb_new):
        @pl.when(c + 3 < G)
        def _():
            conv_start(c + 3)
        w_copy(c).start()

        @pl.when(c >= G - 3)
        def _():
            x_copy(c - (G - 3)).start()
        conv_spec(ug_cur, zb_cur)
        fwd_h(pb_nxt, ug_nxt)
        fwd_u(pb_nxt, ug_nxt)
        conv_inv(c - 1, zb_prev)

        @pl.when(c + 2 < G)
        def _():
            wait_all([w_copy(c - 1), h_copy(c + 2)] + kv_copies(c + 2))
            prep_kv(c + 2, pb_new, True)
            add_skip(c + 1, ug_nxt)

        @pl.when(c + 2 >= G)
        def _():
            w_copy(c - 1).wait()
            add_skip(c + 1, ug_nxt)

    def conv():
        wait_all([fwd_cp, h_copy(0)])
        conv_start(1)
        inv_cp.start()
        prep_h(0, pb_a)
        fwd_h(pb_a, ug_a)
        wait_all([shk_cp] + kv_copies(0))
        conv_start(2)
        setup_taps()
        prep_kv(0, pb_a, False)
        fwd_u(pb_a, ug_a)
        fence([h_copy(1)])
        prep_h(1, pb_b)
        fence([ssmd_cp])
        setup_skip()
        add_skip(0, ug_a)
        conv_spec(ug_a, zb_a, 0, R0)
        fwd_h(pb_b, ug_b)
        fence(kv_copies(1))
        conv_start(3)
        w_copy(0).start()
        prep_kv(1, pb_b, False)
        add_skip(1, ug_b)
        fence([h_copy(2)])
        conv_spec(ug_a, zb_a, R0, 8)
        fwd_u(pb_b, ug_b)
        fence(kv_copies(2) + [inv_cp])
        prep_kv(2, pb_a, True)

        def body(p, carry):
            conv_step(2 * p + 1, ug_b, ug_a, zb_b, zb_a, pb_a, pb_b)
            conv_step(2 * p + 2, ug_a, ug_b, zb_a, zb_b, pb_b, pb_a)
            return carry
        lax.fori_loop(0, G // 2 - 1, body, 0)
        w_copy(G - 1).start()
        conv_spec(ug_b, zb_b)
        conv_inv(G - 2, zb_a)
        fence([x_copy(0)])
        for p in range(NP):
            ln1_piece(0, p)
        conv_inv(G - 1, zb_b)
        wait_all([w_copy(G - 2), w_copy(G - 1)])

    def phase1():
        def body(c, carry):
            @pl.when(c + 1 < NRC)
            def _():
                x_copy(c + 1).wait()

            @pl.when(c + 2 < NRC)
            def _():
                x_copy(c + 2).start()

            @pl.when(c + 2 == NRC)
            def _():
                wo_copy().start()
            cn = jnp.minimum(c + 1, NRC - 1)
            qkv_proj(_unpack(h_s[...]), c, lambda p: ln1_piece(cn, p), 2)
            return carry
        lax.fori_loop(0, NRC, body, 0)
        wo_copy().wait()

    def phase2(ms):
        o = load_o(0)
        z0 = z_ref[0]
        for q in range(2):
            rs = [oproj_tile(o, 0, n, z0, None, q * (RC // 2), RC // 2, True) for n in range(8)]
            if q == 0:
                attention_tail(ms, rs[0:5:2])
            for p in range(q * NP // 2, (q + 1) * NP // 2):
                ln2_piece(0, p, z0)

        def body(c, carry):
            z0 = z_ref[0]
            z1 = z_ref[1]
            h = _unpack(h_s[...])
            o = load_o(c + 1)
            for n in range(8):
                oproj_tile(o, c + 1, n, z1, first=True)
            qkv_proj(h, c, lambda p: ln2_piece(c + 1, p, z0), 1)
            return carry
        lax.fori_loop(0, NRC - 1, body, 0)
        qkv_proj(_unpack(h_s[...]), NRC - 1, None, 0)

    def phase3(ms):
        o = load_o(0)
        attention_tail(ms, [oproj_tile(o, 0, n, z_ref[1]) for n in range(8)])

        def body(c, carry):
            z0 = z_ref[0]
            z1 = z_ref[1]
            zv = zero_vreg()
            o = load_o(c + 1)
            deps = {}
            p = 0
            for t in range(16):
                for _ in range(2 if t < 2 else 1):
                    if p < NP:
                        deps.setdefault(t + 2, []).append(_tok(out_piece(c, p, z0), zv))
                        p += 1
                oproj_tile(o, c + 1, t // 2, z1, deps.get(t), (t % 2) * 128, 128)
            out_copy(c).start()
            return carry
        lax.fori_loop(0, NRC - 2, body, 0)

        c = NRC - 1
        z0 = z_ref[0]
        zv = zero_vreg()
        o = load_o(c)
        deps = {}
        todo = [(c - 1, p) for p in range(NP)]
        for q in range(3):
            for n in range(8):
                t = 8 * q + n
                for cc, p in todo[2 * n:2 * n + 2]:
                    deps.setdefault(t + 2, []).append(_tok(out_piece(cc, p, z0), zv))
                oproj_tile(o, c, n, z0, deps.get(t), TAIL[q], TAIL[q + 1] - TAIL[q])
            (out_copy(c - 1) if q == 0 else tail_copy(q - 1)).start()
            todo = [(c, p) for p in range(TAIL[q] // 16, TAIL[q + 1] // 16)]
        for cc, p in todo:
            out_piece(cc, p, z0)
        tail_copy(2).start()
        wait_all([out_copy(i) for i in range(NRC - 1)] + [tail_copy(q) for q in range(3)])

    zero16 = jnp.zeros((16, 128), u32)

    def qk(g, j, hh, half, dst, z, zk=0, dep=None):
        qt = qt_s[j, pl.ds(pl.multiple_of(g * 64 + hh * 16, 16), 16), :]
        w = _unpack(jnp.concatenate([qt if i == hh else zero16 for i in range(4)], axis=0))
        kh = k_s[g + zk, half * HS // 2:(half + 1) * HS // 2, :]
        m = first = s = None
        for c in range(4):
            ku = kh[c * CH // 2:(c + 1) * CH // 2]
            if dep is not None:
                ku = jnp.concatenate([ku[:CH // 2 - 8], ku[CH // 2 - 8:] | dep], axis=0)
            s = jnp.dot(_unpack(ku), w, preferred_element_type=f32)
            dst[z, c * CH:(c + 1) * CH, :] = s
            mc = jnp.max(s.reshape(CH // 8, 8, 128), axis=0)
            m = mc if m is None else jnp.maximum(m, mc)
            f = pltpu.bitcast(s[0:8], u32)
            first = f if first is None else first | f
        return m, first, s

    def fullmax(m1, m2):
        return jnp.max(jnp.maximum(m1, m2), axis=0, keepdims=True)

    def sm_pv(g, hh, half, src, m, z, dep, trigs):
        mb = jnp.broadcast_to(m, (8, 128))
        mbu = pltpu.bitcast(mb, u32)
        ms = [mb if tr is None else pltpu.bitcast(mbu | tr, f32) for tr in trigs]
        mm = jnp.stack([jnp.stack([ms[4 * st + 3 - kk] for kk in range(4)]) for st in range(2)])
        x = src[z].reshape(2, 4, 4, 4, 8, 128)
        p = jnp.exp2(x - mm[:, None, :, None]).reshape(HS, 128)
        rs = pl.ds(pl.multiple_of(g * 64 + hh * 16, 16), 16)
        vu = vt_s[half * 8:half * 8 + 8, rs, :] | jnp.concatenate([dep, dep], axis=0)[None]
        vu = jnp.concatenate([vu[t] for t in range(8)], axis=1)
        l = _tree_sum(p)
        return jnp.dot(_unpack(vu), p.astype(bf), preferred_element_type=f32), l

    def store_o(g, j, parts):
        outs = [parts[2 * h] * (1.0 / jnp.sum(parts[2 * h + 1], axis=0, keepdims=True)) for h in range(4)]
        o_s[g, pl.ds(pl.multiple_of(j * 64, 64), 64), :] = _pack(jnp.concatenate(outs, axis=0).T)

    LAG = 3
    bufs = {(0, 0): a1, (0, 1): a2, (1, 0): b1, (1, 1): b2}

    def tile_of(t):
        return lax.shift_right_logical(t, 4), t & (NQ - 1)

    def finish_tile(g, j, done, res):
        if done is None:
            parts = []
        else:
            parts = [done[0:32], done[32:40], done[40:72], done[72:80]]
            res = [(done[80:112], done[112:120])] + res
        for h in range(len(res) // 2):
            parts += [res[2 * h][0] + res[2 * h + 1][0], res[2 * h][1] + res[2 * h + 1][1]]
        store_o(g, j, parts)

    def attention(m_init):
        nit = G * NQ // UNR

        def body(it, carry):
            z1 = z_ref[0]
            z2 = z_ref[1]
            zv = zero_vreg()
            g, j0 = tile_of(it * UNR)
            gp, jp = tile_of(jnp.maximum(it * UNR - 1, 0))
            mfull = {(-1, 2): carry[0], (-1, 3): carry[1]}
            mpart = do = ps = po = None
            res = []

            def tg(sv, i):
                return None if sv is None else pltpu.bitcast(sv[i * 8:i * 8 + 8], u32) & zv

            for n in range(8 * UNR):
                u, qh, qhalf = n // 8, (n % 8) // 2, n % 2
                mp, first, cs = qk(g, j0 + u, qh, qhalf, bufs[(qh % 2, qhalf)], z1, z_ref[2 + n], do)
                if qhalf == 0:
                    mpart = mp
                else:
                    mfull[(u, qh)] = fullmax(mpart, mp)
                pu, ph, phalf = (n - LAG) // 8, ((n - LAG) % 8) // 2, (n - LAG) % 2
                trigs = [tg(ps, i) for i in TA] + [tg(po, 0)] + [tg(cs, i) for i in TB]
                o, l = sm_pv(gp if pu < 0 else g, ph, phalf, bufs[(ph % 2, phalf)], mfull[(pu, ph)], z2,
                             first & zv, trigs)
                ps, po, do = cs, o, tg(o, 3)
                res.append((o, l))
                if ph == 3 and phalf == 1:
                    if pu < 0:
                        finish_tile(gp, jp, fin[z2], res)
                    else:
                        finish_tile(g, j0 + pu, None, res)
                    res = []
            fin[z1] = jnp.concatenate([res[0][0] + res[1][0], res[0][1] + res[1][1],
                                       res[2][0] + res[3][0], res[2][1] + res[3][1],
                                       res[4][0], res[4][1]], axis=0)
            return mfull[(UNR - 1, 2)], mfull[(UNR - 1, 3)]

        return lax.fori_loop(0, nit, body, m_init)

    def attention_tail(ms, rs):
        z2 = z_ref[1]
        zv = zero_vreg()
        res = []
        for k, (ph, phalf) in enumerate(((2, 1), (3, 0), (3, 1))):
            trigs = [pltpu.bitcast(rs[k][16 * i:16 * i + 8], u32) & zv for i in range(8)]
            res.append(sm_pv(G - 1, ph, phalf, bufs[(ph % 2, phalf)], ms[ph - 2], z2, trigs[7], trigs))
        finish_tile(G - 1, NQ - 1, fin[z2], res)

    conv()
    phase1()
    ms = attention((jnp.zeros((1, 128), f32), jnp.zeros((1, 128), f32)))
    phase2(ms)
    ms = attention(ms)
    phase3(ms)


@jax.jit
def pallas_interleave_layers__softmax_full_mha__ssm_conv_h3__prompt_kernel(
        A_x, A_wqkv, A_wo, B_q, B_k, B_v, B_shift_k, B_ssm_k, B_ssm_D):
    del B_q
    fwd, inv = _dft_mats()
    scratch = [
        pltpu.VMEM((1, S, D), f32),
        pltpu.VMEM((2, G, S, 128), f32),
        pltpu.VMEM((NQ, D // 2, 128), u32),
        pltpu.VMEM((G, S // 2, 128), u32),
        pltpu.VMEM((NQ, D // 2, 128), u32),
        pltpu.VMEM((G, S // 2, 128), u32),
        pltpu.VMEM((1, HS, 128), f32), pltpu.VMEM((1, HS, 128), f32),
        pltpu.VMEM((1, HS, 128), f32), pltpu.VMEM((1, HS, 128), f32),
        pltpu.VMEM((1, 120, 128), f32),
        pltpu.VMEM((1, S + 8, 128), f32),
        pltpu.VMEM((G, 40, 128), f32),
        pltpu.VMEM((1, 2 * NC, 3, IM, 128), f32),
        pltpu.VMEM((1, 2 * NC, 3, IM, 128), f32),
        pltpu.VMEM((NC, 128, 128), u32),
        pltpu.VMEM((NC, 128, 128), u32),
        pltpu.VMEM((S, 128), u32),
        pltpu.VMEM((S, 128), u32),
        pltpu.VMEM((RC // 2, D), u32),
        pltpu.SMEM((NZ,), i32),
        pltpu.VMEM((S, D), bf),
        pltpu.VMEM((D, 3 * D + 128), bf),
        pltpu.VMEM((D, D + 128), bf),
        pltpu.VMEM((G, S, 128), bf),
        pltpu.VMEM((G, S, 128), bf),
        pltpu.VMEM((D, S + 128), bf),
        pltpu.VMEM((S, D), bf),
        pltpu.VMEM((4, D), bf),
        pltpu.VMEM((G, 128), bf),
        pltpu.VMEM((320, 128), u32),
        pltpu.VMEM((64, 256), u32),
        pltpu.SemaphoreType.DMA((3, G)),
        pltpu.SemaphoreType.DMA((NRC,)),
        pltpu.SemaphoreType.DMA((G + 1,)),
        pltpu.SemaphoreType.DMA((NRC + 2,)),
        pltpu.SemaphoreType.DMA((4,)),
    ]
    hbm = pl.BlockSpec(memory_space=pl.ANY)
    return pl.pallas_call(
        _kernel,
        out_shape=jax.ShapeDtypeStruct((1, S, D), bf),
        in_specs=[hbm] * 10,
        out_specs=hbm,
        scratch_shapes=scratch,
        compiler_params=pltpu.CompilerParams(vmem_limit_bytes=120 * 2**20, disable_bounds_checks=True),
    )(A_x, A_wqkv, A_wo, B_k, B_v, B_shift_k.T, B_ssm_k, B_ssm_D.reshape(G, 128),
      jnp.asarray(fwd), jnp.asarray(inv))
```

```python
import numpy as np
import jax
import jax.numpy as jnp
from jax import lax
import jax.experimental.pallas as pl
import jax.experimental.pallas.tpu as pltpu

S = 2048
D = 1024
DH = 32
G = 8
NQ = 16
HS = S // 2
CH = HS // 4
UNR = 8
NV = 64
LAG = 3
RC = 256
NRC = S // RC
NP = RC // 16
NC = 16
NB = 4
IM = 136
GO = 8
EPS = 1e-5
NZ = 2 + 8 * UNR
QSCALE = float(DH ** -0.5 * np.log2(np.e))
N0 = 18
VT = ('p30,p31,p31,c5,c5,c5,c14,c18/p28,p29,p29,p29,o1,c0,c6,c13',
      'p31,p31,p31,c1,c5,c5,c14,c17/p27,p27,p28,p29,o1,c0,c5,c14')
ET = ('p17,p22,p29,p30,o0,c0,c4,c8/p16,p19,p29,p29,o0,c0,c4,c6',
      'p17,p19,p30,o0,o2,c0,c4,c10/p17,p19,p29,o0,o3,c2,c4,c6')

bf = jnp.bfloat16
f32 = jnp.float32
u32 = jnp.uint32
i32 = jnp.int32
NT = (((1,), (1,)), ((), ()))


def _dft_mats():
    n = np.arange(128)
    f = np.concatenate([np.arange(0, 128, 2), np.arange(1, 128, 2)])
    ang = 2.0 * np.pi * np.outer(f + 0.5, n) / 256.0
    re, im = np.cos(ang), -np.sin(ang)
    inv = np.concatenate([re, im], axis=0).T / 128.0
    fwd = np.concatenate([re, im, re, im - re, im + re], axis=0)

    def pack_rows(a):
        u = np.ascontiguousarray(a, dtype=np.float32).view(np.uint32)
        u = (u + 0x7FFF + ((u >> 16) & 1)) >> 16
        return (u[0::2] | (u[1::2] << 16)).astype(np.uint32)
    return pack_rows(fwd), pack_rows(inv)


def _tree_sum(p):
    n = p.shape[0] // 8
    x = p.reshape(n, 8, 128)
    while n > 1:
        x = x.reshape(n // 2, 2, 8, 128)
        x = x[:, 0] + x[:, 1]
        n //= 2
    return x[0]


def _ln(x):
    m = jnp.mean(x, axis=-1, keepdims=True)
    xc = x - m
    v = jnp.mean(xc * xc, axis=-1, keepdims=True)
    return xc * lax.rsqrt(v + EPS)


def _pack(x):
    return pltpu.bitcast(x.astype(bf), u32)


def _unpack(x):
    return pltpu.bitcast(x, bf)


def _tok(v, zv):
    v = v if v.dtype == u32 else pltpu.bitcast(v, u32)
    while v.shape[1] > 128:
        h = v.shape[1] // 2
        v = v[:, :h] | v[:, h:]
    while v.shape[0] > 8:
        h = v.shape[0] // 2
        v = v[:h] | v[h:]
    return v & zv


def _gate(w, toks):
    if not toks:
        return w
    wu = pltpu.bitcast(w, u32)
    h0 = wu[0:8]
    for t in toks:
        h0 = h0 | t
    return _unpack(jnp.concatenate([h0, wu[8:]], axis=0))


def _kernel(x_hbm, wqkv_hbm, wo_hbm, bk_hbm, bv_hbm, shk_hbm, ssmk_hbm, ssmd_hbm, fwd_hbm, inv_hbm, out_hbm,
            x_s, y_s, qt_s, k_s, vt_s, o_s, kb_s, a1, a2, b1, b2, fin, kf_s, taps_s, ug_a, ug_b, zb_a, zb_b,
            pb_a, pb_b, h_s, z_ref, x_in, wqkv, wo, bk, bv, ssmk, shk, ssmd, fwd_ref, inv_ref,
            sem_c, sem_x, sem_w, sem_o, sem_s):
    out_s = x_in

    def kv_copies(cb):
        cs = pl.ds(pl.multiple_of(cb * 128, 128), 128)
        return [pltpu.make_async_copy(bk_hbm.at[0, :, cs], bk.at[cb % NB], sem_c.at[0, cb]),
                pltpu.make_async_copy(bv_hbm.at[0, :, cs], bv.at[cb % NB], sem_c.at[1, cb])]

    def h_copy(cb):
        cs = pl.ds(pl.multiple_of(cb * 128, 128), 128)
        return pltpu.make_async_copy(ssmk_hbm.at[cs, :], ssmk.at[cb % NB, :, pl.ds(0, S)], sem_c.at[2, cb])

    def x_copy(c):
        rs = pl.ds(pl.multiple_of(c * RC, RC), RC)
        return pltpu.make_async_copy(x_hbm.at[0, rs, :], x_in.at[rs, :], sem_x.at[c])

    def w_copy(c):
        rs = pl.ds(pl.multiple_of(c * 128, 128), 128)
        return pltpu.make_async_copy(wqkv_hbm.at[rs, :], wqkv.at[rs, pl.ds(0, 3 * D)], sem_w.at[c])

    def wo_copy():
        return pltpu.make_async_copy(wo_hbm, wo.at[:, pl.ds(0, D)], sem_w.at[G])

    def out_copy(c):
        rs = pl.ds(pl.multiple_of(c * RC, RC), RC)
        return pltpu.make_async_copy(out_s.at[rs, :], out_hbm.at[0, rs, :], sem_o.at[c])

    TAIL = (0, 128, 192, 256)

    def tail_copy(q):
        rs = pl.ds((NRC - 1) * RC + TAIL[q], TAIL[q + 1] - TAIL[q])
        return pltpu.make_async_copy(out_s.at[rs, :], out_hbm.at[0, rs, :], sem_o.at[NRC - 1 + q])

    def conv_start(c):
        h_copy(c).start()
        for cp in kv_copies(c):
            cp.start()

    def wait_all(cps):
        for cp in cps:
            cp.wait()

    shk_cp, ssmd_cp, fwd_cp, inv_cp = [
        pltpu.make_async_copy(src, dst, sem_s.at[i]) for i, (src, dst) in enumerate(
            ((shk_hbm, shk), (ssmd_hbm, ssmd), (fwd_hbm, fwd_ref), (inv_hbm, inv_ref)))]
    h_copy(0).start()
    fwd_cp.start()
    shk_cp.start()
    ssmd_cp.start()
    for cp in kv_copies(0):
        cp.start()

    for i in range(NZ):
        z_ref[i] = 0
    fin[...] = jnp.ones(fin.shape, f32)
    for buf in (a2, b1, b2):
        buf[...] = jnp.zeros(buf.shape, f32)
    kf_s[0, 0:8, :] = jnp.zeros((8, 128), f32)

    def zero_vreg():
        return jnp.full((8, 128), z_ref[0], i32).astype(u32)

    def fence(cps):
        @pl.when(z_ref[0] == 0)
        def _():
            wait_all(cps)

    TILES = [(0, n) for n in range(8)] + [(2, n) for n in range(8)] + [(1, n) for n in range(8)]

    def qkv_tile(h, c, idx, toks, zv):
        kind, n = TILES[idx]
        col = kind * D + n * 128
        r = jnp.dot(h, _gate(wqkv[:, col:col + 128], toks), preferred_element_type=f32)
        if kind == 1:
            k_s[n, pl.ds(pl.multiple_of(c * (RC // 2), RC // 2), RC // 2), :] = _pack(r)
            return None
        dst = qt_s if kind == 0 else vt_s
        if kind == 0:
            r = r * QSCALE
        pks = []
        for t in range(RC // 128):
            pk = _pack(r[t * 128:(t + 1) * 128, :].T)
            dst[c * (RC // 128) + t, n * 64:(n + 1) * 64, :] = pk
            pks.append(pk)
        return _tok(jnp.concatenate(pks, axis=0), zv)

    def qkv_proj(h, c, piece_fn, first_piece, kb_jobs):
        zv = zero_vreg()
        deps = {}
        for n in range(24):
            done = qkv_tile(h, c, n, deps.get(n), zv)
            if done is not None:
                deps.setdefault(n + 3, []).append(done)
            if n in kb_jobs:
                deps.setdefault(n + 2, []).append(kb_piece(*kb_jobs[n], zv))
            if piece_fn is not None and first_piece <= n < first_piece + NP:
                deps.setdefault(n + 3, []).append(_tok(piece_fn(n - first_piece), zv))

    def kb_plan(g, tiles):
        return {t: (g, 128 * i // len(tiles), 128 * (i + 1) // len(tiles)) for i, t in enumerate(tiles)}

    def kb_piece(g, lo, hi, zv):
        kx = _unpack(k_s[g, 0:NV // 2, :]).astype(f32)
        for d in range(lo, hi):
            v = jnp.broadcast_to(kx[:, d:d + 1], (NV, 128))
            kb_s[g, d] = v
        return _tok(v[NV - 32:], zv)

    def piece_rows(c, p):
        return pl.ds(pl.multiple_of(c * RC + p * 16, 16), 16)

    def ln1_piece(c, p):
        hp = _pack(_ln(x_in[piece_rows(c, p), :].astype(f32)))
        h_s[p * 8:(p + 1) * 8, :] = hp
        return hp

    def gated_x(c, p, z):
        rows = piece_rows(c, p)
        x1 = x_s[z, rows, :]
        y = jnp.concatenate([y_s[0, g, rows, :] + y_s[1, g, rows, :] for g in range(G)], axis=1)
        return x1 + _ln(x1) * y

    def ln2_piece(c, p, z):
        x2 = gated_x(c, p, z)
        x_s[z, piece_rows(c, p), :] = x2
        hp = _pack(_ln(x2))
        h_s[p * 8:(p + 1) * 8, :] = hp
        return hp

    def out_piece(c, p, z):
        v = gated_x(c, p, z)
        out_s[piece_rows(c, p), :] = v.astype(bf)
        return v

    def load_o(c):
        rs = pl.ds(pl.multiple_of(c * (RC // 2), RC // 2), RC // 2)
        return jnp.concatenate([_unpack(o_s[g, rs, :]) for g in range(G)], axis=1)

    def oproj_tile(o, c, n, z, toks=None, r0=0, nr=RC, first=False):
        rows = pl.ds(pl.multiple_of(c * RC + r0, nr), nr)
        cols = slice(n * 128, (n + 1) * 128)
        r = jnp.dot(o[r0:r0 + nr], _gate(wo[:, cols], toks), preferred_element_type=f32)
        x0 = x_in[rows, cols].astype(f32) if first else x_s[z, rows, cols]
        x_s[z, rows, cols] = x0 + r
        return r

    zts = [z_ref[2 + ib] for ib in range(4)]

    def setup_taps():
        taps = shk[...].astype(f32)
        for cb in range(G):
            for t in range(4):
                taps_s[cb, 8 * t:8 * t + 8, :] = jnp.broadcast_to(taps[t:t + 1, cb * 128:(cb + 1) * 128], (8, 128))

    def setup_skip():
        dall = ssmd[...].astype(f32)
        for cb in range(G):
            taps_s[cb, 32:40, :] = jnp.broadcast_to(dall[cb:cb + 1, :], (8, 128))

    def prep_h_chunk(cb, pb, j):
        pb[HS + j * 64:HS + (j + 1) * 64, :] = pltpu.bitcast(ssmk[cb % NB, :, j * 128:(j + 1) * 128], u32)

    def prep_h(cb, pb):
        for j in range(NC):
            prep_h_chunk(cb, pb, j)

    def prep_kv(cb, pb, with_h):
        zs = z_ref[1]
        tp = taps_s[cb, 0:32, :]
        for j in range(NC):
            r0 = j * 128
            if with_h:
                prep_h_chunk(cb, pb, j)
            kf_s[zs, 8 + r0:8 + r0 + 128, :] = bk[cb % NB, r0:r0 + 128, :].astype(f32)
            ks = None
            for t in range(4):
                term = kf_s[zs, 8 + r0 - t:8 + r0 - t + 128, :].reshape(16, 8, 128) * tp[8 * t:8 * t + 8][None]
                ks = term if ks is None else ks + term
            pb[j * 64:(j + 1) * 64, :] = _pack(ks.reshape(128, 128) * bv[cb % NB, r0:r0 + 128, :].astype(f32))

    def fwd_h(pb, ug):
        for m in range(NC):
            hm = lax.dot_general(_unpack(fwd_ref[128:320, :]), _unpack(pb[HS + m * 64:HS + (m + 1) * 64, :]),
                                 NT, preferred_element_type=f32)
            ug[0, NC + m, :, GO:GO + 128, :] = hm.reshape(3, 128, 128)

    def fwd_u(pb, ug):
        for j in range(NC):
            u = jnp.dot(_unpack(fwd_ref[0:128, :]), _unpack(pb[j * 64:(j + 1) * 64, :]),
                        preferred_element_type=f32)
            ug[0, j, 0:2, 0:128, :] = u.reshape(2, 128, 128)

    def add_skip(cb, ug):
        dv = taps_s[cb, 32:40, :][None]
        for e in range(3):
            v = ug[0, NC, e, GO:GO + 128, :].reshape(16, 8, 128)
            ug[0, NC, e, GO:GO + 128, :] = (v - dv if e == 1 else v + dv).reshape(128, 128)

    def spec_item(ug, ib, r):
        zt = zts[ib]
        acc = None
        for j in range(4 * ib + 4):
            u = ug[zt, j:j + 1, 0:2, r:r + 8, :]
            u = jnp.concatenate([u[:, 0:1] + u[:, 1:2], u], axis=1)
            q0 = max(0, j - 4 * ib)
            m0 = NC + 4 * ib - j
            t = ug[zt, m0 + q0:m0 + 4, :, GO + r:GO + r + 8, :] * u
            if acc is None:
                acc = t
            elif q0 == 0:
                acc = acc + t
            else:
                acc = jnp.concatenate([acc[:q0], acc[q0:] + t], axis=0)
        return acc[:, 0] - acc[:, 2], acc[:, 0] + acc[:, 1]

    def overlap_add(yr, yi, prev, r):
        n = 1 if prev is None else 0
        pr = yr[:3] if prev is None else jnp.concatenate([prev[0], yr[:3]], axis=0)
        pi = yi[:3] if prev is None else jnp.concatenate([prev[1], yi[:3]], axis=0)
        if r < 64:
            zr, zi = yr[n:] - pi, yi[n:] + pr
        else:
            zr, zi = yr[n:] + pi, yi[n:] - pr
        if prev is None:
            zr = jnp.concatenate([yr[:1], zr], axis=0)
            zi = jnp.concatenate([yi[:1], zi], axis=0)
        return zr, zi, (yr[3:], yi[3:])

    def conv_spec(ug, zb, lo=0, hi=8):
        for rp in range(lo, hi):
            p0 = p1 = None
            for ib in range(4):
                zr0, zi0, p0 = overlap_add(*spec_item(ug, ib, 16 * rp), p0, 16 * rp)
                zr1, zi1, p1 = overlap_add(*spec_item(ug, ib, 16 * rp + 8), p1, 16 * rp)
                zb[4 * ib:4 * ib + 4, rp * 8:rp * 8 + 8, :] = _pack(jnp.concatenate([zr0, zr1], axis=1))
                zb[4 * ib:4 * ib + 4, 64 + rp * 8:72 + rp * 8, :] = _pack(jnp.concatenate([zi0, zi1], axis=1))

    def conv_inv(cb, zb):
        for i in range(NC):
            for e in range(2):
                y_s[e, cb, i * 128:(i + 1) * 128, :] = jnp.dot(
                    _unpack(inv_ref[:, e * 128:(e + 1) * 128]), _unpack(zb[i, e * 64:(e + 1) * 64, :]),
                    preferred_element_type=f32)

    def conv_step(c, ug_cur, ug_nxt, zb_cur, zb_prev, pb_nxt, pb_new):
        @pl.when(c + 3 < G)
        def _():
            conv_start(c + 3)
        w_copy(c).start()

        @pl.when(c >= G - 3)
        def _():
            x_copy(c - (G - 3)).start()
        conv_spec(ug_cur, zb_cur)
        fwd_h(pb_nxt, ug_nxt)
        fwd_u(pb_nxt, ug_nxt)
        conv_inv(c - 1, zb_prev)

        @pl.when(c + 2 < G)
        def _():
            wait_all([w_copy(c - 1), h_copy(c + 2)] + kv_copies(c + 2))
            prep_kv(c + 2, pb_new, True)
            add_skip(c + 1, ug_nxt)

        @pl.when(c + 2 >= G)
        def _():
            w_copy(c - 1).wait()
            add_skip(c + 1, ug_nxt)

    def conv():
        wait_all([fwd_cp, h_copy(0)])
        conv_start(1)
        inv_cp.start()
        prep_h(0, pb_a)
        fwd_h(pb_a, ug_a)
        wait_all([shk_cp] + kv_copies(0))
        conv_start(2)
        setup_taps()
        prep_kv(0, pb_a, False)
        fwd_u(pb_a, ug_a)
        fence([h_copy(1)])
        prep_h(1, pb_b)
        fence([ssmd_cp])
        setup_skip()
        add_skip(0, ug_a)
        conv_spec(ug_a, zb_a, 0, 4)
        fwd_h(pb_b, ug_b)
        fence(kv_copies(1))
        conv_start(3)
        w_copy(0).start()
        prep_kv(1, pb_b, False)
        add_skip(1, ug_b)
        fence([h_copy(2)])
        conv_spec(ug_a, zb_a, 4, 8)
        fwd_u(pb_b, ug_b)
        fence(kv_copies(2) + [inv_cp])
        prep_kv(2, pb_a, True)

        def body(p, carry):
            conv_step(2 * p + 1, ug_b, ug_a, zb_b, zb_a, pb_a, pb_b)
            conv_step(2 * p + 2, ug_a, ug_b, zb_a, zb_b, pb_b, pb_a)
            return carry
        lax.fori_loop(0, G // 2 - 1, body, 0)
        w_copy(G - 1).start()
        conv_spec(ug_b, zb_b)
        conv_inv(G - 2, zb_a)
        fence([x_copy(0)])
        for p in range(NP):
            ln1_piece(0, p)
        conv_inv(G - 1, zb_b)
        wait_all([w_copy(G - 2), w_copy(G - 1)])
        col = D + (G - 1) * 128
        k_s[G - 1, 0:NV // 2, :] = _pack(jnp.dot(_unpack(h_s[0:NV // 2, :]), wqkv[:, col:col + 128],
                                                 preferred_element_type=f32))

    def phase1():
        def body(c, carry):
            @pl.when(c + 1 < NRC)
            def _():
                x_copy(c + 1).wait()

            @pl.when(c + 2 < NRC)
            def _():
                x_copy(c + 2).start()

            @pl.when(c + 2 == NRC)
            def _():
                wo_copy().start()
            cn = jnp.minimum(c + 1, NRC - 1)
            qkv_proj(_unpack(h_s[...]), c, lambda p: ln1_piece(cn, p), 2, kb_plan((c + G - 1) & (G - 1), range(17, 22)))
            return carry
        lax.fori_loop(0, NRC, body, 0)
        wo_copy().wait()

    def phase2(ms):
        o = load_o(0)
        z0 = z_ref[0]
        for q in range(2):
            rs = [oproj_tile(o, 0, n, z0, None, q * (RC // 2), RC // 2, True) for n in range(8)]
            if q == 0:
                attention_tail(ms, rs[0:5:2])
            for p in range(q * NP // 2, (q + 1) * NP // 2):
                ln2_piece(0, p, z0)

        def body(c, carry):
            z0 = z_ref[0]
            z1 = z_ref[1]
            h = _unpack(h_s[...])
            o = load_o(c + 1)
            for n in range(8):
                oproj_tile(o, c + 1, n, z1, first=True)
            qkv_proj(h, c, lambda p: ln2_piece(c + 1, p, z0), 1, kb_plan(jnp.maximum(c - 1, 0), range(17, 22)))
            return carry
        lax.fori_loop(0, NRC - 1, body, 0)
        qkv_proj(_unpack(h_s[...]), NRC - 1, None, 0,
                 {**kb_plan(G - 2, range(0, 10)), **kb_plan(G - 1, range(10, 20))})

    def phase3(ms):
        o = load_o(0)
        attention_tail(ms, [oproj_tile(o, 0, n, z_ref[1]) for n in range(8)])

        def body(c, carry):
            z0 = z_ref[0]
            z1 = z_ref[1]
            zv = zero_vreg()
            o = load_o(c + 1)
            deps = {}
            p = 0
            for t in range(16):
                for _ in range(2 if t < 2 else 1):
                    if p < NP:
                        deps.setdefault(t + 2, []).append(_tok(out_piece(c, p, z0), zv))
                        p += 1
                oproj_tile(o, c + 1, t // 2, z1, deps.get(t), (t % 2) * 128, 128)
            out_copy(c).start()
            return carry
        lax.fori_loop(0, NRC - 2, body, 0)

        c = NRC - 1
        z0 = z_ref[0]
        zv = zero_vreg()
        o = load_o(c)
        deps = {}
        todo = [(c - 1, p) for p in range(NP)]
        for q in range(3):
            for n in range(8):
                t = 8 * q + n
                for cc, p in todo[2 * n:2 * n + 2]:
                    deps.setdefault(t + 2, []).append(_tok(out_piece(cc, p, z0), zv))
                oproj_tile(o, c, n, z0, deps.get(t), TAIL[q], TAIL[q + 1] - TAIL[q])
            (out_copy(c - 1) if q == 0 else tail_copy(q - 1)).start()
            todo = [(c, p) for p in range(TAIL[q] // 16, TAIL[q + 1] // 16)]
        for cc, p in todo:
            out_piece(cc, p, z0)
        tail_copy(2).start()
        wait_all([out_copy(i) for i in range(NRC - 1)] + [tail_copy(q) for q in range(3)])

    zero16 = jnp.zeros((16, 128), u32)

    def qk(g, j, hh, half, dst, z, zk, dep):
        qt = qt_s[j, pl.ds(pl.multiple_of(g * 64 + hh * 16, 16), 16), :]
        w = _unpack(jnp.concatenate([qt if i == hh else zero16 for i in range(4)], axis=0))
        ch = CH if half == 1 else CH - NV // 4
        r0 = NV if half == 0 else 0
        kh = k_s[g + zk, (half * HS + r0) // 2:(half + 1) * HS // 2, :]
        m = first = s = None
        for c in range(4):
            ku = kh[c * ch // 2:(c + 1) * ch // 2]
            if dep is not None:
                ku = jnp.concatenate([ku[:ch // 2 - 8], ku[ch // 2 - 8:] | dep], axis=0)
            s = jnp.dot(_unpack(ku), w, preferred_element_type=f32)
            dst[z, r0 + c * ch:r0 + (c + 1) * ch, :] = s
            mc = jnp.max(s.reshape(ch // 8, 8, 128), axis=0)
            m = mc if m is None else jnp.maximum(m, mc)
            f = pltpu.bitcast(s[0:8], u32)
            first = f if first is None else first | f
        return m, first, s

    def qk_vpu(g, j, hh, i0, acc, trigs):
        qw16 = qt_s[j, pl.ds(pl.multiple_of(g * 64 + hh * 16, 16), 16), :]
        for k, tr in enumerate(trigs):
            i = i0 + k
            qw = jnp.broadcast_to(qw16[i:i + 1], (8, 128))
            if tr is not None:
                qw = qw | tr
            qb = pltpu.bitcast(jnp.stack([qw << 16, qw & jnp.uint32(0xFFFF0000)]), f32)
            d = hh * 32 + 2 * i
            t = kb_s[g, d:d + 2].reshape(2, NV // 8, 8, 128) * qb[:, None]
            acc = t[0] + t[1] if acc is None else acc + t[0] + t[1]
        return acc

    def fullmax(m1, m2):
        return jnp.max(jnp.maximum(m1, m2), axis=0, keepdims=True)

    def sm_pv(g, hh, half, src, m, z, dep, trigs):
        mb = jnp.broadcast_to(m, (8, 128))
        mbu = pltpu.bitcast(mb, u32)
        ms = [mb if tr is None else pltpu.bitcast(mbu | tr, f32) for tr in trigs]
        mm = jnp.stack([jnp.stack([ms[4 * st + 3 - kk] for kk in range(4)]) for st in range(2)])
        x = src[z].reshape(2, 4, 4, 4, 8, 128)
        p = jnp.exp2(x - mm[:, None, :, None]).reshape(HS, 128)
        rs = pl.ds(pl.multiple_of(g * 64 + hh * 16, 16), 16)
        vu = vt_s[half * 8:half * 8 + 8, rs, :]
        vu = jnp.concatenate([vu[:, 0:8] | dep[None], vu[:, 8:16]], axis=1)
        vu = jnp.concatenate([vu[t] for t in range(8)], axis=1)
        l = _tree_sum(p)
        return jnp.dot(_unpack(vu), p.astype(bf), preferred_element_type=f32), l

    def store_o(g, j, parts):
        outs = [parts[2 * h] * (1.0 / jnp.sum(parts[2 * h + 1], axis=0, keepdims=True)) for h in range(4)]
        o_s[g, pl.ds(pl.multiple_of(j * 64, 64), 64), :] = _pack(jnp.concatenate(outs, axis=0).T)

    bufs = {(0, 0): a1, (0, 1): a2, (1, 0): b1, (1, 1): b2}

    def tile_of(t):
        return lax.shift_right_logical(t, 4), t & (NQ - 1)

    def finish_tile(g, j, done, res):
        if done is None:
            parts = []
        else:
            parts = [done[0:32], done[32:40], done[40:72], done[72:80]]
            res = [(done[80:112], done[112:120])] + res
        for h in range(len(res) // 2):
            parts += [res[2 * h][0] + res[2 * h + 1][0], res[2 * h][1] + res[2 * h + 1][1]]
        store_o(g, j, parts)

    def attention(m_init):
        nit = G * NQ // UNR

        def body(it, carry):
            z1 = z_ref[0]
            z2 = z_ref[1]
            zv = zero_vreg()
            g, j0 = tile_of(it * UNR)
            gp, jp = tile_of(jnp.maximum(it * UNR - 1, 0))
            mfull = {(-1, 2): carry[0], (-1, 3): carry[1]}
            mpart = do = ps = po = vacc = None
            res = []
            cache = {}

            def tg(sv, i):
                if sv is None:
                    return None
                if (id(sv), i) not in cache:
                    cache[(id(sv), i)] = (sv, pltpu.bitcast(sv[i * 8:i * 8 + 8], u32) & zv)
                return cache[(id(sv), i)][1]

            for n in range(8 * UNR):
                u, qh, qhalf = n // 8, (n % 8) // 2, n % 2
                mp, first, cs = qk(g, j0 + u, qh, qhalf, bufs[(qh % 2, qhalf)], z1, z_ref[2 + n], do)
                src = {'p': ps, 'o': po, 'c': cs}
                vtr, etr = [[tg(src[t[0]], int(t[1:])) for t in spec[n >= N0].split('/')[qhalf].split(',')]
                            for spec in (VT, ET)]
                if qhalf == 0:
                    vacc = qk_vpu(g, j0 + u, qh, 0, None, vtr)
                    mpart = mp
                else:
                    vacc = qk_vpu(g, j0 + u, qh, 16 - len(vtr), vacc, vtr)
                    bufs[(qh % 2, 0)][z1, 0:NV, :] = vacc.reshape(NV, 128)
                    mfull[(u, qh)] = fullmax(jnp.maximum(mpart, jnp.max(vacc, axis=0)), mp)
                pu, ph, phalf = (n - LAG) // 8, ((n - LAG) % 8) // 2, (n - LAG) % 2
                o, l = sm_pv(gp if pu < 0 else g, ph, phalf, bufs[(ph % 2, phalf)], mfull[(pu, ph)], z2,
                             first & zv, etr)
                ps, po, do = cs, o, tg(o, 3)
                res.append((o, l))
                if ph == 3 and phalf == 1:
                    if pu < 0:
                        finish_tile(gp, jp, fin[z2], res)
                    else:
                        finish_tile(g, j0 + pu, None, res)
                    res = []
            fin[z1] = jnp.concatenate([res[0][0] + res[1][0], res[0][1] + res[1][1],
                                       res[2][0] + res[3][0], res[2][1] + res[3][1],
                                       res[4][0], res[4][1]], axis=0)
            return mfull[(UNR - 1, 2)], mfull[(UNR - 1, 3)]

        return lax.fori_loop(0, nit, body, m_init)

    def attention_tail(ms, rs):
        z2 = z_ref[1]
        zv = zero_vreg()
        res = []
        for k, (ph, phalf) in enumerate(((2, 1), (3, 0), (3, 1))):
            trigs = [pltpu.bitcast(rs[k][16 * i:16 * i + 8], u32) & zv for i in range(8)]
            res.append(sm_pv(G - 1, ph, phalf, bufs[(ph % 2, phalf)], ms[ph - 2], z2, trigs[7], trigs))
        finish_tile(G - 1, NQ - 1, fin[z2], res)

    conv()
    phase1()
    ms = attention((jnp.zeros((1, 128), f32), jnp.zeros((1, 128), f32)))
    phase2(ms)
    ms = attention(ms)
    phase3(ms)


@jax.jit
def pallas_interleave_layers__softmax_full_mha__ssm_conv_h3__prompt_kernel(
        A_x, A_wqkv, A_wo, B_q, B_k, B_v, B_shift_k, B_ssm_k, B_ssm_D):
    del B_q
    fwd, inv = _dft_mats()
    scratch = [
        pltpu.VMEM((1, S, D), f32),
        pltpu.VMEM((2, G, S, 128), f32),
        pltpu.VMEM((NQ, D // 2, 128), u32),
        pltpu.VMEM((G, S // 2, 128), u32),
        pltpu.VMEM((NQ, D // 2, 128), u32),
        pltpu.VMEM((G, S // 2, 128), u32),
        pltpu.VMEM((G, 128, NV, 128), f32),
        pltpu.VMEM((1, HS, 128), f32), pltpu.VMEM((1, HS, 128), f32),
        pltpu.VMEM((1, HS, 128), f32), pltpu.VMEM((1, HS, 128), f32),
        pltpu.VMEM((1, 120, 128), f32),
        pltpu.VMEM((1, S + 8, 128), f32),
        pltpu.VMEM((G, 40, 128), f32),
        pltpu.VMEM((1, 2 * NC, 3, IM, 128), f32),
        pltpu.VMEM((1, 2 * NC, 3, IM, 128), f32),
        pltpu.VMEM((NC, 128, 128), u32),
        pltpu.VMEM((NC, 128, 128), u32),
        pltpu.VMEM((S, 128), u32),
        pltpu.VMEM((S, 128), u32),
        pltpu.VMEM((RC // 2, D), u32),
        pltpu.SMEM((NZ,), i32),
        pltpu.VMEM((S, D), bf),
        pltpu.VMEM((D, 3 * D + 128), bf),
        pltpu.VMEM((D, D + 128), bf),
        pltpu.VMEM((NB, S, 128), bf),
        pltpu.VMEM((NB, S, 128), bf),
        pltpu.VMEM((NB, 128, S + 128), bf),
        pltpu.VMEM((4, D), bf),
        pltpu.VMEM((G, 128), bf),
        pltpu.VMEM((320, 128), u32),
        pltpu.VMEM((64, 256), u32),
        pltpu.SemaphoreType.DMA((3, G)),
        pltpu.SemaphoreType.DMA((NRC,)),
        pltpu.SemaphoreType.DMA((G + 1,)),
        pltpu.SemaphoreType.DMA((NRC + 2,)),
        pltpu.SemaphoreType.DMA((4,)),
    ]
    hbm = pl.BlockSpec(memory_space=pl.ANY)
    return pl.pallas_call(
        _kernel,
        out_shape=jax.ShapeDtypeStruct((1, S, D), bf),
        in_specs=[hbm] * 10,
        out_specs=hbm,
        scratch_shapes=scratch,
        compiler_params=pltpu.CompilerParams(vmem_limit_bytes=120 * 2**20, disable_bounds_checks=True),
    )(A_x, A_wqkv, A_wo, B_k, B_v, B_shift_k.T, B_ssm_k, B_ssm_D.reshape(G, 128),
      jnp.asarray(fwd), jnp.asarray(inv))
```

```python
import numpy as np
import jax
import jax.numpy as jnp
from jax import lax
import jax.experimental.pallas as pl
import jax.experimental.pallas.tpu as pltpu

S = 2048
D = 1024
DH = 32
G = 8
NQ = 16
HS = S // 2
CH = HS // 4
UNR = 8
NV = 64
LAG = 3
RC = 256
NRC = S // RC
NP = RC // 16
NC = 16
NB = 4
IM = 136
GO = 8
EPS = 1e-5
F2 = 1
LNS2 = 13
KBR2 = range(15, 23)
LNS = 12
KBR = range(15, 22)
NZ = 2 + 8 * UNR
QSCALE = float(DH ** -0.5 * np.log2(np.e))
N0 = 12
VT = ('p30,p31,p31,o3,c5,c5,c14,c18/p28,p29,p29,p29,o1,c0,c6,c13',
      'p31,p31,p31,c1,c5,c5,c14,c17/p26,p27,p28,o1,c1,c4,c7,c16')
ET = ('p17,p22,p29,p30,o0,c0,c4,c8/p16,p19,p29,p29,o0,c0,c4,c6',
      'p19,p20,p30,o0,o1,c0,c4,c10/p17,p19,p29,o0,o3,c2,c6,c6')

bf = jnp.bfloat16
f32 = jnp.float32
u32 = jnp.uint32
i32 = jnp.int32
NT = (((1,), (1,)), ((), ()))


def _dft_mats():
    n = np.arange(128)
    f = np.concatenate([np.arange(0, 128, 2), np.arange(1, 128, 2)])
    ang = 2.0 * np.pi * np.outer(f + 0.5, n) / 256.0
    re, im = np.cos(ang), -np.sin(ang)
    inv = np.concatenate([re, im], axis=0).T / 128.0
    fwd = np.concatenate([re, im, re, im - re, im + re], axis=0)

    def pack_rows(a):
        u = np.ascontiguousarray(a, dtype=np.float32).view(np.uint32)
        u = (u + 0x7FFF + ((u >> 16) & 1)) >> 16
        return (u[0::2] | (u[1::2] << 16)).astype(np.uint32)
    return pack_rows(fwd), pack_rows(inv)


def _tree_sum(p):
    n = p.shape[0] // 8
    x = p.reshape(n, 8, 128)
    while n > 1:
        x = x.reshape(n // 2, 2, 8, 128)
        x = x[:, 0] + x[:, 1]
        n //= 2
    return x[0]


def _ln(x):
    m = jnp.mean(x, axis=-1, keepdims=True)
    xc = x - m
    v = jnp.mean(xc * xc, axis=-1, keepdims=True)
    return xc * lax.rsqrt(v + EPS)


def _pack(x):
    return pltpu.bitcast(x.astype(bf), u32)


def _unpack(x):
    return pltpu.bitcast(x, bf)


def _tok(v, zv):
    v = v if v.dtype == u32 else pltpu.bitcast(v, u32)
    while v.shape[1] > 128:
        h = v.shape[1] // 2
        v = v[:, :h] | v[:, h:]
    while v.shape[0] > 8:
        h = v.shape[0] // 2
        v = v[:h] | v[h:]
    return v & zv


def _gate(w, toks):
    if not toks:
        return w
    wu = pltpu.bitcast(w, u32)
    h0 = wu[0:8]
    for t in toks:
        h0 = h0 | t
    return _unpack(jnp.concatenate([h0, wu[8:]], axis=0))


def _kernel(x_hbm, wqkv_hbm, wo_hbm, bk_hbm, bv_hbm, shk_hbm, ssmk_hbm, ssmd_hbm, fwd_hbm, inv_hbm, out_hbm,
            x_s, y_s, qt_s, k_s, vt_s, o_s, kb_s, a1, a2, b1, b2, fin, kf_s, taps_s, ug_a, ug_b, zb_a, zb_b,
            pb_a, pb_b, h_s, z_ref, x_in, wqkv, wo, bk, bv, ssmk, shk, ssmd, fwd_ref, inv_ref,
            sem_c, sem_x, sem_w, sem_o, sem_s):
    out_s = x_in

    def kv_copies(cb):
        cs = pl.ds(pl.multiple_of(cb * 128, 128), 128)
        return [pltpu.make_async_copy(bk_hbm.at[0, :, cs], bk.at[cb % NB], sem_c.at[0, cb]),
                pltpu.make_async_copy(bv_hbm.at[0, :, cs], bv.at[cb % NB], sem_c.at[1, cb])]

    def h_copy(cb):
        cs = pl.ds(pl.multiple_of(cb * 128, 128), 128)
        return pltpu.make_async_copy(ssmk_hbm.at[cs, :], ssmk.at[cb % NB, :, pl.ds(0, S)], sem_c.at[2, cb])

    def x_copy(c):
        rs = pl.ds(pl.multiple_of(c * RC, RC), RC)
        return pltpu.make_async_copy(x_hbm.at[0, rs, :], x_in.at[rs, :], sem_x.at[c])

    def w_copy(c):
        rs = pl.ds(pl.multiple_of(c * 128, 128), 128)
        return pltpu.make_async_copy(wqkv_hbm.at[rs, :], wqkv.at[rs, pl.ds(0, 3 * D)], sem_w.at[c])

    def wo_copy():
        return pltpu.make_async_copy(wo_hbm, wo.at[:, pl.ds(0, D)], sem_w.at[G])

    def out_copy(c):
        rs = pl.ds(pl.multiple_of(c * RC, RC), RC)
        return pltpu.make_async_copy(out_s.at[rs, :], out_hbm.at[0, rs, :], sem_o.at[c])

    TAIL = (0, 128, 192, 256)

    def tail_copy(q):
        rs = pl.ds((NRC - 1) * RC + TAIL[q], TAIL[q + 1] - TAIL[q])
        return pltpu.make_async_copy(out_s.at[rs, :], out_hbm.at[0, rs, :], sem_o.at[NRC - 1 + q])

    def conv_start(c):
        h_copy(c).start()
        for cp in kv_copies(c):
            cp.start()

    def wait_all(cps):
        for cp in cps:
            cp.wait()

    shk_cp, ssmd_cp, fwd_cp, inv_cp = [
        pltpu.make_async_copy(src, dst, sem_s.at[i]) for i, (src, dst) in enumerate(
            ((shk_hbm, shk), (ssmd_hbm, ssmd), (fwd_hbm, fwd_ref), (inv_hbm, inv_ref)))]
    h_copy(0).start()
    fwd_cp.start()
    shk_cp.start()
    ssmd_cp.start()
    for cp in kv_copies(0):
        cp.start()

    for i in range(NZ):
        z_ref[i] = 0
    fin[...] = jnp.ones(fin.shape, f32)
    for buf in (a2, b1, b2):
        buf[...] = jnp.zeros(buf.shape, f32)
    kf_s[0, 0:8, :] = jnp.zeros((8, 128), f32)

    def zero_vreg():
        return jnp.full((8, 128), z_ref[0], i32).astype(u32)

    def fence(cps):
        @pl.when(z_ref[0] == 0)
        def _():
            wait_all(cps)

    TILES = [(0, n) for n in range(8)] + [(2, n) for n in range(8)] + [(1, n) for n in range(8)]

    def qkv_tile(h, c, idx, toks, zv):
        kind, n = TILES[idx]
        col = kind * D + n * 128
        r = jnp.dot(h, _gate(wqkv[:, col:col + 128], toks), preferred_element_type=f32)
        if kind == 1:
            k_s[n, pl.ds(pl.multiple_of(c * (RC // 2), RC // 2), RC // 2), :] = _pack(r)
            return None
        dst = qt_s if kind == 0 else vt_s
        if kind == 0:
            r = r * QSCALE
        pks = []
        for t in range(RC // 128):
            pk = _pack(r[t * 128:(t + 1) * 128, :].T)
            dst[c * (RC // 128) + t, n * 64:(n + 1) * 64, :] = pk
            pks.append(pk)
        return _tok(jnp.concatenate(pks, axis=0), zv)

    def qkv_proj(h, c, piece_fn, first_piece, kb_jobs, span=NP):
        zv = zero_vreg()
        deps = {}
        for n in range(24):
            done = qkv_tile(h, c, n, deps.get(n), zv)
            if done is not None:
                deps.setdefault(n + 3, []).append(done)
            if n in kb_jobs:
                deps.setdefault(n + 2, []).append(kb_piece(*kb_jobs[n], zv))
            if piece_fn is not None:
                for p in range(NP):
                    if first_piece + p * span // NP == n:
                        deps.setdefault(n + 3, []).append(_tok(piece_fn(p), zv))

    def kb_plan(g, tiles):
        return {t: (g, 128 * i // len(tiles), 128 * (i + 1) // len(tiles)) for i, t in enumerate(tiles)}

    def kb_piece(g, lo, hi, zv):
        kx = _unpack(k_s[g, 0:NV // 2, :]).astype(f32)
        for d in range(lo, hi):
            v = jnp.broadcast_to(kx[:, d:d + 1], (NV, 128))
            kb_s[g, d] = v
        return _tok(v[NV - 32:], zv)

    def early_keys():
        col = D + (G - 1) * 128
        k_s[G - 1, 0:NV // 2, :] = _pack(jnp.dot(_unpack(h_s[0:NV // 2, :]), wqkv[:, col:col + 128],
                                                 preferred_element_type=f32))

    def piece_rows(c, p):
        return pl.ds(pl.multiple_of(c * RC + p * 16, 16), 16)

    def ln1_piece(c, p):
        hp = _pack(_ln(x_in[piece_rows(c, p), :].astype(f32)))
        h_s[p * 8:(p + 1) * 8, :] = hp
        return hp

    def gated_x(c, p, z):
        rows = piece_rows(c, p)
        x1 = x_s[z, rows, :]
        y = jnp.concatenate([y_s[0, g, rows, :] + y_s[1, g, rows, :] for g in range(G)], axis=1)
        return x1 + _ln(x1) * y

    def ln2_piece(c, p, z):
        x2 = gated_x(c, p, z)
        x_s[z, piece_rows(c, p), :] = x2
        hp = _pack(_ln(x2))
        h_s[p * 8:(p + 1) * 8, :] = hp
        return hp

    def out_piece(c, p, z):
        v = gated_x(c, p, z)
        out_s[piece_rows(c, p), :] = v.astype(bf)
        return v

    def load_o(c):
        rs = pl.ds(pl.multiple_of(c * (RC // 2), RC // 2), RC // 2)
        return jnp.concatenate([_unpack(o_s[g, rs, :]) for g in range(G)], axis=1)

    def oproj_tile(o, c, n, z, toks=None, r0=0, nr=RC, first=False):
        rows = pl.ds(pl.multiple_of(c * RC + r0, nr), nr)
        cols = slice(n * 128, (n + 1) * 128)
        r = jnp.dot(o[r0:r0 + nr], _gate(wo[:, cols], toks), preferred_element_type=f32)
        x0 = x_in[rows, cols].astype(f32) if first else x_s[z, rows, cols]
        x_s[z, rows, cols] = x0 + r
        return r

    zts = [z_ref[2 + ib] for ib in range(4)]

    def setup_taps():
        taps = shk[...].astype(f32)
        for cb in range(G):
            for t in range(4):
                taps_s[cb, 8 * t:8 * t + 8, :] = jnp.broadcast_to(taps[t:t + 1, cb * 128:(cb + 1) * 128], (8, 128))

    def setup_skip():
        dall = ssmd[...].astype(f32)
        for cb in range(G):
            taps_s[cb, 32:40, :] = jnp.broadcast_to(dall[cb:cb + 1, :], (8, 128))

    def prep_h_chunk(cb, pb, j):
        pb[HS + j * 64:HS + (j + 1) * 64, :] = pltpu.bitcast(ssmk[cb % NB, :, j * 128:(j + 1) * 128], u32)

    def prep_h(cb, pb):
        for j in range(NC):
            prep_h_chunk(cb, pb, j)

    def prep_kv(cb, pb, with_h):
        zs = z_ref[1]
        tp = taps_s[cb, 0:32, :]
        for j in range(NC):
            r0 = j * 128
            if with_h:
                prep_h_chunk(cb, pb, j)
            kf_s[zs, 8 + r0:8 + r0 + 128, :] = bk[cb % NB, r0:r0 + 128, :].astype(f32)
            ks = None
            for t in range(4):
                term = kf_s[zs, 8 + r0 - t:8 + r0 - t + 128, :].reshape(16, 8, 128) * tp[8 * t:8 * t + 8][None]
                ks = term if ks is None else ks + term
            pb[j * 64:(j + 1) * 64, :] = _pack(ks.reshape(128, 128) * bv[cb % NB, r0:r0 + 128, :].astype(f32))

    def fwd_h(pb, ug):
        for m in range(NC):
            hm = lax.dot_general(_unpack(fwd_ref[128:320, :]), _unpack(pb[HS + m * 64:HS + (m + 1) * 64, :]),
                                 NT, preferred_element_type=f32)
            ug[0, NC + m, :, GO:GO + 128, :] = hm.reshape(3, 128, 128)

    def fwd_u(pb, ug):
        for j in range(NC):
            u = jnp.dot(_unpack(fwd_ref[0:128, :]), _unpack(pb[j * 64:(j + 1) * 64, :]),
                        preferred_element_type=f32)
            ug[0, j, 0:2, 0:128, :] = u.reshape(2, 128, 128)

    def add_skip(cb, ug):
        dv = taps_s[cb, 32:40, :][None]
        for e in range(3):
            v = ug[0, NC, e, GO:GO + 128, :].reshape(16, 8, 128)
            ug[0, NC, e, GO:GO + 128, :] = (v - dv if e == 1 else v + dv).reshape(128, 128)

    def spec_item(ug, ib, r):
        zt = zts[ib]
        acc = None
        for j in range(4 * ib + 4):
            u = ug[zt, j:j + 1, 0:2, r:r + 8, :]
            u = jnp.concatenate([u[:, 0:1] + u[:, 1:2], u], axis=1)
            q0 = max(0, j - 4 * ib)
            m0 = NC + 4 * ib - j
            t = ug[zt, m0 + q0:m0 + 4, :, GO + r:GO + r + 8, :] * u
            if acc is None:
                acc = t
            elif q0 == 0:
                acc = acc + t
            else:
                acc = jnp.concatenate([acc[:q0], acc[q0:] + t], axis=0)
        return acc[:, 0] - acc[:, 2], acc[:, 0] + acc[:, 1]

    def overlap_add(yr, yi, prev, r):
        n = 1 if prev is None else 0
        pr = yr[:3] if prev is None else jnp.concatenate([prev[0], yr[:3]], axis=0)
        pi = yi[:3] if prev is None else jnp.concatenate([prev[1], yi[:3]], axis=0)
        if r < 64:
            zr, zi = yr[n:] - pi, yi[n:] + pr
        else:
            zr, zi = yr[n:] + pi, yi[n:] - pr
        if prev is None:
            zr = jnp.concatenate([yr[:1], zr], axis=0)
            zi = jnp.concatenate([yi[:1], zi], axis=0)
        return zr, zi, (yr[3:], yi[3:])

    def conv_spec(ug, zb, lo=0, hi=8):
        for rp in range(lo, hi):
            p0 = p1 = None
            for ib in range(4):
                zr0, zi0, p0 = overlap_add(*spec_item(ug, ib, 16 * rp), p0, 16 * rp)
                zr1, zi1, p1 = overlap_add(*spec_item(ug, ib, 16 * rp + 8), p1, 16 * rp)
                zb[4 * ib:4 * ib + 4, rp * 8:rp * 8 + 8, :] = _pack(jnp.concatenate([zr0, zr1], axis=1))
                zb[4 * ib:4 * ib + 4, 64 + rp * 8:72 + rp * 8, :] = _pack(jnp.concatenate([zi0, zi1], axis=1))

    def conv_inv(cb, zb):
        for i in range(NC):
            for e in range(2):
                y_s[e, cb, i * 128:(i + 1) * 128, :] = jnp.dot(
                    _unpack(inv_ref[:, e * 128:(e + 1) * 128]), _unpack(zb[i, e * 64:(e + 1) * 64, :]),
                    preferred_element_type=f32)

    def conv_step(c, ug_cur, ug_nxt, zb_cur, zb_prev, pb_nxt, pb_new):
        @pl.when(c + 3 < G)
        def _():
            conv_start(c + 3)
        w_copy(c).start()

        @pl.when(c >= G - 3)
        def _():
            x_copy(c - (G - 3)).start()
        conv_spec(ug_cur, zb_cur)
        fwd_h(pb_nxt, ug_nxt)
        fwd_u(pb_nxt, ug_nxt)
        conv_inv(c - 1, zb_prev)

        @pl.when(c + 2 < G)
        def _():
            wait_all([w_copy(c - 1), h_copy(c + 2)] + kv_copies(c + 2))
            prep_kv(c + 2, pb_new, True)
            add_skip(c + 1, ug_nxt)

        @pl.when(c + 2 >= G)
        def _():
            w_copy(c - 1).wait()
            add_skip(c + 1, ug_nxt)

    def conv():
        wait_all([fwd_cp, h_copy(0)])
        conv_start(1)
        inv_cp.start()
        prep_h(0, pb_a)
        fwd_h(pb_a, ug_a)
        wait_all([shk_cp] + kv_copies(0))
        conv_start(2)
        setup_taps()
        prep_kv(0, pb_a, False)
        fwd_u(pb_a, ug_a)
        fence([h_copy(1)])
        prep_h(1, pb_b)
        fence([ssmd_cp])
        setup_skip()
        add_skip(0, ug_a)
        conv_spec(ug_a, zb_a, 0, 4)
        fwd_h(pb_b, ug_b)
        fence(kv_copies(1))
        conv_start(3)
        w_copy(0).start()
        prep_kv(1, pb_b, False)
        add_skip(1, ug_b)
        fence([h_copy(2)])
        conv_spec(ug_a, zb_a, 4, 8)
        fwd_u(pb_b, ug_b)
        fence(kv_copies(2) + [inv_cp])
        prep_kv(2, pb_a, True)

        def body(p, carry):
            conv_step(2 * p + 1, ug_b, ug_a, zb_b, zb_a, pb_a, pb_b)
            conv_step(2 * p + 2, ug_a, ug_b, zb_a, zb_b, pb_b, pb_a)
            return carry
        lax.fori_loop(0, G // 2 - 1, body, 0)
        w_copy(G - 1).start()
        conv_spec(ug_b, zb_b)
        conv_inv(G - 2, zb_a)
        fence([x_copy(0), w_copy(G - 2), w_copy(G - 1)])
        for p in range(NP):
            ln1_piece(0, p)
        conv_inv(G - 1, zb_b)
        early_keys()

    def phase1():
        def body(c, carry):
            @pl.when(c + 1 < NRC)
            def _():
                x_copy(c + 1).wait()

            @pl.when(c + 2 < NRC)
            def _():
                x_copy(c + 2).start()

            @pl.when(c + 2 == NRC)
            def _():
                wo_copy().start()
            cn = jnp.minimum(c + 1, NRC - 1)
            qkv_proj(_unpack(h_s[...]), c, lambda p: ln1_piece(cn, p), 2, kb_plan((c + G - 1) & (G - 1), KBR), LNS)
            return carry
        lax.fori_loop(0, NRC, body, 0)
        wo_copy().wait()

    def phase2(ms):
        o = load_o(0)
        z0 = z_ref[0]
        for q in range(2):
            rs = [oproj_tile(o, 0, n, z0, None, q * (RC // 2), RC // 2, True) for n in range(8)]
            if q == 0:
                attention_tail(ms, rs[0:5:2])
            for p in range(q * NP // 2, (q + 1) * NP // 2):
                ln2_piece(0, p, z0)
        early_keys()

        def body(c, carry):
            z0 = z_ref[0]
            z1 = z_ref[1]
            h = _unpack(h_s[...])
            o = load_o(c + 1)
            for n in range(8):
                oproj_tile(o, c + 1, n, z1, first=True)
            qkv_proj(h, c, lambda p: ln2_piece(c + 1, p, z0), F2, kb_plan((c + G - 1) & (G - 1), KBR2), LNS2)
            return carry
        lax.fori_loop(0, NRC - 1, body, 0)
        qkv_proj(_unpack(h_s[...]), NRC - 1, None, 0, kb_plan(G - 2, KBR))

    def phase3(ms):
        o = load_o(0)
        attention_tail(ms, [oproj_tile(o, 0, n, z_ref[1]) for n in range(8)])

        def body(c, carry):
            z0 = z_ref[0]
            z1 = z_ref[1]
            zv = zero_vreg()
            o = load_o(c + 1)
            deps = {}
            p = 0
            for t in range(16):
                for _ in range(2 if t < 2 else 1):
                    if p < NP:
                        deps.setdefault(t + 2, []).append(_tok(out_piece(c, p, z0), zv))
                        p += 1
                oproj_tile(o, c + 1, t // 2, z1, deps.get(t), (t % 2) * 128, 128)
            out_copy(c).start()
            return carry
        lax.fori_loop(0, NRC - 2, body, 0)

        c = NRC - 1
        z0 = z_ref[0]
        zv = zero_vreg()
        o = load_o(c)
        deps = {}
        todo = [(c - 1, p) for p in range(NP)]
        for q in range(3):
            for n in range(8):
                t = 8 * q + n
                for cc, p in todo[2 * n:2 * n + 2]:
                    deps.setdefault(t + 2, []).append(_tok(out_piece(cc, p, z0), zv))
                oproj_tile(o, c, n, z0, deps.get(t), TAIL[q], TAIL[q + 1] - TAIL[q])
            (out_copy(c - 1) if q == 0 else tail_copy(q - 1)).start()
            todo = [(c, p) for p in range(TAIL[q] // 16, TAIL[q + 1] // 16)]
        for cc, p in todo:
            out_piece(cc, p, z0)
        tail_copy(2).start()
        wait_all([out_copy(i) for i in range(NRC - 1)] + [tail_copy(q) for q in range(3)])

    zero16 = jnp.zeros((16, 128), u32)

    def qk(g, j, hh, half, dst, z, zk, dep):
        qt = qt_s[j, pl.ds(pl.multiple_of(g * 64 + hh * 16, 16), 16), :]
        w = _unpack(jnp.concatenate([qt if i == hh else zero16 for i in range(4)], axis=0))
        ch = CH if half == 1 else CH - NV // 4
        r0 = NV if half == 0 else 0
        kh = k_s[g + zk, (half * HS + r0) // 2:(half + 1) * HS // 2, :]
        m = first = s = None
        for c in range(4):
            ku = kh[c * ch // 2:(c + 1) * ch // 2]
            if dep is not None:
                ku = jnp.concatenate([ku[:ch // 2 - 8], ku[ch // 2 - 8:] | dep], axis=0)
            s = jnp.dot(_unpack(ku), w, preferred_element_type=f32)
            dst[z, r0 + c * ch:r0 + (c + 1) * ch, :] = s
            mc = jnp.max(s.reshape(ch // 8, 8, 128), axis=0)
            m = mc if m is None else jnp.maximum(m, mc)
            f = pltpu.bitcast(s[0:8], u32)
            first = f if first is None else first | f
        return m, first, s

    def qk_vpu(g, j, hh, i0, acc, trigs):
        qw16 = qt_s[j, pl.ds(pl.multiple_of(g * 64 + hh * 16, 16), 16), :]
        for k, tr in enumerate(trigs):
            i = i0 + k
            qw = jnp.broadcast_to(qw16[i:i + 1], (8, 128))
            if tr is not None:
                qw = qw | tr
            qb = pltpu.bitcast(jnp.stack([qw << 16, qw & jnp.uint32(0xFFFF0000)]), f32)
            d = hh * 32 + 2 * i
            t = kb_s[g, d:d + 2].reshape(2, NV // 8, 8, 128) * qb[:, None]
            acc = t[0] + t[1] if acc is None else acc + t[0] + t[1]
        return acc

    def fullmax(m1, m2):
        return jnp.max(jnp.maximum(m1, m2), axis=0, keepdims=True)

    def sm_pv(g, hh, half, src, m, z, dep, trigs):
        mb = jnp.broadcast_to(m, (8, 128))
        mbu = pltpu.bitcast(mb, u32)
        ms = [mb if tr is None else pltpu.bitcast(mbu | tr, f32) for tr in trigs]
        mm = jnp.stack([jnp.stack([ms[4 * st + 3 - kk] for kk in range(4)]) for st in range(2)])
        x = src[z].reshape(2, 4, 4, 4, 8, 128)
        p = jnp.exp2(x - mm[:, None, :, None]).reshape(HS, 128)
        rs = pl.ds(pl.multiple_of(g * 64 + hh * 16, 16), 16)
        vu = vt_s[half * 8:half * 8 + 8, rs, :]
        vu = jnp.concatenate([vu[:, 0:8] | dep[None], vu[:, 8:16]], axis=1)
        vu = jnp.concatenate([vu[t] for t in range(8)], axis=1)
        l = _tree_sum(p)
        return jnp.dot(_unpack(vu), p.astype(bf), preferred_element_type=f32), l

    def store_o(g, j, parts):
        outs = [parts[2 * h] * (1.0 / jnp.sum(parts[2 * h + 1], axis=0, keepdims=True)) for h in range(4)]
        o_s[g, pl.ds(pl.multiple_of(j * 64, 64), 64), :] = _pack(jnp.concatenate(outs, axis=0).T)

    bufs = {(0, 0): a1, (0, 1): a2, (1, 0): b1, (1, 1): b2}

    def tile_of(t):
        return lax.shift_right_logical(t, 4), t & (NQ - 1)

    def finish_tile(g, j, done, res):
        if done is None:
            parts = []
        else:
            parts = [done[0:32], done[32:40], done[40:72], done[72:80]]
            res = [(done[80:112], done[112:120])] + res
        for h in range(len(res) // 2):
            parts += [res[2 * h][0] + res[2 * h + 1][0], res[2 * h][1] + res[2 * h + 1][1]]
        store_o(g, j, parts)

    def attention(m_init):
        nit = G * NQ // UNR

        def body(it, carry):
            z1 = z_ref[0]
            z2 = z_ref[1]
            zv = zero_vreg()
            g, j0 = tile_of(it * UNR)
            gp, jp = tile_of(jnp.maximum(it * UNR - 1, 0))
            mfull = {(-1, 2): carry[0], (-1, 3): carry[1]}
            mpart = do = ps = po = vacc = None
            res = []
            cache = {}

            def tg(sv, i):
                if sv is None:
                    return None
                if (id(sv), i) not in cache:
                    cache[(id(sv), i)] = (sv, pltpu.bitcast(sv[i * 8:i * 8 + 8], u32) & zv)
                return cache[(id(sv), i)][1]

            for n in range(8 * UNR):
                u, qh, qhalf = n // 8, (n % 8) // 2, n % 2
                mp, first, cs = qk(g, j0 + u, qh, qhalf, bufs[(qh % 2, qhalf)], z1, z_ref[2 + n], do)
                src = {'p': ps, 'o': po, 'c': cs}
                vtr, etr = [[tg(src[t[0]], int(t[1:])) for t in spec[n >= N0].split('/')[qhalf].split(',')]
                            for spec in (VT, ET)]
                if qhalf == 0:
                    vacc = qk_vpu(g, j0 + u, qh, 0, None, vtr)
                    mpart = mp
                else:
                    vacc = qk_vpu(g, j0 + u, qh, 16 - len(vtr), vacc, vtr)
                    bufs[(qh % 2, 0)][z1, 0:NV, :] = vacc.reshape(NV, 128)
                    mfull[(u, qh)] = fullmax(jnp.maximum(mpart, jnp.max(vacc, axis=0)), mp)
                pu, ph, phalf = (n - LAG) // 8, ((n - LAG) % 8) // 2, (n - LAG) % 2
                o, l = sm_pv(gp if pu < 0 else g, ph, phalf, bufs[(ph % 2, phalf)], mfull[(pu, ph)], z2,
                             first & zv, etr)
                ps, po, do = cs, o, tg(o, 3)
                res.append((o, l))
                if ph == 3 and phalf == 1:
                    if pu < 0:
                        finish_tile(gp, jp, fin[z2], res)
                    else:
                        finish_tile(g, j0 + pu, None, res)
                    res = []
            fin[z1] = jnp.concatenate([res[0][0] + res[1][0], res[0][1] + res[1][1],
                                       res[2][0] + res[3][0], res[2][1] + res[3][1],
                                       res[4][0], res[4][1]], axis=0)
            return mfull[(UNR - 1, 2)], mfull[(UNR - 1, 3)]

        return lax.fori_loop(0, nit, body, m_init)

    def attention_tail(ms, rs):
        z2 = z_ref[1]
        zv = zero_vreg()
        res = []
        for k, (ph, phalf) in enumerate(((2, 1), (3, 0), (3, 1))):
            trigs = [pltpu.bitcast(rs[k][16 * i:16 * i + 8], u32) & zv for i in range(8)]
            res.append(sm_pv(G - 1, ph, phalf, bufs[(ph % 2, phalf)], ms[ph - 2], z2, trigs[7], trigs))
        finish_tile(G - 1, NQ - 1, fin[z2], res)

    conv()
    phase1()
    ms = attention((jnp.zeros((1, 128), f32), jnp.zeros((1, 128), f32)))
    phase2(ms)
    ms = attention(ms)
    phase3(ms)


@jax.jit
def pallas_interleave_layers__softmax_full_mha__ssm_conv_h3__prompt_kernel(
        A_x, A_wqkv, A_wo, B_q, B_k, B_v, B_shift_k, B_ssm_k, B_ssm_D):
    del B_q
    fwd, inv = _dft_mats()
    scratch = [
        pltpu.VMEM((1, S, D), f32),
        pltpu.VMEM((2, G, S, 128), f32),
        pltpu.VMEM((NQ, D // 2, 128), u32),
        pltpu.VMEM((G, S // 2, 128), u32),
        pltpu.VMEM((NQ, D // 2, 128), u32),
        pltpu.VMEM((G, S // 2, 128), u32),
        pltpu.VMEM((G, 128, NV, 128), f32),
        pltpu.VMEM((1, HS, 128), f32), pltpu.VMEM((1, HS, 128), f32),
        pltpu.VMEM((1, HS, 128), f32), pltpu.VMEM((1, HS, 128), f32),
        pltpu.VMEM((1, 120, 128), f32),
        pltpu.VMEM((1, S + 8, 128), f32),
        pltpu.VMEM((G, 40, 128), f32),
        pltpu.VMEM((1, 2 * NC, 3, IM, 128), f32),
        pltpu.VMEM((1, 2 * NC, 3, IM, 128), f32),
        pltpu.VMEM((NC, 128, 128), u32),
        pltpu.VMEM((NC, 128, 128), u32),
        pltpu.VMEM((S, 128), u32),
        pltpu.VMEM((S, 128), u32),
        pltpu.VMEM((RC // 2, D), u32),
        pltpu.SMEM((NZ,), i32),
        pltpu.VMEM((S, D), bf),
        pltpu.VMEM((D, 3 * D + 128), bf),
        pltpu.VMEM((D, D + 128), bf),
        pltpu.VMEM((NB, S, 128), bf),
        pltpu.VMEM((NB, S, 128), bf),
        pltpu.VMEM((NB, 128, S + 128), bf),
        pltpu.VMEM((4, D), bf),
        pltpu.VMEM((G, 128), bf),
        pltpu.VMEM((320, 128), u32),
        pltpu.VMEM((64, 256), u32),
        pltpu.SemaphoreType.DMA((3, G)),
        pltpu.SemaphoreType.DMA((NRC,)),
        pltpu.SemaphoreType.DMA((G + 1,)),
        pltpu.SemaphoreType.DMA((NRC + 2,)),
        pltpu.SemaphoreType.DMA((4,)),
    ]
    hbm = pl.BlockSpec(memory_space=pl.ANY)
    return pl.pallas_call(
        _kernel,
        out_shape=jax.ShapeDtypeStruct((1, S, D), bf),
        in_specs=[hbm] * 10,
        out_specs=hbm,
        scratch_shapes=scratch,
        compiler_params=pltpu.CompilerParams(vmem_limit_bytes=120 * 2**20, disable_bounds_checks=True),
    )(A_x, A_wqkv, A_wo, B_k, B_v, B_shift_k.T, B_ssm_k, B_ssm_D.reshape(G, 128),
      jnp.asarray(fwd), jnp.asarray(inv))
```

```python
import numpy as np
import jax
import jax.numpy as jnp
from jax import lax
import jax.experimental.pallas as pl
import jax.experimental.pallas.tpu as pltpu

S = 2048
D = 1024
DH = 32
G = 8
NQ = 16
HS = S // 2
CH = HS // 4
UNR = 8
NE = 0
TSRC = 2
JOBS0 = {0: (240, 240, 240, 240), 16: (240, 240, 240, 224)}[NE]
NV = 64 + NE
LAG = 3
RC = 256
NRC = S // RC
NP = RC // 16
NC = 16
NB = 4
IM = 136
GO = 8
EPS = 1e-5
F2 = 1
LNS2 = 13
KBR2 = range(15, 23)
LNS = 12
KBR = range(15, 22)
NZ = 2 + 8 * UNR
QSCALE = float(DH ** -0.5 * np.log2(np.e))
N0 = 12
VT = ('p30,p31,p31,o3,c5,c5,c14,c17/p28,p29,p29,o0,o1,c0,c6,c13',
      'p28,p31,p31,p31,p31,p31,c1,c17/p26,p27,p29,o0,c0,c4,c7,c17')
ET = ('p17,p22,p29,p30,o0,c0,c4,c8/p16,p19,p29,p29,o0,c0,c4,c6',
      'p19,p21,p30,o0,o0,c0,c4,c10/p17,p18,p29,o0,o1,o3,c3,c5')

bf = jnp.bfloat16
f32 = jnp.float32
u32 = jnp.uint32
i32 = jnp.int32
NT = (((1,), (1,)), ((), ()))


def _dft_mats():
    n = np.arange(128)
    f = np.concatenate([np.arange(0, 128, 2), np.arange(1, 128, 2)])
    ang = 2.0 * np.pi * np.outer(f + 0.5, n) / 256.0
    re, im = np.cos(ang), -np.sin(ang)
    inv = np.concatenate([re, im], axis=0).T / 128.0
    fwd = np.concatenate([re, im, re, im - re, im + re], axis=0)

    def pack_rows(a):
        u = np.ascontiguousarray(a, dtype=np.float32).view(np.uint32)
        u = (u + 0x7FFF + ((u >> 16) & 1)) >> 16
        return (u[0::2] | (u[1::2] << 16)).astype(np.uint32)
    return pack_rows(fwd), pack_rows(inv)


def _tree_sum(p):
    n = p.shape[0] // 8
    x = p.reshape(n, 8, 128)
    while n > 1:
        x = x.reshape(n // 2, 2, 8, 128)
        x = x[:, 0] + x[:, 1]
        n //= 2
    return x[0]


def _ln(x):
    m = jnp.mean(x, axis=-1, keepdims=True)
    xc = x - m
    v = jnp.mean(xc * xc, axis=-1, keepdims=True)
    return xc * lax.rsqrt(v + EPS)


def _pack(x):
    return pltpu.bitcast(x.astype(bf), u32)


def _unpack(x):
    return pltpu.bitcast(x, bf)


def _tok(v, zv):
    v = v if v.dtype == u32 else pltpu.bitcast(v, u32)
    while v.shape[1] > 128:
        h = v.shape[1] // 2
        v = v[:, :h] | v[:, h:]
    while v.shape[0] > 8:
        h = v.shape[0] // 2
        v = v[:h] | v[h:]
    return v & zv


def _gate(w, toks):
    if not toks:
        return w
    wu = pltpu.bitcast(w, u32)
    h0 = wu[0:8]
    for t in toks:
        h0 = h0 | t
    return _unpack(jnp.concatenate([h0, wu[8:]], axis=0))


def _kernel(x_hbm, wqkv_hbm, wo_hbm, bk_hbm, bv_hbm, shk_hbm, ssmk_hbm, ssmd_hbm, fwd_hbm, inv_hbm, out_hbm,
            x_s, y_s, qt_s, k_s, vt_s, o_s, kb_s, a1, a2, b1, b2, fin, kf_s, taps_s, ug_a, ug_b, zb_a, zb_b,
            pb_a, pb_b, h_s, z_ref, x_in, wqkv, wo, bk, bv, ssmk, shk, ssmd, fwd_ref, inv_ref,
            sem_c, sem_x, sem_w, sem_o, sem_s):
    out_s = x_in

    def kv_copies(cb):
        cs = pl.ds(pl.multiple_of(cb * 128, 128), 128)
        return [pltpu.make_async_copy(bk_hbm.at[0, :, cs], bk.at[cb % NB], sem_c.at[0, cb]),
                pltpu.make_async_copy(bv_hbm.at[0, :, cs], bv.at[cb % NB], sem_c.at[1, cb])]

    def h_copy(cb):
        cs = pl.ds(pl.multiple_of(cb * 128, 128), 128)
        return pltpu.make_async_copy(ssmk_hbm.at[cs, :], ssmk.at[cb % NB, :, pl.ds(0, S)], sem_c.at[2, cb])

    def x_copy(c):
        rs = pl.ds(pl.multiple_of(c * RC, RC), RC)
        return pltpu.make_async_copy(x_hbm.at[0, rs, :], x_in.at[rs, :], sem_x.at[c])

    def w_copy(c):
        rs = pl.ds(pl.multiple_of(c * 128, 128), 128)
        return pltpu.make_async_copy(wqkv_hbm.at[rs, :], wqkv.at[rs, pl.ds(0, 3 * D)], sem_w.at[c])

    def wo_copy():
        return pltpu.make_async_copy(wo_hbm, wo.at[:, pl.ds(0, D)], sem_w.at[G])

    def out_copy(c):
        rs = pl.ds(pl.multiple_of(c * RC, RC), RC)
        return pltpu.make_async_copy(out_s.at[rs, :], out_hbm.at[0, rs, :], sem_o.at[c])

    TAIL = (0, 128, 192, 256)

    def tail_copy(q):
        rs = pl.ds((NRC - 1) * RC + TAIL[q], TAIL[q + 1] - TAIL[q])
        return pltpu.make_async_copy(out_s.at[rs, :], out_hbm.at[0, rs, :], sem_o.at[NRC - 1 + q])

    def conv_start(c):
        h_copy(c).start()
        for cp in kv_copies(c):
            cp.start()

    def wait_all(cps):
        for cp in cps:
            cp.wait()

    shk_cp, ssmd_cp, fwd_cp, inv_cp = [
        pltpu.make_async_copy(src, dst, sem_s.at[i]) for i, (src, dst) in enumerate(
            ((shk_hbm, shk), (ssmd_hbm, ssmd), (fwd_hbm, fwd_ref), (inv_hbm, inv_ref)))]
    h_copy(0).start()
    fwd_cp.start()
    shk_cp.start()
    ssmd_cp.start()
    for cp in kv_copies(0):
        cp.start()

    for i in range(NZ):
        z_ref[i] = 0
    fin[...] = jnp.ones(fin.shape, f32)
    for buf in (a2, b1, b2):
        buf[...] = jnp.zeros(buf.shape, f32)
    kf_s[0, 0:8, :] = jnp.zeros((8, 128), f32)

    def zero_vreg():
        return jnp.full((8, 128), z_ref[0], i32).astype(u32)

    def fence(cps):
        @pl.when(z_ref[0] == 0)
        def _():
            wait_all(cps)

    TILES = [(0, n) for n in range(8)] + [(2, n) for n in range(8)] + [(1, n) for n in range(8)]

    def qkv_tile(h, c, idx, toks, zv):
        kind, n = TILES[idx]
        col = kind * D + n * 128
        r = jnp.dot(h, _gate(wqkv[:, col:col + 128], toks), preferred_element_type=f32)
        if kind == 1:
            k_s[n, pl.ds(pl.multiple_of(c * (RC // 2), RC // 2), RC // 2), :] = _pack(r)
            return None
        dst = qt_s if kind == 0 else vt_s
        if kind == 0:
            r = r * QSCALE
        pks = []
        for t in range(RC // 128):
            pk = _pack(r[t * 128:(t + 1) * 128, :].T)
            dst[c * (RC // 128) + t, n * 64:(n + 1) * 64, :] = pk
            pks.append(pk)
        return _tok(jnp.concatenate(pks, axis=0), zv)

    def qkv_proj(h, c, piece_fn, first_piece, kb_jobs, span=NP):
        zv = zero_vreg()
        deps = {}
        for n in range(24):
            done = qkv_tile(h, c, n, deps.get(n), zv)
            if done is not None:
                deps.setdefault(n + 3, []).append(done)
            if n in kb_jobs:
                deps.setdefault(n + 2, []).append(kb_piece(*kb_jobs[n], zv))
            if piece_fn is not None:
                for p in range(NP):
                    if first_piece + p * span // NP == n:
                        deps.setdefault(n + 3, []).append(_tok(piece_fn(p), zv))

    def kb_plan(g, tiles):
        return {t: (g, 128 * i // len(tiles), 128 * (i + 1) // len(tiles)) for i, t in enumerate(tiles)}

    def kb_piece(g, lo, hi, zv):
        kx = _unpack(k_s[g, 0:NV // 2, :]).astype(f32)
        for d in range(lo, hi):
            v = jnp.broadcast_to(kx[:, d:d + 1], (NV, 128))
            kb_s[g, d] = v[0:64]
            if NE:
                kbx(g, d, 1)[...] = v[64:NV]
        return _tok(v[NV - 32:], zv)

    def early_keys():
        col = D + (G - 1) * 128
        k_s[G - 1, 0:NV // 2, :] = _pack(jnp.dot(_unpack(h_s[0:NV // 2, :]), wqkv[:, col:col + 128],
                                                 preferred_element_type=f32))

    def piece_rows(c, p):
        return pl.ds(pl.multiple_of(c * RC + p * 16, 16), 16)

    def ln1_piece(c, p):
        hp = _pack(_ln(x_in[piece_rows(c, p), :].astype(f32)))
        h_s[p * 8:(p + 1) * 8, :] = hp
        return hp

    def gated_x(c, p, z):
        rows = piece_rows(c, p)
        x1 = x_s[z, rows, :]
        y = jnp.concatenate([y_s[0, g, rows, :] + y_s[1, g, rows, :] for g in range(G)], axis=1)
        return x1 + _ln(x1) * y

    def ln2_piece(c, p, z):
        x2 = gated_x(c, p, z)
        x_s[z, piece_rows(c, p), :] = x2
        hp = _pack(_ln(x2))
        h_s[p * 8:(p + 1) * 8, :] = hp
        return hp

    def out_piece(c, p, z):
        v = gated_x(c, p, z)
        out_s[piece_rows(c, p), :] = v.astype(bf)
        return v

    def load_o(c):
        rs = pl.ds(pl.multiple_of(c * (RC // 2), RC // 2), RC // 2)
        return jnp.concatenate([_unpack(o_s[g, rs, :]) for g in range(G)], axis=1)

    def oproj_tile(o, c, n, z, toks=None, r0=0, nr=RC, first=False):
        rows = pl.ds(pl.multiple_of(c * RC + r0, nr), nr)
        cols = slice(n * 128, (n + 1) * 128)
        r = jnp.dot(o[r0:r0 + nr], _gate(wo[:, cols], toks), preferred_element_type=f32)
        x0 = x_in[rows, cols].astype(f32) if first else x_s[z, rows, cols]
        x_s[z, rows, cols] = x0 + r
        return r

    zts = [z_ref[2 + ib] for ib in range(4)]

    def setup_taps():
        taps = shk[...].astype(f32)
        for cb in range(G):
            for t in range(4):
                taps_s[cb, 8 * t:8 * t + 8, :] = jnp.broadcast_to(taps[t:t + 1, cb * 128:(cb + 1) * 128], (8, 128))

    def setup_skip():
        dall = ssmd[...].astype(f32)
        for cb in range(G):
            taps_s[cb, 32:40, :] = jnp.broadcast_to(dall[cb:cb + 1, :], (8, 128))

    def prep_h_chunk(cb, pb, j):
        pb[HS + j * 64:HS + (j + 1) * 64, :] = pltpu.bitcast(ssmk[cb % NB, :, j * 128:(j + 1) * 128], u32)

    def prep_h(cb, pb):
        for j in range(NC):
            prep_h_chunk(cb, pb, j)

    def prep_kv(cb, pb, with_h):
        zs = z_ref[1]
        tp = taps_s[cb, 0:32, :]
        for j in range(NC):
            r0 = j * 128
            if with_h:
                prep_h_chunk(cb, pb, j)
            kf_s[zs, 8 + r0:8 + r0 + 128, :] = bk[cb % NB, r0:r0 + 128, :].astype(f32)
            ks = None
            for t in range(4):
                term = kf_s[zs, 8 + r0 - t:8 + r0 - t + 128, :].reshape(16, 8, 128) * tp[8 * t:8 * t + 8][None]
                ks = term if ks is None else ks + term
            pb[j * 64:(j + 1) * 64, :] = _pack(ks.reshape(128, 128) * bv[cb % NB, r0:r0 + 128, :].astype(f32))

    def fwd_h(pb, ug):
        for m in range(NC):
            hm = lax.dot_general(_unpack(fwd_ref[128:320, :]), _unpack(pb[HS + m * 64:HS + (m + 1) * 64, :]),
                                 NT, preferred_element_type=f32)
            ug[0, NC + m, :, GO:GO + 128, :] = hm.reshape(3, 128, 128)

    def fwd_u(pb, ug):
        for j in range(NC):
            u = jnp.dot(_unpack(fwd_ref[0:128, :]), _unpack(pb[j * 64:(j + 1) * 64, :]),
                        preferred_element_type=f32)
            ug[0, j, 0:2, 0:128, :] = u.reshape(2, 128, 128)

    def add_skip(cb, ug):
        dv = taps_s[cb, 32:40, :][None]
        for e in range(3):
            v = ug[0, NC, e, GO:GO + 128, :].reshape(16, 8, 128)
            ug[0, NC, e, GO:GO + 128, :] = (v - dv if e == 1 else v + dv).reshape(128, 128)

    def spec_item(ug, ib, r):
        zt = zts[ib]
        acc = None
        for j in range(4 * ib + 4):
            u = ug[zt, j:j + 1, 0:2, r:r + 8, :]
            u = jnp.concatenate([u[:, 0:1] + u[:, 1:2], u], axis=1)
            q0 = max(0, j - 4 * ib)
            m0 = NC + 4 * ib - j
            t = ug[zt, m0 + q0:m0 + 4, :, GO + r:GO + r + 8, :] * u
            if acc is None:
                acc = t
            elif q0 == 0:
                acc = acc + t
            else:
                acc = jnp.concatenate([acc[:q0], acc[q0:] + t], axis=0)
        return acc[:, 0] - acc[:, 2], acc[:, 0] + acc[:, 1]

    def overlap_add(yr, yi, prev, r):
        n = 1 if prev is None else 0
        pr = yr[:3] if prev is None else jnp.concatenate([prev[0], yr[:3]], axis=0)
        pi = yi[:3] if prev is None else jnp.concatenate([prev[1], yi[:3]], axis=0)
        if r < 64:
            zr, zi = yr[n:] - pi, yi[n:] + pr
        else:
            zr, zi = yr[n:] + pi, yi[n:] - pr
        if prev is None:
            zr = jnp.concatenate([yr[:1], zr], axis=0)
            zi = jnp.concatenate([yi[:1], zi], axis=0)
        return zr, zi, (yr[3:], yi[3:])

    def conv_spec(ug, zb, lo=0, hi=8):
        for rp in range(lo, hi):
            p0 = p1 = None
            for ib in range(4):
                zr0, zi0, p0 = overlap_add(*spec_item(ug, ib, 16 * rp), p0, 16 * rp)
                zr1, zi1, p1 = overlap_add(*spec_item(ug, ib, 16 * rp + 8), p1, 16 * rp)
                zb[4 * ib:4 * ib + 4, rp * 8:rp * 8 + 8, :] = _pack(jnp.concatenate([zr0, zr1], axis=1))
                zb[4 * ib:4 * ib + 4, 64 + rp * 8:72 + rp * 8, :] = _pack(jnp.concatenate([zi0, zi1], axis=1))

    def conv_inv(cb, zb):
        for i in range(NC):
            for e in range(2):
                y_s[e, cb, i * 128:(i + 1) * 128, :] = jnp.dot(
                    _unpack(inv_ref[:, e * 128:(e + 1) * 128]), _unpack(zb[i, e * 64:(e + 1) * 64, :]),
                    preferred_element_type=f32)

    def conv_step(c, ug_cur, ug_nxt, zb_cur, zb_prev, pb_nxt, pb_new):
        @pl.when(c + 3 < G)
        def _():
            conv_start(c + 3)
        w_copy(c).start()

        @pl.when(c >= G - 3)
        def _():
            x_copy(c - (G - 3)).start()
        conv_spec(ug_cur, zb_cur)
        fwd_h(pb_nxt, ug_nxt)
        fwd_u(pb_nxt, ug_nxt)
        conv_inv(c - 1, zb_prev)

        @pl.when(c + 2 < G)
        def _():
            wait_all([w_copy(c - 1), h_copy(c + 2)] + kv_copies(c + 2))
            prep_kv(c + 2, pb_new, True)
            add_skip(c + 1, ug_nxt)

        @pl.when(c + 2 >= G)
        def _():
            w_copy(c - 1).wait()
            add_skip(c + 1, ug_nxt)

    def conv():
        wait_all([fwd_cp, h_copy(0)])
        conv_start(1)
        inv_cp.start()
        prep_h(0, pb_a)
        fwd_h(pb_a, ug_a)
        wait_all([shk_cp] + kv_copies(0))
        conv_start(2)
        setup_taps()
        prep_kv(0, pb_a, False)
        fwd_u(pb_a, ug_a)
        fence([h_copy(1)])
        prep_h(1, pb_b)
        fence([ssmd_cp])
        setup_skip()
        add_skip(0, ug_a)
        conv_spec(ug_a, zb_a, 0, 4)
        fwd_h(pb_b, ug_b)
        fence(kv_copies(1))
        conv_start(3)
        w_copy(0).start()
        prep_kv(1, pb_b, False)
        add_skip(1, ug_b)
        fence([h_copy(2)])
        conv_spec(ug_a, zb_a, 4, 8)
        fwd_u(pb_b, ug_b)
        fence(kv_copies(2) + [inv_cp])
        prep_kv(2, pb_a, True)

        def body(p, carry):
            conv_step(2 * p + 1, ug_b, ug_a, zb_b, zb_a, pb_a, pb_b)
            conv_step(2 * p + 2, ug_a, ug_b, zb_a, zb_b, pb_b, pb_a)
            return carry
        lax.fori_loop(0, G // 2 - 1, body, 0)
        w_copy(G - 1).start()
        conv_spec(ug_b, zb_b)
        conv_inv(G - 2, zb_a)
        fence([x_copy(0), w_copy(G - 2), w_copy(G - 1)])
        for p in range(NP):
            ln1_piece(0, p)
        conv_inv(G - 1, zb_b)
        early_keys()

    def phase1():
        def body(c, carry):
            @pl.when(c + 1 < NRC)
            def _():
                x_copy(c + 1).wait()

            @pl.when(c + 2 < NRC)
            def _():
                x_copy(c + 2).start()

            @pl.when(c + 2 == NRC)
            def _():
                wo_copy().start()
            cn = jnp.minimum(c + 1, NRC - 1)
            qkv_proj(_unpack(h_s[...]), c, lambda p: ln1_piece(cn, p), 2, kb_plan((c + G - 1) & (G - 1), KBR), LNS)
            return carry
        lax.fori_loop(0, NRC, body, 0)
        wo_copy().wait()

    def phase2(ms):
        o = load_o(0)
        z0 = z_ref[0]
        for q in range(2):
            rs = [oproj_tile(o, 0, n, z0, None, q * (RC // 2), RC // 2, True) for n in range(8)]
            if q == 0:
                attention_tail(ms, rs[0:5:2])
            for p in range(q * NP // 2, (q + 1) * NP // 2):
                ln2_piece(0, p, z0)
        early_keys()

        def body(c, carry):
            z0 = z_ref[0]
            z1 = z_ref[1]
            h = _unpack(h_s[...])
            o = load_o(c + 1)
            for n in range(8):
                oproj_tile(o, c + 1, n, z1, first=True)
            qkv_proj(h, c, lambda p: ln2_piece(c + 1, p, z0), F2, kb_plan((c + G - 1) & (G - 1), KBR2), LNS2)
            return carry
        lax.fori_loop(0, NRC - 1, body, 0)
        qkv_proj(_unpack(h_s[...]), NRC - 1, None, 0, kb_plan(G - 2, KBR))

    def phase3(ms):
        o = load_o(0)
        attention_tail(ms, [oproj_tile(o, 0, n, z_ref[1]) for n in range(8)])

        def body(c, carry):
            z0 = z_ref[0]
            z1 = z_ref[1]
            zv = zero_vreg()
            o = load_o(c + 1)
            deps = {}
            p = 0
            for t in range(16):
                for _ in range(2 if t < 2 else 1):
                    if p < NP:
                        deps.setdefault(t + 2, []).append(_tok(out_piece(c, p, z0), zv))
                        p += 1
                oproj_tile(o, c + 1, t // 2, z1, deps.get(t), (t % 2) * 128, 128)
            out_copy(c).start()
            return carry
        lax.fori_loop(0, NRC - 2, body, 0)

        c = NRC - 1
        z0 = z_ref[0]
        zv = zero_vreg()
        o = load_o(c)
        deps = {}
        todo = [(c - 1, p) for p in range(NP)]
        for q in range(3):
            for n in range(8):
                t = 8 * q + n
                for cc, p in todo[2 * n:2 * n + 2]:
                    deps.setdefault(t + 2, []).append(_tok(out_piece(cc, p, z0), zv))
                oproj_tile(o, c, n, z0, deps.get(t), TAIL[q], TAIL[q + 1] - TAIL[q])
            (out_copy(c - 1) if q == 0 else tail_copy(q - 1)).start()
            todo = [(c, p) for p in range(TAIL[q] // 16, TAIL[q + 1] // 16)]
        for cc, p in todo:
            out_piece(cc, p, z0)
        tail_copy(2).start()
        wait_all([out_copy(i) for i in range(NRC - 1)] + [tail_copy(q) for q in range(3)])

    zero16 = jnp.zeros((16, 128), u32)

    def after(x, src, never):
        if src is None:
            return x
        src = pltpu.bitcast(src, x.dtype)
        if x.ndim == 3:
            return jnp.where(never[None], src[None], x)
        return jnp.where(never, src, x)

    def qk(g, j, hh, half, dst, z, zk, dep, never):
        qt = qt_s[j, pl.ds(pl.multiple_of(g * 64 + hh * 16, 16), 16), :]
        w = _unpack(jnp.concatenate([qt if i == hh else zero16 for i in range(4)], axis=0))
        r0 = NV if half == 0 else 0
        kh = k_s[g + zk, (half * HS + r0) // 2:(half + 1) * HS // 2, :]
        m = s0 = None
        lo = 0
        for c in range(4):
            ch = CH if half == 1 else JOBS0[c]
            ku = kh[lo // 2:(lo + ch) // 2]
            ku = jnp.concatenate([ku[:ch // 2 - 8], after(ku[ch // 2 - 8:], dep, never)], axis=0)
            s = jnp.dot(_unpack(ku), w, preferred_element_type=f32)
            dst[z, r0 + lo:r0 + lo + ch, :] = s
            mc = jnp.max(s.reshape(ch // 8, 8, 128), axis=0)
            m = mc if m is None else jnp.maximum(m, mc)
            if c == TSRC:
                s0 = s
            lo += ch
        return m, s0

    def kbx(g, col, n):
        k = (col % 64) // 8
        return (ug_a if col < 64 else ug_b).at[0, 4 * g + k // 3, k % 3, pl.ds((col % 8) * NE, n * NE), :]

    def qk_vpu(g, j, hh, i0, acc, trigs, never):
        qw16 = qt_s[j, pl.ds(pl.multiple_of(g * 64 + hh * 16, 16), 16), :]
        for k, tr in enumerate(trigs):
            i = i0 + k
            qw = after(jnp.broadcast_to(qw16[i:i + 1], (8, 128)), tr, never)
            qb = pltpu.bitcast(jnp.stack([qw << 16, qw & jnp.uint32(0xFFFF0000)]), f32)
            d = hh * 32 + 2 * i
            kb = kb_s[g, d:d + 2].reshape(2, 8, 8, 128)
            if NE:
                kb = jnp.concatenate([kb, kbx(g, d, 2)[...].reshape(2, NE // 8, 8, 128)], axis=1)
            t = kb * qb[:, None]
            acc = t[0] + t[1] if acc is None else acc + t[0] + t[1]
        return acc

    def fullmax(m1, m2):
        return jnp.max(jnp.maximum(m1, m2), axis=0, keepdims=True)

    def sm_pv(g, hh, half, src, m, z, dep, trigs, never):
        mb = jnp.broadcast_to(m, (8, 128))
        ms = [after(mb, tr, never) for tr in trigs]
        mm = jnp.stack([jnp.stack([ms[4 * st + 3 - kk] for kk in range(4)]) for st in range(2)])
        x = src[z].reshape(2, 4, 4, 4, 8, 128)
        p = jnp.exp2(x - mm[:, None, :, None]).reshape(HS, 128)
        rs = pl.ds(pl.multiple_of(g * 64 + hh * 16, 16), 16)
        vu = vt_s[half * 8:half * 8 + 8, rs, :]
        vu = jnp.concatenate([after(vu[:, 0:8], dep, never), vu[:, 8:16]], axis=1)
        vu = jnp.concatenate([vu[t] for t in range(8)], axis=1)
        l = _tree_sum(p)
        return jnp.dot(_unpack(vu), p.astype(bf), preferred_element_type=f32), l

    def store_o(g, j, parts):
        outs = [parts[2 * h] * (1.0 / jnp.sum(parts[2 * h + 1], axis=0, keepdims=True)) for h in range(4)]
        o_s[g, pl.ds(pl.multiple_of(j * 64, 64), 64), :] = _pack(jnp.concatenate(outs, axis=0).T)

    bufs = {(0, 0): a1, (0, 1): a2, (1, 0): b1, (1, 1): b2}

    def tile_of(t):
        return lax.shift_right_logical(t, 4), t & (NQ - 1)

    def finish_tile(g, j, done, res):
        if done is None:
            parts = []
        else:
            parts = [done[0:32], done[32:40], done[40:72], done[72:80]]
            res = [(done[80:112], done[112:120])] + res
        for h in range(len(res) // 2):
            parts += [res[2 * h][0] + res[2 * h + 1][0], res[2 * h][1] + res[2 * h + 1][1]]
        store_o(g, j, parts)

    def attention(m_init):
        nit = G * NQ // UNR

        def body(it, carry):
            z1 = z_ref[0]
            z2 = z_ref[1]
            never = zero_vreg() != 0
            g, j0 = tile_of(it * UNR)
            gp, jp = tile_of(jnp.maximum(it * UNR - 1, 0))
            mfull = {(-1, 2): carry[0], (-1, 3): carry[1]}
            mpart = do = ps = po = vacc = None
            res = []

            def tg(sv, i):
                return None if sv is None else sv[i * 8:i * 8 + 8]

            for n in range(8 * UNR):
                u, qh, qhalf = n // 8, (n % 8) // 2, n % 2
                mp, cs = qk(g, j0 + u, qh, qhalf, bufs[(qh % 2, qhalf)], z1, z_ref[2 + n], do, never)
                src = {'p': ps, 'o': po, 'c': cs}
                vtr, etr = [[tg(src[t[0]], int(t[1:])) for t in spec[n >= N0].split('/')[qhalf].split(',')]
                            for spec in (VT, ET)]
                if qhalf == 0:
                    vacc = qk_vpu(g, j0 + u, qh, 0, None, vtr, never)
                    mpart = mp
                else:
                    vacc = qk_vpu(g, j0 + u, qh, 16 - len(vtr), vacc, vtr, never)
                    bufs[(qh % 2, 0)][z1, 0:NV, :] = vacc.reshape(NV, 128)
                    mfull[(u, qh)] = fullmax(jnp.maximum(mpart, jnp.max(vacc, axis=0)), mp)
                pu, ph, phalf = (n - LAG) // 8, ((n - LAG) % 8) // 2, (n - LAG) % 2
                o, l = sm_pv(gp if pu < 0 else g, ph, phalf, bufs[(ph % 2, phalf)], mfull[(pu, ph)], z2,
                             tg(cs, 0), etr, never)
                ps, po, do = cs, o, tg(o, 3)
                res.append((o, l))
                if ph == 3 and phalf == 1:
                    if pu < 0:
                        finish_tile(gp, jp, fin[z2], res)
                    else:
                        finish_tile(g, j0 + pu, None, res)
                    res = []
            fin[z1] = jnp.concatenate([res[0][0] + res[1][0], res[0][1] + res[1][1],
                                       res[2][0] + res[3][0], res[2][1] + res[3][1],
                                       res[4][0], res[4][1]], axis=0)
            return mfull[(UNR - 1, 2)], mfull[(UNR - 1, 3)]

        return lax.fori_loop(0, nit, body, m_init)

    def attention_tail(ms, rs):
        z2 = z_ref[1]
        never = zero_vreg() != 0
        res = []
        for k, (ph, phalf) in enumerate(((2, 1), (3, 0), (3, 1))):
            trigs = [rs[k][16 * i:16 * i + 8] for i in range(8)]
            res.append(sm_pv(G - 1, ph, phalf, bufs[(ph % 2, phalf)], ms[ph - 2], z2, trigs[7], trigs, never))
        finish_tile(G - 1, NQ - 1, fin[z2], res)

    conv()
    phase1()
    ms = attention((jnp.zeros((1, 128), f32), jnp.zeros((1, 128), f32)))
    phase2(ms)
    ms = attention(ms)
    phase3(ms)


@jax.jit
def pallas_interleave_layers__softmax_full_mha__ssm_conv_h3__prompt_kernel(
        A_x, A_wqkv, A_wo, B_q, B_k, B_v, B_shift_k, B_ssm_k, B_ssm_D):
    del B_q
    fwd, inv = _dft_mats()
    scratch = [
        pltpu.VMEM((1, S, D), f32),
        pltpu.VMEM((2, G, S, 128), f32),
        pltpu.VMEM((NQ, D // 2, 128), u32),
        pltpu.VMEM((G, S // 2, 128), u32),
        pltpu.VMEM((NQ, D // 2, 128), u32),
        pltpu.VMEM((G, S // 2, 128), u32),
        pltpu.VMEM((G, 128, 64, 128), f32),
        pltpu.VMEM((1, HS, 128), f32), pltpu.VMEM((1, HS, 128), f32),
        pltpu.VMEM((1, HS, 128), f32), pltpu.VMEM((1, HS, 128), f32),
        pltpu.VMEM((1, 120, 128), f32),
        pltpu.VMEM((1, S + 8, 128), f32),
        pltpu.VMEM((G, 40, 128), f32),
        pltpu.VMEM((1, 2 * NC, 3, IM, 128), f32),
        pltpu.VMEM((1, 2 * NC, 3, IM, 128), f32),
        pltpu.VMEM((NC, 128, 128), u32),
        pltpu.VMEM((NC, 128, 128), u32),
        pltpu.VMEM((S, 128), u32),
        pltpu.VMEM((S, 128), u32),
        pltpu.VMEM((RC // 2, D), u32),
        pltpu.SMEM((NZ,), i32),
        pltpu.VMEM((S, D), bf),
        pltpu.VMEM((D, 3 * D + 128), bf),
        pltpu.VMEM((D, D + 128), bf),
        pltpu.VMEM((NB, S, 128), bf),
        pltpu.VMEM((NB, S, 128), bf),
        pltpu.VMEM((NB, 128, S + 128), bf),
        pltpu.VMEM((4, D), bf),
        pltpu.VMEM((G, 128), bf),
        pltpu.VMEM((320, 128), u32),
        pltpu.VMEM((64, 256), u32),
        pltpu.SemaphoreType.DMA((3, G)),
        pltpu.SemaphoreType.DMA((NRC,)),
        pltpu.SemaphoreType.DMA((G + 1,)),
        pltpu.SemaphoreType.DMA((NRC + 2,)),
        pltpu.SemaphoreType.DMA((4,)),
    ]
    hbm = pl.BlockSpec(memory_space=pl.ANY)
    return pl.pallas_call(
        _kernel,
        out_shape=jax.ShapeDtypeStruct((1, S, D), bf),
        in_specs=[hbm] * 10,
        out_specs=hbm,
        scratch_shapes=scratch,
        compiler_params=pltpu.CompilerParams(vmem_limit_bytes=120 * 2**20, disable_bounds_checks=True),
    )(A_x, A_wqkv, A_wo, B_k, B_v, B_shift_k.T, B_ssm_k, B_ssm_D.reshape(G, 128),
      jnp.asarray(fwd), jnp.asarray(inv))
```

```python
import numpy as np
import jax
import jax.numpy as jnp
from jax import lax
import jax.experimental.pallas as pl
import jax.experimental.pallas.tpu as pltpu

S = 2048
D = 1024
DH = 32
G = 8
NQ = 16
HS = S // 2
CH = HS // 4
UNR = 8
NE = 0
TSRC = 2
JOBS0 = {0: (240, 240, 240, 240), 16: (240, 240, 240, 224)}[NE]
NV = 64 + NE
LAG = 3
RC = 256
NRC = S // RC
NP = RC // 16
NC = 16
NB = 4
IM = 136
GO = 8
EPS = 1e-5
HEAD = (0, 128, 256)
HD = 4
HP = 1
TD = 6
F2 = 1
LNS2 = 13
KBR2 = range(15, 23)
LNS = 12
KBR = range(15, 22)
NZ = 2 + 8 * UNR
QSCALE = float(DH ** -0.5 * np.log2(np.e))
N0 = 12
VT = ('p30,p31,p31,o3,c5,c5,c14,c17/p28,p29,p29,o1,o2,c0,c6,c13',
      'p28,p31,p31,p31,p31,p31,c1,c17/p26,p27,p27,o0,c0,c4,c5,c16')
ET = ('p17,p20,p29,p30,o0,c0,c4,c8/p16,p19,p29,p29,o0,c0,c4,c6',
      'p21,p21,p30,o0,o0,c0,c4,c10/p17,p18,p29,o0,o1,o3,c3,c6')

bf = jnp.bfloat16
f32 = jnp.float32
u32 = jnp.uint32
i32 = jnp.int32
NT = (((1,), (1,)), ((), ()))


def _dft_mats():
    n = np.arange(128)
    f = np.concatenate([np.arange(0, 128, 2), np.arange(1, 128, 2)])
    ang = 2.0 * np.pi * np.outer(f + 0.5, n) / 256.0
    re, im = np.cos(ang), -np.sin(ang)
    inv = np.concatenate([re, im], axis=0).T / 128.0
    fwd = np.concatenate([re, im, re, im - re, im + re], axis=0)

    def pack_rows(a):
        u = np.ascontiguousarray(a, dtype=np.float32).view(np.uint32)
        u = (u + 0x7FFF + ((u >> 16) & 1)) >> 16
        return (u[0::2] | (u[1::2] << 16)).astype(np.uint32)
    return pack_rows(fwd), pack_rows(inv)


def _tree_sum(p):
    n = p.shape[0] // 8
    x = p.reshape(n, 8, 128)
    while n > 1:
        x = x.reshape(n // 2, 2, 8, 128)
        x = x[:, 0] + x[:, 1]
        n //= 2
    return x[0]


def _ln(x):
    m = jnp.mean(x, axis=-1, keepdims=True)
    xc = x - m
    v = jnp.mean(xc * xc, axis=-1, keepdims=True)
    return xc * lax.rsqrt(v + EPS)


def _pack(x):
    return pltpu.bitcast(x.astype(bf), u32)


def _unpack(x):
    return pltpu.bitcast(x, bf)


def _tok(v, zv):
    v = v if v.dtype == u32 else pltpu.bitcast(v, u32)
    while v.shape[1] > 128:
        h = v.shape[1] // 2
        v = v[:, :h] | v[:, h:]
    while v.shape[0] > 8:
        h = v.shape[0] // 2
        v = v[:h] | v[h:]
    return v & zv


def _gate(w, toks):
    if not toks:
        return w
    wu = pltpu.bitcast(w, u32)
    h0 = wu[0:8]
    for t in toks:
        h0 = h0 | t
    return _unpack(jnp.concatenate([h0, wu[8:]], axis=0))


def _kernel(x_hbm, wqkv_hbm, wo_hbm, bk_hbm, bv_hbm, shk_hbm, ssmk_hbm, ssmd_hbm, fwd_hbm, inv_hbm, out_hbm,
            x_s, y_s, qt_s, k_s, vt_s, o_s, kb_s, a1, a2, b1, b2, fin, kf_s, taps_s, ug_a, ug_b, zb_a, zb_b,
            pb_a, pb_b, h_s, z_ref, x_in, wqkv, wo, bk, bv, ssmk, shk, ssmd, fwd_ref, inv_ref,
            sem_c, sem_x, sem_w, sem_o, sem_s):
    out_s = x_in

    def kv_copies(cb):
        cs = pl.ds(pl.multiple_of(cb * 128, 128), 128)
        return [pltpu.make_async_copy(bk_hbm.at[0, :, cs], bk.at[cb % NB], sem_c.at[0, cb]),
                pltpu.make_async_copy(bv_hbm.at[0, :, cs], bv.at[cb % NB], sem_c.at[1, cb])]

    def h_copy(cb):
        cs = pl.ds(pl.multiple_of(cb * 128, 128), 128)
        return pltpu.make_async_copy(ssmk_hbm.at[cs, :], ssmk.at[cb % NB, :, pl.ds(0, S)], sem_c.at[2, cb])

    def x_copy(c):
        rs = pl.ds(pl.multiple_of(c * RC, RC), RC)
        return pltpu.make_async_copy(x_hbm.at[0, rs, :], x_in.at[rs, :], sem_x.at[c])

    def w_copy(c):
        rs = pl.ds(pl.multiple_of(c * 128, 128), 128)
        return pltpu.make_async_copy(wqkv_hbm.at[rs, :], wqkv.at[rs, pl.ds(0, 3 * D)], sem_w.at[c])

    def wo_copy():
        return pltpu.make_async_copy(wo_hbm, wo.at[:, pl.ds(0, D)], sem_w.at[G])

    def out_copy(c):
        rs = pl.ds(pl.multiple_of(c * RC, RC), RC)
        return pltpu.make_async_copy(out_s.at[rs, :], out_hbm.at[0, rs, :], sem_o.at[c])

    TAIL = (0, 128, 192, 256)

    def tail_copy(q):
        rs = pl.ds((NRC - 1) * RC + TAIL[q], TAIL[q + 1] - TAIL[q])
        return pltpu.make_async_copy(out_s.at[rs, :], out_hbm.at[0, rs, :], sem_o.at[NRC - 1 + q])

    def conv_start(c):
        h_copy(c).start()
        for cp in kv_copies(c):
            cp.start()

    def wait_all(cps):
        for cp in cps:
            cp.wait()

    shk_cp, ssmd_cp, fwd_cp, inv_cp = [
        pltpu.make_async_copy(src, dst, sem_s.at[i]) for i, (src, dst) in enumerate(
            ((shk_hbm, shk), (ssmd_hbm, ssmd), (fwd_hbm, fwd_ref), (inv_hbm, inv_ref)))]
    h_copy(0).start()
    fwd_cp.start()
    shk_cp.start()
    ssmd_cp.start()
    for cp in kv_copies(0):
        cp.start()

    for i in range(NZ):
        z_ref[i] = 0
    fin[...] = jnp.ones(fin.shape, f32)
    for buf in (a2, b1, b2):
        buf[...] = jnp.zeros(buf.shape, f32)
    kf_s[0, 0:8, :] = jnp.zeros((8, 128), f32)

    def zero_vreg():
        return jnp.full((8, 128), z_ref[0], i32).astype(u32)

    def fence(cps):
        @pl.when(z_ref[0] == 0)
        def _():
            wait_all(cps)

    TILES = [(0, n) for n in range(8)] + [(2, n) for n in range(8)] + [(1, n) for n in range(8)]

    def qkv_tile(h, c, idx, toks, zv):
        kind, n = TILES[idx]
        col = kind * D + n * 128
        r = jnp.dot(h, _gate(wqkv[:, col:col + 128], toks), preferred_element_type=f32)
        if kind == 1:
            k_s[n, pl.ds(pl.multiple_of(c * (RC // 2), RC // 2), RC // 2), :] = _pack(r)
            return None
        dst = qt_s if kind == 0 else vt_s
        if kind == 0:
            r = r * QSCALE
        pks = []
        for t in range(RC // 128):
            pk = _pack(r[t * 128:(t + 1) * 128, :].T)
            dst[c * (RC // 128) + t, n * 64:(n + 1) * 64, :] = pk
            pks.append(pk)
        return _tok(jnp.concatenate(pks, axis=0), zv)

    def qkv_proj(h, c, piece_fn, first_piece, kb_jobs, span=NP):
        zv = zero_vreg()
        deps = {}
        for n in range(24):
            done = qkv_tile(h, c, n, deps.get(n), zv)
            if done is not None:
                deps.setdefault(n + 3, []).append(done)
            if n in kb_jobs:
                deps.setdefault(n + 2, []).append(kb_piece(*kb_jobs[n], zv))
            if piece_fn is not None:
                for p in range(NP):
                    if first_piece + p * span // NP == n:
                        deps.setdefault(n + 3, []).append(_tok(piece_fn(p), zv))

    def kb_plan(g, tiles):
        return {t: (g, 128 * i // len(tiles), 128 * (i + 1) // len(tiles)) for i, t in enumerate(tiles)}

    def kb_piece(g, lo, hi, zv):
        kx = _unpack(k_s[g, 0:NV // 2, :]).astype(f32)
        for d in range(lo, hi):
            v = jnp.broadcast_to(kx[:, d:d + 1], (NV, 128))
            kb_s[g, d] = v[0:64]
            if NE:
                kbx(g, d, 1)[...] = v[64:NV]
        return _tok(v[NV - 32:], zv)

    def early_keys():
        col = D + (G - 1) * 128
        k_s[G - 1, 0:NV // 2, :] = _pack(jnp.dot(_unpack(h_s[0:NV // 2, :]), wqkv[:, col:col + 128],
                                                 preferred_element_type=f32))

    def piece_rows(c, p):
        return pl.ds(pl.multiple_of(c * RC + p * 16, 16), 16)

    def ln1_piece(c, p):
        hp = _pack(_ln(x_in[piece_rows(c, p), :].astype(f32)))
        h_s[p * 8:(p + 1) * 8, :] = hp
        return hp

    def gated_x(c, p, z):
        rows = piece_rows(c, p)
        x1 = x_s[z, rows, :]
        y = jnp.concatenate([y_s[0, g, rows, :] + y_s[1, g, rows, :] for g in range(G)], axis=1)
        return x1 + _ln(x1) * y

    def ln2_piece(c, p, z):
        x2 = gated_x(c, p, z)
        x_s[z, piece_rows(c, p), :] = x2
        hp = _pack(_ln(x2))
        h_s[p * 8:(p + 1) * 8, :] = hp
        return hp

    def out_piece(c, p, z):
        v = gated_x(c, p, z)
        out_s[piece_rows(c, p), :] = v.astype(bf)
        return v

    def load_o(c):
        rs = pl.ds(pl.multiple_of(c * (RC // 2), RC // 2), RC // 2)
        return jnp.concatenate([_unpack(o_s[g, rs, :]) for g in range(G)], axis=1)

    def oproj_tile(o, c, n, z, toks=None, r0=0, nr=RC, first=False):
        rows = pl.ds(pl.multiple_of(c * RC + r0, 64), nr)
        cols = slice(n * 128, (n + 1) * 128)
        r = jnp.dot(o[r0:r0 + nr], _gate(wo[:, cols], toks), preferred_element_type=f32)
        x0 = x_in[rows, cols].astype(f32) if first else x_s[z, rows, cols]
        x_s[z, rows, cols] = x0 + r
        return r

    zts = [z_ref[2 + ib] for ib in range(4)]

    def setup_taps():
        taps = shk[...].astype(f32)
        for cb in range(G):
            for t in range(4):
                taps_s[cb, 8 * t:8 * t + 8, :] = jnp.broadcast_to(taps[t:t + 1, cb * 128:(cb + 1) * 128], (8, 128))

    def setup_skip():
        dall = ssmd[...].astype(f32)
        for cb in range(G):
            taps_s[cb, 32:40, :] = jnp.broadcast_to(dall[cb:cb + 1, :], (8, 128))

    def prep_h_chunk(cb, pb, j):
        pb[HS + j * 64:HS + (j + 1) * 64, :] = pltpu.bitcast(ssmk[cb % NB, :, j * 128:(j + 1) * 128], u32)

    def prep_h(cb, pb):
        for j in range(NC):
            prep_h_chunk(cb, pb, j)

    def prep_kv(cb, pb, with_h):
        zs = z_ref[1]
        tp = taps_s[cb, 0:32, :]
        for j in range(NC):
            r0 = j * 128
            if with_h:
                prep_h_chunk(cb, pb, j)
            kf_s[zs, 8 + r0:8 + r0 + 128, :] = bk[cb % NB, r0:r0 + 128, :].astype(f32)
            ks = None
            for t in range(4):
                term = kf_s[zs, 8 + r0 - t:8 + r0 - t + 128, :].reshape(16, 8, 128) * tp[8 * t:8 * t + 8][None]
                ks = term if ks is None else ks + term
            pb[j * 64:(j + 1) * 64, :] = _pack(ks.reshape(128, 128) * bv[cb % NB, r0:r0 + 128, :].astype(f32))

    def fwd_h(pb, ug):
        for m in range(NC):
            hm = lax.dot_general(_unpack(fwd_ref[128:320, :]), _unpack(pb[HS + m * 64:HS + (m + 1) * 64, :]),
                                 NT, preferred_element_type=f32)
            ug[0, NC + m, :, GO:GO + 128, :] = hm.reshape(3, 128, 128)

    def fwd_u(pb, ug):
        for j in range(NC):
            u = jnp.dot(_unpack(fwd_ref[0:128, :]), _unpack(pb[j * 64:(j + 1) * 64, :]),
                        preferred_element_type=f32)
            ug[0, j, 0:2, 0:128, :] = u.reshape(2, 128, 128)

    def add_skip(cb, ug):
        dv = taps_s[cb, 32:40, :][None]
        for e in range(3):
            v = ug[0, NC, e, GO:GO + 128, :].reshape(16, 8, 128)
            ug[0, NC, e, GO:GO + 128, :] = (v - dv if e == 1 else v + dv).reshape(128, 128)

    def spec_item(ug, ib, r):
        zt = zts[ib]
        acc = None
        for j in range(4 * ib + 4):
            u = ug[zt, j:j + 1, 0:2, r:r + 8, :]
            u = jnp.concatenate([u[:, 0:1] + u[:, 1:2], u], axis=1)
            q0 = max(0, j - 4 * ib)
            m0 = NC + 4 * ib - j
            t = ug[zt, m0 + q0:m0 + 4, :, GO + r:GO + r + 8, :] * u
            if acc is None:
                acc = t
            elif q0 == 0:
                acc = acc + t
            else:
                acc = jnp.concatenate([acc[:q0], acc[q0:] + t], axis=0)
        return acc[:, 0] - acc[:, 2], acc[:, 0] + acc[:, 1]

    def overlap_add(yr, yi, prev, r):
        n = 1 if prev is None else 0
        pr = yr[:3] if prev is None else jnp.concatenate([prev[0], yr[:3]], axis=0)
        pi = yi[:3] if prev is None else jnp.concatenate([prev[1], yi[:3]], axis=0)
        if r < 64:
            zr, zi = yr[n:] - pi, yi[n:] + pr
        else:
            zr, zi = yr[n:] + pi, yi[n:] - pr
        if prev is None:
            zr = jnp.concatenate([yr[:1], zr], axis=0)
            zi = jnp.concatenate([yi[:1], zi], axis=0)
        return zr, zi, (yr[3:], yi[3:])

    def conv_spec(ug, zb, lo=0, hi=8):
        for rp in range(lo, hi):
            p0 = p1 = None
            for ib in range(4):
                zr0, zi0, p0 = overlap_add(*spec_item(ug, ib, 16 * rp), p0, 16 * rp)
                zr1, zi1, p1 = overlap_add(*spec_item(ug, ib, 16 * rp + 8), p1, 16 * rp)
                zb[4 * ib:4 * ib + 4, rp * 8:rp * 8 + 8, :] = _pack(jnp.concatenate([zr0, zr1], axis=1))
                zb[4 * ib:4 * ib + 4, 64 + rp * 8:72 + rp * 8, :] = _pack(jnp.concatenate([zi0, zi1], axis=1))

    def conv_inv(cb, zb):
        for i in range(NC):
            for e in range(2):
                y_s[e, cb, i * 128:(i + 1) * 128, :] = jnp.dot(
                    _unpack(inv_ref[:, e * 128:(e + 1) * 128]), _unpack(zb[i, e * 64:(e + 1) * 64, :]),
                    preferred_element_type=f32)

    def conv_step(c, ug_cur, ug_nxt, zb_cur, zb_prev, pb_nxt, pb_new):
        @pl.when(c + 3 < G)
        def _():
            conv_start(c + 3)
        w_copy(c).start()

        @pl.when(c >= G - 3)
        def _():
            x_copy(c - (G - 3)).start()
        conv_spec(ug_cur, zb_cur)
        fwd_h(pb_nxt, ug_nxt)
        fwd_u(pb_nxt, ug_nxt)
        conv_inv(c - 1, zb_prev)

        @pl.when(c + 2 < G)
        def _():
            wait_all([w_copy(c - 1), h_copy(c + 2)] + kv_copies(c + 2))
            prep_kv(c + 2, pb_new, True)
            add_skip(c + 1, ug_nxt)

        @pl.when(c + 2 >= G)
        def _():
            w_copy(c - 1).wait()
            add_skip(c + 1, ug_nxt)

    def conv():
        wait_all([fwd_cp, h_copy(0)])
        conv_start(1)
        inv_cp.start()
        prep_h(0, pb_a)
        fwd_h(pb_a, ug_a)
        wait_all([shk_cp] + kv_copies(0))
        conv_start(2)
        setup_taps()
        prep_kv(0, pb_a, False)
        fwd_u(pb_a, ug_a)
        fence([h_copy(1)])
        prep_h(1, pb_b)
        fence([ssmd_cp])
        setup_skip()
        add_skip(0, ug_a)
        conv_spec(ug_a, zb_a, 0, 4)
        fwd_h(pb_b, ug_b)
        fence(kv_copies(1))
        conv_start(3)
        w_copy(0).start()
        prep_kv(1, pb_b, False)
        add_skip(1, ug_b)
        fence([h_copy(2)])
        conv_spec(ug_a, zb_a, 4, 8)
        fwd_u(pb_b, ug_b)
        fence(kv_copies(2) + [inv_cp])
        prep_kv(2, pb_a, True)

        def body(p, carry):
            conv_step(2 * p + 1, ug_b, ug_a, zb_b, zb_a, pb_a, pb_b)
            conv_step(2 * p + 2, ug_a, ug_b, zb_a, zb_b, pb_b, pb_a)
            return carry
        lax.fori_loop(0, G // 2 - 1, body, 0)
        w_copy(G - 1).start()
        conv_spec(ug_b, zb_b)
        conv_inv(G - 2, zb_a)
        fence([x_copy(0), w_copy(G - 2), w_copy(G - 1)])
        for p in range(NP):
            ln1_piece(0, p)
        conv_inv(G - 1, zb_b)
        early_keys()

    def phase1():
        def body(c, carry):
            @pl.when(c + 1 < NRC)
            def _():
                x_copy(c + 1).wait()

            @pl.when(c + 2 < NRC)
            def _():
                x_copy(c + 2).start()

            @pl.when(c + 2 == NRC)
            def _():
                wo_copy().start()
            cn = jnp.minimum(c + 1, NRC - 1)
            qkv_proj(_unpack(h_s[...]), c, lambda p: ln1_piece(cn, p), 2, kb_plan((c + G - 1) & (G - 1), KBR), LNS)
            return carry
        lax.fori_loop(0, NRC, body, 0)
        wo_copy().wait()

    def phase2(ms):
        o = load_o(0)
        z0 = z_ref[0]
        zv = zero_vreg()
        deps = {}
        todo = []
        for q in range(len(HEAD) - 1):
            rs = []
            for n in range(8):
                t = 8 * q + n
                for p in todo[HP * n:HP * n + HP]:
                    deps.setdefault(t + HD, []).append(_tok(ln2_piece(0, p, z0), zv))
                rs.append(oproj_tile(o, 0, n, z0, deps.get(t), HEAD[q], HEAD[q + 1] - HEAD[q], True))
            if q == 0:
                deps.setdefault(11, []).append(attention_tail(ms, rs[0:5:2]))
            todo = list(range(HEAD[q] // 16, HEAD[q + 1] // 16))
        for p in todo:
            ln2_piece(0, p, z0)
        early_keys()

        def body(c, carry):
            z0 = z_ref[0]
            z1 = z_ref[1]
            h = _unpack(h_s[...])
            o = load_o(c + 1)
            for n in range(8):
                oproj_tile(o, c + 1, n, z1, first=True)
            qkv_proj(h, c, lambda p: ln2_piece(c + 1, p, z0), F2, kb_plan((c + G - 1) & (G - 1), KBR2), LNS2)
            return carry
        lax.fori_loop(0, NRC - 1, body, 0)
        qkv_proj(_unpack(h_s[...]), NRC - 1, None, 0, kb_plan(G - 2, KBR))

    def phase3(ms):
        o = load_o(0)
        done = attention_tail(ms, [oproj_tile(o, 0, n, z_ref[1]) for n in range(3)])
        for n in range(3, 8):
            oproj_tile(o, 0, n, z_ref[1], [done] if n == 6 else None)

        def body(c, carry):
            z0 = z_ref[0]
            z1 = z_ref[1]
            zv = zero_vreg()
            o = load_o(c + 1)
            deps = {}
            p = 0
            for t in range(16):
                for _ in range(2 if t < 2 else 1):
                    if p < NP:
                        deps.setdefault(t + 2, []).append(_tok(out_piece(c, p, z0), zv))
                        p += 1
                oproj_tile(o, c + 1, t // 2, z1, deps.get(t), (t % 2) * 128, 128)
            out_copy(c).start()
            return carry
        lax.fori_loop(0, NRC - 2, body, 0)

        c = NRC - 1
        z0 = z_ref[0]
        zv = zero_vreg()
        o = load_o(c)
        deps = {}
        todo = [(c - 1, p) for p in range(NP)]
        for q in range(3):
            for n in range(8):
                t = 8 * q + n
                for cc, p in todo[2 * n:2 * n + 2]:
                    deps.setdefault(t + (2 if q == 0 else TD), []).append(_tok(out_piece(cc, p, z0), zv))
                oproj_tile(o, c, n, z0, deps.get(t), TAIL[q], TAIL[q + 1] - TAIL[q])
            if q == 1:
                out_copy(c - 1).start()
            if q > 0:
                tail_copy(q - 1).start()
            todo = [(c, p) for p in range(TAIL[q] // 16, TAIL[q + 1] // 16)]
        for cc, p in todo:
            out_piece(cc, p, z0)
        tail_copy(2).start()
        wait_all([out_copy(i) for i in range(NRC - 1)] + [tail_copy(q) for q in range(3)])

    zero16 = jnp.zeros((16, 128), u32)

    def after(x, src, never):
        if src is None:
            return x
        src = pltpu.bitcast(src, x.dtype)
        if x.ndim == 3:
            return jnp.where(never[None], src[None], x)
        return jnp.where(never, src, x)

    def qk(g, j, hh, half, dst, z, zk, dep, never):
        qt = qt_s[j, pl.ds(pl.multiple_of(g * 64 + hh * 16, 16), 16), :]
        w = _unpack(jnp.concatenate([qt if i == hh else zero16 for i in range(4)], axis=0))
        r0 = NV if half == 0 else 0
        kh = k_s[g + zk, (half * HS + r0) // 2:(half + 1) * HS // 2, :]
        m = s0 = None
        lo = 0
        for c in range(4):
            ch = CH if half == 1 else JOBS0[c]
            ku = kh[lo // 2:(lo + ch) // 2]
            ku = jnp.concatenate([ku[:ch // 2 - 8], after(ku[ch // 2 - 8:], dep, never)], axis=0)
            s = jnp.dot(_unpack(ku), w, preferred_element_type=f32)
            dst[z, r0 + lo:r0 + lo + ch, :] = s
            mc = jnp.max(s.reshape(ch // 8, 8, 128), axis=0)
            m = mc if m is None else jnp.maximum(m, mc)
            if c == TSRC:
                s0 = s
            lo += ch
        return m, s0

    def kbx(g, col, n):
        k = (col % 64) // 8
        return (ug_a if col < 64 else ug_b).at[0, 4 * g + k // 3, k % 3, pl.ds((col % 8) * NE, n * NE), :]

    def qk_vpu(g, j, hh, i0, acc, trigs, never):
        qw16 = qt_s[j, pl.ds(pl.multiple_of(g * 64 + hh * 16, 16), 16), :]
        for k, tr in enumerate(trigs):
            i = i0 + k
            qw = after(jnp.broadcast_to(qw16[i:i + 1], (8, 128)), tr, never)
            qb = pltpu.bitcast(jnp.stack([qw << 16, qw & jnp.uint32(0xFFFF0000)]), f32)
            d = hh * 32 + 2 * i
            kb = kb_s[g, d:d + 2].reshape(2, 8, 8, 128)
            if NE:
                kb = jnp.concatenate([kb, kbx(g, d, 2)[...].reshape(2, NE // 8, 8, 128)], axis=1)
            t = kb * qb[:, None]
            acc = t[0] + t[1] if acc is None else acc + t[0] + t[1]
        return acc

    def fullmax(m1, m2):
        return jnp.max(jnp.maximum(m1, m2), axis=0, keepdims=True)

    def sm_pv(g, hh, half, src, m, z, dep, trigs, never):
        mb = jnp.broadcast_to(m, (8, 128))
        ms = [after(mb, tr, never) for tr in trigs]
        mm = jnp.stack([jnp.stack([ms[4 * st + 3 - kk] for kk in range(4)]) for st in range(2)])
        x = src[z].reshape(2, 4, 4, 4, 8, 128)
        p = jnp.exp2(x - mm[:, None, :, None]).reshape(HS, 128)
        rs = pl.ds(pl.multiple_of(g * 64 + hh * 16, 16), 16)
        vu = vt_s[half * 8:half * 8 + 8, rs, :]
        vu = jnp.concatenate([after(vu[:, 0:8], dep, never), vu[:, 8:16]], axis=1)
        vu = jnp.concatenate([vu[t] for t in range(8)], axis=1)
        l = _tree_sum(p)
        return jnp.dot(_unpack(vu), p.astype(bf), preferred_element_type=f32), l

    def store_o(g, j, parts):
        outs = [parts[2 * h] * (1.0 / jnp.sum(parts[2 * h + 1], axis=0, keepdims=True)) for h in range(4)]
        ot = _pack(jnp.concatenate(outs, axis=0).T)
        o_s[g, pl.ds(pl.multiple_of(j * 64, 64), 64), :] = ot
        return ot

    bufs = {(0, 0): a1, (0, 1): a2, (1, 0): b1, (1, 1): b2}

    def tile_of(t):
        return lax.shift_right_logical(t, 4), t & (NQ - 1)

    def finish_tile(g, j, done, res):
        if done is None:
            parts = []
        else:
            parts = [done[0:32], done[32:40], done[40:72], done[72:80]]
            res = [(done[80:112], done[112:120])] + res
        for h in range(len(res) // 2):
            parts += [res[2 * h][0] + res[2 * h + 1][0], res[2 * h][1] + res[2 * h + 1][1]]
        return store_o(g, j, parts)

    def attention(m_init):
        nit = G * NQ // UNR

        def body(it, carry):
            z1 = z_ref[0]
            z2 = z_ref[1]
            never = zero_vreg() != 0
            g, j0 = tile_of(it * UNR)
            gp, jp = tile_of(jnp.maximum(it * UNR - 1, 0))
            mfull = {(-1, 2): carry[0], (-1, 3): carry[1]}
            mpart = do = ps = po = vacc = None
            res = []

            def tg(sv, i):
                return None if sv is None else sv[i * 8:i * 8 + 8]

            for n in range(8 * UNR):
                u, qh, qhalf = n // 8, (n % 8) // 2, n % 2
                mp, cs = qk(g, j0 + u, qh, qhalf, bufs[(qh % 2, qhalf)], z1, z_ref[2 + n], do, never)
                src = {'p': ps, 'o': po, 'c': cs}
                vtr, etr = [[tg(src[t[0]], int(t[1:])) for t in spec[n >= N0].split('/')[qhalf].split(',')]
                            for spec in (VT, ET)]
                if qhalf == 0:
                    vacc = qk_vpu(g, j0 + u, qh, 0, None, vtr, never)
                    mpart = mp
                else:
                    vacc = qk_vpu(g, j0 + u, qh, 16 - len(vtr), vacc, vtr, never)
                    bufs[(qh % 2, 0)][z1, 0:NV, :] = vacc.reshape(NV, 128)
                    mfull[(u, qh)] = fullmax(jnp.maximum(mpart, jnp.max(vacc, axis=0)), mp)
                pu, ph, phalf = (n - LAG) // 8, ((n - LAG) % 8) // 2, (n - LAG) % 2
                o, l = sm_pv(gp if pu < 0 else g, ph, phalf, bufs[(ph % 2, phalf)], mfull[(pu, ph)], z2,
                             tg(cs, 0), etr, never)
                ps, po, do = cs, o, tg(o, 3)
                res.append((o, l))
                if ph == 3 and phalf == 1:
                    if pu < 0:
                        finish_tile(gp, jp, fin[z2], res)
                    else:
                        finish_tile(g, j0 + pu, None, res)
                    res = []
            fin[z1] = jnp.concatenate([res[0][0] + res[1][0], res[0][1] + res[1][1],
                                       res[2][0] + res[3][0], res[2][1] + res[3][1],
                                       res[4][0], res[4][1]], axis=0)
            return mfull[(UNR - 1, 2)], mfull[(UNR - 1, 3)]

        return lax.fori_loop(0, nit, body, m_init)

    def attention_tail(ms, rs):
        z2 = z_ref[1]
        never = zero_vreg() != 0
        res = []
        for k, (ph, phalf) in enumerate(((2, 1), (3, 0), (3, 1))):
            trigs = [rs[k][16 * i:16 * i + 8] for i in range(8)]
            res.append(sm_pv(G - 1, ph, phalf, bufs[(ph % 2, phalf)], ms[ph - 2], z2, trigs[7], trigs, never))
        return _tok(finish_tile(G - 1, NQ - 1, fin[z2], res), zero_vreg())

    conv()
    phase1()
    ms = attention((jnp.zeros((1, 128), f32), jnp.zeros((1, 128), f32)))
    phase2(ms)
    ms = attention(ms)
    phase3(ms)


@jax.jit
def pallas_interleave_layers__softmax_full_mha__ssm_conv_h3__prompt_kernel(
        A_x, A_wqkv, A_wo, B_q, B_k, B_v, B_shift_k, B_ssm_k, B_ssm_D):
    del B_q
    fwd, inv = _dft_mats()
    scratch = [
        pltpu.VMEM((1, S, D), f32),
        pltpu.VMEM((2, G, S, 128), f32),
        pltpu.VMEM((NQ, D // 2, 128), u32),
        pltpu.VMEM((G, S // 2, 128), u32),
        pltpu.VMEM((NQ, D // 2, 128), u32),
        pltpu.VMEM((G, S // 2, 128), u32),
        pltpu.VMEM((G, 128, 64, 128), f32),
        pltpu.VMEM((1, HS, 128), f32), pltpu.VMEM((1, HS, 128), f32),
        pltpu.VMEM((1, HS, 128), f32), pltpu.VMEM((1, HS, 128), f32),
        pltpu.VMEM((1, 120, 128), f32),
        pltpu.VMEM((1, S + 8, 128), f32),
        pltpu.VMEM((G, 40, 128), f32),
        pltpu.VMEM((1, 2 * NC, 3, IM, 128), f32),
        pltpu.VMEM((1, 2 * NC, 3, IM, 128), f32),
        pltpu.VMEM((NC, 128, 128), u32),
        pltpu.VMEM((NC, 128, 128), u32),
        pltpu.VMEM((S, 128), u32),
        pltpu.VMEM((S, 128), u32),
        pltpu.VMEM((RC // 2, D), u32),
        pltpu.SMEM((NZ,), i32),
        pltpu.VMEM((S, D), bf),
        pltpu.VMEM((D, 3 * D + 128), bf),
        pltpu.VMEM((D, D + 128), bf),
        pltpu.VMEM((NB, S, 128), bf),
        pltpu.VMEM((NB, S, 128), bf),
        pltpu.VMEM((NB, 128, S + 128), bf),
        pltpu.VMEM((4, D), bf),
        pltpu.VMEM((G, 128), bf),
        pltpu.VMEM((320, 128), u32),
        pltpu.VMEM((64, 256), u32),
        pltpu.SemaphoreType.DMA((3, G)),
        pltpu.SemaphoreType.DMA((NRC,)),
        pltpu.SemaphoreType.DMA((G + 1,)),
        pltpu.SemaphoreType.DMA((NRC + 2,)),
        pltpu.SemaphoreType.DMA((4,)),
    ]
    hbm = pl.BlockSpec(memory_space=pl.ANY)
    return pl.pallas_call(
        _kernel,
        out_shape=jax.ShapeDtypeStruct((1, S, D), bf),
        in_specs=[hbm] * 10,
        out_specs=hbm,
        scratch_shapes=scratch,
        compiler_params=pltpu.CompilerParams(vmem_limit_bytes=120 * 2**20, disable_bounds_checks=True),
    )(A_x, A_wqkv, A_wo, B_k, B_v, B_shift_k.T, B_ssm_k, B_ssm_D.reshape(G, 128),
      jnp.asarray(fwd), jnp.asarray(inv))
```

```python
import numpy as np
import jax
import jax.numpy as jnp
from jax import lax
import jax.experimental.pallas as pl
import jax.experimental.pallas.tpu as pltpu

S = 2048
D = 1024
DH = 32
G = 8
NQ = 16
HS = S // 2
UNR = 8
NV = 64
LAG = 3
RC = 256
NRC = S // RC
NP = RC // 16
NC = 16
NB = 4
IM = 136
GO = 8
EPS = 1e-5
NZ = 2 + 8 * UNR
QSCALE = float(DH ** -0.5 * np.log2(np.e))
N0 = 12
VT = ('p30,p31,p31,o3,c5,c5,c14,c17/p28,p29,p29,o1,o2,c0,c6,c13',
      'p28,p31,p31,p31,p31,p31,c1,c17/p26,p27,p27,o0,c0,c4,c5,c16')
ET = ('p17,p20,p29,p30,o0,c0,c4,c8/p16,p19,p29,p29,o0,c0,c4,c6',
      'p21,p21,p30,o0,o0,c0,c4,c10/p17,p18,p29,o0,o1,o3,c3,c6')

bf = jnp.bfloat16
f32 = jnp.float32
u32 = jnp.uint32
i32 = jnp.int32
NT = (((1,), (1,)), ((), ()))


def _dft_mats():
    n = np.arange(128)
    f = np.concatenate([np.arange(0, 128, 2), np.arange(1, 128, 2)])
    ang = 2.0 * np.pi * np.outer(f + 0.5, n) / 256.0
    re, im = np.cos(ang), -np.sin(ang)
    inv = np.concatenate([re, im], axis=0).T / 128.0
    fwd = np.concatenate([re, im, re, im - re, im + re], axis=0)

    def pack_rows(a):
        u = np.ascontiguousarray(a, dtype=np.float32).view(np.uint32)
        u = (u + 0x7FFF + ((u >> 16) & 1)) >> 16
        return (u[0::2] | (u[1::2] << 16)).astype(np.uint32)
    return pack_rows(fwd), pack_rows(inv)


def _tree_sum(p):
    n = p.shape[0] // 8
    x = p.reshape(n, 8, 128)
    while n > 1:
        x = x.reshape(n // 2, 2, 8, 128)
        x = x[:, 0] + x[:, 1]
        n //= 2
    return x[0]


def _ln(x):
    m = jnp.mean(x, axis=-1, keepdims=True)
    xc = x - m
    v = jnp.mean(xc * xc, axis=-1, keepdims=True)
    return xc * lax.rsqrt(v + EPS)


def _pack(x):
    return pltpu.bitcast(x.astype(bf), u32)


def _unpack(x):
    return pltpu.bitcast(x, bf)


def _tok(v, zv):
    v = v if v.dtype == u32 else pltpu.bitcast(v, u32)
    while v.shape[1] > 128:
        h = v.shape[1] // 2
        v = v[:, :h] | v[:, h:]
    while v.shape[0] > 8:
        h = v.shape[0] // 2
        v = v[:h] | v[h:]
    return v & zv


def _gate(w, toks):
    if not toks:
        return w
    wu = pltpu.bitcast(w, u32)
    h0 = wu[0:8]
    for t in toks:
        h0 = h0 | t
    return _unpack(jnp.concatenate([h0, wu[8:]], axis=0))


def _kernel(x_hbm, wqkv_hbm, wo_hbm, bk_hbm, bv_hbm, shk_hbm, ssmk_hbm, ssmd_hbm, fwd_hbm, inv_hbm, out_hbm,
            x_s, y_s, qt_s, k_s, vt_s, o_s, kb_s, a1, a2, b1, b2, fin, kf_s, taps_s, ug_a, ug_b, zb_a, zb_b,
            pb_a, pb_b, h_s, z_ref, x_in, wqkv, wo, bk, bv, ssmk, shk, ssmd, fwd_ref, inv_ref,
            sem_c, sem_x, sem_w, sem_o, sem_s):
    out_s = x_in

    def kv_copies(cb):
        cs = pl.ds(pl.multiple_of(cb * 128, 128), 128)
        return [pltpu.make_async_copy(bk_hbm.at[0, :, cs], bk.at[cb % NB], sem_c.at[0, cb]),
                pltpu.make_async_copy(bv_hbm.at[0, :, cs], bv.at[cb % NB], sem_c.at[1, cb])]

    def h_copy(cb):
        cs = pl.ds(pl.multiple_of(cb * 128, 128), 128)
        return pltpu.make_async_copy(ssmk_hbm.at[cs, :], ssmk.at[cb % NB, :, pl.ds(0, S)], sem_c.at[2, cb])

    def x_copy(c):
        rs = pl.ds(pl.multiple_of(c * RC, RC), RC)
        return pltpu.make_async_copy(x_hbm.at[0, rs, :], x_in.at[rs, :], sem_x.at[c])

    def w_copy(c):
        rs = pl.ds(pl.multiple_of(c * 128, 128), 128)
        return pltpu.make_async_copy(wqkv_hbm.at[rs, :], wqkv.at[rs, pl.ds(0, 3 * D)], sem_w.at[c])

    def wo_copy():
        return pltpu.make_async_copy(wo_hbm, wo.at[:, pl.ds(0, D)], sem_w.at[G])

    def out_copy(c):
        rs = pl.ds(pl.multiple_of(c * RC, RC), RC)
        return pltpu.make_async_copy(out_s.at[rs, :], out_hbm.at[0, rs, :], sem_o.at[c])

    TAIL = (0, 128, 192, 256)

    def tail_copy(q):
        rs = pl.ds((NRC - 1) * RC + TAIL[q], TAIL[q + 1] - TAIL[q])
        return pltpu.make_async_copy(out_s.at[rs, :], out_hbm.at[0, rs, :], sem_o.at[NRC - 1 + q])

    def conv_start(c):
        h_copy(c).start()
        for cp in kv_copies(c):
            cp.start()

    def wait_all(cps):
        for cp in cps:
            cp.wait()

    shk_cp, ssmd_cp, fwd_cp, inv_cp = [
        pltpu.make_async_copy(src, dst, sem_s.at[i]) for i, (src, dst) in enumerate(
            ((shk_hbm, shk), (ssmd_hbm, ssmd), (fwd_hbm, fwd_ref), (inv_hbm, inv_ref)))]
    h_copy(0).start()
    fwd_cp.start()
    shk_cp.start()
    ssmd_cp.start()
    for cp in kv_copies(0):
        cp.start()

    for i in range(NZ):
        z_ref[i] = 0
    fin[...] = jnp.ones(fin.shape, f32)
    for buf in (a2, b1, b2):
        buf[...] = jnp.zeros(buf.shape, f32)
    kf_s[0, 0:8, :] = jnp.zeros((8, 128), f32)

    def zero_vreg():
        return jnp.full((8, 128), z_ref[0], i32).astype(u32)

    def fence(cps):
        @pl.when(z_ref[0] == 0)
        def _():
            wait_all(cps)

    TILES = [(0, n) for n in range(8)] + [(2, n) for n in range(8)] + [(1, n) for n in range(8)]

    def qkv_tile(h, c, idx, toks, zv):
        kind, n = TILES[idx]
        col = kind * D + n * 128
        r = jnp.dot(h, _gate(wqkv[:, col:col + 128], toks), preferred_element_type=f32)
        if kind == 1:
            k_s[n, pl.ds(pl.multiple_of(c * (RC // 2), RC // 2), RC // 2), :] = _pack(r)
            return None
        dst = qt_s if kind == 0 else vt_s
        if kind == 0:
            r = r * QSCALE
        pks = []
        for t in range(RC // 128):
            pk = _pack(r[t * 128:(t + 1) * 128, :].T)
            dst[c * (RC // 128) + t, n * 64:(n + 1) * 64, :] = pk
            pks.append(pk)
        return _tok(jnp.concatenate(pks, axis=0), zv)

    def qkv_proj(h, c, piece_fn, first_piece, kb_jobs, span=NP):
        zv = zero_vreg()
        deps = {}
        for n in range(24):
            done = qkv_tile(h, c, n, deps.get(n), zv)
            if done is not None:
                deps.setdefault(n + 3, []).append(done)
            if n in kb_jobs:
                deps.setdefault(n + 2, []).append(kb_piece(*kb_jobs[n], zv))
            if piece_fn is not None:
                for p in range(NP):
                    if first_piece + p * span // NP == n:
                        deps.setdefault(n + 3, []).append(_tok(piece_fn(p), zv))

    def kb_plan(g, tiles):
        return {t: (g, 128 * i // len(tiles), 128 * (i + 1) // len(tiles)) for i, t in enumerate(tiles)}

    def kb_piece(g, lo, hi, zv):
        kx = _unpack(k_s[g, 0:NV // 2, :]).astype(f32)
        for d in range(lo, hi):
            v = jnp.broadcast_to(kx[:, d:d + 1], (NV, 128))
            kb_s[g, d] = v
        return _tok(v[NV - 32:], zv)

    def early_keys():
        col = D + (G - 1) * 128
        k_s[G - 1, 0:NV // 2, :] = _pack(jnp.dot(_unpack(h_s[0:NV // 2, :]), wqkv[:, col:col + 128],
                                                 preferred_element_type=f32))

    def piece_rows(c, p):
        return pl.ds(pl.multiple_of(c * RC + p * 16, 16), 16)

    def ln1_piece(c, p):
        hp = _pack(_ln(x_in[piece_rows(c, p), :].astype(f32)))
        h_s[p * 8:(p + 1) * 8, :] = hp
        return hp

    def gated_x(c, p, z):
        rows = piece_rows(c, p)
        x1 = x_s[z, rows, :]
        y = jnp.concatenate([y_s[0, g, rows, :] + y_s[1, g, rows, :] for g in range(G)], axis=1)
        return x1 + _ln(x1) * y

    def ln2_piece(c, p, z):
        x2 = gated_x(c, p, z)
        x_s[z, piece_rows(c, p), :] = x2
        hp = _pack(_ln(x2))
        h_s[p * 8:(p + 1) * 8, :] = hp
        return hp

    def out_piece(c, p, z):
        v = gated_x(c, p, z)
        out_s[piece_rows(c, p), :] = v.astype(bf)
        return v

    def load_o(c):
        rs = pl.ds(pl.multiple_of(c * (RC // 2), RC // 2), RC // 2)
        return jnp.concatenate([_unpack(o_s[g, rs, :]) for g in range(G)], axis=1)

    def oproj_tile(o, c, n, z, toks=None, r0=0, nr=RC, first=False):
        rows = pl.ds(pl.multiple_of(c * RC + r0, 64), nr)
        cols = slice(n * 128, (n + 1) * 128)
        r = jnp.dot(o[r0:r0 + nr], _gate(wo[:, cols], toks), preferred_element_type=f32)
        x0 = x_in[rows, cols].astype(f32) if first else x_s[z, rows, cols]
        x_s[z, rows, cols] = x0 + r
        return r

    zts = [z_ref[2 + ib] for ib in range(4)]

    def setup_taps():
        taps = shk[...].astype(f32)
        for cb in range(G):
            for t in range(4):
                taps_s[cb, 8 * t:8 * t + 8, :] = jnp.broadcast_to(taps[t:t + 1, cb * 128:(cb + 1) * 128], (8, 128))

    def setup_skip():
        dall = ssmd[...].astype(f32)
        for cb in range(G):
            taps_s[cb, 32:40, :] = jnp.broadcast_to(dall[cb:cb + 1, :], (8, 128))

    def prep_h_chunk(cb, pb, j):
        pb[HS + j * 64:HS + (j + 1) * 64, :] = pltpu.bitcast(ssmk[cb % NB, :, j * 128:(j + 1) * 128], u32)

    def prep_h(cb, pb):
        for j in range(NC):
            prep_h_chunk(cb, pb, j)

    def prep_kv(cb, pb, with_h):
        zs = z_ref[1]
        tp = taps_s[cb, 0:32, :]
        for j in range(NC):
            r0 = j * 128
            if with_h:
                prep_h_chunk(cb, pb, j)
            kf_s[zs, 8 + r0:8 + r0 + 128, :] = bk[cb % NB, r0:r0 + 128, :].astype(f32)
            ks = None
            for t in range(4):
                term = kf_s[zs, 8 + r0 - t:8 + r0 - t + 128, :].reshape(16, 8, 128) * tp[8 * t:8 * t + 8][None]
                ks = term if ks is None else ks + term
            pb[j * 64:(j + 1) * 64, :] = _pack(ks.reshape(128, 128) * bv[cb % NB, r0:r0 + 128, :].astype(f32))

    def fwd_h(pb, ug):
        for m in range(NC):
            hm = lax.dot_general(_unpack(fwd_ref[128:320, :]), _unpack(pb[HS + m * 64:HS + (m + 1) * 64, :]),
                                 NT, preferred_element_type=f32)
            ug[0, NC + m, :, GO:GO + 128, :] = hm.reshape(3, 128, 128)

    def fwd_u(pb, ug):
        for j in range(NC):
            u = jnp.dot(_unpack(fwd_ref[0:128, :]), _unpack(pb[j * 64:(j + 1) * 64, :]),
                        preferred_element_type=f32)
            ug[0, j, 0:2, 0:128, :] = u.reshape(2, 128, 128)

    def add_skip(cb, ug):
        dv = taps_s[cb, 32:40, :][None]
        for e in range(3):
            v = ug[0, NC, e, GO:GO + 128, :].reshape(16, 8, 128)
            ug[0, NC, e, GO:GO + 128, :] = (v - dv if e == 1 else v + dv).reshape(128, 128)

    def spec_item(ug, ib, r):
        zt = zts[ib]
        acc = None
        for j in range(4 * ib + 4):
            u = ug[zt, j:j + 1, 0:2, r:r + 8, :]
            u = jnp.concatenate([u[:, 0:1] + u[:, 1:2], u], axis=1)
            q0 = max(0, j - 4 * ib)
            m0 = NC + 4 * ib - j
            t = ug[zt, m0 + q0:m0 + 4, :, GO + r:GO + r + 8, :] * u
            if acc is None:
                acc = t
            elif q0 == 0:
                acc = acc + t
            else:
                acc = jnp.concatenate([acc[:q0], acc[q0:] + t], axis=0)
        return acc[:, 0] - acc[:, 2], acc[:, 0] + acc[:, 1]

    def overlap_add(yr, yi, prev, r):
        n = 1 if prev is None else 0
        pr = yr[:3] if prev is None else jnp.concatenate([prev[0], yr[:3]], axis=0)
        pi = yi[:3] if prev is None else jnp.concatenate([prev[1], yi[:3]], axis=0)
        if r < 64:
            zr, zi = yr[n:] - pi, yi[n:] + pr
        else:
            zr, zi = yr[n:] + pi, yi[n:] - pr
        if prev is None:
            zr = jnp.concatenate([yr[:1], zr], axis=0)
            zi = jnp.concatenate([yi[:1], zi], axis=0)
        return zr, zi, (yr[3:], yi[3:])

    def conv_spec(ug, zb, lo=0, hi=8):
        for rp in range(lo, hi):
            p0 = p1 = None
            for ib in range(4):
                zr0, zi0, p0 = overlap_add(*spec_item(ug, ib, 16 * rp), p0, 16 * rp)
                zr1, zi1, p1 = overlap_add(*spec_item(ug, ib, 16 * rp + 8), p1, 16 * rp)
                zb[4 * ib:4 * ib + 4, rp * 8:rp * 8 + 8, :] = _pack(jnp.concatenate([zr0, zr1], axis=1))
                zb[4 * ib:4 * ib + 4, 64 + rp * 8:72 + rp * 8, :] = _pack(jnp.concatenate([zi0, zi1], axis=1))

    def conv_inv(cb, zb):
        for i in range(NC):
            for e in range(2):
                y_s[e, cb, i * 128:(i + 1) * 128, :] = jnp.dot(
                    _unpack(inv_ref[:, e * 128:(e + 1) * 128]), _unpack(zb[i, e * 64:(e + 1) * 64, :]),
                    preferred_element_type=f32)

    def conv_step(c, ug_cur, ug_nxt, zb_cur, zb_prev, pb_nxt, pb_new):
        @pl.when(c + 3 < G)
        def _():
            conv_start(c + 3)
        w_copy(c).start()

        @pl.when(c >= G - 3)
        def _():
            x_copy(c - (G - 3)).start()
        conv_spec(ug_cur, zb_cur)
        fwd_h(pb_nxt, ug_nxt)
        fwd_u(pb_nxt, ug_nxt)
        conv_inv(c - 1, zb_prev)

        @pl.when(c + 2 < G)
        def _():
            wait_all([w_copy(c - 1), h_copy(c + 2)] + kv_copies(c + 2))
            prep_kv(c + 2, pb_new, True)
            add_skip(c + 1, ug_nxt)

        @pl.when(c + 2 >= G)
        def _():
            w_copy(c - 1).wait()
            add_skip(c + 1, ug_nxt)

    def conv():
        wait_all([fwd_cp, h_copy(0)])
        conv_start(1)
        inv_cp.start()
        prep_h(0, pb_a)
        fwd_h(pb_a, ug_a)
        wait_all([shk_cp] + kv_copies(0))
        conv_start(2)
        setup_taps()
        prep_kv(0, pb_a, False)
        fwd_u(pb_a, ug_a)
        fence([h_copy(1)])
        prep_h(1, pb_b)
        fence([ssmd_cp])
        setup_skip()
        add_skip(0, ug_a)
        conv_spec(ug_a, zb_a, 0, 4)
        fwd_h(pb_b, ug_b)
        fence(kv_copies(1))
        conv_start(3)
        w_copy(0).start()
        prep_kv(1, pb_b, False)
        add_skip(1, ug_b)
        fence([h_copy(2)])
        conv_spec(ug_a, zb_a, 4, 8)
        fwd_u(pb_b, ug_b)
        fence(kv_copies(2) + [inv_cp])
        prep_kv(2, pb_a, True)

        def body(p, carry):
            conv_step(2 * p + 1, ug_b, ug_a, zb_b, zb_a, pb_a, pb_b)
            conv_step(2 * p + 2, ug_a, ug_b, zb_a, zb_b, pb_b, pb_a)
            return carry
        lax.fori_loop(0, G // 2 - 1, body, 0)
        w_copy(G - 1).start()
        conv_spec(ug_b, zb_b)
        conv_inv(G - 2, zb_a)
        fence([x_copy(0), w_copy(G - 2), w_copy(G - 1)])
        for p in range(NP):
            ln1_piece(0, p)
        conv_inv(G - 1, zb_b)
        early_keys()

    def phase1():
        def body(c, carry):
            @pl.when(c + 1 < NRC)
            def _():
                x_copy(c + 1).wait()

            @pl.when(c + 2 < NRC)
            def _():
                x_copy(c + 2).start()

            @pl.when(c + 2 == NRC)
            def _():
                wo_copy().start()
            cn = jnp.minimum(c + 1, NRC - 1)
            qkv_proj(_unpack(h_s[...]), c, lambda p: ln1_piece(cn, p), 2,
                     kb_plan((c + G - 1) & (G - 1), range(15, 22)), 12)
            return carry
        lax.fori_loop(0, NRC, body, 0)
        wo_copy().wait()

    def phase2(ms):
        o = load_o(0)
        z0 = z_ref[0]
        zv = zero_vreg()
        deps = {}
        todo = []
        for q in range(2):
            rs = []
            for n in range(8):
                t = 8 * q + n
                for p in todo[n:n + 1]:
                    deps.setdefault(t + 4, []).append(_tok(ln2_piece(0, p, z0), zv))
                rs.append(oproj_tile(o, 0, n, z0, deps.get(t), q * (RC // 2), RC // 2, True))
            if q == 0:
                deps.setdefault(11, []).append(attention_tail(ms, rs[0:5:2]))
            todo = list(range(q * NP // 2, (q + 1) * NP // 2))
        for p in todo:
            ln2_piece(0, p, z0)
        early_keys()

        def body(c, carry):
            z0 = z_ref[0]
            z1 = z_ref[1]
            h = _unpack(h_s[...])
            o = load_o(c + 1)
            for n in range(8):
                oproj_tile(o, c + 1, n, z1, first=True)
            qkv_proj(h, c, lambda p: ln2_piece(c + 1, p, z0), 1,
                     kb_plan((c + G - 1) & (G - 1), range(15, 23)), 13)
            return carry
        lax.fori_loop(0, NRC - 1, body, 0)
        qkv_proj(_unpack(h_s[...]), NRC - 1, None, 0, kb_plan(G - 2, range(15, 22)))

    def phase3(ms):
        o = load_o(0)
        done = attention_tail(ms, [oproj_tile(o, 0, n, z_ref[1]) for n in range(3)])
        for n in range(3, 8):
            oproj_tile(o, 0, n, z_ref[1], [done] if n == 6 else None)

        def body(c, carry):
            z0 = z_ref[0]
            z1 = z_ref[1]
            zv = zero_vreg()
            o = load_o(c + 1)
            deps = {}
            p = 0
            for t in range(16):
                for _ in range(2 if t < 2 else 1):
                    if p < NP:
                        deps.setdefault(t + 2, []).append(_tok(out_piece(c, p, z0), zv))
                        p += 1
                oproj_tile(o, c + 1, t // 2, z1, deps.get(t), (t % 2) * 128, 128)
            out_copy(c).start()
            return carry
        lax.fori_loop(0, NRC - 2, body, 0)

        c = NRC - 1
        z0 = z_ref[0]
        zv = zero_vreg()
        o = load_o(c)
        deps = {}
        todo = [(c - 1, p) for p in range(NP)]
        for q in range(3):
            for n in range(8):
                t = 8 * q + n
                for cc, p in todo[2 * n:2 * n + 2]:
                    deps.setdefault(t + (2 if q == 0 else 6), []).append(_tok(out_piece(cc, p, z0), zv))
                oproj_tile(o, c, n, z0, deps.get(t), TAIL[q], TAIL[q + 1] - TAIL[q])
            if q == 1:
                out_copy(c - 1).start()
            if q > 0:
                tail_copy(q - 1).start()
            todo = [(c, p) for p in range(TAIL[q] // 16, TAIL[q + 1] // 16)]
        for cc, p in todo:
            out_piece(cc, p, z0)
        tail_copy(2).start()
        wait_all([out_copy(i) for i in range(NRC - 1)] + [tail_copy(q) for q in range(3)])

    zero16 = jnp.zeros((16, 128), u32)

    def after(x, src, never):
        if src is None:
            return x
        src = pltpu.bitcast(src, x.dtype)
        if x.ndim == 3:
            return jnp.where(never[None], src[None], x)
        return jnp.where(never, src, x)

    def qk(g, j, hh, half, dst, z, zk, dep, never):
        qt = qt_s[j, pl.ds(pl.multiple_of(g * 64 + hh * 16, 16), 16), :]
        w = _unpack(jnp.concatenate([qt if i == hh else zero16 for i in range(4)], axis=0))
        r0 = NV if half == 0 else 0
        kh = k_s[g + zk, (half * HS + r0) // 2:(half + 1) * HS // 2, :]
        ch = (HS - r0) // 4
        m = s2 = None
        for c in range(4):
            ku = kh[c * ch // 2:(c + 1) * ch // 2]
            ku = jnp.concatenate([ku[:ch // 2 - 8], after(ku[ch // 2 - 8:], dep, never)], axis=0)
            s = jnp.dot(_unpack(ku), w, preferred_element_type=f32)
            dst[z, r0 + c * ch:r0 + (c + 1) * ch, :] = s
            mc = jnp.max(s.reshape(ch // 8, 8, 128), axis=0)
            m = mc if m is None else jnp.maximum(m, mc)
            if c == 2:
                s2 = s
        return m, s2

    def qk_vpu(g, j, hh, i0, acc, trigs, never):
        qw16 = qt_s[j, pl.ds(pl.multiple_of(g * 64 + hh * 16, 16), 16), :]
        for k, tr in enumerate(trigs):
            i = i0 + k
            qw = after(jnp.broadcast_to(qw16[i:i + 1], (8, 128)), tr, never)
            qb = pltpu.bitcast(jnp.stack([qw << 16, qw & jnp.uint32(0xFFFF0000)]), f32)
            d = hh * 32 + 2 * i
            t = kb_s[g, d:d + 2].reshape(2, NV // 8, 8, 128) * qb[:, None]
            acc = t[0] + t[1] if acc is None else acc + t[0] + t[1]
        return acc

    def fullmax(m1, m2):
        return jnp.max(jnp.maximum(m1, m2), axis=0, keepdims=True)

    def sm_pv(g, hh, half, src, m, z, dep, trigs, never):
        mb = jnp.broadcast_to(m, (8, 128))
        ms = [after(mb, tr, never) for tr in trigs]
        mm = jnp.stack([jnp.stack([ms[4 * st + 3 - kk] for kk in range(4)]) for st in range(2)])
        x = src[z].reshape(2, 4, 4, 4, 8, 128)
        p = jnp.exp2(x - mm[:, None, :, None]).reshape(HS, 128)
        rs = pl.ds(pl.multiple_of(g * 64 + hh * 16, 16), 16)
        vu = vt_s[half * 8:half * 8 + 8, rs, :]
        vu = jnp.concatenate([after(vu[:, 0:8], dep, never), vu[:, 8:16]], axis=1)
        vu = jnp.concatenate([vu[t] for t in range(8)], axis=1)
        l = _tree_sum(p)
        return jnp.dot(_unpack(vu), p.astype(bf), preferred_element_type=f32), l

    def store_o(g, j, parts):
        outs = [parts[2 * h] * (1.0 / jnp.sum(parts[2 * h + 1], axis=0, keepdims=True)) for h in range(4)]
        ot = _pack(jnp.concatenate(outs, axis=0).T)
        o_s[g, pl.ds(pl.multiple_of(j * 64, 64), 64), :] = ot
        return ot

    bufs = {(0, 0): a1, (0, 1): a2, (1, 0): b1, (1, 1): b2}

    def tile_of(t):
        return lax.shift_right_logical(t, 4), t & (NQ - 1)

    def finish_tile(g, j, done, res):
        if done is None:
            parts = []
        else:
            parts = [done[0:32], done[32:40], done[40:72], done[72:80]]
            res = [(done[80:112], done[112:120])] + res
        for h in range(len(res) // 2):
            parts += [res[2 * h][0] + res[2 * h + 1][0], res[2 * h][1] + res[2 * h + 1][1]]
        return store_o(g, j, parts)

    def attention(m_init):
        nit = G * NQ // UNR

        def body(it, carry):
            z1 = z_ref[0]
            z2 = z_ref[1]
            never = zero_vreg() != 0
            g, j0 = tile_of(it * UNR)
            gp, jp = tile_of(jnp.maximum(it * UNR - 1, 0))
            mfull = {(-1, 2): carry[0], (-1, 3): carry[1]}
            mpart = do = ps = po = vacc = None
            res = []

            def tg(sv, i):
                return None if sv is None else sv[i * 8:i * 8 + 8]

            for n in range(8 * UNR):
                u, qh, qhalf = n // 8, (n % 8) // 2, n % 2
                mp, cs = qk(g, j0 + u, qh, qhalf, bufs[(qh % 2, qhalf)], z1, z_ref[2 + n], do, never)
                src = {'p': ps, 'o': po, 'c': cs}
                vtr, etr = [[tg(src[t[0]], int(t[1:])) for t in spec[n >= N0].split('/')[qhalf].split(',')]
                            for spec in (VT, ET)]
                if qhalf == 0:
                    vacc = qk_vpu(g, j0 + u, qh, 0, None, vtr, never)
                    mpart = mp
                else:
                    vacc = qk_vpu(g, j0 + u, qh, 16 - len(vtr), vacc, vtr, never)
                    bufs[(qh % 2, 0)][z1, 0:NV, :] = vacc.reshape(NV, 128)
                    mfull[(u, qh)] = fullmax(jnp.maximum(mpart, jnp.max(vacc, axis=0)), mp)
                pu, ph, phalf = (n - LAG) // 8, ((n - LAG) % 8) // 2, (n - LAG) % 2
                o, l = sm_pv(gp if pu < 0 else g, ph, phalf, bufs[(ph % 2, phalf)], mfull[(pu, ph)], z2,
                             tg(cs, 0), etr, never)
                ps, po, do = cs, o, tg(o, 3)
                res.append((o, l))
                if ph == 3 and phalf == 1:
                    if pu < 0:
                        finish_tile(gp, jp, fin[z2], res)
                    else:
                        finish_tile(g, j0 + pu, None, res)
                    res = []
            fin[z1] = jnp.concatenate([res[0][0] + res[1][0], res[0][1] + res[1][1],
                                       res[2][0] + res[3][0], res[2][1] + res[3][1],
                                       res[4][0], res[4][1]], axis=0)
            return mfull[(UNR - 1, 2)], mfull[(UNR - 1, 3)]

        return lax.fori_loop(0, nit, body, m_init)

    def attention_tail(ms, rs):
        z2 = z_ref[1]
        never = zero_vreg() != 0
        res = []
        for k, (ph, phalf) in enumerate(((2, 1), (3, 0), (3, 1))):
            trigs = [rs[k][16 * i:16 * i + 8] for i in range(8)]
            res.append(sm_pv(G - 1, ph, phalf, bufs[(ph % 2, phalf)], ms[ph - 2], z2, trigs[7], trigs, never))
        return _tok(finish_tile(G - 1, NQ - 1, fin[z2], res), zero_vreg())

    conv()
    phase1()
    ms = attention((jnp.zeros((1, 128), f32), jnp.zeros((1, 128), f32)))
    phase2(ms)
    ms = attention(ms)
    phase3(ms)


@jax.jit
def pallas_interleave_layers__softmax_full_mha__ssm_conv_h3__prompt_kernel(
        A_x, A_wqkv, A_wo, B_q, B_k, B_v, B_shift_k, B_ssm_k, B_ssm_D):
    del B_q
    fwd, inv = _dft_mats()
    scratch = [
        pltpu.VMEM((1, S, D), f32),
        pltpu.VMEM((2, G, S, 128), f32),
        pltpu.VMEM((NQ, D // 2, 128), u32),
        pltpu.VMEM((G, S // 2, 128), u32),
        pltpu.VMEM((NQ, D // 2, 128), u32),
        pltpu.VMEM((G, S // 2, 128), u32),
        pltpu.VMEM((G, 128, NV, 128), f32),
        pltpu.VMEM((1, HS, 128), f32), pltpu.VMEM((1, HS, 128), f32),
        pltpu.VMEM((1, HS, 128), f32), pltpu.VMEM((1, HS, 128), f32),
        pltpu.VMEM((1, 120, 128), f32),
        pltpu.VMEM((1, S + 8, 128), f32),
        pltpu.VMEM((G, 40, 128), f32),
        pltpu.VMEM((1, 2 * NC, 3, IM, 128), f32),
        pltpu.VMEM((1, 2 * NC, 3, IM, 128), f32),
        pltpu.VMEM((NC, 128, 128), u32),
        pltpu.VMEM((NC, 128, 128), u32),
        pltpu.VMEM((S, 128), u32),
        pltpu.VMEM((S, 128), u32),
        pltpu.VMEM((RC // 2, D), u32),
        pltpu.SMEM((NZ,), i32),
        pltpu.VMEM((S, D), bf),
        pltpu.VMEM((D, 3 * D + 128), bf),
        pltpu.VMEM((D, D + 128), bf),
        pltpu.VMEM((NB, S, 128), bf),
        pltpu.VMEM((NB, S, 128), bf),
        pltpu.VMEM((NB, 128, S + 128), bf),
        pltpu.VMEM((4, D), bf),
        pltpu.VMEM((G, 128), bf),
        pltpu.VMEM((320, 128), u32),
        pltpu.VMEM((64, 256), u32),
        pltpu.SemaphoreType.DMA((3, G)),
        pltpu.SemaphoreType.DMA((NRC,)),
        pltpu.SemaphoreType.DMA((G + 1,)),
        pltpu.SemaphoreType.DMA((NRC + 2,)),
        pltpu.SemaphoreType.DMA((4,)),
    ]
    hbm = pl.BlockSpec(memory_space=pl.ANY)
    return pl.pallas_call(
        _kernel,
        out_shape=jax.ShapeDtypeStruct((1, S, D), bf),
        in_specs=[hbm] * 10,
        out_specs=hbm,
        scratch_shapes=scratch,
        compiler_params=pltpu.CompilerParams(vmem_limit_bytes=120 * 2**20, disable_bounds_checks=True),
    )(A_x, A_wqkv, A_wo, B_k, B_v, B_shift_k.T, B_ssm_k, B_ssm_D.reshape(G, 128),
      jnp.asarray(fwd), jnp.asarray(inv))
```

```python
import numpy as np
import jax
import jax.numpy as jnp
from jax import lax
import jax.experimental.pallas as pl
import jax.experimental.pallas.tpu as pltpu

S = 2048
D = 1024
DH = 32
G = 8
NQ = 16
HS = S // 2
UNR = 8
NV = 64
LAG = 3
RC = 256
NRC = S // RC
NP = RC // 16
NC = 16
NB = 4
IM = 136
GO = 8
EPS = 1e-5
NZ = 2 + 8 * UNR
QSCALE = float(DH ** -0.5 * np.log2(np.e))
VT = 'p24,p25,p26,p26,p28,p30,p31,p31,o0,o3,c0,c8,c9,c15,c16,c17/p23,p23,p26,p27,p28,p29,p29,o0,o3,c4,c4,c12,c15,c16,c18,c20'
ET = 'p18,p30,o0,o0,o1,c0,c2,c10/p18,p19,p24,p29,o0,o3,c4,c9'

bf = jnp.bfloat16
f32 = jnp.float32
u32 = jnp.uint32
i32 = jnp.int32
NT = (((1,), (1,)), ((), ()))


def _dft_mats():
    n = np.arange(128)
    f = np.concatenate([np.arange(0, 128, 2), np.arange(1, 128, 2)])
    ang = 2.0 * np.pi * np.outer(f + 0.5, n) / 256.0
    re, im = np.cos(ang), -np.sin(ang)
    inv = np.concatenate([re, im], axis=0).T / 128.0
    fwd = np.concatenate([re, im, re, im - re, im + re], axis=0)

    def pack_rows(a):
        u = np.ascontiguousarray(a, dtype=np.float32).view(np.uint32)
        u = (u + 0x7FFF + ((u >> 16) & 1)) >> 16
        return (u[0::2] | (u[1::2] << 16)).astype(np.uint32)
    return pack_rows(fwd), pack_rows(inv)


def _tree_sum(p):
    n = p.shape[0] // 8
    x = p.reshape(n, 8, 128)
    while n > 1:
        x = x.reshape(n // 2, 2, 8, 128)
        x = x[:, 0] + x[:, 1]
        n //= 2
    return x[0]


def _ln(x):
    m = jnp.mean(x, axis=-1, keepdims=True)
    xc = x - m
    v = jnp.mean(xc * xc, axis=-1, keepdims=True)
    return xc * lax.rsqrt(v + EPS)


def _pack(x):
    return pltpu.bitcast(x.astype(bf), u32)


def _unpack(x):
    return pltpu.bitcast(x, bf)


def _tok(v, zv):
    v = v if v.dtype == u32 else pltpu.bitcast(v, u32)
    while v.shape[1] > 128:
        h = v.shape[1] // 2
        v = v[:, :h] | v[:, h:]
    while v.shape[0] > 8:
        h = v.shape[0] // 2
        v = v[:h] | v[h:]
    return v & zv


def _gate(w, toks):
    if not toks:
        return w
    wu = pltpu.bitcast(w, u32)
    h0 = wu[0:8]
    for t in toks:
        h0 = h0 | t
    return _unpack(jnp.concatenate([h0, wu[8:]], axis=0))


def _kernel(x_hbm, wqkv_hbm, wo_hbm, bk_hbm, bv_hbm, shk_hbm, ssmk_hbm, ssmd_hbm, fwd_hbm, inv_hbm, out_hbm,
            x_s, y_s, qt_s, k_s, vt_s, o_s, kb_s, a1, a2, b1, b2, fin, kf_s, taps_s, ug_a, ug_b, zb_a, zb_b,
            pb_a, pb_b, h_s, z_ref, x_in, wqkv, wo, bk, bv, ssmk, shk, ssmd, fwd_ref, inv_ref,
            sem_c, sem_x, sem_w, sem_o, sem_s):
    out_s = x_in

    def kv_copies(cb):
        cs = pl.ds(pl.multiple_of(cb * 128, 128), 128)
        return [pltpu.make_async_copy(bk_hbm.at[0, :, cs], bk.at[cb % NB], sem_c.at[0, cb]),
                pltpu.make_async_copy(bv_hbm.at[0, :, cs], bv.at[cb % NB], sem_c.at[1, cb])]

    def h_copy(cb):
        cs = pl.ds(pl.multiple_of(cb * 128, 128), 128)
        return pltpu.make_async_copy(ssmk_hbm.at[cs, :], ssmk.at[cb % NB, :, pl.ds(0, S)], sem_c.at[2, cb])

    def x_copy(c):
        rs = pl.ds(pl.multiple_of(c * RC, RC), RC)
        return pltpu.make_async_copy(x_hbm.at[0, rs, :], x_in.at[rs, :], sem_x.at[c])

    def w_copy(c):
        rs = pl.ds(pl.multiple_of(c * 128, 128), 128)
        return pltpu.make_async_copy(wqkv_hbm.at[rs, :], wqkv.at[rs, pl.ds(0, 3 * D)], sem_w.at[c])

    def wo_copy():
        return pltpu.make_async_copy(wo_hbm, wo.at[:, pl.ds(0, D)], sem_w.at[G])

    def out_copy(c):
        rs = pl.ds(pl.multiple_of(c * RC, RC), RC)
        return pltpu.make_async_copy(out_s.at[rs, :], out_hbm.at[0, rs, :], sem_o.at[c])

    TAIL = (0, 128, 192, 256)

    def tail_copy(q):
        rs = pl.ds((NRC - 1) * RC + TAIL[q], TAIL[q + 1] - TAIL[q])
        return pltpu.make_async_copy(out_s.at[rs, :], out_hbm.at[0, rs, :], sem_o.at[NRC - 1 + q])

    def conv_start(c):
        h_copy(c).start()
        for cp in kv_copies(c):
            cp.start()

    def wait_all(cps):
        for cp in cps:
            cp.wait()

    shk_cp, ssmd_cp, fwd_cp, inv_cp = [
        pltpu.make_async_copy(src, dst, sem_s.at[i]) for i, (src, dst) in enumerate(
            ((shk_hbm, shk), (ssmd_hbm, ssmd), (fwd_hbm, fwd_ref), (inv_hbm, inv_ref)))]
    h_copy(0).start()
    fwd_cp.start()
    shk_cp.start()
    ssmd_cp.start()
    for cp in kv_copies(0):
        cp.start()

    for i in range(NZ):
        z_ref[i] = 0
    fin[...] = jnp.ones(fin.shape, f32)
    for buf in (a2, b1, b2):
        buf[...] = jnp.zeros(buf.shape, f32)
    kf_s[0, 0:8, :] = jnp.zeros((8, 128), f32)

    def zero_vreg():
        return jnp.full((8, 128), z_ref[0], i32).astype(u32)

    def fence(cps):
        @pl.when(z_ref[0] == 0)
        def _():
            wait_all(cps)

    TILES = [(0, n) for n in range(8)] + [(2, n) for n in range(8)] + [(1, n) for n in range(8)]

    def qkv_tile(h, c, idx, toks, zv):
        kind, n = TILES[idx]
        col = kind * D + n * 128
        r = jnp.dot(h, _gate(wqkv[:, col:col + 128], toks), preferred_element_type=f32)
        if kind == 1:
            k_s[n, pl.ds(pl.multiple_of(c * (RC // 2), RC // 2), RC // 2), :] = _pack(r)
            return None
        dst = qt_s if kind == 0 else vt_s
        if kind == 0:
            r = r * QSCALE
        pks = []
        for t in range(RC // 128):
            pk = _pack(r[t * 128:(t + 1) * 128, :].T)
            dst[c * (RC // 128) + t, n * 64:(n + 1) * 64, :] = pk
            pks.append(pk)
        return _tok(jnp.concatenate(pks, axis=0), zv)

    def qkv_proj(h, c, piece_fn, first_piece, kb_jobs, span=NP):
        zv = zero_vreg()
        deps = {}
        for n in range(24):
            done = qkv_tile(h, c, n, deps.get(n), zv)
            if done is not None:
                deps.setdefault(n + 3, []).append(done)
            if n in kb_jobs:
                deps.setdefault(n + 2, []).append(kb_piece(*kb_jobs[n], zv))
            if piece_fn is not None:
                for p in range(NP):
                    if first_piece + p * span // NP == n:
                        deps.setdefault(n + 3, []).append(_tok(piece_fn(p), zv))

    def kb_plan(g, tiles):
        return {t: (g, 128 * i // len(tiles), 128 * (i + 1) // len(tiles)) for i, t in enumerate(tiles)}

    def kb_piece(g, lo, hi, zv):
        kx = _unpack(k_s[g, 0:NV // 2, :]).astype(f32)
        for d in range(lo, hi):
            v = jnp.broadcast_to(kx[:, d:d + 1], (NV, 128))
            kb_s[g, d] = v
        return _tok(v[NV - 32:], zv)

    def early_keys():
        col = D + (G - 1) * 128
        k_s[G - 1, 0:NV // 2, :] = _pack(jnp.dot(_unpack(h_s[0:NV // 2, :]), wqkv[:, col:col + 128],
                                                 preferred_element_type=f32))

    def piece_rows(c, p):
        return pl.ds(pl.multiple_of(c * RC + p * 16, 16), 16)

    def ln1_piece(c, p):
        hp = _pack(_ln(x_in[piece_rows(c, p), :].astype(f32)))
        h_s[p * 8:(p + 1) * 8, :] = hp
        return hp

    def gated_x(c, p, z):
        rows = piece_rows(c, p)
        x1 = x_s[z, rows, :]
        y = jnp.concatenate([y_s[0, g, rows, :] + y_s[1, g, rows, :] for g in range(G)], axis=1)
        return x1 + _ln(x1) * y

    def ln2_piece(c, p, z):
        x2 = gated_x(c, p, z)
        x_s[z, piece_rows(c, p), :] = x2
        hp = _pack(_ln(x2))
        h_s[p * 8:(p + 1) * 8, :] = hp
        return hp

    def out_piece(c, p, z):
        v = gated_x(c, p, z)
        out_s[piece_rows(c, p), :] = v.astype(bf)
        return v

    def load_o(c):
        rs = pl.ds(pl.multiple_of(c * (RC // 2), RC // 2), RC // 2)
        return jnp.concatenate([_unpack(o_s[g, rs, :]) for g in range(G)], axis=1)

    def oproj_tile(o, c, n, z, toks=None, r0=0, nr=RC, first=False):
        rows = pl.ds(pl.multiple_of(c * RC + r0, 64), nr)
        cols = slice(n * 128, (n + 1) * 128)
        r = jnp.dot(o[r0:r0 + nr], _gate(wo[:, cols], toks), preferred_element_type=f32)
        x0 = x_in[rows, cols].astype(f32) if first else x_s[z, rows, cols]
        x_s[z, rows, cols] = x0 + r
        return r

    zts = [z_ref[2 + ib] for ib in range(4)]

    def setup_taps():
        taps = shk[...].astype(f32)
        for cb in range(G):
            for t in range(4):
                taps_s[cb, 8 * t:8 * t + 8, :] = jnp.broadcast_to(taps[t:t + 1, cb * 128:(cb + 1) * 128], (8, 128))

    def setup_skip():
        dall = ssmd[...].astype(f32)
        for cb in range(G):
            taps_s[cb, 32:40, :] = jnp.broadcast_to(dall[cb:cb + 1, :], (8, 128))

    def prep_h_chunk(cb, pb, j):
        pb[HS + j * 64:HS + (j + 1) * 64, :] = pltpu.bitcast(ssmk[cb % NB, :, j * 128:(j + 1) * 128], u32)

    def prep_h(cb, pb):
        for j in range(NC):
            prep_h_chunk(cb, pb, j)

    def prep_kv(cb, pb, with_h):
        zs = z_ref[1]
        tp = taps_s[cb, 0:32, :]
        for j in range(NC):
            r0 = j * 128
            if with_h:
                prep_h_chunk(cb, pb, j)
            kf_s[zs, 8 + r0:8 + r0 + 128, :] = bk[cb % NB, r0:r0 + 128, :].astype(f32)
            ks = None
            for t in range(4):
                term = kf_s[zs, 8 + r0 - t:8 + r0 - t + 128, :].reshape(16, 8, 128) * tp[8 * t:8 * t + 8][None]
                ks = term if ks is None else ks + term
            pb[j * 64:(j + 1) * 64, :] = _pack(ks.reshape(128, 128) * bv[cb % NB, r0:r0 + 128, :].astype(f32))

    def fwd_h(pb, ug):
        for m in range(NC):
            hm = lax.dot_general(_unpack(fwd_ref[128:320, :]), _unpack(pb[HS + m * 64:HS + (m + 1) * 64, :]),
                                 NT, preferred_element_type=f32)
            ug[0, NC + m, :, GO:GO + 128, :] = hm.reshape(3, 128, 128)

    def fwd_u(pb, ug):
        for j in range(NC):
            u = jnp.dot(_unpack(fwd_ref[0:128, :]), _unpack(pb[j * 64:(j + 1) * 64, :]),
                        preferred_element_type=f32)
            ug[0, j, 0:2, 0:128, :] = u.reshape(2, 128, 128)

    def add_skip(cb, ug):
        dv = taps_s[cb, 32:40, :][None]
        for e in range(3):
            v = ug[0, NC, e, GO:GO + 128, :].reshape(16, 8, 128)
            ug[0, NC, e, GO:GO + 128, :] = (v - dv if e == 1 else v + dv).reshape(128, 128)

    def spec_item(ug, ib, r):
        zt = zts[ib]
        acc = None
        for j in range(4 * ib + 4):
            u = ug[zt, j:j + 1, 0:2, r:r + 8, :]
            u = jnp.concatenate([u[:, 0:1] + u[:, 1:2], u], axis=1)
            q0 = max(0, j - 4 * ib)
            m0 = NC + 4 * ib - j
            t = ug[zt, m0 + q0:m0 + 4, :, GO + r:GO + r + 8, :] * u
            if acc is None:
                acc = t
            elif q0 == 0:
                acc = acc + t
            else:
                acc = jnp.concatenate([acc[:q0], acc[q0:] + t], axis=0)
        return acc[:, 0] - acc[:, 2], acc[:, 0] + acc[:, 1]

    def overlap_add(yr, yi, prev, r):
        n = 1 if prev is None else 0
        pr = yr[:3] if prev is None else jnp.concatenate([prev[0], yr[:3]], axis=0)
        pi = yi[:3] if prev is None else jnp.concatenate([prev[1], yi[:3]], axis=0)
        if r < 64:
            zr, zi = yr[n:] - pi, yi[n:] + pr
        else:
            zr, zi = yr[n:] + pi, yi[n:] - pr
        if prev is None:
            zr = jnp.concatenate([yr[:1], zr], axis=0)
            zi = jnp.concatenate([yi[:1], zi], axis=0)
        return zr, zi, (yr[3:], yi[3:])

    def conv_spec(ug, zb, lo=0, hi=8):
        for rp in range(lo, hi):
            p0 = p1 = None
            for ib in range(4):
                zr0, zi0, p0 = overlap_add(*spec_item(ug, ib, 16 * rp), p0, 16 * rp)
                zr1, zi1, p1 = overlap_add(*spec_item(ug, ib, 16 * rp + 8), p1, 16 * rp)
                zb[4 * ib:4 * ib + 4, rp * 8:rp * 8 + 8, :] = _pack(jnp.concatenate([zr0, zr1], axis=1))
                zb[4 * ib:4 * ib + 4, 64 + rp * 8:72 + rp * 8, :] = _pack(jnp.concatenate([zi0, zi1], axis=1))

    def conv_inv(cb, zb):
        for i in range(NC):
            for e in range(2):
                y_s[e, cb, i * 128:(i + 1) * 128, :] = jnp.dot(
                    _unpack(inv_ref[:, e * 128:(e + 1) * 128]), _unpack(zb[i, e * 64:(e + 1) * 64, :]),
                    preferred_element_type=f32)

    def conv_step(c, ug_cur, ug_nxt, zb_cur, zb_prev, pb_nxt, pb_new):
        @pl.when(c + 3 < G)
        def _():
            conv_start(c + 3)
        w_copy(c).start()

        @pl.when(c >= G - 3)
        def _():
            x_copy(c - (G - 3)).start()
        conv_spec(ug_cur, zb_cur)
        fwd_h(pb_nxt, ug_nxt)
        fwd_u(pb_nxt, ug_nxt)
        conv_inv(c - 1, zb_prev)

        @pl.when(c + 2 < G)
        def _():
            wait_all([w_copy(c - 1), h_copy(c + 2)] + kv_copies(c + 2))
            prep_kv(c + 2, pb_new, True)
            add_skip(c + 1, ug_nxt)

        @pl.when(c + 2 >= G)
        def _():
            w_copy(c - 1).wait()
            add_skip(c + 1, ug_nxt)

    def conv():
        wait_all([fwd_cp, h_copy(0)])
        conv_start(1)
        inv_cp.start()
        prep_h(0, pb_a)
        fwd_h(pb_a, ug_a)
        wait_all([shk_cp] + kv_copies(0))
        conv_start(2)
        setup_taps()
        prep_kv(0, pb_a, False)
        fwd_u(pb_a, ug_a)
        fence([h_copy(1)])
        prep_h(1, pb_b)
        fence([ssmd_cp])
        setup_skip()
        add_skip(0, ug_a)
        conv_spec(ug_a, zb_a, 0, 4)
        fwd_h(pb_b, ug_b)
        fence(kv_copies(1))
        conv_start(3)
        w_copy(0).start()
        prep_kv(1, pb_b, False)
        add_skip(1, ug_b)
        fence([h_copy(2)])
        conv_spec(ug_a, zb_a, 4, 8)
        fwd_u(pb_b, ug_b)
        fence(kv_copies(2) + [inv_cp])
        prep_kv(2, pb_a, True)

        def body(p, carry):
            conv_step(2 * p + 1, ug_b, ug_a, zb_b, zb_a, pb_a, pb_b)
            conv_step(2 * p + 2, ug_a, ug_b, zb_a, zb_b, pb_b, pb_a)
            return carry
        lax.fori_loop(0, G // 2 - 1, body, 0)
        w_copy(G - 1).start()
        conv_spec(ug_b, zb_b)
        conv_inv(G - 2, zb_a)
        fence([x_copy(0), w_copy(G - 2), w_copy(G - 1)])
        for p in range(NP):
            ln1_piece(0, p)
        conv_inv(G - 1, zb_b)
        early_keys()

    def phase1():
        def body(c, carry):
            @pl.when(c + 1 < NRC)
            def _():
                x_copy(c + 1).wait()

            @pl.when(c + 2 < NRC)
            def _():
                x_copy(c + 2).start()

            @pl.when(c + 2 == NRC)
            def _():
                wo_copy().start()
            cn = jnp.minimum(c + 1, NRC - 1)
            qkv_proj(_unpack(h_s[...]), c, lambda p: ln1_piece(cn, p), 2,
                     kb_plan((c + G - 1) & (G - 1), range(15, 22)), 12)
            return carry
        lax.fori_loop(0, NRC, body, 0)
        wo_copy().wait()

    def phase2(ms):
        o = load_o(0)
        z0 = z_ref[0]
        zv = zero_vreg()
        deps = {}
        todo = []
        for q in range(2):
            rs = []
            for n in range(8):
                t = 8 * q + n
                for p in todo[n:n + 1]:
                    deps.setdefault(t + 4, []).append(_tok(ln2_piece(0, p, z0), zv))
                rs.append(oproj_tile(o, 0, n, z0, deps.get(t), q * (RC // 2), RC // 2, True))
            if q == 0:
                deps.setdefault(11, []).append(attention_tail(ms, rs[0:5:2]))
            todo = list(range(q * NP // 2, (q + 1) * NP // 2))
        for p in todo:
            ln2_piece(0, p, z0)
        early_keys()

        def body(c, carry):
            z0 = z_ref[0]
            z1 = z_ref[1]
            h = _unpack(h_s[...])
            o = load_o(c + 1)
            for n in range(8):
                oproj_tile(o, c + 1, n, z1, first=True)
            qkv_proj(h, c, lambda p: ln2_piece(c + 1, p, z0), 1,
                     kb_plan((c + G - 1) & (G - 1), range(15, 23)), 13)
            return carry
        lax.fori_loop(0, NRC - 1, body, 0)
        qkv_proj(_unpack(h_s[...]), NRC - 1, None, 0, kb_plan(G - 2, range(15, 22)))

    def phase3(ms):
        o = load_o(0)
        done = attention_tail(ms, [oproj_tile(o, 0, n, z_ref[1]) for n in range(3)])
        for n in range(3, 8):
            oproj_tile(o, 0, n, z_ref[1], [done] if n == 6 else None)

        def body(c, carry):
            z0 = z_ref[0]
            z1 = z_ref[1]
            zv = zero_vreg()
            o = load_o(c + 1)
            deps = {}
            p = 0
            for t in range(16):
                for _ in range(2 if t < 2 else 1):
                    if p < NP:
                        deps.setdefault(t + 2, []).append(_tok(out_piece(c, p, z0), zv))
                        p += 1
                oproj_tile(o, c + 1, t // 2, z1, deps.get(t), (t % 2) * 128, 128)
            out_copy(c).start()
            return carry
        lax.fori_loop(0, NRC - 2, body, 0)

        c = NRC - 1
        z0 = z_ref[0]
        zv = zero_vreg()
        o = load_o(c)
        deps = {}
        todo = [(c - 1, p) for p in range(NP)]
        for q in range(3):
            for n in range(8):
                t = 8 * q + n
                for cc, p in todo[2 * n:2 * n + 2]:
                    deps.setdefault(t + (2 if q == 0 else 6), []).append(_tok(out_piece(cc, p, z0), zv))
                oproj_tile(o, c, n, z0, deps.get(t), TAIL[q], TAIL[q + 1] - TAIL[q])
            if q == 1:
                out_copy(c - 1).start()
            if q > 0:
                tail_copy(q - 1).start()
            todo = [(c, p) for p in range(TAIL[q] // 16, TAIL[q + 1] // 16)]
        for cc, p in todo:
            out_piece(cc, p, z0)
        tail_copy(2).start()
        wait_all([out_copy(i) for i in range(NRC - 1)] + [tail_copy(q) for q in range(3)])

    zero16 = jnp.zeros((16, 128), u32)

    def after(x, src, never):
        if src is None:
            return x
        src = pltpu.bitcast(src, x.dtype)
        if x.ndim == 3:
            return jnp.where(never[None], src[None], x)
        return jnp.where(never, src, x)

    def qk(g, j, hh, half, dst, z, zk, dep, never):
        qt = qt_s[j, pl.ds(pl.multiple_of(g * 64 + hh * 16, 16), 16), :]
        w = _unpack(jnp.concatenate([qt if i == hh else zero16 for i in range(4)], axis=0))
        r0 = NV if half == 0 else 0
        kh = k_s[g + zk, (half * HS + r0) // 2:(half + 1) * HS // 2, :]
        ch = (HS - r0) // 4
        m = s2 = None
        for c in range(4):
            ku = kh[c * ch // 2:(c + 1) * ch // 2]
            ku = jnp.concatenate([ku[:ch // 2 - 8], after(ku[ch // 2 - 8:], dep, never)], axis=0)
            s = jnp.dot(_unpack(ku), w, preferred_element_type=f32)
            dst[z, r0 + c * ch:r0 + (c + 1) * ch, :] = s
            mc = jnp.max(s.reshape(ch // 8, 8, 128), axis=0)
            m = mc if m is None else jnp.maximum(m, mc)
            if c == 2:
                s2 = s
        return m, s2

    def qk_vpu(g, j, hh, half, trigs, never):
        qw16 = qt_s[j, pl.ds(pl.multiple_of(g * 64 + hh * 16, 16), 16), :]
        rows = slice(half * NV // 2, (half + 1) * NV // 2)
        acc = None
        for i, tr in enumerate(trigs):
            qw = after(jnp.broadcast_to(qw16[i:i + 1], (8, 128)), tr, never)
            qb = pltpu.bitcast(jnp.stack([qw << 16, qw & jnp.uint32(0xFFFF0000)]), f32)
            d = hh * 32 + 2 * i
            t = kb_s[g, d:d + 2, rows, :].reshape(2, NV // 16, 8, 128) * qb[:, None]
            acc = t[0] + t[1] if acc is None else acc + t[0] + t[1]
        return acc

    def fullmax(m1, m2):
        return jnp.max(jnp.maximum(m1, m2), axis=0, keepdims=True)

    def sm_pv(g, hh, half, src, m, z, dep, trigs, never):
        mb = jnp.broadcast_to(m, (8, 128))
        ms = [after(mb, tr, never) for tr in trigs]
        mm = jnp.stack([jnp.stack([ms[4 * st + 3 - kk] for kk in range(4)]) for st in range(2)])
        x = src[z].reshape(2, 4, 4, 4, 8, 128)
        p = jnp.exp2(x - mm[:, None, :, None]).reshape(HS, 128)
        rs = pl.ds(pl.multiple_of(g * 64 + hh * 16, 16), 16)
        vu = vt_s[half * 8:half * 8 + 8, rs, :]
        vu = jnp.concatenate([after(vu[:, 0:8], dep, never), vu[:, 8:16]], axis=1)
        vu = jnp.concatenate([vu[t] for t in range(8)], axis=1)
        l = _tree_sum(p)
        return jnp.dot(_unpack(vu), p.astype(bf), preferred_element_type=f32), l

    def store_o(g, j, parts):
        outs = [parts[2 * h] * (1.0 / jnp.sum(parts[2 * h + 1], axis=0, keepdims=True)) for h in range(4)]
        ot = _pack(jnp.concatenate(outs, axis=0).T)
        o_s[g, pl.ds(pl.multiple_of(j * 64, 64), 64), :] = ot
        return ot

    bufs = {(0, 0): a1, (0, 1): a2, (1, 0): b1, (1, 1): b2}

    def tile_of(t):
        return lax.shift_right_logical(t, 4), t & (NQ - 1)

    def finish_tile(g, j, done, res):
        if done is None:
            parts = []
        else:
            parts = [done[0:32], done[32:40], done[40:72], done[72:80]]
            res = [(done[80:112], done[112:120])] + res
        for h in range(len(res) // 2):
            parts += [res[2 * h][0] + res[2 * h + 1][0], res[2 * h][1] + res[2 * h + 1][1]]
        return store_o(g, j, parts)

    def attention(m_init):
        nit = G * NQ // UNR

        def body(it, carry):
            z1 = z_ref[0]
            z2 = z_ref[1]
            never = zero_vreg() != 0
            g, j0 = tile_of(it * UNR)
            gp, jp = tile_of(jnp.maximum(it * UNR - 1, 0))
            mfull = {(-1, 2): carry[0], (-1, 3): carry[1]}
            mpart = do = ps = po = None
            res = []

            def tg(sv, i):
                return None if sv is None else sv[i * 8:i * 8 + 8]

            for n in range(8 * UNR):
                u, qh, qhalf = n // 8, (n % 8) // 2, n % 2
                mp, cs = qk(g, j0 + u, qh, qhalf, bufs[(qh % 2, qhalf)], z1, z_ref[2 + n], do, never)
                src = {'p': ps, 'o': po, 'c': cs}
                vtr, etr = [[tg(src[t[0]], int(t[1:])) for t in spec.split('/')[qhalf].split(',')]
                            for spec in (VT, ET)]
                sv = qk_vpu(g, j0 + u, qh, qhalf, vtr, never)
                bufs[(qh % 2, 0)][z1, qhalf * NV // 2:(qhalf + 1) * NV // 2, :] = sv.reshape(NV // 2, 128)
                mp = jnp.maximum(mp, jnp.max(sv, axis=0))
                if qhalf == 0:
                    mpart = mp
                else:
                    mfull[(u, qh)] = fullmax(mpart, mp)
                pu, ph, phalf = (n - LAG) // 8, ((n - LAG) % 8) // 2, (n - LAG) % 2
                o, l = sm_pv(gp if pu < 0 else g, ph, phalf, bufs[(ph % 2, phalf)], mfull[(pu, ph)], z2,
                             tg(cs, 0), etr, never)
                ps, po, do = cs, o, tg(o, 3)
                res.append((o, l))
                if ph == 3 and phalf == 1:
                    if pu < 0:
                        finish_tile(gp, jp, fin[z2], res)
                    else:
                        finish_tile(g, j0 + pu, None, res)
                    res = []
            fin[z1] = jnp.concatenate([res[0][0] + res[1][0], res[0][1] + res[1][1],
                                       res[2][0] + res[3][0], res[2][1] + res[3][1],
                                       res[4][0], res[4][1]], axis=0)
            return mfull[(UNR - 1, 2)], mfull[(UNR - 1, 3)]

        return lax.fori_loop(0, nit, body, m_init)

    def attention_tail(ms, rs):
        z2 = z_ref[1]
        never = zero_vreg() != 0
        res = []
        for k, (ph, phalf) in enumerate(((2, 1), (3, 0), (3, 1))):
            trigs = [rs[k][16 * i:16 * i + 8] for i in range(8)]
            res.append(sm_pv(G - 1, ph, phalf, bufs[(ph % 2, phalf)], ms[ph - 2], z2, trigs[7], trigs, never))
        return _tok(finish_tile(G - 1, NQ - 1, fin[z2], res), zero_vreg())

    conv()
    phase1()
    ms = attention((jnp.zeros((1, 128), f32), jnp.zeros((1, 128), f32)))
    phase2(ms)
    ms = attention(ms)
    phase3(ms)


@jax.jit
def pallas_interleave_layers__softmax_full_mha__ssm_conv_h3__prompt_kernel(
        A_x, A_wqkv, A_wo, B_q, B_k, B_v, B_shift_k, B_ssm_k, B_ssm_D):
    del B_q
    fwd, inv = _dft_mats()
    scratch = [
        pltpu.VMEM((1, S, D), f32),
        pltpu.VMEM((2, G, S, 128), f32),
        pltpu.VMEM((NQ, D // 2, 128), u32),
        pltpu.VMEM((G, S // 2, 128), u32),
        pltpu.VMEM((NQ, D // 2, 128), u32),
        pltpu.VMEM((G, S // 2, 128), u32),
        pltpu.VMEM((G, 128, NV, 128), f32),
        pltpu.VMEM((1, HS, 128), f32), pltpu.VMEM((1, HS, 128), f32),
        pltpu.VMEM((1, HS, 128), f32), pltpu.VMEM((1, HS, 128), f32),
        pltpu.VMEM((1, 120, 128), f32),
        pltpu.VMEM((1, S + 8, 128), f32),
        pltpu.VMEM((G, 40, 128), f32),
        pltpu.VMEM((1, 2 * NC, 3, IM, 128), f32),
        pltpu.VMEM((1, 2 * NC, 3, IM, 128), f32),
        pltpu.VMEM((NC, 128, 128), u32),
        pltpu.VMEM((NC, 128, 128), u32),
        pltpu.VMEM((S, 128), u32),
        pltpu.VMEM((S, 128), u32),
        pltpu.VMEM((RC // 2, D), u32),
        pltpu.SMEM((NZ,), i32),
        pltpu.VMEM((S, D), bf),
        pltpu.VMEM((D, 3 * D + 128), bf),
        pltpu.VMEM((D, D + 128), bf),
        pltpu.VMEM((NB, S, 128), bf),
        pltpu.VMEM((NB, S, 128), bf),
        pltpu.VMEM((NB, 128, S + 128), bf),
        pltpu.VMEM((4, D), bf),
        pltpu.VMEM((G, 128), bf),
        pltpu.VMEM((320, 128), u32),
        pltpu.VMEM((64, 256), u32),
        pltpu.SemaphoreType.DMA((3, G)),
        pltpu.SemaphoreType.DMA((NRC,)),
        pltpu.SemaphoreType.DMA((G + 1,)),
        pltpu.SemaphoreType.DMA((NRC + 2,)),
        pltpu.SemaphoreType.DMA((4,)),
    ]
    hbm = pl.BlockSpec(memory_space=pl.ANY)
    return pl.pallas_call(
        _kernel,
        out_shape=jax.ShapeDtypeStruct((1, S, D), bf),
        in_specs=[hbm] * 10,
        out_specs=hbm,
        scratch_shapes=scratch,
        compiler_params=pltpu.CompilerParams(vmem_limit_bytes=120 * 2**20, disable_bounds_checks=True),
    )(A_x, A_wqkv, A_wo, B_k, B_v, B_shift_k.T, B_ssm_k, B_ssm_D.reshape(G, 128),
      jnp.asarray(fwd), jnp.asarray(inv))
```

```python
import numpy as np
import jax
import jax.numpy as jnp
from jax import lax
import jax.experimental.pallas as pl
import jax.experimental.pallas.tpu as pltpu

S = 2048
D = 1024
DH = 32
G = 8
NQ = 16
HS = S // 2
UNR = 8
NV = 64
LAG = 3
RC = 256
NRC = S // RC
NP = RC // 16
NC = 16
NB = 4
IM = 136
GO = 8
EPS = 1e-5
NZ = 2 + 8 * UNR
QSCALE = float(DH ** -0.5 * np.log2(np.e))
VT = 'p24,p25,p26,p26,p28,p30,p31,p31,o0,o3,c0,c8,c9,c15,c16,c17/p23,p23,p26,p27,p28,p29,p29,o0,o3,c4,c4,c12,c15,c16,c18,c20'
ET = 'p18,p30,o0,o0,o1,c0,c2,c10/p18,p19,p24,p29,o0,o3,c4,c9'

bf = jnp.bfloat16
f32 = jnp.float32
u32 = jnp.uint32
i32 = jnp.int32
NT = (((1,), (1,)), ((), ()))


def _dft_mats():
    n = np.arange(128)
    f = np.concatenate([np.arange(0, 128, 2), np.arange(1, 128, 2)])
    ang = 2.0 * np.pi * np.outer(f + 0.5, n) / 256.0
    re, im = np.cos(ang), -np.sin(ang)
    inv = np.concatenate([re, im], axis=0).T / 128.0
    fwd = np.concatenate([re, im, re, im - re, im + re], axis=0)

    def pack_rows(a):
        u = np.ascontiguousarray(a, dtype=np.float32).view(np.uint32)
        u = (u + 0x7FFF + ((u >> 16) & 1)) >> 16
        return (u[0::2] | (u[1::2] << 16)).astype(np.uint32)
    return pack_rows(fwd), pack_rows(inv)


def _tree_sum(p):
    n = p.shape[0] // 8
    x = p.reshape(n, 8, 128)
    while n > 1:
        x = x.reshape(n // 2, 2, 8, 128)
        x = x[:, 0] + x[:, 1]
        n //= 2
    return x[0]


def _ln(x):
    m = jnp.mean(x, axis=-1, keepdims=True)
    xc = x - m
    v = jnp.mean(xc * xc, axis=-1, keepdims=True)
    return xc * lax.rsqrt(v + EPS)


def _pack(x):
    return pltpu.bitcast(x.astype(bf), u32)


def _unpack(x):
    return pltpu.bitcast(x, bf)


def _tok(v, zv):
    v = v if v.dtype == u32 else pltpu.bitcast(v, u32)
    while v.shape[1] > 128:
        h = v.shape[1] // 2
        v = v[:, :h] | v[:, h:]
    while v.shape[0] > 8:
        h = v.shape[0] // 2
        v = v[:h] | v[h:]
    return v & zv


def _gate(w, toks):
    if not toks:
        return w
    wu = pltpu.bitcast(w, u32)
    h0 = wu[0:8]
    for t in toks:
        h0 = h0 | t
    return _unpack(jnp.concatenate([h0, wu[8:]], axis=0))


def _kernel(x_hbm, wqkv_hbm, wo_hbm, bk_hbm, bv_hbm, shk_hbm, ssmk_hbm, ssmd_hbm, fwd_hbm, inv_hbm, out_hbm,
            x_s, y_s, qt_s, k_s, vt_s, o_s, kb_s, a1, a2, b1, b2, fin, kf_s, taps_s, ug_a, ug_b, zb_a, zb_b,
            pb_a, pb_b, h_s, z_ref, x_in, wqkv, wo, bk, bv, ssmk, shk, ssmd, fwd_ref, inv_ref,
            sem_c, sem_x, sem_w, sem_o, sem_s):
    out_s = x_in

    def kv_copies(cb):
        cs = pl.ds(pl.multiple_of(cb * 128, 128), 128)
        return [pltpu.make_async_copy(bk_hbm.at[0, :, cs], bk.at[cb % NB], sem_c.at[0, cb]),
                pltpu.make_async_copy(bv_hbm.at[0, :, cs], bv.at[cb % NB], sem_c.at[1, cb])]

    def h_copy(cb):
        cs = pl.ds(pl.multiple_of(cb * 128, 128), 128)
        return pltpu.make_async_copy(ssmk_hbm.at[cs, :], ssmk.at[cb % NB, :, pl.ds(0, S)], sem_c.at[2, cb])

    def x_copy(c):
        rs = pl.ds(pl.multiple_of(c * RC, RC), RC)
        return pltpu.make_async_copy(x_hbm.at[0, rs, :], x_in.at[rs, :], sem_x.at[c])

    def w_copy(c):
        rs = pl.ds(pl.multiple_of(c * 128, 128), 128)
        return pltpu.make_async_copy(wqkv_hbm.at[rs, :], wqkv.at[rs, pl.ds(0, 3 * D)], sem_w.at[c])

    def wo_copy():
        return pltpu.make_async_copy(wo_hbm, wo.at[:, pl.ds(0, D)], sem_w.at[G])

    def out_copy(c):
        rs = pl.ds(pl.multiple_of(c * RC, RC), RC)
        return pltpu.make_async_copy(out_s.at[rs, :], out_hbm.at[0, rs, :], sem_o.at[c])

    TAIL = (0, 128, 192, 256)

    def tail_copy(q):
        rs = pl.ds((NRC - 1) * RC + TAIL[q], TAIL[q + 1] - TAIL[q])
        return pltpu.make_async_copy(out_s.at[rs, :], out_hbm.at[0, rs, :], sem_o.at[NRC - 1 + q])

    def conv_start(c):
        h_copy(c).start()
        for cp in kv_copies(c):
            cp.start()

    def wait_all(cps):
        for cp in cps:
            cp.wait()

    shk_cp, ssmd_cp, fwd_cp, inv_cp = [
        pltpu.make_async_copy(src, dst, sem_s.at[i]) for i, (src, dst) in enumerate(
            ((shk_hbm, shk), (ssmd_hbm, ssmd), (fwd_hbm, fwd_ref), (inv_hbm, inv_ref)))]
    h_copy(0).start()
    fwd_cp.start()
    shk_cp.start()
    ssmd_cp.start()
    for cp in kv_copies(0):
        cp.start()

    for i in range(NZ):
        z_ref[i] = 0
    fin[...] = jnp.ones(fin.shape, f32)
    for buf in (a2, b1, b2):
        buf[...] = jnp.zeros(buf.shape, f32)
    kf_s[0, 0:8, :] = jnp.zeros((8, 128), f32)

    def zero_vreg():
        return jnp.full((8, 128), z_ref[0], i32).astype(u32)

    def fence(cps):
        @pl.when(z_ref[0] == 0)
        def _():
            wait_all(cps)

    TILES = [(0, n) for n in range(8)] + [(2, n) for n in range(8)] + [(1, n) for n in range(8)]

    def qkv_tile(h, c, idx, toks, zv):
        kind, n = TILES[idx]
        col = kind * D + n * 128
        r = jnp.dot(h, _gate(wqkv[:, col:col + 128], toks), preferred_element_type=f32)
        if kind == 1:
            k_s[n, pl.ds(pl.multiple_of(c * (RC // 2), RC // 2), RC // 2), :] = _pack(r)
            return None
        dst = qt_s if kind == 0 else vt_s
        if kind == 0:
            r = r * QSCALE
        pks = []
        for t in range(RC // 128):
            pk = _pack(r[t * 128:(t + 1) * 128, :].T)
            dst[c * (RC // 128) + t, n * 64:(n + 1) * 64, :] = pk
            pks.append(pk)
        return _tok(jnp.concatenate(pks, axis=0), zv)

    def qkv_proj(h, c, piece_fn, first_piece, kb_jobs, span=NP):
        zv = zero_vreg()
        deps = {}
        for n in range(24):
            done = qkv_tile(h, c, n, deps.get(n), zv)
            if done is not None:
                deps.setdefault(n + 3, []).append(done)
            if n in kb_jobs:
                deps.setdefault(n + 2, []).append(kb_piece(*kb_jobs[n], zv))
            if piece_fn is not None:
                for p in range(NP):
                    if first_piece + p * span // NP == n:
                        deps.setdefault(n + 3, []).append(_tok(piece_fn(p), zv))

    def kb_plan(g, tiles):
        return {t: (g, 128 * i // len(tiles), 128 * (i + 1) // len(tiles)) for i, t in enumerate(tiles)}

    def kb_piece(g, lo, hi, zv):
        kx = _unpack(k_s[g, 0:NV // 2, :]).astype(f32)
        for d in range(lo, hi):
            v = jnp.broadcast_to(kx[:, d:d + 1], (NV, 128))
            kb_s[g, d] = v
        return _tok(v[NV - 32:], zv)

    def early_keys():
        col = D + (G - 1) * 128
        k_s[G - 1, 0:NV // 2, :] = _pack(jnp.dot(_unpack(h_s[0:NV // 2, :]), wqkv[:, col:col + 128],
                                                 preferred_element_type=f32))

    def piece_rows(c, p):
        return pl.ds(pl.multiple_of(c * RC + p * 16, 16), 16)

    def ln1_piece(c, p):
        hp = _pack(_ln(x_in[piece_rows(c, p), :].astype(f32)))
        h_s[p * 8:(p + 1) * 8, :] = hp
        return hp

    def gated_x(c, p, z):
        rows = piece_rows(c, p)
        x1 = x_s[z, rows, :]
        y = jnp.concatenate([y_s[0, g, rows, :] + y_s[1, g, rows, :] for g in range(G)], axis=1)
        return x1 + _ln(x1) * y

    def ln2_piece(c, p, z):
        x2 = gated_x(c, p, z)
        x_s[z, piece_rows(c, p), :] = x2
        hp = _pack(_ln(x2))
        h_s[p * 8:(p + 1) * 8, :] = hp
        return hp

    def out_piece(c, p, z):
        v = gated_x(c, p, z)
        out_s[piece_rows(c, p), :] = v.astype(bf)
        return v

    def load_o(c):
        rs = pl.ds(pl.multiple_of(c * (RC // 2), RC // 2), RC // 2)
        return jnp.concatenate([_unpack(o_s[g, rs, :]) for g in range(G)], axis=1)

    def oproj_tile(o, c, n, z, toks=None, r0=0, nr=RC, first=False):
        rows = pl.ds(pl.multiple_of(c * RC + r0, 64), nr)
        cols = slice(n * 128, (n + 1) * 128)
        r = jnp.dot(o[r0:r0 + nr], _gate(wo[:, cols], toks), preferred_element_type=f32)
        x0 = x_in[rows, cols].astype(f32) if first else x_s[z, rows, cols]
        x_s[z, rows, cols] = x0 + r
        return r

    zts = [z_ref[2 + ib] for ib in range(4)]

    def setup_taps():
        taps = shk[...].astype(f32)
        for cb in range(G):
            for t in range(4):
                taps_s[cb, 8 * t:8 * t + 8, :] = jnp.broadcast_to(taps[t:t + 1, cb * 128:(cb + 1) * 128], (8, 128))

    def setup_skip():
        dall = ssmd[...].astype(f32)
        for cb in range(G):
            taps_s[cb, 32:40, :] = jnp.broadcast_to(dall[cb:cb + 1, :], (8, 128))

    def prep_h_chunk(cb, pb, j):
        pb[HS + j * 64:HS + (j + 1) * 64, :] = pltpu.bitcast(ssmk[cb % NB, :, j * 128:(j + 1) * 128], u32)

    def prep_h(cb, pb):
        for j in range(NC):
            prep_h_chunk(cb, pb, j)

    def prep_kv(cb, pb, with_h):
        zs = z_ref[1]
        tp = taps_s[cb, 0:32, :]
        for j in range(NC):
            r0 = j * 128
            if with_h:
                prep_h_chunk(cb, pb, j)
            kf_s[zs, 8 + r0:8 + r0 + 128, :] = bk[cb % NB, r0:r0 + 128, :].astype(f32)
            ks = None
            for t in range(4):
                term = kf_s[zs, 8 + r0 - t:8 + r0 - t + 128, :].reshape(16, 8, 128) * tp[8 * t:8 * t + 8][None]
                ks = term if ks is None else ks + term
            pb[j * 64:(j + 1) * 64, :] = _pack(ks.reshape(128, 128) * bv[cb % NB, r0:r0 + 128, :].astype(f32))

    def fwd_h(pb, ug):
        for m in range(NC):
            hm = lax.dot_general(_unpack(fwd_ref[128:320, :]), _unpack(pb[HS + m * 64:HS + (m + 1) * 64, :]),
                                 NT, preferred_element_type=f32)
            ug[0, NC + m, :, GO:GO + 128, :] = hm.reshape(3, 128, 128)

    def fwd_u(pb, ug):
        for j in range(NC):
            u = jnp.dot(_unpack(fwd_ref[0:128, :]), _unpack(pb[j * 64:(j + 1) * 64, :]),
                        preferred_element_type=f32)
            ug[0, j, 0:2, 0:128, :] = u.reshape(2, 128, 128)

    def add_skip(cb, ug):
        dv = taps_s[cb, 32:40, :][None]
        for e in range(3):
            v = ug[0, NC, e, GO:GO + 128, :].reshape(16, 8, 128)
            ug[0, NC, e, GO:GO + 128, :] = (v - dv if e == 1 else v + dv).reshape(128, 128)

    def spec_item(ug, ib, r):
        zt = zts[ib]
        acc = None
        for j in range(4 * ib + 4):
            u = ug[zt, j:j + 1, 0:2, r:r + 8, :]
            u = jnp.concatenate([u[:, 0:1] + u[:, 1:2], u], axis=1)
            q0 = max(0, j - 4 * ib)
            m0 = NC + 4 * ib - j
            t = ug[zt, m0 + q0:m0 + 4, :, GO + r:GO + r + 8, :] * u
            if acc is None:
                acc = t
            elif q0 == 0:
                acc = acc + t
            else:
                acc = jnp.concatenate([acc[:q0], acc[q0:] + t], axis=0)
        return acc[:, 0] - acc[:, 2], acc[:, 0] + acc[:, 1]

    def overlap_add(yr, yi, prev, r):
        n = 1 if prev is None else 0
        pr = yr[:3] if prev is None else jnp.concatenate([prev[0], yr[:3]], axis=0)
        pi = yi[:3] if prev is None else jnp.concatenate([prev[1], yi[:3]], axis=0)
        if r < 64:
            zr, zi = yr[n:] - pi, yi[n:] + pr
        else:
            zr, zi = yr[n:] + pi, yi[n:] - pr
        if prev is None:
            zr = jnp.concatenate([yr[:1], zr], axis=0)
            zi = jnp.concatenate([yi[:1], zi], axis=0)
        return zr, zi, (yr[3:], yi[3:])

    def conv_spec(ug, zb, lo=0, hi=8):
        for rp in range(lo, hi):
            p0 = p1 = None
            for ib in range(4):
                zr0, zi0, p0 = overlap_add(*spec_item(ug, ib, 16 * rp), p0, 16 * rp)
                zr1, zi1, p1 = overlap_add(*spec_item(ug, ib, 16 * rp + 8), p1, 16 * rp)
                zb[4 * ib:4 * ib + 4, rp * 8:rp * 8 + 8, :] = _pack(jnp.concatenate([zr0, zr1], axis=1))
                zb[4 * ib:4 * ib + 4, 64 + rp * 8:72 + rp * 8, :] = _pack(jnp.concatenate([zi0, zi1], axis=1))

    def conv_inv(cb, zb):
        for i in range(NC):
            for e in range(2):
                y_s[e, cb, i * 128:(i + 1) * 128, :] = jnp.dot(
                    _unpack(inv_ref[:, e * 128:(e + 1) * 128]), _unpack(zb[i, e * 64:(e + 1) * 64, :]),
                    preferred_element_type=f32)

    def conv_step(c, ug_cur, ug_nxt, zb_cur, zb_prev, pb_nxt, pb_new):
        @pl.when(c + 3 < G)
        def _():
            conv_start(c + 3)
        w_copy(c).start()

        @pl.when(c >= G - 3)
        def _():
            x_copy(c - (G - 3)).start()
        conv_spec(ug_cur, zb_cur)
        conv_inv(c - 1, zb_prev)
        fwd_u(pb_nxt, ug_nxt)
        fwd_h(pb_nxt, ug_nxt)

        @pl.when(c + 2 < G)
        def _():
            wait_all([w_copy(c - 1), h_copy(c + 2)] + kv_copies(c + 2))
            prep_kv(c + 2, pb_new, True)
            add_skip(c + 1, ug_nxt)

        @pl.when(c + 2 >= G)
        def _():
            w_copy(c - 1).wait()
            add_skip(c + 1, ug_nxt)

    def conv():
        wait_all([fwd_cp, h_copy(0)])
        conv_start(1)
        inv_cp.start()
        prep_h(0, pb_a)
        fwd_h(pb_a, ug_a)
        wait_all([shk_cp] + kv_copies(0))
        conv_start(2)
        setup_taps()
        prep_kv(0, pb_a, False)
        fwd_u(pb_a, ug_a)
        fence([h_copy(1)])
        prep_h(1, pb_b)
        fence([ssmd_cp])
        setup_skip()
        add_skip(0, ug_a)
        conv_spec(ug_a, zb_a, 0, 4)
        fwd_h(pb_b, ug_b)
        fence(kv_copies(1))
        conv_start(3)
        w_copy(0).start()
        prep_kv(1, pb_b, False)
        add_skip(1, ug_b)
        fence([h_copy(2)])
        conv_spec(ug_a, zb_a, 4, 8)
        fwd_u(pb_b, ug_b)
        fence(kv_copies(2) + [inv_cp])
        prep_kv(2, pb_a, True)

        def body(p, carry):
            conv_step(2 * p + 1, ug_b, ug_a, zb_b, zb_a, pb_a, pb_b)
            conv_step(2 * p + 2, ug_a, ug_b, zb_a, zb_b, pb_b, pb_a)
            return carry
        lax.fori_loop(0, G // 2 - 1, body, 0)
        w_copy(G - 1).start()
        conv_spec(ug_b, zb_b)
        conv_inv(G - 2, zb_a)
        fence([x_copy(0), w_copy(G - 2), w_copy(G - 1)])
        for p in range(NP):
            ln1_piece(0, p)
        conv_inv(G - 1, zb_b)
        early_keys()

    def phase1():
        def body(c, carry):
            @pl.when(c + 1 < NRC)
            def _():
                x_copy(c + 1).wait()

            @pl.when(c + 2 < NRC)
            def _():
                x_copy(c + 2).start()

            @pl.when(c + 2 == NRC)
            def _():
                wo_copy().start()
            cn = jnp.minimum(c + 1, NRC - 1)
            qkv_proj(_unpack(h_s[...]), c, lambda p: ln1_piece(cn, p), 2,
                     kb_plan((c + G - 1) & (G - 1), range(15, 22)), 12)
            return carry
        lax.fori_loop(0, NRC, body, 0)
        wo_copy().wait()

    def phase2(ms):
        o = load_o(0)
        z0 = z_ref[0]
        zv = zero_vreg()
        deps = {}
        todo = []
        for q in range(2):
            rs = []
            for n in range(8):
                t = 8 * q + n
                for p in todo[n:n + 1]:
                    deps.setdefault(t + 4, []).append(_tok(ln2_piece(0, p, z0), zv))
                rs.append(oproj_tile(o, 0, n, z0, deps.get(t), q * (RC // 2), RC // 2, True))
            if q == 0:
                deps.setdefault(11, []).append(attention_tail(ms, rs[0:5:2]))
            todo = list(range(q * NP // 2, (q + 1) * NP // 2))
        for p in todo:
            ln2_piece(0, p, z0)
        early_keys()

        def body(c, carry):
            z0 = z_ref[0]
            z1 = z_ref[1]
            h = _unpack(h_s[...])
            o = load_o(c + 1)
            for n in range(8):
                oproj_tile(o, c + 1, n, z1, first=True)
            qkv_proj(h, c, lambda p: ln2_piece(c + 1, p, z0), 1,
                     kb_plan((c + G - 1) & (G - 1), range(15, 23)), 13)
            return carry
        lax.fori_loop(0, NRC - 1, body, 0)
        qkv_proj(_unpack(h_s[...]), NRC - 1, None, 0, kb_plan(G - 2, range(15, 22)))

    def phase3(ms):
        o = load_o(0)
        done = attention_tail(ms, [oproj_tile(o, 0, n, z_ref[1]) for n in range(3)])
        for n in range(3, 8):
            oproj_tile(o, 0, n, z_ref[1], [done] if n == 6 else None)

        def body(c, carry):
            z0 = z_ref[0]
            z1 = z_ref[1]
            zv = zero_vreg()
            o = load_o(c + 1)
            deps = {}
            p = 0
            for t in range(16):
                for _ in range(2 if t < 2 else 1):
                    if p < NP:
                        deps.setdefault(t + 2, []).append(_tok(out_piece(c, p, z0), zv))
                        p += 1
                oproj_tile(o, c + 1, t // 2, z1, deps.get(t), (t % 2) * 128, 128)
            out_copy(c).start()
            return carry
        lax.fori_loop(0, NRC - 2, body, 0)

        c = NRC - 1
        z0 = z_ref[0]
        zv = zero_vreg()
        o = load_o(c)
        deps = {}
        todo = [(c - 1, p) for p in range(NP)]
        for q in range(3):
            for n in range(8):
                t = 8 * q + n
                for cc, p in todo[2 * n:2 * n + 2]:
                    deps.setdefault(t + (2 if q == 0 else 6), []).append(_tok(out_piece(cc, p, z0), zv))
                oproj_tile(o, c, n, z0, deps.get(t), TAIL[q], TAIL[q + 1] - TAIL[q])
            if q == 1:
                out_copy(c - 1).start()
            if q > 0:
                tail_copy(q - 1).start()
            todo = [(c, p) for p in range(TAIL[q] // 16, TAIL[q + 1] // 16)]
        for cc, p in todo:
            out_piece(cc, p, z0)
        tail_copy(2).start()
        wait_all([out_copy(i) for i in range(NRC - 1)] + [tail_copy(q) for q in range(3)])

    zero16 = jnp.zeros((16, 128), u32)

    def after(x, src, never):
        if src is None:
            return x
        src = pltpu.bitcast(src, x.dtype)
        if x.ndim == 3:
            return jnp.where(never[None], src[None], x)
        return jnp.where(never, src, x)

    def qk(g, j, hh, half, dst, z, zk, dep, never):
        qt = qt_s[j, pl.ds(pl.multiple_of(g * 64 + hh * 16, 16), 16), :]
        w = _unpack(jnp.concatenate([qt if i == hh else zero16 for i in range(4)], axis=0))
        r0 = NV if half == 0 else 0
        kh = k_s[g + zk, (half * HS + r0) // 2:(half + 1) * HS // 2, :]
        ch = (HS - r0) // 4
        m = s2 = None
        for c in range(4):
            ku = kh[c * ch // 2:(c + 1) * ch // 2]
            ku = jnp.concatenate([ku[:ch // 2 - 8], after(ku[ch // 2 - 8:], dep, never)], axis=0)
            s = jnp.dot(_unpack(ku), w, preferred_element_type=f32)
            dst[z, r0 + c * ch:r0 + (c + 1) * ch, :] = s
            mc = jnp.max(s.reshape(ch // 8, 8, 128), axis=0)
            m = mc if m is None else jnp.maximum(m, mc)
            if c == 2:
                s2 = s
        return m, s2

    def qk_vpu(g, j, hh, half, trigs, never):
        qw16 = qt_s[j, pl.ds(pl.multiple_of(g * 64 + hh * 16, 16), 16), :]
        qw = jnp.broadcast_to(qw16[:, None, :], (16, 8, 128))
        if all(tr is not None for tr in trigs):
            qw = jnp.where(never[None], pltpu.bitcast(jnp.stack(trigs), u32), qw)
        else:
            qw = jnp.stack([after(qw[i], tr, never) for i, tr in enumerate(trigs)])
        qb = jnp.stack([qw << 16, qw & jnp.uint32(0xFFFF0000)], axis=1).reshape(32, 1, 8, 128)
        kb = kb_s[g, hh * 32:hh * 32 + 32, half * NV // 2:(half + 1) * NV // 2, :]
        return jnp.sum(kb.reshape(32, NV // 16, 8, 128) * pltpu.bitcast(qb, f32), axis=0)

    def fullmax(m1, m2):
        return jnp.max(jnp.maximum(m1, m2), axis=0, keepdims=True)

    def sm_pv(g, hh, half, src, m, z, dep, trigs, never):
        mb = jnp.broadcast_to(m, (8, 128))
        ms = [after(mb, tr, never) for tr in trigs]
        mm = jnp.stack([jnp.stack([ms[4 * st + 3 - kk] for kk in range(4)]) for st in range(2)])
        x = src[z].reshape(2, 4, 4, 4, 8, 128)
        p = jnp.exp2(x - mm[:, None, :, None]).reshape(HS, 128)
        rs = pl.ds(pl.multiple_of(g * 64 + hh * 16, 16), 16)
        vu = vt_s[half * 8:half * 8 + 8, rs, :]
        vu = jnp.concatenate([after(vu[:, 0:8], dep, never), vu[:, 8:16]], axis=1)
        vu = jnp.concatenate([vu[t] for t in range(8)], axis=1)
        l = _tree_sum(p)
        return jnp.dot(_unpack(vu), p.astype(bf), preferred_element_type=f32), l

    def store_o(g, j, parts):
        outs = [parts[2 * h] * (1.0 / jnp.sum(parts[2 * h + 1], axis=0, keepdims=True)) for h in range(4)]
        ot = _pack(jnp.concatenate(outs, axis=0).T)
        o_s[g, pl.ds(pl.multiple_of(j * 64, 64), 64), :] = ot
        return ot

    bufs = {(0, 0): a1, (0, 1): a2, (1, 0): b1, (1, 1): b2}

    def tile_of(t):
        return lax.shift_right_logical(t, 4), t & (NQ - 1)

    def finish_tile(g, j, done, res):
        if done is None:
            parts = []
        else:
            parts = [done[0:32], done[32:40], done[40:72], done[72:80]]
            res = [(done[80:112], done[112:120])] + res
        for h in range(len(res) // 2):
            parts += [res[2 * h][0] + res[2 * h + 1][0], res[2 * h][1] + res[2 * h + 1][1]]
        return store_o(g, j, parts)

    def attention(m_init):
        nit = G * NQ // UNR

        def body(it, carry):
            z1 = z_ref[0]
            z2 = z_ref[1]
            never = zero_vreg() != 0
            g, j0 = tile_of(it * UNR)
            gp, jp = tile_of(jnp.maximum(it * UNR - 1, 0))
            mfull = {(-1, 2): carry[0], (-1, 3): carry[1]}
            mpart = do = ps = po = None
            res = []

            def tg(sv, i):
                return None if sv is None else sv[i * 8:i * 8 + 8]

            for n in range(8 * UNR):
                u, qh, qhalf = n // 8, (n % 8) // 2, n % 2
                mp, cs = qk(g, j0 + u, qh, qhalf, bufs[(qh % 2, qhalf)], z1, z_ref[2 + n], do, never)
                src = {'p': ps, 'o': po, 'c': cs}
                vtr, etr = [[tg(src[t[0]], int(t[1:])) for t in spec.split('/')[qhalf].split(',')]
                            for spec in (VT, ET)]
                sv = qk_vpu(g, j0 + u, qh, qhalf, vtr, never)
                bufs[(qh % 2, 0)][z1, qhalf * NV // 2:(qhalf + 1) * NV // 2, :] = sv.reshape(NV // 2, 128)
                mp = jnp.maximum(mp, jnp.max(sv, axis=0))
                if qhalf == 0:
                    mpart = mp
                else:
                    mfull[(u, qh)] = fullmax(mpart, mp)
                pu, ph, phalf = (n - LAG) // 8, ((n - LAG) % 8) // 2, (n - LAG) % 2
                o, l = sm_pv(gp if pu < 0 else g, ph, phalf, bufs[(ph % 2, phalf)], mfull[(pu, ph)], z2,
                             tg(cs, 0), etr, never)
                ps, po, do = cs, o, tg(o, 3)
                res.append((o, l))
                if ph == 3 and phalf == 1:
                    if pu < 0:
                        finish_tile(gp, jp, fin[z2], res)
                    else:
                        finish_tile(g, j0 + pu, None, res)
                    res = []
            fin[z1] = jnp.concatenate([res[0][0] + res[1][0], res[0][1] + res[1][1],
                                       res[2][0] + res[3][0], res[2][1] + res[3][1],
                                       res[4][0], res[4][1]], axis=0)
            return mfull[(UNR - 1, 2)], mfull[(UNR - 1, 3)]

        return lax.fori_loop(0, nit, body, m_init)

    def attention_tail(ms, rs):
        z2 = z_ref[1]
        never = zero_vreg() != 0
        res = []
        for k, (ph, phalf) in enumerate(((2, 1), (3, 0), (3, 1))):
            trigs = [rs[k][16 * i:16 * i + 8] for i in range(8)]
            res.append(sm_pv(G - 1, ph, phalf, bufs[(ph % 2, phalf)], ms[ph - 2], z2, trigs[7], trigs, never))
        return _tok(finish_tile(G - 1, NQ - 1, fin[z2], res), zero_vreg())

    conv()
    phase1()
    ms = attention((jnp.zeros((1, 128), f32), jnp.zeros((1, 128), f32)))
    phase2(ms)
    ms = attention(ms)
    phase3(ms)


@jax.jit
def pallas_interleave_layers__softmax_full_mha__ssm_conv_h3__prompt_kernel(
        A_x, A_wqkv, A_wo, B_q, B_k, B_v, B_shift_k, B_ssm_k, B_ssm_D):
    del B_q
    fwd, inv = _dft_mats()
    scratch = [
        pltpu.VMEM((1, S, D), f32),
        pltpu.VMEM((2, G, S, 128), f32),
        pltpu.VMEM((NQ, D // 2, 128), u32),
        pltpu.VMEM((G, S // 2, 128), u32),
        pltpu.VMEM((NQ, D // 2, 128), u32),
        pltpu.VMEM((G, S // 2, 128), u32),
        pltpu.VMEM((G, 128, NV, 128), f32),
        pltpu.VMEM((1, HS, 128), f32), pltpu.VMEM((1, HS, 128), f32),
        pltpu.VMEM((1, HS, 128), f32), pltpu.VMEM((1, HS, 128), f32),
        pltpu.VMEM((1, 120, 128), f32),
        pltpu.VMEM((1, S + 8, 128), f32),
        pltpu.VMEM((G, 40, 128), f32),
        pltpu.VMEM((1, 2 * NC, 3, IM, 128), f32),
        pltpu.VMEM((1, 2 * NC, 3, IM, 128), f32),
        pltpu.VMEM((NC, 128, 128), u32),
        pltpu.VMEM((NC, 128, 128), u32),
        pltpu.VMEM((S, 128), u32),
        pltpu.VMEM((S, 128), u32),
        pltpu.VMEM((RC // 2, D), u32),
        pltpu.SMEM((NZ,), i32),
        pltpu.VMEM((S, D), bf),
        pltpu.VMEM((D, 3 * D + 128), bf),
        pltpu.VMEM((D, D + 128), bf),
        pltpu.VMEM((NB, S, 128), bf),
        pltpu.VMEM((NB, S, 128), bf),
        pltpu.VMEM((NB, 128, S + 128), bf),
        pltpu.VMEM((4, D), bf),
        pltpu.VMEM((G, 128), bf),
        pltpu.VMEM((320, 128), u32),
        pltpu.VMEM((64, 256), u32),
        pltpu.SemaphoreType.DMA((3, G)),
        pltpu.SemaphoreType.DMA((NRC,)),
        pltpu.SemaphoreType.DMA((G + 1,)),
        pltpu.SemaphoreType.DMA((NRC + 2,)),
        pltpu.SemaphoreType.DMA((4,)),
    ]
    hbm = pl.BlockSpec(memory_space=pl.ANY)
    return pl.pallas_call(
        _kernel,
        out_shape=jax.ShapeDtypeStruct((1, S, D), bf),
        in_specs=[hbm] * 10,
        out_specs=hbm,
        scratch_shapes=scratch,
        compiler_params=pltpu.CompilerParams(vmem_limit_bytes=120 * 2**20, disable_bounds_checks=True),
    )(A_x, A_wqkv, A_wo, B_k, B_v, B_shift_k.T, B_ssm_k, B_ssm_D.reshape(G, 128),
      jnp.asarray(fwd), jnp.asarray(inv))
```
